```python
import jax
import jax.numpy as jnp

def _softmax(x, axis=-1):
    return jax.nn.softmax(x, axis=axis)
def _gelu(x):
    return jax.nn.gelu(x, approximate=True)
def _silu(x):
    return jax.nn.silu(x)
def _sigmoid(x):
    return jax.nn.sigmoid(x)
def _layernorm(x, axis=-1, eps=1e-5):
    m = jnp.mean(x, axis=axis, keepdims=True)
    v = jnp.var(x, axis=axis, keepdims=True)
    return (x - m) / jnp.sqrt(v + eps)
def _scatter_add(tgt, idx, src, axis=0):
    return tgt.at[idx].add(src)
def _segment_sum(src, seg, n):
    return jax.ops.segment_sum(src, seg, n)
class _Rng:
    def __init__(self, key):
        self._k = key
    def _next(self):
        self._k, sub = jax.random.split(self._k)
        return sub
    def normal(self, shape):
        return jax.random.normal(self._next(), shape, dtype=jnp.bfloat16)
    def randint(self, lo, hi, shape):
        return jax.random.randint(self._next(), shape, lo, hi, dtype=jnp.int32)
    def uniform(self, shape, lo=0.0, hi=1.0):
        return jax.random.uniform(self._next(), shape, jnp.bfloat16, lo, hi)
    def permutation(self, n):
        return jax.random.permutation(self._next(), n)


kernel_name = 'parallel_sum__sliding_local_dilated__glu_gated_bilinear__prompt'

def setup_inputs():
    _rng = _Rng(jax.random.key(int.from_bytes(__import__("os").urandom(4), "little")))
    _w = (lambda a: (lambda t: t.astype(jnp.bfloat16) if jnp.issubdtype(t.dtype, jnp.floating) else t)(jnp.asarray(a)))
    def _A_setup():
        B, S, D = 1, 2048, 1024
        return {
            "x": _w((lambda *s: _rng.normal(s) * 0.05)(B, S, D)),
            "wqkv": _w((lambda *s: _rng.normal(s) * 0.05)(D, 3 * D)),
            "wo": _w((lambda *s: _rng.normal(s) * 0.05)(D, D)),
        }
    _A_in = _A_setup()

    def _B_setup():
        B, S, D, F = 1, 2048, 1024, 3584
        return {
            "x": _w((lambda *s: _rng.normal(s) * 0.05)(B, S, D)),
            "w_gate": _w((lambda *s: _rng.normal(s) * 0.05)(D, F) * (D ** -0.5)),
            "w_up": _w((lambda *s: _rng.normal(s) * 0.05)(D, F) * (D ** -0.5)),
            "w_down": _w((lambda *s: _rng.normal(s) * 0.05)(F, D) * (F ** -0.5)),
        }
    _B_in = _B_setup()

    return {
        "A_x": _A_in["x"],
        "A_wqkv": _A_in["wqkv"],
        "A_wo": _A_in["wo"],
        "B_x": _B_in["x"],
        "B_w_gate": _B_in["w_gate"],
        "B_w_up": _B_in["w_up"],
        "B_w_down": _B_in["w_down"],
    }

def reference(A_x, A_wqkv, A_wo, B_x, B_w_gate, B_w_up, B_w_down):
    def _A_ref(x, wqkv, wo):
        B, S, D = x.shape
        H = 32; Dh = D // H
        W, dil = 8, 2
        qkv = (lambda x, *d: x.transpose(*d))((x @ wqkv).reshape(B, S, 3, H, Dh), 2, 0, 3, 1, 4)
        q, k, v = qkv[0], qkv[1], qkv[2]
        scale = Dh ** -0.5
        pos = jnp.arange(S)
        off = jnp.arange(W) * dil
        idx = pos[:, None] - off[None, :]
        mask = idx >= 0
        idx_c = jnp.where(mask, idx, 0).reshape(-1)
        kg = k[:, :, idx_c, :].reshape(B, H, S, W, Dh)
        vg = v[:, :, idx_c, :].reshape(B, H, S, W, Dh)
        logits = jnp.einsum("bhsd,bhswd->bhsw", q, kg) * scale
        logits = jnp.where(mask[None, None, :, :], logits, -1e9)
        attn = _softmax(logits, axis=-1)
        o = jnp.einsum("bhsw,bhswd->bhsd", attn, vg)
        return (lambda x, *d: x.transpose(*d))(o, 0, 2, 1, 3).reshape(B, S, D) @ wo

    def _B_ref(x, w_gate, w_up, w_down):
        g = jnp.einsum("bsd,df->bsf", x, w_gate)
        u = jnp.einsum("bsd,df->bsf", x, w_up)
        h = g * u
        return jnp.einsum("bsf,fd->bsd", h, w_down)

    x = A_x
    xn = _layernorm(x, axis=-1)
    return x + _A_ref(xn, A_wqkv, A_wo) + _B_ref(xn, B_w_gate, B_w_up, B_w_down)
```

```python
import functools

import jax
import jax.numpy as jnp
from jax import lax
from jax.experimental import pallas as pl
from jax.experimental.pallas import tpu as pltpu

S, D, F = 2048, 1024, 3584
H, DH, WIN, DIL = 32, 32, 8, 2
TM = 256
HM = TM // 2
NB = S // TM
HD = D // 2
FC = 256
NCH = F // 2 // FC
HALO = 16
NG = D // 128
EPS = 1e-5
NEG = -1e9
BF = jnp.bfloat16
F32 = jnp.float32
LOG2E = 1.4426950408889634
NSTEPS = 16


def _at(step):
    return min(step, NSTEPS - 1)


def _dot(a, b):
    return jnp.dot(a, b, preferred_element_type=F32)


def _butterfly(vs):
    lane = lax.broadcasted_iota(jnp.int32, vs[0].shape, 1)
    for b in range(3):
        sh = 4 << b
        bit = (lane & sh) != 0
        new = list(vs)
        for i0 in range(NG):
            if i0 & (1 << b):
                continue
            i1 = i0 | (1 << b)
            new[i0] = jnp.where(bit, pltpu.roll(vs[i1], sh, 1), vs[i0])
            new[i1] = jnp.where(bit, vs[i1], pltpu.roll(vs[i0], 128 - sh, 1))
        vs = new
    return vs


def _sum4(x):
    lane = lax.broadcasted_iota(jnp.int32, x.shape, 1)
    x = x + jnp.where((lane & 1) != 0, pltpu.roll(x, 1, 1), pltpu.roll(x, 127, 1))
    x = x + jnp.where((lane & 2) != 0, pltpu.roll(x, 2, 1), pltpu.roll(x, 126, 1))
    return x


def _lhs_combos(a11, a12, a21, a22):
    return [a11 + a22, a21 + a22, a11, a22, a11 + a12, a21 - a11, a12 - a22]


def _strassen_out(m):
    return (m[0] + m[3] - m[4] + m[6], m[2] + m[4], m[1] + m[3], m[0] - m[1] + m[2] + m[5])


def _layernorm(x):
    x = x.astype(F32)
    mean = jnp.mean(x, axis=-1, keepdims=True)
    xc = x - mean
    var = jnp.mean(xc * xc, axis=-1, keepdims=True)
    return xc * lax.rsqrt(var + EPS)


def _kernel(x_hbm, wqkv_hbm, wo_hbm, wg_hbm, wu_hbm, wd_hbm, o_ref,
            x_scr, wqkv, wo, rawg, rawu, rawd, cg, cu, cd,
            xn_scr, s_scr, q_scr, k_scr, v_scr, o_scr,
            sem_x, sem_w, sem_raw):
    s = pl.program_id(0)

    def x_copy(b):
        return pltpu.make_async_copy(x_hbm.at[pl.ds(b * TM, TM), :], x_scr.at[pl.ds(b * TM, TM), :], sem_x.at[b])

    def wqkv_copy(j):
        return pltpu.make_async_copy(wqkv_hbm.at[:, pl.ds(j * D, D)], wqkv.at[:, pl.ds(j * D, D)], sem_w.at[j])

    def wo_copy():
        return pltpu.make_async_copy(wo_hbm, wo, sem_w.at[3])

    def raw_copies(c):
        return [
            pltpu.make_async_copy(wg_hbm.at[:, pl.ds(c * FC, FC)], rawg.at[c, :, pl.ds(0, FC)], sem_raw.at[c, 0]),
            pltpu.make_async_copy(wg_hbm.at[:, pl.ds(F // 2 + c * FC, FC)], rawg.at[c, :, pl.ds(FC, FC)], sem_raw.at[c, 1]),
            pltpu.make_async_copy(wu_hbm.at[:, pl.ds(c * FC, FC)], rawu.at[c, :, pl.ds(0, FC)], sem_raw.at[c, 2]),
            pltpu.make_async_copy(wu_hbm.at[:, pl.ds(F // 2 + c * FC, FC)], rawu.at[c, :, pl.ds(FC, FC)], sem_raw.at[c, 3]),
            pltpu.make_async_copy(wd_hbm.at[pl.ds(c * FC, FC), :], rawd.at[c, pl.ds(0, FC), :], sem_raw.at[c, 4]),
            pltpu.make_async_copy(wd_hbm.at[pl.ds(F // 2 + c * FC, FC), :], rawd.at[c, pl.ds(FC, FC), :], sem_raw.at[c, 5]),
        ]

    def ln_block(b):
        r0 = pl.multiple_of(b * TM, TM)
        RC = 16
        for r in range(0, HM, RC):
            top = _layernorm(x_scr[pl.ds(r0 + r, RC), :])
            bot = _layernorm(x_scr[pl.ds(r0 + HM + r, RC), :])
            xn_scr[r:r + RC, :] = top.astype(BF)
            xn_scr[HM + r:HM + r + RC, :] = bot.astype(BF)
            cs = _lhs_combos(top[:, :HD], top[:, HD:], bot[:, :HD], bot[:, HD:])
            for j in range(7):
                s_scr[b, j, r:r + RC, :] = cs[j].astype(BF)

    @pl.when(s == 0)
    def _():
        x_copy(0).start()
        wqkv_copy(0).start()
        x_copy(1).start()
        wqkv_copy(1).start()
        wqkv_copy(2).start()
        for c in range(2):
            for cp in raw_copies(c):
                cp.start(priority=1)
        x_copy(2).start()
        k_scr[:, 0:HALO, :] = jnp.zeros((NG, HALO, 128), F32)
        v_scr[:, 0:HALO, :] = jnp.zeros((NG, HALO, 128), F32)
        x_copy(0).wait()
        ln_block(0)
        x_copy(1).wait()
        for j in range(3):
            wqkv_copy(j).wait()

    @pl.when(s == _at(1))
    def _():
        for b in range(3, NB):
            x_copy(b).start()
        for c in range(2, NCH):
            for cp in raw_copies(c):
                cp.start(priority=1)
        wo_copy().start(priority=1)

    for c in range(NCH):
        @pl.when(s == _at(c + 1))
        def _():
            for cp in raw_copies(c):
                cp.wait()
            if c + 2 < NB:
                x_copy(c + 2).wait()

    @pl.when(s == _at(NB))
    def _():
        wo_copy().wait()

    @pl.when(s < NB)
    def _():
        xn = xn_scr[...]
        ln_block(jnp.minimum(s + 1, NB - 1))
        r0 = pl.multiple_of(s * TM, TM)
        RC = 16
        for sec, (dst, off) in enumerate(((q_scr, 0), (k_scr, HALO), (v_scr, HALO))):
            y = _dot(xn, wqkv[:, sec * D:(sec + 1) * D])
            for r in range(0, TM, RC):
                vs = _butterfly([y[r:r + RC, g * 128:(g + 1) * 128] for g in range(NG)])
                for g in range(NG):
                    dst[g, pl.ds(r0 + off + r, RC), :] = vs[g]
        c = lax.rem(s + (NCH - 1), NCH)

        def build(raw, cmb, kq, nq):
            RB = 16
            for r in range(0, kq, RB):
                b11 = raw[c, r:r + RB, 0:nq].astype(F32)
                b12 = raw[c, r:r + RB, nq:2 * nq].astype(F32)
                b21 = raw[c, kq + r:kq + r + RB, 0:nq].astype(F32)
                b22 = raw[c, kq + r:kq + r + RB, nq:2 * nq].astype(F32)
                cmb[c, 0, r:r + RB, :] = (b11 + b22).astype(BF)
                cmb[c, 1, r:r + RB, :] = (b12 - b22).astype(BF)
                cmb[c, 2, r:r + RB, :] = (b21 - b11).astype(BF)
                cmb[c, 3, r:r + RB, :] = (b11 + b12).astype(BF)
                cmb[c, 4, r:r + RB, :] = (b21 + b22).astype(BF)

        build(rawg, cg, HD, FC)
        build(rawu, cu, HD, FC)
        build(rawd, cd, FC, HD)

    @pl.when(s >= NB)
    def _():
        i = s - NB
        r0 = pl.multiple_of(i * TM, TM)

        def wlist(raw, cmb, c, kq, nq):
            return [cmb[c, 0], raw[c, 0:kq, 0:nq], cmb[c, 1], cmb[c, 2],
                    raw[c, kq:2 * kq, nq:2 * nq], cmb[c, 3], cmb[c, 4]]

        RA = 8
        cexp = (DH ** -0.5) * LOG2E

        def attn_rows(r):
            q = [q_scr[g, pl.ds(r0 + r, RA), :] for g in range(NG)]
            sw = []
            for w in range(WIN):
                acc = None
                for g in range(NG):
                    t = q[g] * k_scr[g, pl.ds(r0 + r + HALO - DIL * w, RA), :]
                    acc = t if acc is None else acc + t
                acc = _sum4(acc)
                if r < HALO and w > 0:
                    row = lax.broadcasted_iota(jnp.int32, (RA, 128), 0) + (r0 + r)
                    acc = jnp.where(row >= DIL * w, acc, NEG)
                sw.append(acc)
            m = sw[0]
            for w in range(1, WIN):
                m = jnp.maximum(m, sw[w])
            e = [jnp.exp2((sw[w] - m) * cexp) for w in range(WIN)]
            den = e[0]
            for w in range(1, WIN):
                den = den + e[w]
            inv = 1.0 / den
            p = [e[w] * inv for w in range(WIN)]
            o = []
            for g in range(NG):
                acc = None
                for w in range(WIN):
                    t = p[w] * v_scr[g, pl.ds(r0 + r + HALO - DIL * w, RA), :]
                    acc = t if acc is None else acc + t
                o.append(acc)
            o = _butterfly(o)
            return jnp.concatenate(o, axis=1)

        sl = [s_scr[i, j] for j in range(7)]
        acc = [None] * 7
        o_parts = []
        n_att = TM // RA
        per = -(-n_att // (NCH - 1))
        for c in range(NCH):
            wg_l = wlist(rawg, cg, c, HD, FC)
            wu_l = wlist(rawu, cu, c, HD, FC)
            wd_l = wlist(rawd, cd, c, FC, HD)
            g = _strassen_out([_dot(sl[j], wg_l[j]) for j in range(7)])
            u = _strassen_out([_dot(sl[j], wu_l[j]) for j in range(7)])
            hq = [g[t] * u[t] for t in range(4)]
            hl = [t.astype(BF) for t in _lhs_combos(*hq)]
            for j in range(7):
                y = _dot(hl[j], wd_l[j])
                acc[j] = y if acc[j] is None else acc[j] + y
            for a in range(c * per, min((c + 1) * per, n_att), 2):
                o2 = jnp.concatenate([attn_rows(a * RA), attn_rows((a + 1) * RA)], axis=0)
                o_scr[a * RA:(a + 2) * RA, :] = o2.astype(BF)
        ao = _dot(o_scr[...], wo[...])
        y11, y12, y21, y22 = _strassen_out(acc)
        x = x_scr[pl.ds(r0, TM), :].astype(F32)
        o_ref[0:HM, 0:HD] = (x[0:HM, 0:HD] + ao[0:HM, 0:HD] + y11).astype(o_ref.dtype)
        o_ref[0:HM, HD:D] = (x[0:HM, HD:D] + ao[0:HM, HD:D] + y12).astype(o_ref.dtype)
        o_ref[HM:TM, 0:HD] = (x[HM:TM, 0:HD] + ao[HM:TM, 0:HD] + y21).astype(o_ref.dtype)
        o_ref[HM:TM, HD:D] = (x[HM:TM, HD:D] + ao[HM:TM, HD:D] + y22).astype(o_ref.dtype)


@jax.jit
def pallas_parallel_sum__sliding_local_dilated__glu_gated_bilinear__prompt_kernel(
    A_x: jax.Array,
    A_wqkv: jax.Array,
    A_wo: jax.Array,
    B_x: jax.Array,
    B_w_gate: jax.Array,
    B_w_up: jax.Array,
    B_w_down: jax.Array,
):
    del B_x
    x = A_x.reshape(S, D)
    hbm = pl.BlockSpec(memory_space=pl.ANY)
    out = pl.pallas_call(
        _kernel,
        grid=(NSTEPS,),
        in_specs=[hbm] * 6,
        out_specs=pl.BlockSpec((TM, D), lambda s: (jnp.maximum(s - NB, 0), 0)),
        out_shape=jax.ShapeDtypeStruct((S, D), A_x.dtype),
        scratch_shapes=[
            pltpu.VMEM((S, D), BF),
            pltpu.VMEM((D, 3 * D), BF),
            pltpu.VMEM((D, D), BF),
            pltpu.VMEM((NCH, D, 2 * FC), BF),
            pltpu.VMEM((NCH, D, 2 * FC), BF),
            pltpu.VMEM((NCH, 2 * FC, D), BF),
            pltpu.VMEM((NCH, 5, HD, FC), BF),
            pltpu.VMEM((NCH, 5, HD, FC), BF),
            pltpu.VMEM((NCH, 5, FC, HD), BF),
            pltpu.VMEM((TM, D), BF),
            pltpu.VMEM((NB, 7, HM, HD), BF),
            pltpu.VMEM((NG, S, 128), F32),
            pltpu.VMEM((NG, S + HALO, 128), F32),
            pltpu.VMEM((NG, S + HALO, 128), F32),
            pltpu.VMEM((TM, D), BF),
            pltpu.SemaphoreType.DMA((NB,)),
            pltpu.SemaphoreType.DMA((4,)),
            pltpu.SemaphoreType.DMA((NCH, 6)),
        ],
        compiler_params=pltpu.CompilerParams(
            dimension_semantics=("arbitrary",),
            vmem_limit_bytes=124 * 1024 * 1024,
        ),
        name="fused_attn_ffn",
    )(x, A_wqkv, A_wo, B_w_gate, B_w_up, B_w_down)
    return out.reshape(A_x.shape)
```

```python
import functools

import jax
import jax.numpy as jnp
from jax import lax
from jax.experimental import pallas as pl
from jax.experimental.pallas import tpu as pltpu

S, D, F = 2048, 1024, 3584
H, DH, WIN, DIL = 32, 32, 8, 2
TM = 256
HM = TM // 2
NB = S // TM
HD = D // 2
FC = 256
NCH = F // 2 // FC
HALO = 16
NG = D // 128
EPS = 1e-5
NEG = -1e9
BF = jnp.bfloat16
F32 = jnp.float32
LOG2E = 1.4426950408889634
NSTEPS = 16


def _at(step):
    return min(step, NSTEPS - 1)


def _dot(a, b):
    return jnp.dot(a, b, preferred_element_type=F32)


def _butterfly(vs):
    lane = lax.broadcasted_iota(jnp.int32, vs[0].shape, 1)
    for b in range(3):
        sh = 4 << b
        bit = (lane & sh) != 0
        new = list(vs)
        for i0 in range(NG):
            if i0 & (1 << b):
                continue
            i1 = i0 | (1 << b)
            new[i0] = jnp.where(bit, pltpu.roll(vs[i1], sh, 1), vs[i0])
            new[i1] = jnp.where(bit, vs[i1], pltpu.roll(vs[i0], 128 - sh, 1))
        vs = new
    return vs


def _sum4(x):
    lane = lax.broadcasted_iota(jnp.int32, x.shape, 1)
    x = x + jnp.where((lane & 1) != 0, pltpu.roll(x, 1, 1), pltpu.roll(x, 127, 1))
    x = x + jnp.where((lane & 2) != 0, pltpu.roll(x, 2, 1), pltpu.roll(x, 126, 1))
    return x


def _dep32(x, tok, never):
    return jnp.where(never, pltpu.bitcast(tok, x.dtype), x)


def _gate(m, tok, never):
    t = pltpu.bitcast(m[0:16, 0:128], F32)
    t = pltpu.bitcast(_dep32(t, tok, never), BF)
    top = jnp.concatenate([t, m[0:16, 128:]], axis=1)
    return jnp.concatenate([top, m[16:]], axis=0)


def _lhs_combos(a11, a12, a21, a22):
    return [a11 + a22, a21 + a22, a11, a22, a11 + a12, a21 - a11, a12 - a22]


def _strassen_out(m):
    return (m[0] + m[3] - m[4] + m[6], m[2] + m[4], m[1] + m[3], m[0] - m[1] + m[2] + m[5])


def _layernorm(x):
    x = x.astype(F32)
    mean = jnp.mean(x, axis=-1, keepdims=True)
    xc = x - mean
    var = jnp.mean(xc * xc, axis=-1, keepdims=True)
    return xc * lax.rsqrt(var + EPS)


def _kernel(x_hbm, wqkv_hbm, wo_hbm, wg_hbm, wu_hbm, wd_hbm, o_ref,
            x_scr, wqkv, wo, rawg, rawu, rawd, cg, cu, cd,
            xn_scr, s_scr, q_scr, k_scr, v_scr, o_scr,
            sem_x, sem_w, sem_raw):
    s = pl.program_id(0)

    def x_copy(b):
        return pltpu.make_async_copy(x_hbm.at[pl.ds(b * TM, TM), :], x_scr.at[pl.ds(b * TM, TM), :], sem_x.at[b])

    def wqkv_copy(j):
        return pltpu.make_async_copy(wqkv_hbm.at[:, pl.ds(j * D, D)], wqkv.at[:, pl.ds(j * D, D)], sem_w.at[j])

    def wo_copy():
        return pltpu.make_async_copy(wo_hbm, wo, sem_w.at[3])

    def raw_copies(c):
        return [
            pltpu.make_async_copy(wg_hbm.at[:, pl.ds(c * FC, FC)], rawg.at[c, :, pl.ds(0, FC)], sem_raw.at[c, 0]),
            pltpu.make_async_copy(wg_hbm.at[:, pl.ds(F // 2 + c * FC, FC)], rawg.at[c, :, pl.ds(FC, FC)], sem_raw.at[c, 1]),
            pltpu.make_async_copy(wu_hbm.at[:, pl.ds(c * FC, FC)], rawu.at[c, :, pl.ds(0, FC)], sem_raw.at[c, 2]),
            pltpu.make_async_copy(wu_hbm.at[:, pl.ds(F // 2 + c * FC, FC)], rawu.at[c, :, pl.ds(FC, FC)], sem_raw.at[c, 3]),
            pltpu.make_async_copy(wd_hbm.at[pl.ds(c * FC, FC), :], rawd.at[c, pl.ds(0, FC), :], sem_raw.at[c, 4]),
            pltpu.make_async_copy(wd_hbm.at[pl.ds(F // 2 + c * FC, FC), :], rawd.at[c, pl.ds(FC, FC), :], sem_raw.at[c, 5]),
        ]

    def ln_block(b):
        r0 = pl.multiple_of(b * TM, TM)
        RC = 16
        for r in range(0, HM, RC):
            top = _layernorm(x_scr[pl.ds(r0 + r, RC), :])
            bot = _layernorm(x_scr[pl.ds(r0 + HM + r, RC), :])
            xn_scr[r:r + RC, :] = top.astype(BF)
            xn_scr[HM + r:HM + r + RC, :] = bot.astype(BF)
            cs = _lhs_combos(top[:, :HD], top[:, HD:], bot[:, :HD], bot[:, HD:])
            for j in range(7):
                s_scr[b, j, r:r + RC, :] = cs[j].astype(BF)

    @pl.when(s == 0)
    def _():
        x_copy(0).start()
        wqkv_copy(0).start()
        x_copy(1).start()
        wqkv_copy(1).start()
        wqkv_copy(2).start()
        for c in range(2):
            for cp in raw_copies(c):
                cp.start(priority=1)
        x_copy(2).start()
        k_scr[:, 0:HALO, :] = jnp.zeros((NG, HALO, 128), F32)
        v_scr[:, 0:HALO, :] = jnp.zeros((NG, HALO, 128), F32)
        x_copy(0).wait()
        ln_block(0)
        x_copy(1).wait()
        for j in range(3):
            wqkv_copy(j).wait()

    @pl.when(s == _at(1))
    def _():
        for b in range(3, NB):
            x_copy(b).start()
        for c in range(2, NCH):
            for cp in raw_copies(c):
                cp.start(priority=1)
        wo_copy().start(priority=1)

    for c in range(NCH):
        @pl.when(s == _at(c + 1))
        def _():
            for cp in raw_copies(c):
                cp.wait()
            if c + 2 < NB:
                x_copy(c + 2).wait()

    @pl.when(s == _at(NB))
    def _():
        wo_copy().wait()

    @pl.when(s < NB)
    def _():
        xn = xn_scr[...]
        ln_block(jnp.minimum(s + 1, NB - 1))
        r0 = pl.multiple_of(s * TM, TM)
        RC = 16
        for sec, (dst, off) in enumerate(((q_scr, 0), (k_scr, HALO), (v_scr, HALO))):
            y = _dot(xn, wqkv[:, sec * D:(sec + 1) * D])
            for r in range(0, TM, RC):
                vs = _butterfly([y[r:r + RC, g * 128:(g + 1) * 128] for g in range(NG)])
                for g in range(NG):
                    dst[g, pl.ds(r0 + off + r, RC), :] = vs[g]
        c = lax.rem(s + (NCH - 1), NCH)

        def build(raw, cmb, kq, nq):
            RB = 16
            for r in range(0, kq, RB):
                b11 = raw[c, r:r + RB, 0:nq].astype(F32)
                b12 = raw[c, r:r + RB, nq:2 * nq].astype(F32)
                b21 = raw[c, kq + r:kq + r + RB, 0:nq].astype(F32)
                b22 = raw[c, kq + r:kq + r + RB, nq:2 * nq].astype(F32)
                cmb[c, 0, r:r + RB, :] = (b11 + b22).astype(BF)
                cmb[c, 1, r:r + RB, :] = (b12 - b22).astype(BF)
                cmb[c, 2, r:r + RB, :] = (b21 - b11).astype(BF)
                cmb[c, 3, r:r + RB, :] = (b11 + b12).astype(BF)
                cmb[c, 4, r:r + RB, :] = (b21 + b22).astype(BF)

        build(rawg, cg, HD, FC)
        build(rawu, cu, HD, FC)
        build(rawd, cd, FC, HD)

    @pl.when(s >= NB)
    def _():
        i = s - NB
        r0 = pl.multiple_of(i * TM, TM)

        def wlist(raw, cmb, c, kq, nq):
            return [cmb[c, 0], raw[c, 0:kq, 0:nq], cmb[c, 1], cmb[c, 2],
                    raw[c, kq:2 * kq, nq:2 * nq], cmb[c, 3], cmb[c, 4]]

        RA = 8
        cexp = (DH ** -0.5) * LOG2E

        never = lax.broadcasted_iota(jnp.int32, (8, 128), 0) < jnp.minimum(s, 0)

        def attn_rows(r, tok):
            q = [q_scr[g, pl.ds(r0 + r, RA), :] for g in range(NG)]
            if tok is not None:
                q = [_dep32(t, tok, never) for t in q]
            sw = []
            for w in range(WIN):
                acc = None
                for g in range(NG):
                    t = q[g] * k_scr[g, pl.ds(r0 + r + HALO - DIL * w, RA), :]
                    acc = t if acc is None else acc + t
                acc = _sum4(acc)
                if r < HALO and w > 0:
                    row = lax.broadcasted_iota(jnp.int32, (RA, 128), 0) + (r0 + r)
                    acc = jnp.where(row >= DIL * w, acc, NEG)
                sw.append(acc)
            m = sw[0]
            for w in range(1, WIN):
                m = jnp.maximum(m, sw[w])
            e = [jnp.exp2((sw[w] - m) * cexp) for w in range(WIN)]
            den = e[0]
            for w in range(1, WIN):
                den = den + e[w]
            inv = 1.0 / den
            p = [e[w] * inv for w in range(WIN)]
            o = []
            for g in range(NG):
                acc = None
                for w in range(WIN):
                    t = p[w] * v_scr[g, pl.ds(r0 + r + HALO - DIL * w, RA), :]
                    acc = t if acc is None else acc + t
                o.append(acc)
            o = _butterfly(o)
            return jnp.concatenate(o, axis=1), o[0]

        sl = [s_scr[i, j] for j in range(7)]
        acc = [None] * 7
        o_parts = []
        n_att = TM // RA
        per = 6
        tok = None
        for c in range(NCH):
            wg_l = wlist(rawg, cg, c, HD, FC)
            wu_l = wlist(rawu, cu, c, HD, FC)
            wd_l = wlist(rawd, cd, c, FC, HD)
            slc = sl
            g = _strassen_out([_dot(slc[j], wg_l[j]) for j in range(7)])
            u = _strassen_out([_dot(slc[j], wu_l[j]) for j in range(7)])
            hq = [g[t] * u[t] for t in range(4)]
            hl = [t.astype(BF) for t in _lhs_combos(*hq)]
            for j in range(7):
                y = _dot(hl[j], wd_l[j])
                acc[j] = y if acc[j] is None else acc[j] + y
            for a in range(c * per, min((c + 1) * per, n_att), 2):
                oa, tok = attn_rows(a * RA, tok)
                ob, tok = attn_rows((a + 1) * RA, tok)
                o2 = jnp.concatenate([oa, ob], axis=0)
                o_scr[a * RA:(a + 2) * RA, :] = o2.astype(BF)
        ao = _dot(o_scr[...], wo[...])
        y11, y12, y21, y22 = _strassen_out(acc)
        x = x_scr[pl.ds(r0, TM), :].astype(F32)
        o_ref[0:HM, 0:HD] = (x[0:HM, 0:HD] + ao[0:HM, 0:HD] + y11).astype(o_ref.dtype)
        o_ref[0:HM, HD:D] = (x[0:HM, HD:D] + ao[0:HM, HD:D] + y12).astype(o_ref.dtype)
        o_ref[HM:TM, 0:HD] = (x[HM:TM, 0:HD] + ao[HM:TM, 0:HD] + y21).astype(o_ref.dtype)
        o_ref[HM:TM, HD:D] = (x[HM:TM, HD:D] + ao[HM:TM, HD:D] + y22).astype(o_ref.dtype)


@jax.jit
def pallas_parallel_sum__sliding_local_dilated__glu_gated_bilinear__prompt_kernel(
    A_x: jax.Array,
    A_wqkv: jax.Array,
    A_wo: jax.Array,
    B_x: jax.Array,
    B_w_gate: jax.Array,
    B_w_up: jax.Array,
    B_w_down: jax.Array,
):
    del B_x
    x = A_x.reshape(S, D)
    hbm = pl.BlockSpec(memory_space=pl.ANY)
    out = pl.pallas_call(
        _kernel,
        grid=(NSTEPS,),
        in_specs=[hbm] * 6,
        out_specs=pl.BlockSpec((TM, D), lambda s: (jnp.maximum(s - NB, 0), 0)),
        out_shape=jax.ShapeDtypeStruct((S, D), A_x.dtype),
        scratch_shapes=[
            pltpu.VMEM((S, D), BF),
            pltpu.VMEM((D, 3 * D), BF),
            pltpu.VMEM((D, D), BF),
            pltpu.VMEM((NCH, D, 2 * FC), BF),
            pltpu.VMEM((NCH, D, 2 * FC), BF),
            pltpu.VMEM((NCH, 2 * FC, D), BF),
            pltpu.VMEM((NCH, 5, HD, FC), BF),
            pltpu.VMEM((NCH, 5, HD, FC), BF),
            pltpu.VMEM((NCH, 5, FC, HD), BF),
            pltpu.VMEM((TM, D), BF),
            pltpu.VMEM((NB, 7, HM, HD), BF),
            pltpu.VMEM((NG, S, 128), F32),
            pltpu.VMEM((NG, S + HALO, 128), F32),
            pltpu.VMEM((NG, S + HALO, 128), F32),
            pltpu.VMEM((TM, D), BF),
            pltpu.SemaphoreType.DMA((NB,)),
            pltpu.SemaphoreType.DMA((4,)),
            pltpu.SemaphoreType.DMA((NCH, 6)),
        ],
        compiler_params=pltpu.CompilerParams(
            dimension_semantics=("arbitrary",),
            vmem_limit_bytes=124 * 1024 * 1024,
        ),
        name="fused_attn_ffn",
    )(x, A_wqkv, A_wo, B_w_gate, B_w_up, B_w_down)
    return out.reshape(A_x.shape)
```

```python
import functools

import jax
import jax.numpy as jnp
from jax import lax
from jax.experimental import pallas as pl
from jax.experimental.pallas import tpu as pltpu

S, D, F = 2048, 1024, 3584
H, DH, WIN, DIL = 32, 32, 8, 2
TM = 256
HM = TM // 2
NB = S // TM
HD = D // 2
FC = 256
NCH = F // 2 // FC
HALO = 16
NG = D // 128
EPS = 1e-5
NEG = -1e9
BF = jnp.bfloat16
F32 = jnp.float32
LOG2E = 1.4426950408889634
NSTEPS = 16
ROLL_EVERY = 3
LN_FIRST = False


def _at(step):
    return min(step, NSTEPS - 1)


def _dot(a, b):
    return jnp.dot(a, b, preferred_element_type=F32)


def _butterfly(vs):
    lane = lax.broadcasted_iota(jnp.int32, vs[0].shape, 1)
    for b in range(3):
        sh = 4 << b
        bit = (lane & sh) != 0
        new = list(vs)
        for i0 in range(NG):
            if i0 & (1 << b):
                continue
            i1 = i0 | (1 << b)
            new[i0] = jnp.where(bit, pltpu.roll(vs[i1], sh, 1), vs[i0])
            new[i1] = jnp.where(bit, vs[i1], pltpu.roll(vs[i0], 128 - sh, 1))
        vs = new
    return vs


def _sum4(x):
    lane = lax.broadcasted_iota(jnp.int32, x.shape, 1)
    x = x + jnp.where((lane & 1) != 0, pltpu.roll(x, 1, 1), pltpu.roll(x, 127, 1))
    x = x + jnp.where((lane & 2) != 0, pltpu.roll(x, 2, 1), pltpu.roll(x, 126, 1))
    return x


def _dep32(x, tok, never):
    return jnp.where(never, pltpu.bitcast(tok, x.dtype), x)


def _gate(m, tok, never):
    t = pltpu.bitcast(m[0:16, 0:128], F32)
    t = pltpu.bitcast(_dep32(t, tok, never), BF)
    top = jnp.concatenate([t, m[0:16, 128:]], axis=1)
    if m.shape[0] == 16:
        return top
    return jnp.concatenate([top, m[16:]], axis=0)


def _lhs_combos(a11, a12, a21, a22):
    return [a11 + a22, a21 + a22, a11, a22, a11 + a12, a21 - a11, a12 - a22]


def _strassen_out(m):
    return (m[0] + m[3] - m[4] + m[6], m[2] + m[4], m[1] + m[3], m[0] - m[1] + m[2] + m[5])


def _layernorm(x):
    x = x.astype(F32)
    mean = jnp.mean(x, axis=-1, keepdims=True)
    xc = x - mean
    var = jnp.mean(xc * xc, axis=-1, keepdims=True)
    return xc * lax.rsqrt(var + EPS)


def _kernel(x_hbm, wqkv_hbm, wo_hbm, wg_hbm, wu_hbm, wd_hbm, o_ref,
            x_scr, wqkv, wo, rawg, rawu, rawd, cg, cu, cd,
            xn_scr, s_scr, q_scr, k_scr, v_scr, o_scr,
            sem_x, sem_w, sem_raw):
    s = pl.program_id(0)

    def x_copy(b):
        return pltpu.make_async_copy(x_hbm.at[pl.ds(b * TM, TM), :], x_scr.at[pl.ds(b * TM, TM), :], sem_x.at[b])

    def wqkv_copy(j):
        return pltpu.make_async_copy(wqkv_hbm.at[:, pl.ds(j * D, D)], wqkv.at[:, pl.ds(j * D, D)], sem_w.at[j])

    def wo_copy():
        return pltpu.make_async_copy(wo_hbm, wo, sem_w.at[3])

    def raw_copies(c):
        return [
            pltpu.make_async_copy(wg_hbm.at[:, pl.ds(c * FC, FC)], rawg.at[c, :, pl.ds(0, FC)], sem_raw.at[c, 0]),
            pltpu.make_async_copy(wg_hbm.at[:, pl.ds(F // 2 + c * FC, FC)], rawg.at[c, :, pl.ds(FC, FC)], sem_raw.at[c, 1]),
            pltpu.make_async_copy(wu_hbm.at[:, pl.ds(c * FC, FC)], rawu.at[c, :, pl.ds(0, FC)], sem_raw.at[c, 2]),
            pltpu.make_async_copy(wu_hbm.at[:, pl.ds(F // 2 + c * FC, FC)], rawu.at[c, :, pl.ds(FC, FC)], sem_raw.at[c, 3]),
            pltpu.make_async_copy(wd_hbm.at[pl.ds(c * FC, FC), :], rawd.at[c, pl.ds(0, FC), :], sem_raw.at[c, 4]),
            pltpu.make_async_copy(wd_hbm.at[pl.ds(F // 2 + c * FC, FC), :], rawd.at[c, pl.ds(FC, FC), :], sem_raw.at[c, 5]),
        ]

    never = lax.broadcasted_iota(jnp.int32, (8, 128), 0) < jnp.minimum(s, 0)

    def ln_block(b, chain=False):
        r0 = pl.multiple_of(b * TM, TM)
        RC = 16
        tok = None
        for r in range(0, HM, RC):
            xt = x_scr[pl.ds(r0 + r, RC), :]
            xb = x_scr[pl.ds(r0 + HM + r, RC), :]
            if tok is not None:
                xt = _gate(xt, tok, never)
                xb = _gate(xb, tok, never)
            top = _layernorm(xt)
            bot = _layernorm(xb)
            if chain:
                tok = top[0:8, 0:128] + bot[0:8, 0:128]
            xn_scr[r:r + RC, :] = top.astype(BF)
            xn_scr[HM + r:HM + r + RC, :] = bot.astype(BF)
            cs = _lhs_combos(top[:, :HD], top[:, HD:], bot[:, :HD], bot[:, HD:])
            for j in range(7):
                s_scr[b, j, r:r + RC, :] = cs[j].astype(BF)
        return tok

    @pl.when(s == 0)
    def _():
        x_copy(0).start()
        wqkv_copy(0).start()
        x_copy(1).start()
        wqkv_copy(1).start()
        wqkv_copy(2).start()
        for c in range(2):
            for cp in raw_copies(c):
                cp.start(priority=1)
        x_copy(2).start()
        k_scr[:, 0:HALO, :] = jnp.zeros((NG, HALO, 128), F32)
        v_scr[:, 0:HALO, :] = jnp.zeros((NG, HALO, 128), F32)
        x_copy(0).wait()
        ln_block(0)
        x_copy(1).wait()
        for j in range(3):
            wqkv_copy(j).wait()

    @pl.when(s == _at(1))
    def _():
        for b in range(3, NB):
            x_copy(b).start()
        for c in range(2, NCH):
            for cp in raw_copies(c):
                cp.start(priority=1)
        wo_copy().start(priority=1)

    for c in range(NCH):
        @pl.when(s == _at(c + 1))
        def _():
            for cp in raw_copies(c):
                cp.wait()
            if c + 2 < NB:
                x_copy(c + 2).wait()

    @pl.when(s == _at(NB))
    def _():
        wo_copy().wait()

    @pl.when(s < NB)
    def _():
        xn = xn_scr[...]
        r0 = pl.multiple_of(s * TM, TM)
        RC = 16
        ys = [_dot(xn, wqkv[:, sec * D:(sec + 1) * D]) for sec in (1, 2, 0)]
        tok = ln_block(jnp.minimum(s + 1, NB - 1), chain=True)
        c = lax.rem(s + (NCH - 1), NCH)
        never4 = lax.broadcasted_iota(jnp.int32, (4, 128), 0) < jnp.minimum(s, 0)

        def build(raw, cmb, kq, nq, tok):
            def ld(r, n, tok4):
                t = pltpu.bitcast(raw[c, r:r + 8, n:n + 128], F32)
                return pltpu.bitcast(_dep32(t, tok4, never4), BF).astype(F32)

            for r in range(0, kq, 16):
                for n0 in range(0, nq, 128):
                    cnt[0] += 1
                    if cnt[0] % ROLL_EVERY == 0:
                        tok = pltpu.roll(tok, 1, 1)
                    tok4 = tok[0:4]
                    b11, b12, b21, b22 = [
                        jnp.concatenate([ld(rr, nn, tok4), ld(rr + 8, nn, tok4)], axis=0)
                        for rr, nn in ((r, n0), (r, nq + n0), (kq + r, n0), (kq + r, nq + n0))]
                    outs = [(b11 + b22).astype(BF), (b12 - b22).astype(BF), (b21 - b11).astype(BF),
                            (b11 + b12).astype(BF), (b21 + b22).astype(BF)]
                    for j in range(5):
                        cmb[c, j, r:r + 16, n0:n0 + 128] = outs[j]
                    tok = pltpu.bitcast(outs[0], F32)
            return tok

        cnt = [0]
        if not LN_FIRST:
            tok = jnp.zeros((8, 128), F32)
        tok = build(rawg, cg, HD, FC, tok)
        tok = build(rawu, cu, HD, FC, tok)
        tok = build(rawd, cd, FC, HD, tok)
        for y, dst in ((ys[0], k_scr), (ys[1], v_scr)):
            for r in range(0, TM, RC):
                vs = _butterfly([y[r:r + RC, g * 128:(g + 1) * 128] for g in range(NG)])
                for g in range(NG):
                    dst[g, pl.ds(r0 + HALO + r, RC), :] = vs[g]
        for g in range(NG):
            q_scr[g, pl.ds(r0, TM), :] = ys[2][:, g * 128:(g + 1) * 128]

    @pl.when(s >= NB)
    def _():
        i = s - NB
        r0 = pl.multiple_of(i * TM, TM)

        def wlist(raw, cmb, c, kq, nq):
            return [cmb[c, 0], raw[c, 0:kq, 0:nq], cmb[c, 1], cmb[c, 2],
                    raw[c, kq:2 * kq, nq:2 * nq], cmb[c, 3], cmb[c, 4]]

        RA = 8
        cexp = (DH ** -0.5) * LOG2E

        def attn_rows(r, tok):
            q = [q_scr[g, pl.ds(r0 + r, RA), :] for g in range(NG)]
            if tok is not None:
                q = [_dep32(t, tok, never) for t in q]
            q = _butterfly(q)
            sw = []
            for w in range(WIN):
                acc = None
                for g in range(NG):
                    t = q[g] * k_scr[g, pl.ds(r0 + r + HALO - DIL * w, RA), :]
                    acc = t if acc is None else acc + t
                acc = _sum4(acc)
                if r < HALO and w > 0:
                    row = lax.broadcasted_iota(jnp.int32, (RA, 128), 0) + (r0 + r)
                    acc = jnp.where(row >= DIL * w, acc, NEG)
                sw.append(acc)
            m = sw[0]
            for w in range(1, WIN):
                m = jnp.maximum(m, sw[w])
            e = [jnp.exp2((sw[w] - m) * cexp) for w in range(WIN)]
            den = e[0]
            for w in range(1, WIN):
                den = den + e[w]
            inv = 1.0 / den
            p = [e[w] * inv for w in range(WIN)]
            o = []
            for g in range(NG):
                acc = None
                for w in range(WIN):
                    t = p[w] * v_scr[g, pl.ds(r0 + r + HALO - DIL * w, RA), :]
                    acc = t if acc is None else acc + t
                o.append(acc)
            o = _butterfly(o)
            return jnp.concatenate(o, axis=1), o[0]

        sl = [s_scr[i, j] for j in range(7)]
        acc = [None] * 7
        o_parts = []
        n_att = TM // RA
        per = 6
        tok = None
        for c in range(NCH):
            wg_l = wlist(rawg, cg, c, HD, FC)
            wu_l = wlist(rawu, cu, c, HD, FC)
            wd_l = wlist(rawd, cd, c, FC, HD)
            slc = sl
            g = _strassen_out([_dot(slc[j], wg_l[j]) for j in range(7)])
            u = _strassen_out([_dot(slc[j], wu_l[j]) for j in range(7)])
            hq = [g[t] * u[t] for t in range(4)]
            hl = [t.astype(BF) for t in _lhs_combos(*hq)]
            for j in range(7):
                y = _dot(hl[j], wd_l[j])
                acc[j] = y if acc[j] is None else acc[j] + y
            for a in range(c * per, min((c + 1) * per, n_att), 2):
                oa, tok = attn_rows(a * RA, tok)
                ob, tok = attn_rows((a + 1) * RA, tok)
                o2 = jnp.concatenate([oa, ob], axis=0)
                o_scr[a * RA:(a + 2) * RA, :] = o2.astype(BF)
        ao = _dot(o_scr[...], wo[...])
        y11, y12, y21, y22 = _strassen_out(acc)
        x = x_scr[pl.ds(r0, TM), :].astype(F32)
        o_ref[0:HM, 0:HD] = (x[0:HM, 0:HD] + ao[0:HM, 0:HD] + y11).astype(o_ref.dtype)
        o_ref[0:HM, HD:D] = (x[0:HM, HD:D] + ao[0:HM, HD:D] + y12).astype(o_ref.dtype)
        o_ref[HM:TM, 0:HD] = (x[HM:TM, 0:HD] + ao[HM:TM, 0:HD] + y21).astype(o_ref.dtype)
        o_ref[HM:TM, HD:D] = (x[HM:TM, HD:D] + ao[HM:TM, HD:D] + y22).astype(o_ref.dtype)


@jax.jit
def pallas_parallel_sum__sliding_local_dilated__glu_gated_bilinear__prompt_kernel(
    A_x: jax.Array,
    A_wqkv: jax.Array,
    A_wo: jax.Array,
    B_x: jax.Array,
    B_w_gate: jax.Array,
    B_w_up: jax.Array,
    B_w_down: jax.Array,
):
    del B_x
    x = A_x.reshape(S, D)
    hbm = pl.BlockSpec(memory_space=pl.ANY)
    out = pl.pallas_call(
        _kernel,
        grid=(NSTEPS,),
        in_specs=[hbm] * 6,
        out_specs=pl.BlockSpec((TM, D), lambda s: (jnp.maximum(s - NB, 0), 0)),
        out_shape=jax.ShapeDtypeStruct((S, D), A_x.dtype),
        scratch_shapes=[
            pltpu.VMEM((S, D), BF),
            pltpu.VMEM((D, 3 * D), BF),
            pltpu.VMEM((D, D), BF),
            pltpu.VMEM((NCH, D, 2 * FC), BF),
            pltpu.VMEM((NCH, D, 2 * FC), BF),
            pltpu.VMEM((NCH, 2 * FC, D), BF),
            pltpu.VMEM((NCH, 5, HD, FC), BF),
            pltpu.VMEM((NCH, 5, HD, FC), BF),
            pltpu.VMEM((NCH, 5, FC, HD), BF),
            pltpu.VMEM((TM, D), BF),
            pltpu.VMEM((NB, 7, HM, HD), BF),
            pltpu.VMEM((NG, S, 128), F32),
            pltpu.VMEM((NG, S + HALO, 128), F32),
            pltpu.VMEM((NG, S + HALO, 128), F32),
            pltpu.VMEM((TM, D), BF),
            pltpu.SemaphoreType.DMA((NB,)),
            pltpu.SemaphoreType.DMA((4,)),
            pltpu.SemaphoreType.DMA((NCH, 6)),
        ],
        compiler_params=pltpu.CompilerParams(
            dimension_semantics=("arbitrary",),
            vmem_limit_bytes=124 * 1024 * 1024,
        ),
        name="fused_attn_ffn",
    )(x, A_wqkv, A_wo, B_w_gate, B_w_up, B_w_down)
    return out.reshape(A_x.shape)
```

```python
import functools

import jax
import jax.numpy as jnp
from jax import lax
from jax.experimental import pallas as pl
from jax.experimental.pallas import tpu as pltpu

S, D, F = 2048, 1024, 3584
H, DH, WIN, DIL = 32, 32, 8, 2
TM = 256
HM = TM // 2
NB = S // TM
HD = D // 2
FC = 256
NCH = F // 2 // FC
HALO = 16
NG = D // 128
EPS = 1e-5
NEG = -1e9
BF = jnp.bfloat16
F32 = jnp.float32
LOG2E = 1.4426950408889634
NSTEPS = 16
WC = 512
NWC = 3 * D // WC
ROLL_EVERY = 3
LN_FIRST = False


def _dot(a, b):
    return jnp.dot(a, b, preferred_element_type=F32)


def _butterfly(vs):
    lane = lax.broadcasted_iota(jnp.int32, vs[0].shape, 1)
    for b in range(3):
        sh = 4 << b
        bit = (lane & sh) != 0
        new = list(vs)
        for i0 in range(NG):
            if i0 & (1 << b):
                continue
            i1 = i0 | (1 << b)
            new[i0] = jnp.where(bit, pltpu.roll(vs[i1], sh, 1), vs[i0])
            new[i1] = jnp.where(bit, vs[i1], pltpu.roll(vs[i0], 128 - sh, 1))
        vs = new
    return vs


def _sum4(x):
    lane = lax.broadcasted_iota(jnp.int32, x.shape, 1)
    x = x + jnp.where((lane & 1) != 0, pltpu.roll(x, 1, 1), pltpu.roll(x, 127, 1))
    x = x + jnp.where((lane & 2) != 0, pltpu.roll(x, 2, 1), pltpu.roll(x, 126, 1))
    return x


def _dep32(x, tok, never):
    return jnp.where(never, pltpu.bitcast(tok, x.dtype), x)


def _gate(m, tok, never):
    t = pltpu.bitcast(m[0:16, 0:128], F32)
    t = pltpu.bitcast(_dep32(t, tok, never), BF)
    top = jnp.concatenate([t, m[0:16, 128:]], axis=1)
    if m.shape[0] == 16:
        return top
    return jnp.concatenate([top, m[16:]], axis=0)


def _lhs_combos(a11, a12, a21, a22):
    return [a11 + a22, a21 + a22, a11, a22, a11 + a12, a21 - a11, a12 - a22]


def _strassen_out(m):
    return (m[0] + m[3] - m[4] + m[6], m[2] + m[4], m[1] + m[3], m[0] - m[1] + m[2] + m[5])


def _layernorm(x):
    x = x.astype(F32)
    mean = jnp.mean(x, axis=-1, keepdims=True)
    xc = x - mean
    var = jnp.mean(xc * xc, axis=-1, keepdims=True)
    return xc * lax.rsqrt(var + EPS)


def _kernel(x_hbm, wqkv_hbm, wo_hbm, wg_hbm, wu_hbm, wd_hbm, o_ref,
            x_scr, wqkv, wo, rawg, rawu, rawd, cg, cu, cd,
            xn_scr, s_scr, q_scr, kv_scr, o_scr,
            sem_x, sem_w, sem_raw):
    s = pl.program_id(0)
    k_scr = kv_scr.at[0]
    v_scr = kv_scr.at[1]

    def x_copy(b):
        return pltpu.make_async_copy(x_hbm.at[pl.ds(b * TM, TM), :], x_scr.at[pl.ds(b * TM, TM), :], sem_x.at[b])

    def wqkv_copy(k):
        return pltpu.make_async_copy(wqkv_hbm.at[:, pl.ds(k * WC, WC)], wqkv.at[k], sem_w.at[k])

    def wo_copy():
        return pltpu.make_async_copy(wo_hbm, wo, sem_w.at[NWC])

    def raw_copies(c):
        return [
            pltpu.make_async_copy(wg_hbm.at[:, pl.ds(c * FC, FC)], rawg.at[c, :, pl.ds(0, FC)], sem_raw.at[c, 0]),
            pltpu.make_async_copy(wg_hbm.at[:, pl.ds(F // 2 + c * FC, FC)], rawg.at[c, :, pl.ds(FC, FC)], sem_raw.at[c, 1]),
            pltpu.make_async_copy(wu_hbm.at[:, pl.ds(c * FC, FC)], rawu.at[c, :, pl.ds(0, FC)], sem_raw.at[c, 2]),
            pltpu.make_async_copy(wu_hbm.at[:, pl.ds(F // 2 + c * FC, FC)], rawu.at[c, :, pl.ds(FC, FC)], sem_raw.at[c, 3]),
            pltpu.make_async_copy(wd_hbm.at[pl.ds(c * FC, FC), :], rawd.at[c, pl.ds(0, FC), :], sem_raw.at[c, 4]),
            pltpu.make_async_copy(wd_hbm.at[pl.ds(F // 2 + c * FC, FC), :], rawd.at[c, pl.ds(FC, FC), :], sem_raw.at[c, 5]),
        ]

    never = lax.broadcasted_iota(jnp.int32, (8, 128), 0) < jnp.minimum(s, 0)

    def ln_unit(b, r, tok):
        RC = 16
        r0 = pl.multiple_of(b * TM + r, RC)
        xt = x_scr[pl.ds(r0, RC), :]
        xb = x_scr[pl.ds(r0 + HM, RC), :]
        if tok is not None:
            xt = _gate(xt, tok, never)
            xb = _gate(xb, tok, never)
        top = _layernorm(xt)
        bot = _layernorm(xb)
        xn_scr[pl.ds(r, RC), :] = top.astype(BF)
        xn_scr[pl.ds(HM + r, RC), :] = bot.astype(BF)
        cs = _lhs_combos(top[:, :HD], top[:, HD:], bot[:, :HD], bot[:, HD:])
        for j in range(7):
            s_scr[b, j, pl.ds(r, RC), :] = cs[j].astype(BF)
        return top[0:8, 0:128] + bot[0:8, 0:128]

    def ln_block(b, chain=False):
        tok = None
        for r in range(0, HM, 16):
            t = ln_unit(b, r, tok)
            tok = t if chain else None
        return tok

    def store_kv(y, dst, r0):
        RC = 16
        for r in range(0, TM, RC):
            vs = _butterfly([y[r:r + RC, g * 128:(g + 1) * 128] for g in range(NG)])
            for g in range(NG):
                dst[g, pl.ds(r0 + HALO + r, RC), :] = vs[g]

    def store_q(y, r0):
        for g in range(NG):
            q_scr[g, pl.ds(r0, TM), :] = y[:, g * 128:(g + 1) * 128]

    @pl.when(s == 0)
    def _():
        x_copy(0).start(priority=1)

        def issue(j, carry):
            @pl.when(j == 1)
            def _():
                x_copy(1).start(priority=1)

            wqkv_copy(lax.rem(j + 2, NWC)).start(priority=1)
            return carry

        lax.fori_loop(0, NWC, issue, 0)
        for cp in raw_copies(0):
            cp.start(priority=1)
        x_copy(2).start(priority=1)
        k_scr[:, 0:HALO, :] = jnp.zeros((NG, HALO, 128), F32)
        v_scr[:, 0:HALO, :] = jnp.zeros((NG, HALO, 128), F32)
        x_copy(0).wait()
        ln_block(0)
        xn = xn_scr[...]

        def body(j, carry):
            k = lax.rem(j + 2, NWC)
            wqkv_copy(k).wait()

            @pl.when(j == 1)
            def _():
                x_copy(1).wait()

            half = lax.rem(j, 2)
            sec = jnp.maximum(lax.div(j, 2) - 1, 0)
            src = pl.multiple_of((sec + 1) * TM + half * HM, HM)
            dstr = pl.multiple_of(HALO + half * HM, 16)
            for r in range(0, HM, 16):
                vs = _butterfly([q_scr[g, pl.ds(src + r, 16), :] for g in range(NG)])
                for g in range(NG):
                    kv_scr[sec, g, pl.ds(dstr + r, 16), :] = vs[g]
            lb = jnp.minimum(j, 1)
            u0 = 2 * jnp.clip(j - 1, 0, 3)
            tok = ln_unit(lb, pl.multiple_of(u0 * 16, 16), None)
            ln_unit(lb, pl.multiple_of(u0 * 16 + 16, 16), tok)
            y = _dot(xn, wqkv[k])
            rb = pl.multiple_of(lax.rem(lax.div(j, 2) + 1, 3) * TM, TM)
            for gg in range(WC // 128):
                q_scr[half * (WC // 128) + gg, pl.ds(rb, TM), :] = y[:, gg * 128:(gg + 1) * 128]
            return carry

        lax.fori_loop(0, NWC, body, 0)

    @pl.when(s < NCH - 1)
    def _():
        for cp in raw_copies(s + 1):
            cp.start(priority=1)

    @pl.when(s < NB - 3)
    def _():
        x_copy(s + 3).start(priority=1)

    @pl.when(s == NCH - 1)
    def _():
        wo_copy().start(priority=1)

    @pl.when(jnp.logical_and(s >= 1, s < NB))
    def _():
        for cp in raw_copies(s - 1):
            cp.wait()

    @pl.when(jnp.logical_and(s >= 1, s < NB - 1))
    def _():
        x_copy(s + 1).wait()

    @pl.when(s == NB)
    def _():
        wo_copy().wait()

    @pl.when(jnp.logical_and(s >= 1, s < NB))
    def _():
        xn = xn_scr[...]
        r0 = pl.multiple_of(s * TM, TM)
        ys = [jnp.concatenate([_dot(xn, wqkv[2 * sec]), _dot(xn, wqkv[2 * sec + 1])], axis=1) for sec in (1, 2, 0)]
        tok = ln_block(jnp.minimum(s + 1, NB - 1), chain=True)
        c = s - 1
        never4 = lax.broadcasted_iota(jnp.int32, (4, 128), 0) < jnp.minimum(s, 0)

        def build(raw, cmb, kq, nq, tok):
            def ld(r, n, tok4):
                t = pltpu.bitcast(raw[c, r:r + 8, n:n + 128], F32)
                return pltpu.bitcast(_dep32(t, tok4, never4), BF).astype(F32)

            for r in range(0, kq, 16):
                for n0 in range(0, nq, 128):
                    cnt[0] += 1
                    if cnt[0] % ROLL_EVERY == 0:
                        tok = pltpu.roll(tok, 1, 1)
                    tok4 = tok[0:4]
                    b11, b12, b21, b22 = [
                        jnp.concatenate([ld(rr, nn, tok4), ld(rr + 8, nn, tok4)], axis=0)
                        for rr, nn in ((r, n0), (r, nq + n0), (kq + r, n0), (kq + r, nq + n0))]
                    outs = [(b11 + b22).astype(BF), (b12 - b22).astype(BF), (b21 - b11).astype(BF),
                            (b11 + b12).astype(BF), (b21 + b22).astype(BF)]
                    for j in range(5):
                        cmb[c, j, r:r + 16, n0:n0 + 128] = outs[j]
                    tok = pltpu.bitcast(outs[0], F32)
            return tok

        cnt = [0]
        if not LN_FIRST:
            tok = jnp.zeros((8, 128), F32)
        tok = build(rawg, cg, HD, FC, tok)
        tok = build(rawu, cu, HD, FC, tok)
        tok = build(rawd, cd, FC, HD, tok)
        store_kv(ys[0], k_scr, r0)
        store_kv(ys[1], v_scr, r0)
        store_q(ys[2], r0)

    if NSTEPS < 2 * NB:
        @pl.when(s == NSTEPS - 1)
        def _():
            l = NSTEPS - 1
            for c in (l, l + 1):
                if c < NCH:
                    for cp in raw_copies(c):
                        cp.wait()
            for b in (l + 2, l + 3):
                if b < NB:
                    x_copy(b).wait()
            if NCH - 1 <= l < NB:
                wo_copy().wait()

    @pl.when(s >= NB)
    def _():
        i = s - NB
        r0 = pl.multiple_of(i * TM, TM)

        def wlist(raw, cmb, c, kq, nq):
            return [cmb[c, 0], raw[c, 0:kq, 0:nq], cmb[c, 1], cmb[c, 2],
                    raw[c, kq:2 * kq, nq:2 * nq], cmb[c, 3], cmb[c, 4]]

        RA = 8
        cexp = (DH ** -0.5) * LOG2E

        def attn_rows(r, tok):
            q = [q_scr[g, pl.ds(r0 + r, RA), :] for g in range(NG)]
            if tok is not None:
                q = [_dep32(t, tok, never) for t in q]
            q = _butterfly(q)
            sw = []
            for w in range(WIN):
                acc = None
                for g in range(NG):
                    t = q[g] * k_scr[g, pl.ds(r0 + r + HALO - DIL * w, RA), :]
                    acc = t if acc is None else acc + t
                acc = _sum4(acc)
                if r < HALO and w > 0:
                    row = lax.broadcasted_iota(jnp.int32, (RA, 128), 0) + (r0 + r)
                    acc = jnp.where(row >= DIL * w, acc, NEG)
                sw.append(acc)
            m = sw[0]
            for w in range(1, WIN):
                m = jnp.maximum(m, sw[w])
            e = [jnp.exp2((sw[w] - m) * cexp) for w in range(WIN)]
            den = e[0]
            for w in range(1, WIN):
                den = den + e[w]
            inv = 1.0 / den
            p = [e[w] * inv for w in range(WIN)]
            o = []
            for g in range(NG):
                acc = None
                for w in range(WIN):
                    t = p[w] * v_scr[g, pl.ds(r0 + r + HALO - DIL * w, RA), :]
                    acc = t if acc is None else acc + t
                o.append(acc)
            o = _butterfly(o)
            return jnp.concatenate(o, axis=1), o[0]

        sl = [s_scr[i, j] for j in range(7)]
        acc = [None] * 7
        o_parts = []
        n_att = TM // RA
        per = 6
        tok = None
        for c in range(NCH):
            wg_l = wlist(rawg, cg, c, HD, FC)
            wu_l = wlist(rawu, cu, c, HD, FC)
            wd_l = wlist(rawd, cd, c, FC, HD)
            slc = sl
            g = _strassen_out([_dot(slc[j], wg_l[j]) for j in range(7)])
            u = _strassen_out([_dot(slc[j], wu_l[j]) for j in range(7)])
            hq = [g[t] * u[t] for t in range(4)]
            hl = [t.astype(BF) for t in _lhs_combos(*hq)]
            for j in range(7):
                y = _dot(hl[j], wd_l[j])
                acc[j] = y if acc[j] is None else acc[j] + y
            for a in range(c * per, min((c + 1) * per, n_att), 2):
                oa, tok = attn_rows(a * RA, tok)
                ob, tok = attn_rows((a + 1) * RA, tok)
                o2 = jnp.concatenate([oa, ob], axis=0)
                o_scr[a * RA:(a + 2) * RA, :] = o2.astype(BF)
        ao = _dot(o_scr[...], wo[...])
        y11, y12, y21, y22 = _strassen_out(acc)
        x = x_scr[pl.ds(r0, TM), :].astype(F32)
        o_ref[0:HM, 0:HD] = (x[0:HM, 0:HD] + ao[0:HM, 0:HD] + y11).astype(o_ref.dtype)
        o_ref[0:HM, HD:D] = (x[0:HM, HD:D] + ao[0:HM, HD:D] + y12).astype(o_ref.dtype)
        o_ref[HM:TM, 0:HD] = (x[HM:TM, 0:HD] + ao[HM:TM, 0:HD] + y21).astype(o_ref.dtype)
        o_ref[HM:TM, HD:D] = (x[HM:TM, HD:D] + ao[HM:TM, HD:D] + y22).astype(o_ref.dtype)


@jax.jit
def pallas_parallel_sum__sliding_local_dilated__glu_gated_bilinear__prompt_kernel(
    A_x: jax.Array,
    A_wqkv: jax.Array,
    A_wo: jax.Array,
    B_x: jax.Array,
    B_w_gate: jax.Array,
    B_w_up: jax.Array,
    B_w_down: jax.Array,
):
    del B_x
    x = A_x.reshape(S, D)
    hbm = pl.BlockSpec(memory_space=pl.ANY)
    out = pl.pallas_call(
        _kernel,
        grid=(NSTEPS,),
        in_specs=[hbm] * 6,
        out_specs=pl.BlockSpec((TM, D), lambda s: (jnp.maximum(s - NB, 0), 0)),
        out_shape=jax.ShapeDtypeStruct((S, D), A_x.dtype),
        scratch_shapes=[
            pltpu.VMEM((S, D), BF),
            pltpu.VMEM((NWC, D, WC), BF),
            pltpu.VMEM((D, D), BF),
            pltpu.VMEM((NCH, D, 2 * FC), BF),
            pltpu.VMEM((NCH, D, 2 * FC), BF),
            pltpu.VMEM((NCH, 2 * FC, D), BF),
            pltpu.VMEM((NCH, 5, HD, FC), BF),
            pltpu.VMEM((NCH, 5, HD, FC), BF),
            pltpu.VMEM((NCH, 5, FC, HD), BF),
            pltpu.VMEM((TM, D), BF),
            pltpu.VMEM((NB, 7, HM, HD), BF),
            pltpu.VMEM((NG, S, 128), F32),
            pltpu.VMEM((2, NG, S + HALO, 128), F32),
            pltpu.VMEM((TM, D), BF),
            pltpu.SemaphoreType.DMA((NB,)),
            pltpu.SemaphoreType.DMA((NWC + 1,)),
            pltpu.SemaphoreType.DMA((NCH, 6)),
        ],
        compiler_params=pltpu.CompilerParams(
            dimension_semantics=("arbitrary",),
            vmem_limit_bytes=124 * 1024 * 1024,
        ),
        name="fused_attn_ffn",
    )(x, A_wqkv, A_wo, B_w_gate, B_w_up, B_w_down)
    return out.reshape(A_x.shape)
```

```python
import functools

import jax
import jax.numpy as jnp
from jax import lax
from jax.experimental import pallas as pl
from jax.experimental.pallas import tpu as pltpu

S, D, F = 2048, 1024, 3584
H, DH, WIN, DIL = 32, 32, 8, 2
TM = 256
HM = TM // 2
NB = S // TM
HD = D // 2
FC = 256
NCH = F // 2 // FC
HALO = 16
NG = D // 128
EPS = 1e-5
NEG = -1e9
BF = jnp.bfloat16
F32 = jnp.float32
U32 = jnp.uint32
LOG2E = 1.4426950408889634
NA = 8
TA = (S - TM) // NA
NSTEPS = 17
WC = 512
NWC = 3 * D // WC
ROLL_EVERY = 1000
LN_FIRST = False
N_EUP = 4


def _dot(a, b):
    return jnp.dot(a, b, preferred_element_type=F32)


def _butterfly(vs):
    lane = lax.broadcasted_iota(jnp.int32, vs[0].shape, 1)
    for b in range(3):
        sh = 4 << b
        bit = (lane & sh) != 0
        new = list(vs)
        for i0 in range(NG):
            if i0 & (1 << b):
                continue
            i1 = i0 | (1 << b)
            new[i0] = jnp.where(bit, pltpu.roll(vs[i1], sh, 1), vs[i0])
            new[i1] = jnp.where(bit, vs[i1], pltpu.roll(vs[i0], 128 - sh, 1))
        vs = new
    return vs


def _sum4(x):
    lane = lax.broadcasted_iota(jnp.int32, x.shape, 1)
    x = x + jnp.where((lane & 1) != 0, pltpu.roll(x, 1, 1), pltpu.roll(x, 127, 1))
    x = x + jnp.where((lane & 2) != 0, pltpu.roll(x, 2, 1), pltpu.roll(x, 126, 1))
    return x


def _dep32(x, tok, never):
    return jnp.where(never, pltpu.bitcast(tok, x.dtype), x)


def _gate(m, tok, never):
    t = pltpu.bitcast(m[0:16, 0:128], F32)
    t = pltpu.bitcast(_dep32(t, tok, never), BF)
    top = jnp.concatenate([t, m[0:16, 128:]], axis=1)
    if m.shape[0] == 16:
        return top
    return jnp.concatenate([top, m[16:]], axis=0)


def _pack(y):
    return pltpu.bitcast(y.astype(BF), U32)


def _unpack(w):
    return pltpu.bitcast(w, BF).astype(F32)


def _lhs_combos(a11, a12, a21, a22):
    return [a11 + a22, a21 + a22, a11, a22, a11 + a12, a21 - a11, a12 - a22]


def _strassen_out(m):
    return (m[0] + m[3] - m[4] + m[6], m[2] + m[4], m[1] + m[3], m[0] - m[1] + m[2] + m[5])


def _layernorm(x):
    x = x.astype(F32)
    mean = jnp.mean(x, axis=-1, keepdims=True)
    xc = x - mean
    var = jnp.mean(xc * xc, axis=-1, keepdims=True)
    return xc * lax.rsqrt(var + EPS)


def _kernel(x_hbm, wqkv_hbm, wo_hbm, wg_hbm, wu_hbm, wd_hbm, o_ref,
            x_scr, wqkv, wo, rawg, rawu, rawd, cg, cu, cd,
            xn_scr, s_scr, q_scr, kv_scr, o_scr,
            sem_x, sem_w, sem_raw):
    s = pl.program_id(0)
    k_scr = kv_scr.at[0]
    v_scr = kv_scr.at[1]

    def x_copy(b):
        return pltpu.make_async_copy(x_hbm.at[pl.ds(b * TM, TM), :], x_scr.at[pl.ds(b * TM, TM), :], sem_x.at[b])

    def wqkv_copy(k):
        return pltpu.make_async_copy(wqkv_hbm.at[:, pl.ds(k * WC, WC)], wqkv.at[k], sem_w.at[k])

    def wo_copy():
        return pltpu.make_async_copy(wo_hbm, wo, sem_w.at[NWC])

    def raw_copies(c):
        return [
            pltpu.make_async_copy(wg_hbm.at[:, pl.ds(c * FC, FC)], rawg.at[c, :, pl.ds(0, FC)], sem_raw.at[c, 0]),
            pltpu.make_async_copy(wg_hbm.at[:, pl.ds(F // 2 + c * FC, FC)], rawg.at[c, :, pl.ds(FC, FC)], sem_raw.at[c, 1]),
            pltpu.make_async_copy(wu_hbm.at[:, pl.ds(c * FC, FC)], rawu.at[c, :, pl.ds(0, FC)], sem_raw.at[c, 2]),
            pltpu.make_async_copy(wu_hbm.at[:, pl.ds(F // 2 + c * FC, FC)], rawu.at[c, :, pl.ds(FC, FC)], sem_raw.at[c, 3]),
            pltpu.make_async_copy(wd_hbm.at[pl.ds(c * FC, FC), :], rawd.at[c, pl.ds(0, FC), :], sem_raw.at[c, 4]),
            pltpu.make_async_copy(wd_hbm.at[pl.ds(F // 2 + c * FC, FC), :], rawd.at[c, pl.ds(FC, FC), :], sem_raw.at[c, 5]),
        ]

    never = lax.broadcasted_iota(jnp.int32, (8, 128), 0) < jnp.minimum(s, 0)

    def ln_unit(b, r, tok):
        RC = 16
        r0 = pl.multiple_of(b * TM + r, RC)
        xt = x_scr[pl.ds(r0, RC), :]
        xb = x_scr[pl.ds(r0 + HM, RC), :]
        if tok is not None:
            xt = _gate(xt, tok, never)
            xb = _gate(xb, tok, never)
        top = _layernorm(xt)
        bot = _layernorm(xb)
        xn_scr[pl.ds(r0, RC), :] = top.astype(BF)
        xn_scr[pl.ds(r0 + HM, RC), :] = bot.astype(BF)
        cs = _lhs_combos(top[:, :HD], top[:, HD:], bot[:, :HD], bot[:, HD:])
        for j in range(7):
            s_scr[b, j, pl.ds(r, RC), :] = cs[j].astype(BF)
        return top[0:8, 0:128] + bot[0:8, 0:128]

    def ln_block(b, chain=False):
        tok = None
        for r in range(0, HM, 16):
            t = ln_unit(b, r, tok)
            tok = t if chain else None
        return tok

    def store_kv(y, dst, r0):
        p0 = pl.multiple_of((r0 + HALO) // 2, 8)
        for r in range(0, y.shape[0], 16):
            vs = _butterfly([_pack(y[r:r + 16, g * 128:(g + 1) * 128]) for g in range(NG)])
            for g in range(NG):
                dst[g, pl.ds(p0 + r // 2, 8), :] = vs[g]

    def store_q(y, r0):
        p0 = pl.multiple_of(r0 // 2, 8)
        for g in range(NG):
            q_scr[g, pl.ds(p0, y.shape[0] // 2), :] = _pack(y[:, g * 128:(g + 1) * 128])

    @pl.when(s == 0)
    def _():
        x_copy(0).start(priority=1)

        def issue(j, carry):
            @pl.when(j == 1)
            def _():
                x_copy(1).start(priority=1)

            wqkv_copy(lax.rem(j + 2, NWC)).start(priority=1)
            return carry

        lax.fori_loop(0, NWC, issue, 0)
        x_copy(2).start(priority=1)
        k_scr[:, 0:HALO // 2, :] = jnp.zeros((NG, HALO // 2, 128), U32)
        v_scr[:, 0:HALO // 2, :] = jnp.zeros((NG, HALO // 2, 128), U32)
        x_copy(0).wait()
        ln_block(0)
        xn = xn_scr[0:TM, :]

        def body(j, carry):
            k = lax.rem(j + 2, NWC)
            wqkv_copy(k).wait()

            @pl.when(j == 1)
            def _():
                x_copy(1).wait()

            half = lax.rem(j, 2)
            sec = jnp.maximum(lax.div(j, 2) - 1, 0)
            src = pl.multiple_of(((sec + 1) * TM + half * HM) // 2, HM // 2)
            dstr = pl.multiple_of((HALO + half * HM) // 2, 8)
            for r in range(0, HM // 2, 8):
                vs = _butterfly([q_scr[g, pl.ds(src + r, 8), :] for g in range(NG)])
                for g in range(NG):
                    kv_scr[sec, g, pl.ds(dstr + r, 8), :] = vs[g]
            lb = jnp.minimum(j, 1)
            u0 = 2 * jnp.clip(j - 1, 0, 3)
            tok = ln_unit(lb, pl.multiple_of(u0 * 16, 16), None)
            ln_unit(lb, pl.multiple_of(u0 * 16 + 16, 16), tok)
            y = _dot(xn, wqkv[k])
            rb = pl.multiple_of(lax.rem(lax.div(j, 2) + 1, 3) * (TM // 2), TM // 2)
            for gg in range(WC // 128):
                q_scr[half * (WC // 128) + gg, pl.ds(rb, TM // 2), :] = _pack(y[:, gg * 128:(gg + 1) * 128])
            return carry

        lax.fori_loop(0, NWC, body, 0)

    @pl.when(s < NCH)
    def _():
        for cp in raw_copies(s):
            cp.start(priority=1)

    @pl.when(s < NB - 3)
    def _():
        x_copy(s + 3).start(priority=1)

    @pl.when(s == NCH)
    def _():
        wo_copy().start(priority=1)

    @pl.when(jnp.logical_and(s >= 2, s <= NA))
    def _():
        for cp in raw_copies(s - 2):
            cp.wait()

    @pl.when(jnp.logical_and(s >= 1, s < NB - 1))
    def _():
        x_copy(s + 1).wait()

    @pl.when(s == NA + 1)
    def _():
        wo_copy().wait()

    @pl.when(jnp.logical_and(s >= 1, s <= NA))
    def _():
        r0 = pl.multiple_of(TM + (s - 1) * TA, 16)
        xn = xn_scr[pl.ds(r0, TA), :]
        ys = [jnp.concatenate([_dot(xn, wqkv[2 * sec]), _dot(xn, wqkv[2 * sec + 1])], axis=1) for sec in (1, 2, 0)]
        tok = ln_block(jnp.minimum(s + 1, NB - 1), chain=True)
        c = lax.rem(s + (NCH - 2), NCH)
        never4 = lax.broadcasted_iota(jnp.int32, (4, 128), 0) < jnp.minimum(s, 0)

        def build(raw, cmb, kq, nq, tok):
            def ld(r, n, tok4):
                t = pltpu.bitcast(raw[c, r:r + 8, n:n + 128], F32)
                return pltpu.bitcast(_dep32(t, tok4, never4), BF).astype(F32)

            for r in range(0, kq, 16):
                for n0 in range(0, nq, 128):
                    cnt[0] += 1
                    if cnt[0] % ROLL_EVERY == 0:
                        tok = pltpu.roll(tok, 1, 1)
                    for _ in range(N_EUP):
                        tok = jnp.exp2(tok)
                    tok4 = tok[0:4]
                    b11, b12, b21, b22 = [
                        jnp.concatenate([ld(rr, nn, tok4), ld(rr + 8, nn, tok4)], axis=0)
                        for rr, nn in ((r, n0), (r, nq + n0), (kq + r, n0), (kq + r, nq + n0))]
                    outs = [(b11 + b22).astype(BF), (b12 - b22).astype(BF), (b21 - b11).astype(BF),
                            (b11 + b12).astype(BF), (b21 + b22).astype(BF)]
                    for j in range(5):
                        cmb[c, j, r:r + 16, n0:n0 + 128] = outs[j]
                    tok = pltpu.bitcast(outs[0], F32)
            return tok

        cnt = [0]
        if not LN_FIRST:
            tok = jnp.zeros((8, 128), F32)
        tok = build(rawg, cg, HD, FC, tok)
        tok = build(rawu, cu, HD, FC, tok)
        tok = build(rawd, cd, FC, HD, tok)
        store_kv(ys[0], k_scr, r0)
        store_kv(ys[1], v_scr, r0)
        store_q(ys[2], r0)

    if NSTEPS < NA + 1 + NB:
        @pl.when(s == NSTEPS - 1)
        def _():
            l = NSTEPS - 1
            for c in (l - 1, l):
                if 0 <= c < NCH:
                    for cp in raw_copies(c):
                        cp.wait()
            for b in (l + 2, l + 3):
                if b < NB:
                    x_copy(b).wait()
            if NCH <= l <= NA:
                wo_copy().wait()

    @pl.when(s > NA)
    def _():
        i = s - (NA + 1)
        r0 = pl.multiple_of(i * TM, TM)

        def wlist(raw, cmb, c, kq, nq):
            return [cmb[c, 0], raw[c, 0:kq, 0:nq], cmb[c, 1], cmb[c, 2],
                    raw[c, kq:2 * kq, nq:2 * nq], cmb[c, 3], cmb[c, 4]]

        RA = 16
        cexp = (DH ** -0.5) * LOG2E
        p0 = pl.multiple_of(r0 // 2, 8)

        def attn_rows(r, tok):
            qp = [q_scr[g, pl.ds(p0 + r // 2, 8), :] for g in range(NG)]
            if tok is not None:
                qp = [_dep32(t, tok, never) for t in qp]
            q = [_unpack(t) for t in _butterfly(qp)]
            kb = p0 + (r + HALO) // 2
            sw = []
            for w in range(WIN):
                acc = None
                for g in range(NG):
                    t = q[g] * _unpack(k_scr[g, pl.ds(kb - w, 8), :])
                    acc = t if acc is None else acc + t
                acc = _sum4(acc)
                if r < HALO and w > 0:
                    row = lax.broadcasted_iota(jnp.int32, (RA, 128), 0) + (r0 + r)
                    acc = jnp.where(row >= DIL * w, acc, NEG)
                sw.append(acc)
            m = sw[0]
            for w in range(1, WIN):
                m = jnp.maximum(m, sw[w])
            e = [jnp.exp2((sw[w] - m) * cexp) for w in range(WIN)]
            den = e[0]
            for w in range(1, WIN):
                den = den + e[w]
            inv = 1.0 / den
            p = [e[w] * inv for w in range(WIN)]
            o = []
            for g in range(NG):
                acc = None
                for w in range(WIN):
                    t = p[w] * _unpack(v_scr[g, pl.ds(kb - w, 8), :])
                    acc = t if acc is None else acc + t
                o.append(_pack(acc))
            o = _butterfly(o)
            for g in range(NG):
                o_scr[r:r + RA, g * 128:(g + 1) * 128] = pltpu.bitcast(o[g], BF)
            return o[0]

        sl = [s_scr[i, j] for j in range(7)]
        acc = [None] * 7
        o_parts = []
        n_att = TM // RA
        per = 3
        tok = None
        for c in range(NCH):
            wg_l = wlist(rawg, cg, c, HD, FC)
            wu_l = wlist(rawu, cu, c, HD, FC)
            wd_l = wlist(rawd, cd, c, FC, HD)
            slc = sl
            g = _strassen_out([_dot(slc[j], wg_l[j]) for j in range(7)])
            u = _strassen_out([_dot(slc[j], wu_l[j]) for j in range(7)])
            hq = [g[t] * u[t] for t in range(4)]
            hl = [t.astype(BF) for t in _lhs_combos(*hq)]
            for j in range(7):
                y = _dot(hl[j], wd_l[j])
                acc[j] = y if acc[j] is None else acc[j] + y
            for a in range(c * per, min((c + 1) * per, n_att)):
                tok = attn_rows(a * RA, tok)
        ao = _dot(o_scr[...], wo[...])
        y11, y12, y21, y22 = _strassen_out(acc)
        x = x_scr[pl.ds(r0, TM), :].astype(F32)
        o_ref[0:HM, 0:HD] = (x[0:HM, 0:HD] + ao[0:HM, 0:HD] + y11).astype(o_ref.dtype)
        o_ref[0:HM, HD:D] = (x[0:HM, HD:D] + ao[0:HM, HD:D] + y12).astype(o_ref.dtype)
        o_ref[HM:TM, 0:HD] = (x[HM:TM, 0:HD] + ao[HM:TM, 0:HD] + y21).astype(o_ref.dtype)
        o_ref[HM:TM, HD:D] = (x[HM:TM, HD:D] + ao[HM:TM, HD:D] + y22).astype(o_ref.dtype)


@jax.jit
def pallas_parallel_sum__sliding_local_dilated__glu_gated_bilinear__prompt_kernel(
    A_x: jax.Array,
    A_wqkv: jax.Array,
    A_wo: jax.Array,
    B_x: jax.Array,
    B_w_gate: jax.Array,
    B_w_up: jax.Array,
    B_w_down: jax.Array,
):
    del B_x
    x = A_x.reshape(S, D)
    hbm = pl.BlockSpec(memory_space=pl.ANY)
    out = pl.pallas_call(
        _kernel,
        grid=(NSTEPS,),
        in_specs=[hbm] * 6,
        out_specs=pl.BlockSpec((TM, D), lambda s: (jnp.maximum(s - (NA + 1), 0), 0)),
        out_shape=jax.ShapeDtypeStruct((S, D), A_x.dtype),
        scratch_shapes=[
            pltpu.VMEM((S, D), BF),
            pltpu.VMEM((NWC, D, WC), BF),
            pltpu.VMEM((D, D), BF),
            pltpu.VMEM((NCH, D, 2 * FC), BF),
            pltpu.VMEM((NCH, D, 2 * FC), BF),
            pltpu.VMEM((NCH, 2 * FC, D), BF),
            pltpu.VMEM((NCH, 5, HD, FC), BF),
            pltpu.VMEM((NCH, 5, HD, FC), BF),
            pltpu.VMEM((NCH, 5, FC, HD), BF),
            pltpu.VMEM((S, D), BF),
            pltpu.VMEM((NB, 7, HM, HD), BF),
            pltpu.VMEM((NG, S // 2, 128), U32),
            pltpu.VMEM((2, NG, (S + HALO) // 2, 128), U32),
            pltpu.VMEM((TM, D), BF),
            pltpu.SemaphoreType.DMA((NB,)),
            pltpu.SemaphoreType.DMA((NWC + 1,)),
            pltpu.SemaphoreType.DMA((NCH, 6)),
        ],
        compiler_params=pltpu.CompilerParams(
            dimension_semantics=("arbitrary",),
            vmem_limit_bytes=124 * 1024 * 1024,
        ),
        name="fused_attn_ffn",
    )(x, A_wqkv, A_wo, B_w_gate, B_w_up, B_w_down)
    return out.reshape(A_x.shape)
```

```python
import functools

import jax
import jax.numpy as jnp
from jax import lax
from jax.experimental import pallas as pl
from jax.experimental.pallas import tpu as pltpu

S, D, F = 2048, 1024, 3584
H, DH, WIN, DIL = 32, 32, 8, 2
TM = 256
HM = TM // 2
NB = S // TM
HD = D // 2
FC = 256
NCH = F // 2 // FC
HALO = 16
NG = D // 128
EPS = 1e-5
NEG = -1e9
BF = jnp.bfloat16
F32 = jnp.float32
U32 = jnp.uint32
LOG2E = 1.4426950408889634
NA = 8
TA = (S - TM) // NA
NSTEPS = 17
WC = 512
NWC = 3 * D // WC
ROLL_EVERY = 1000
LN_FIRST = False
N_EUP = 4
CHAIN_HALVES = True
XOR_TOK = False


def _dot(a, b):
    return jnp.dot(a, b, preferred_element_type=F32)


def _butterfly(vs):
    lane = lax.broadcasted_iota(jnp.int32, vs[0].shape, 1)
    for b in range(3):
        sh = 4 << b
        bit = (lane & sh) != 0
        new = list(vs)
        for i0 in range(NG):
            if i0 & (1 << b):
                continue
            i1 = i0 | (1 << b)
            new[i0] = jnp.where(bit, pltpu.roll(vs[i1], sh, 1), vs[i0])
            new[i1] = jnp.where(bit, vs[i1], pltpu.roll(vs[i0], 128 - sh, 1))
        vs = new
    return vs


def _sum4(x):
    lane = lax.broadcasted_iota(jnp.int32, x.shape, 1)
    x = x + jnp.where((lane & 1) != 0, pltpu.roll(x, 1, 1), pltpu.roll(x, 127, 1))
    x = x + jnp.where((lane & 2) != 0, pltpu.roll(x, 2, 1), pltpu.roll(x, 126, 1))
    return x


def _dep32(x, tok, never):
    return jnp.where(never, pltpu.bitcast(tok, x.dtype), x)


def _gate(m, tok, never):
    t = pltpu.bitcast(m[0:16, 0:128], F32)
    t = pltpu.bitcast(_dep32(t, tok, never), BF)
    top = jnp.concatenate([t, m[0:16, 128:]], axis=1)
    if m.shape[0] == 16:
        return top
    return jnp.concatenate([top, m[16:]], axis=0)


def _pack(y):
    return pltpu.bitcast(y.astype(BF), U32)


def _unpack(w):
    return pltpu.bitcast(w, BF).astype(F32)


def _lhs_combos(a11, a12, a21, a22):
    return [a11 + a22, a21 + a22, a11, a22, a11 + a12, a21 - a11, a12 - a22]


def _strassen_out(m):
    return (m[0] + m[3] - m[4] + m[6], m[2] + m[4], m[1] + m[3], m[0] - m[1] + m[2] + m[5])


def _layernorm(x):
    x = x.astype(F32)
    mean = jnp.mean(x, axis=-1, keepdims=True)
    xc = x - mean
    var = jnp.mean(xc * xc, axis=-1, keepdims=True)
    return xc * lax.rsqrt(var + EPS)


def _kernel(x_hbm, wqkv_hbm, wo_hbm, wg_hbm, wu_hbm, wd_hbm, o_ref,
            x_scr, wqkv, wo, rawg, rawu, rawd, cg, cu, cd,
            xn_scr, s_scr, q_scr, kv_scr, o_scr,
            sem_x, sem_w, sem_raw):
    s = pl.program_id(0)
    k_scr = kv_scr.at[0]
    v_scr = kv_scr.at[1]

    def x_copy(b):
        return pltpu.make_async_copy(x_hbm.at[pl.ds(b * TM, TM), :], x_scr.at[pl.ds(b * TM, TM), :], sem_x.at[b])

    def wqkv_copy(k):
        return pltpu.make_async_copy(wqkv_hbm.at[:, pl.ds(k * WC, WC)], wqkv.at[k], sem_w.at[k])

    def wo_copy():
        return pltpu.make_async_copy(wo_hbm, wo, sem_w.at[NWC])

    def raw_copies(c):
        return [
            pltpu.make_async_copy(wg_hbm.at[:, pl.ds(c * FC, FC)], rawg.at[c, :, pl.ds(0, FC)], sem_raw.at[c, 0]),
            pltpu.make_async_copy(wg_hbm.at[:, pl.ds(F // 2 + c * FC, FC)], rawg.at[c, :, pl.ds(FC, FC)], sem_raw.at[c, 1]),
            pltpu.make_async_copy(wu_hbm.at[:, pl.ds(c * FC, FC)], rawu.at[c, :, pl.ds(0, FC)], sem_raw.at[c, 2]),
            pltpu.make_async_copy(wu_hbm.at[:, pl.ds(F // 2 + c * FC, FC)], rawu.at[c, :, pl.ds(FC, FC)], sem_raw.at[c, 3]),
            pltpu.make_async_copy(wd_hbm.at[pl.ds(c * FC, FC), :], rawd.at[c, pl.ds(0, FC), :], sem_raw.at[c, 4]),
            pltpu.make_async_copy(wd_hbm.at[pl.ds(F // 2 + c * FC, FC), :], rawd.at[c, pl.ds(FC, FC), :], sem_raw.at[c, 5]),
        ]

    never = lax.broadcasted_iota(jnp.int32, (8, 128), 0) < jnp.minimum(s, 0)

    def ln_unit(b, r, tok):
        RC = 16
        r0 = pl.multiple_of(b * TM + r, RC)
        xt = x_scr[pl.ds(r0, RC), :]
        xb = x_scr[pl.ds(r0 + HM, RC), :]
        if tok is not None:
            xt = _gate(xt, tok, never)
            xb = _gate(xb, tok, never)
        top = _layernorm(xt)
        bot = _layernorm(xb)
        xn_scr[pl.ds(r0, RC), :] = top.astype(BF)
        xn_scr[pl.ds(r0 + HM, RC), :] = bot.astype(BF)
        cs = _lhs_combos(top[:, :HD], top[:, HD:], bot[:, :HD], bot[:, HD:])
        for j in range(7):
            s_scr[b, j, pl.ds(r, RC), :] = cs[j].astype(BF)
        return top[0:8, 0:128] + bot[0:8, 0:128]

    def ln_block(b, chain=False):
        tok = None
        for r in range(0, HM, 16):
            t = ln_unit(b, r, tok)
            tok = t if chain else None
        return tok

    def store_kv(y, dst, r0):
        for r in range(0, y.shape[0], 16):
            vs = _butterfly([_pack(y[r:r + 16, g * 128:(g + 1) * 128]) for g in range(NG)])
            for g in range(NG):
                dst[g, pl.ds(r0 + HALO + r, 16), :] = _unpack(vs[g])

    def store_q(y, r0):
        p0 = pl.multiple_of(r0 // 2, 8)
        for g in range(NG):
            q_scr[g, pl.ds(p0, y.shape[0] // 2), :] = _pack(y[:, g * 128:(g + 1) * 128])

    @pl.when(s == 0)
    def _():
        x_copy(0).start(priority=1)

        def issue(j, carry):
            @pl.when(j == 1)
            def _():
                x_copy(1).start(priority=1)

            wqkv_copy(lax.rem(j + 2, NWC)).start(priority=1)
            return carry

        lax.fori_loop(0, NWC, issue, 0)
        x_copy(2).start(priority=1)
        k_scr[:, 0:HALO, :] = jnp.zeros((NG, HALO, 128), F32)
        v_scr[:, 0:HALO, :] = jnp.zeros((NG, HALO, 128), F32)
        x_copy(0).wait()
        ln_block(0)
        xn = xn_scr[0:TM, :]

        def body(j, carry):
            k = lax.rem(j + 2, NWC)
            wqkv_copy(k).wait()

            @pl.when(j == 1)
            def _():
                x_copy(1).wait()

            half = lax.rem(j, 2)
            sec = jnp.maximum(lax.div(j, 2) - 1, 0)
            src = pl.multiple_of(((sec + 1) * TM + half * HM) // 2, HM // 2)
            dstr = pl.multiple_of(HALO + half * HM, 16)
            for r in range(0, HM // 2, 8):
                vs = _butterfly([q_scr[g, pl.ds(src + r, 8), :] for g in range(NG)])
                for g in range(NG):
                    kv_scr[sec, g, pl.ds(dstr + 2 * r, 16), :] = _unpack(vs[g])
            lb = jnp.minimum(j, 1)
            u0 = 2 * jnp.clip(j - 1, 0, 3)
            tok = ln_unit(lb, pl.multiple_of(u0 * 16, 16), None)
            ln_unit(lb, pl.multiple_of(u0 * 16 + 16, 16), tok)
            y = _dot(xn, wqkv[k])
            rb = pl.multiple_of(lax.rem(lax.div(j, 2) + 1, 3) * (TM // 2), TM // 2)
            for gg in range(WC // 128):
                q_scr[half * (WC // 128) + gg, pl.ds(rb, TM // 2), :] = _pack(y[:, gg * 128:(gg + 1) * 128])
            return carry

        lax.fori_loop(0, NWC, body, 0)

    @pl.when(s < NCH)
    def _():
        for cp in raw_copies(s):
            cp.start(priority=1)

    @pl.when(s < NB - 3)
    def _():
        x_copy(s + 3).start(priority=1)

    @pl.when(s == NCH)
    def _():
        wo_copy().start(priority=1)

    @pl.when(jnp.logical_and(s >= 2, s <= NA))
    def _():
        for cp in raw_copies(s - 2):
            cp.wait()

    @pl.when(jnp.logical_and(s >= 1, s < NB - 1))
    def _():
        x_copy(s + 1).wait()

    @pl.when(s == NA + 1)
    def _():
        wo_copy().wait()

    @pl.when(jnp.logical_and(s >= 1, s <= NA))
    def _():
        r0 = pl.multiple_of(TM + (s - 1) * TA, 16)
        xn = xn_scr[pl.ds(r0, TA), :]
        ys = [jnp.concatenate([_dot(xn, wqkv[2 * sec]), _dot(xn, wqkv[2 * sec + 1])], axis=1) for sec in (1, 2, 0)]
        tok = ln_block(jnp.minimum(s + 1, NB - 1), chain=True)
        c = lax.rem(s + (NCH - 2), NCH)
        never4 = lax.broadcasted_iota(jnp.int32, (4, 128), 0) < jnp.minimum(s, 0)

        def build(raw, cmb, kq, nq, tok):
            def ld(r, n, tok4):
                t = pltpu.bitcast(raw[c, r:r + 8, n:n + 128], F32)
                return pltpu.bitcast(_dep32(t, tok4, never4), BF).astype(F32)

            for r in range(0, kq, 16):
                for n0 in range(0, nq, 128):
                    cnt[0] += 1
                    if cnt[0] % ROLL_EVERY == 0:
                        tok = pltpu.roll(tok, 1, 1)
                    for _ in range(N_EUP):
                        tok = jnp.exp2(tok)
                    tok4 = tok[0:4]
                    b11, b12, b21, b22 = [
                        jnp.concatenate([ld(rr, nn, tok4), ld(rr + 8, nn, tok4)], axis=0)
                        for rr, nn in ((r, n0), (r, nq + n0), (kq + r, n0), (kq + r, nq + n0))]
                    outs = [(b11 + b22).astype(BF), (b12 - b22).astype(BF), (b21 - b11).astype(BF),
                            (b11 + b12).astype(BF), (b21 + b22).astype(BF)]
                    for j in range(5):
                        cmb[c, j, r:r + 16, n0:n0 + 128] = outs[j]
                    tok = pltpu.bitcast(outs[0], F32)
            return tok

        cnt = [0]
        if not LN_FIRST:
            tok = jnp.zeros((8, 128), F32)
        tok = build(rawg, cg, HD, FC, tok)
        tok = build(rawu, cu, HD, FC, tok)
        tok = build(rawd, cd, FC, HD, tok)
        store_kv(ys[0], k_scr, r0)
        store_kv(ys[1], v_scr, r0)
        store_q(ys[2], r0)

    if NSTEPS < NA + 1 + NB:
        @pl.when(s == NSTEPS - 1)
        def _():
            l = NSTEPS - 1
            for c in (l - 1, l):
                if 0 <= c < NCH:
                    for cp in raw_copies(c):
                        cp.wait()
            for b in (l + 2, l + 3):
                if b < NB:
                    x_copy(b).wait()
            if NCH <= l <= NA:
                wo_copy().wait()

    @pl.when(s > NA)
    def _():
        i = s - (NA + 1)
        r0 = pl.multiple_of(i * TM, TM)

        def wlist(raw, cmb, c, kq, nq):
            return [cmb[c, 0], raw[c, 0:kq, 0:nq], cmb[c, 1], cmb[c, 2],
                    raw[c, kq:2 * kq, nq:2 * nq], cmb[c, 3], cmb[c, 4]]

        RA = 16
        cexp = (DH ** -0.5) * LOG2E
        p0 = pl.multiple_of(r0 // 2, 8)
        never16 = lax.broadcasted_iota(jnp.int32, (16, 128), 0) < jnp.minimum(s, 0)

        def attn_half(q, r):
            sw = []
            for w in range(WIN):
                acc = None
                for g in range(NG):
                    t = q[g] * k_scr[g, pl.ds(r0 + r + HALO - DIL * w, 8), :]
                    acc = t if acc is None else acc + t
                acc = _sum4(acc)
                if r < HALO and w > 0:
                    row = lax.broadcasted_iota(jnp.int32, (8, 128), 0) + (r0 + r)
                    acc = jnp.where(row >= DIL * w, acc, NEG)
                sw.append(acc)
            m = sw[0]
            for w in range(1, WIN):
                m = jnp.maximum(m, sw[w])
            e = [jnp.exp2((sw[w] - m) * cexp) for w in range(WIN)]
            den = e[0]
            for w in range(1, WIN):
                den = den + e[w]
            inv = 1.0 / den
            p = [e[w] * inv for w in range(WIN)]
            o = []
            for g in range(NG):
                acc = None
                for w in range(WIN):
                    t = p[w] * v_scr[g, pl.ds(r0 + r + HALO - DIL * w, 8), :]
                    acc = t if acc is None else acc + t
                o.append(acc)
            return o

        def attn_rows(r, tok):
            qp = [q_scr[g, pl.ds(p0 + r // 2, 8), :] for g in range(NG)]
            if tok is not None:
                qp = [_dep32(t, tok, never) for t in qp]
            q = [_unpack(t) for t in _butterfly(qp)]
            o0 = attn_half([t[0:8] for t in q], r)
            q1 = [t[8:16] for t in q]
            if CHAIN_HALVES:
                q1 = [_dep32(t, o0[NG - 1], never) for t in q1]
            o1 = attn_half(q1, r + 8)
            o = _butterfly([_pack(jnp.concatenate([o0[g], o1[g]], axis=0)) for g in range(NG)])
            for g in range(NG):
                o_scr[r:r + RA, g * 128:(g + 1) * 128] = pltpu.bitcast(o[g], BF)
            tok = o[0]
            if XOR_TOK:
                for g in range(1, NG):
                    tok = tok ^ o[g]
            return tok

        sl = [s_scr[i, j] for j in range(7)]
        acc = [None] * 7
        o_parts = []
        n_att = TM // RA
        per = 3
        tok = None
        for c in range(NCH):
            wg_l = wlist(rawg, cg, c, HD, FC)
            wu_l = wlist(rawu, cu, c, HD, FC)
            wd_l = wlist(rawd, cd, c, FC, HD)
            slc = sl
            g = _strassen_out([_dot(slc[j], wg_l[j]) for j in range(7)])
            u = _strassen_out([_dot(slc[j], wu_l[j]) for j in range(7)])
            hq = [g[t] * u[t] for t in range(4)]
            hl = [t.astype(BF) for t in _lhs_combos(*hq)]
            for j in range(7):
                y = _dot(hl[j], wd_l[j])
                acc[j] = y if acc[j] is None else acc[j] + y
            for a in range(c * per, min((c + 1) * per, n_att)):
                tok = attn_rows(a * RA, tok)
        ao = _dot(o_scr[...], wo[...])
        y11, y12, y21, y22 = _strassen_out(acc)
        x = x_scr[pl.ds(r0, TM), :].astype(F32)
        o_ref[0:HM, 0:HD] = (x[0:HM, 0:HD] + ao[0:HM, 0:HD] + y11).astype(o_ref.dtype)
        o_ref[0:HM, HD:D] = (x[0:HM, HD:D] + ao[0:HM, HD:D] + y12).astype(o_ref.dtype)
        o_ref[HM:TM, 0:HD] = (x[HM:TM, 0:HD] + ao[HM:TM, 0:HD] + y21).astype(o_ref.dtype)
        o_ref[HM:TM, HD:D] = (x[HM:TM, HD:D] + ao[HM:TM, HD:D] + y22).astype(o_ref.dtype)


@jax.jit
def pallas_parallel_sum__sliding_local_dilated__glu_gated_bilinear__prompt_kernel(
    A_x: jax.Array,
    A_wqkv: jax.Array,
    A_wo: jax.Array,
    B_x: jax.Array,
    B_w_gate: jax.Array,
    B_w_up: jax.Array,
    B_w_down: jax.Array,
):
    del B_x
    x = A_x.reshape(S, D)
    hbm = pl.BlockSpec(memory_space=pl.ANY)
    out = pl.pallas_call(
        _kernel,
        grid=(NSTEPS,),
        in_specs=[hbm] * 6,
        out_specs=pl.BlockSpec((TM, D), lambda s: (jnp.maximum(s - (NA + 1), 0), 0)),
        out_shape=jax.ShapeDtypeStruct((S, D), A_x.dtype),
        scratch_shapes=[
            pltpu.VMEM((S, D), BF),
            pltpu.VMEM((NWC, D, WC), BF),
            pltpu.VMEM((D, D), BF),
            pltpu.VMEM((NCH, D, 2 * FC), BF),
            pltpu.VMEM((NCH, D, 2 * FC), BF),
            pltpu.VMEM((NCH, 2 * FC, D), BF),
            pltpu.VMEM((NCH, 5, HD, FC), BF),
            pltpu.VMEM((NCH, 5, HD, FC), BF),
            pltpu.VMEM((NCH, 5, FC, HD), BF),
            pltpu.VMEM((S, D), BF),
            pltpu.VMEM((NB, 7, HM, HD), BF),
            pltpu.VMEM((NG, S // 2, 128), U32),
            pltpu.VMEM((2, NG, S + HALO, 128), F32),
            pltpu.VMEM((TM, D), BF),
            pltpu.SemaphoreType.DMA((NB,)),
            pltpu.SemaphoreType.DMA((NWC + 1,)),
            pltpu.SemaphoreType.DMA((NCH, 6)),
        ],
        compiler_params=pltpu.CompilerParams(
            dimension_semantics=("arbitrary",),
            vmem_limit_bytes=124 * 1024 * 1024,
        ),
        name="fused_attn_ffn",
    )(x, A_wqkv, A_wo, B_w_gate, B_w_up, B_w_down)
    return out.reshape(A_x.shape)
```

```python
import functools

import jax
import jax.numpy as jnp
from jax import lax
from jax.experimental import pallas as pl
from jax.experimental.pallas import tpu as pltpu

S, D, F = 2048, 1024, 3584
H, DH, WIN, DIL = 32, 32, 8, 2
TM = 256
HM = TM // 2
NB = S // TM
HD = D // 2
FC = 256
NCH = F // 2 // FC
HALO = 16
NG = D // 128
EPS = 1e-5
NEG = -1e9
BF = jnp.bfloat16
F32 = jnp.float32
U32 = jnp.uint32
LOG2E = 1.4426950408889634
NA = 8
TA = (S - TM) // NA
NSTEPS = 17
WC = 512
NWC = 3 * D // WC
ROLL_EVERY = 1000
LN_FIRST = False
N_EUP = 4
CHAIN_HALVES = True
XOR_TOK = False


def _dot(a, b):
    return jnp.dot(a, b, preferred_element_type=F32)


def _butterfly(vs):
    lane = lax.broadcasted_iota(jnp.int32, vs[0].shape, 1)
    for b in range(3):
        sh = 4 << b
        bit = (lane & sh) != 0
        new = list(vs)
        for i0 in range(NG):
            if i0 & (1 << b):
                continue
            i1 = i0 | (1 << b)
            new[i0] = jnp.where(bit, pltpu.roll(vs[i1], sh, 1), vs[i0])
            new[i1] = jnp.where(bit, vs[i1], pltpu.roll(vs[i0], 128 - sh, 1))
        vs = new
    return vs


def _sum4(x):
    lane = lax.broadcasted_iota(jnp.int32, x.shape, 1)
    x = x + jnp.where((lane & 1) != 0, pltpu.roll(x, 1, 1), pltpu.roll(x, 127, 1))
    x = x + jnp.where((lane & 2) != 0, pltpu.roll(x, 2, 1), pltpu.roll(x, 126, 1))
    return x


def _dep32(x, tok, never):
    return jnp.where(never, pltpu.bitcast(tok, x.dtype), x)


def _gate(m, tok, never):
    t = pltpu.bitcast(m[0:16, 0:128], F32)
    t = pltpu.bitcast(_dep32(t, tok, never), BF)
    top = jnp.concatenate([t, m[0:16, 128:]], axis=1)
    if m.shape[0] == 16:
        return top
    return jnp.concatenate([top, m[16:]], axis=0)


def _pack(y):
    return pltpu.bitcast(y.astype(BF), U32)


def _unpack(w):
    return pltpu.bitcast(w, BF).astype(F32)


def _lhs_combos(a11, a12, a21, a22):
    return [a11 + a22, a21 + a22, a11, a22, a11 + a12, a21 - a11, a12 - a22]


def _strassen_out(m):
    return (m[0] + m[3] - m[4] + m[6], m[2] + m[4], m[1] + m[3], m[0] - m[1] + m[2] + m[5])


def _layernorm(x):
    x = x.astype(F32)
    mean = jnp.mean(x, axis=-1, keepdims=True)
    xc = x - mean
    var = jnp.mean(xc * xc, axis=-1, keepdims=True)
    return xc * lax.rsqrt(var + EPS)


def _kernel(x_hbm, wqkv_hbm, wo_hbm, wg_hbm, wu_hbm, wd_hbm, o_ref,
            x_scr, wqkv, wo, rawg, rawu, rawd, cg, cu, cd,
            xn_scr, s_scr, q_scr, kv_scr, o_scr,
            sem_x, sem_w, sem_raw):
    s = pl.program_id(0)
    k_scr = kv_scr.at[0]
    v_scr = kv_scr.at[1]

    def x_copy(b):
        return pltpu.make_async_copy(x_hbm.at[pl.ds(b * TM, TM), :], x_scr.at[pl.ds(b * TM, TM), :], sem_x.at[b])

    def wqkv_copy(k):
        return pltpu.make_async_copy(wqkv_hbm.at[:, pl.ds(k * WC, WC)], wqkv.at[k], sem_w.at[k])

    def wo_copy():
        return pltpu.make_async_copy(wo_hbm, wo, sem_w.at[NWC])

    def raw_copies(c):
        return [
            pltpu.make_async_copy(wg_hbm.at[:, pl.ds(c * FC, FC)], rawg.at[c, :, pl.ds(0, FC)], sem_raw.at[c, 0]),
            pltpu.make_async_copy(wg_hbm.at[:, pl.ds(F // 2 + c * FC, FC)], rawg.at[c, :, pl.ds(FC, FC)], sem_raw.at[c, 1]),
            pltpu.make_async_copy(wu_hbm.at[:, pl.ds(c * FC, FC)], rawu.at[c, :, pl.ds(0, FC)], sem_raw.at[c, 2]),
            pltpu.make_async_copy(wu_hbm.at[:, pl.ds(F // 2 + c * FC, FC)], rawu.at[c, :, pl.ds(FC, FC)], sem_raw.at[c, 3]),
            pltpu.make_async_copy(wd_hbm.at[pl.ds(c * FC, FC), :], rawd.at[c, pl.ds(0, FC), :], sem_raw.at[c, 4]),
            pltpu.make_async_copy(wd_hbm.at[pl.ds(F // 2 + c * FC, FC), :], rawd.at[c, pl.ds(FC, FC), :], sem_raw.at[c, 5]),
        ]

    never = lax.broadcasted_iota(jnp.int32, (8, 128), 0) < jnp.minimum(s, 0)

    def ln_unit(b, r, tok):
        RC = 16
        r0 = pl.multiple_of(b * TM + r, RC)
        xt = x_scr[pl.ds(r0, RC), :]
        xb = x_scr[pl.ds(r0 + HM, RC), :]
        if tok is not None:
            xt = _gate(xt, tok, never)
            xb = _gate(xb, tok, never)
        top = _layernorm(xt)
        bot = _layernorm(xb)
        xn_scr[pl.ds(r0, RC), :] = top.astype(BF)
        xn_scr[pl.ds(r0 + HM, RC), :] = bot.astype(BF)
        cs = _lhs_combos(top[:, :HD], top[:, HD:], bot[:, :HD], bot[:, HD:])
        for j in range(7):
            s_scr[b, j, pl.ds(r, RC), :] = cs[j].astype(BF)
        return top[0:8, 0:128] + bot[0:8, 0:128]

    def ln_block(b, chain=False):
        tok = None
        for r in range(0, HM, 16):
            t = ln_unit(b, r, tok)
            tok = t if chain else None
        return tok

    def store_kv(y, dst, r0):
        for r in range(0, y.shape[0], 16):
            vs = _butterfly([_pack(y[r:r + 16, g * 128:(g + 1) * 128]) for g in range(NG)])
            for g in range(NG):
                dst[g, pl.ds(r0 + HALO + r, 16), :] = _unpack(vs[g])

    def store_q(y, r0):
        p0 = pl.multiple_of(r0 // 2, 8)
        for g in range(NG):
            q_scr[g, pl.ds(p0, y.shape[0] // 2), :] = _pack(y[:, g * 128:(g + 1) * 128])

    @pl.when(s == 0)
    def _():
        x_copy(0).start(priority=1)

        def issue(j, carry):
            @pl.when(j == 1)
            def _():
                x_copy(1).start(priority=1)

            wqkv_copy(lax.rem(j + 2, NWC)).start(priority=1)
            return carry

        lax.fori_loop(0, NWC, issue, 0)
        x_copy(2).start(priority=1)
        k_scr[:, 0:HALO, :] = jnp.zeros((NG, HALO, 128), F32)
        v_scr[:, 0:HALO, :] = jnp.zeros((NG, HALO, 128), F32)
        x_copy(0).wait()
        ln_block(0)
        xn = xn_scr[0:TM, :]

        def body(j, carry):
            k = lax.rem(j + 2, NWC)
            wqkv_copy(k).wait()

            @pl.when(j == 1)
            def _():
                x_copy(1).wait()

            half = lax.rem(j, 2)
            sec = jnp.maximum(lax.div(j, 2) - 1, 0)
            src = pl.multiple_of(((sec + 1) * TM + half * HM) // 2, HM // 2)
            dstr = pl.multiple_of(HALO + half * HM, 16)
            for r in range(0, HM // 2, 8):
                vs = _butterfly([q_scr[g, pl.ds(src + r, 8), :] for g in range(NG)])
                for g in range(NG):
                    kv_scr[sec, g, pl.ds(dstr + 2 * r, 16), :] = _unpack(vs[g])
            lb = jnp.minimum(j, 1)
            u0 = 2 * jnp.clip(j - 1, 0, 3)
            tok = ln_unit(lb, pl.multiple_of(u0 * 16, 16), None)
            ln_unit(lb, pl.multiple_of(u0 * 16 + 16, 16), tok)
            y = _dot(xn, wqkv[k])
            rb = pl.multiple_of(lax.rem(lax.div(j, 2) + 1, 3) * (TM // 2), TM // 2)
            for gg in range(WC // 128):
                q_scr[half * (WC // 128) + gg, pl.ds(rb, TM // 2), :] = _pack(y[:, gg * 128:(gg + 1) * 128])
            return carry

        lax.fori_loop(0, NWC, body, 0)

    @pl.when(s <= NA + 1)
    def _():
        @pl.when(s < NCH)
        def _():
            for cp in raw_copies(s):
                cp.start(priority=1)

        @pl.when(s < NB - 3)
        def _():
            x_copy(s + 3).start(priority=1)

        @pl.when(s == NCH)
        def _():
            wo_copy().start(priority=1)

        @pl.when(jnp.logical_and(s >= 2, s <= NA))
        def _():
            for cp in raw_copies(s - 2):
                cp.wait()

        @pl.when(jnp.logical_and(s >= 1, s < NB - 1))
        def _():
            x_copy(s + 1).wait()

        @pl.when(s == NA + 1)
        def _():
            wo_copy().wait()

    @pl.when(jnp.logical_and(s >= 1, s <= NA))
    def _():
        r0 = pl.multiple_of(TM + (s - 1) * TA, 16)
        xn = xn_scr[pl.ds(r0, TA), :]
        ys = [jnp.concatenate([_dot(xn, wqkv[2 * sec]), _dot(xn, wqkv[2 * sec + 1])], axis=1) for sec in (1, 2, 0)]
        tok = ln_block(jnp.minimum(s + 1, NB - 1), chain=True)
        c = lax.rem(s + (NCH - 2), NCH)
        never4 = lax.broadcasted_iota(jnp.int32, (4, 128), 0) < jnp.minimum(s, 0)

        def build(raw, cmb, kq, nq, tok):
            def ld(r, n, tok4):
                t = pltpu.bitcast(raw[c, r:r + 8, n:n + 128], F32)
                return pltpu.bitcast(_dep32(t, tok4, never4), BF).astype(F32)

            for r in range(0, kq, 16):
                for n0 in range(0, nq, 128):
                    cnt[0] += 1
                    if cnt[0] % ROLL_EVERY == 0:
                        tok = pltpu.roll(tok, 1, 1)
                    for _ in range(N_EUP):
                        tok = jnp.exp2(tok)
                    tok4 = tok[0:4]
                    b11, b12, b21, b22 = [
                        jnp.concatenate([ld(rr, nn, tok4), ld(rr + 8, nn, tok4)], axis=0)
                        for rr, nn in ((r, n0), (r, nq + n0), (kq + r, n0), (kq + r, nq + n0))]
                    outs = [(b11 + b22).astype(BF), (b12 - b22).astype(BF), (b21 - b11).astype(BF),
                            (b11 + b12).astype(BF), (b21 + b22).astype(BF)]
                    for j in range(5):
                        cmb[c, j, r:r + 16, n0:n0 + 128] = outs[j]
                    tok = pltpu.bitcast(outs[0], F32)
            return tok

        cnt = [0]
        if not LN_FIRST:
            tok = jnp.zeros((8, 128), F32)
        tok = build(rawg, cg, HD, FC, tok)
        tok = build(rawu, cu, HD, FC, tok)
        tok = build(rawd, cd, FC, HD, tok)
        store_kv(ys[0], k_scr, r0)
        store_kv(ys[1], v_scr, r0)
        store_q(ys[2], r0)

    if NSTEPS < NA + 1 + NB:
        @pl.when(s == NSTEPS - 1)
        def _():
            l = NSTEPS - 1
            for c in (l - 1, l):
                if 0 <= c < NCH:
                    for cp in raw_copies(c):
                        cp.wait()
            for b in (l + 2, l + 3):
                if b < NB:
                    x_copy(b).wait()
            if NCH <= l <= NA:
                wo_copy().wait()

    @pl.when(s > NA)
    def _():
        i = s - (NA + 1)
        r0 = pl.multiple_of(i * TM, TM)

        def wlist(raw, cmb, c, kq, nq):
            return [cmb[c, 0], raw[c, 0:kq, 0:nq], cmb[c, 1], cmb[c, 2],
                    raw[c, kq:2 * kq, nq:2 * nq], cmb[c, 3], cmb[c, 4]]

        RA = 16
        cexp = (DH ** -0.5) * LOG2E
        p0 = pl.multiple_of(r0 // 2, 8)
        never16 = lax.broadcasted_iota(jnp.int32, (16, 128), 0) < jnp.minimum(s, 0)

        def attn_half(q, r):
            sw = []
            for w in range(WIN):
                acc = None
                for g in range(NG):
                    t = q[g] * k_scr[g, pl.ds(r0 + r + HALO - DIL * w, 8), :]
                    acc = t if acc is None else acc + t
                acc = _sum4(acc)
                if r < HALO and w > 0:
                    row = lax.broadcasted_iota(jnp.int32, (8, 128), 0) + (r0 + r)
                    acc = jnp.where(row >= DIL * w, acc, NEG)
                sw.append(acc)
            m = sw[0]
            for w in range(1, WIN):
                m = jnp.maximum(m, sw[w])
            e = [jnp.exp2((sw[w] - m) * cexp) for w in range(WIN)]
            den = e[0]
            for w in range(1, WIN):
                den = den + e[w]
            inv = 1.0 / den
            p = [e[w] * inv for w in range(WIN)]
            o = []
            for g in range(NG):
                acc = None
                for w in range(WIN):
                    t = p[w] * v_scr[g, pl.ds(r0 + r + HALO - DIL * w, 8), :]
                    acc = t if acc is None else acc + t
                o.append(acc)
            return o

        def attn_rows(r, tok):
            qp = [q_scr[g, pl.ds(p0 + r // 2, 8), :] for g in range(NG)]
            if tok is not None:
                qp = [_dep32(t, tok, never) for t in qp]
            q = [_unpack(t) for t in _butterfly(qp)]
            o0 = attn_half([t[0:8] for t in q], r)
            q1 = [t[8:16] for t in q]
            if CHAIN_HALVES:
                q1 = [_dep32(t, o0[NG - 1], never) for t in q1]
            o1 = attn_half(q1, r + 8)
            o = _butterfly([_pack(jnp.concatenate([o0[g], o1[g]], axis=0)) for g in range(NG)])
            for g in range(NG):
                o_scr[r:r + RA, g * 128:(g + 1) * 128] = pltpu.bitcast(o[g], BF)
            tok = o[0]
            if XOR_TOK:
                for g in range(1, NG):
                    tok = tok ^ o[g]
            return tok

        sl = [s_scr[i, j] for j in range(7)]
        acc = [None] * 7
        o_parts = []
        n_att = TM // RA
        per = 3
        tok = None
        for c in range(NCH):
            wg_l = wlist(rawg, cg, c, HD, FC)
            wu_l = wlist(rawu, cu, c, HD, FC)
            wd_l = wlist(rawd, cd, c, FC, HD)
            slc = sl
            g = _strassen_out([_dot(slc[j], wg_l[j]) for j in range(7)])
            u = _strassen_out([_dot(slc[j], wu_l[j]) for j in range(7)])
            hq = [g[t] * u[t] for t in range(4)]
            hl = [t.astype(BF) for t in _lhs_combos(*hq)]
            for j in range(7):
                y = _dot(hl[j], wd_l[j])
                acc[j] = y if acc[j] is None else acc[j] + y
            for a in range(c * per, min((c + 1) * per, n_att)):
                tok = attn_rows(a * RA, tok)
        ao = _dot(o_scr[...], wo[...])
        y11, y12, y21, y22 = _strassen_out(acc)
        x = x_scr[pl.ds(r0, TM), :].astype(F32)
        o_ref[0:HM, 0:HD] = (x[0:HM, 0:HD] + ao[0:HM, 0:HD] + y11).astype(o_ref.dtype)
        o_ref[0:HM, HD:D] = (x[0:HM, HD:D] + ao[0:HM, HD:D] + y12).astype(o_ref.dtype)
        o_ref[HM:TM, 0:HD] = (x[HM:TM, 0:HD] + ao[HM:TM, 0:HD] + y21).astype(o_ref.dtype)
        o_ref[HM:TM, HD:D] = (x[HM:TM, HD:D] + ao[HM:TM, HD:D] + y22).astype(o_ref.dtype)


@jax.jit
def pallas_parallel_sum__sliding_local_dilated__glu_gated_bilinear__prompt_kernel(
    A_x: jax.Array,
    A_wqkv: jax.Array,
    A_wo: jax.Array,
    B_x: jax.Array,
    B_w_gate: jax.Array,
    B_w_up: jax.Array,
    B_w_down: jax.Array,
):
    del B_x
    x = A_x.reshape(S, D)
    hbm = pl.BlockSpec(memory_space=pl.ANY)
    out = pl.pallas_call(
        _kernel,
        grid=(NSTEPS,),
        in_specs=[hbm] * 6,
        out_specs=pl.BlockSpec((TM, D), lambda s: (jnp.maximum(s - (NA + 1), 0), 0)),
        out_shape=jax.ShapeDtypeStruct((S, D), A_x.dtype),
        scratch_shapes=[
            pltpu.VMEM((S, D), BF),
            pltpu.VMEM((NWC, D, WC), BF),
            pltpu.VMEM((D, D), BF),
            pltpu.VMEM((NCH, D, 2 * FC), BF),
            pltpu.VMEM((NCH, D, 2 * FC), BF),
            pltpu.VMEM((NCH, 2 * FC, D), BF),
            pltpu.VMEM((NCH, 5, HD, FC), BF),
            pltpu.VMEM((NCH, 5, HD, FC), BF),
            pltpu.VMEM((NCH, 5, FC, HD), BF),
            pltpu.VMEM((S, D), BF),
            pltpu.VMEM((NB, 7, HM, HD), BF),
            pltpu.VMEM((NG, S // 2, 128), U32),
            pltpu.VMEM((2, NG, S + HALO, 128), F32),
            pltpu.VMEM((TM, D), BF),
            pltpu.SemaphoreType.DMA((NB,)),
            pltpu.SemaphoreType.DMA((NWC + 1,)),
            pltpu.SemaphoreType.DMA((NCH, 6)),
        ],
        compiler_params=pltpu.CompilerParams(
            dimension_semantics=("arbitrary",),
            vmem_limit_bytes=124 * 1024 * 1024,
            disable_bounds_checks=True,
        ),
        name="fused_attn_ffn",
    )(x, A_wqkv, A_wo, B_w_gate, B_w_up, B_w_down)
    return out.reshape(A_x.shape)
```

```python
import functools

import jax
import jax.numpy as jnp
from jax import lax
from jax.experimental import pallas as pl
from jax.experimental.pallas import tpu as pltpu

S, D, F = 2048, 1024, 3584
H, DH, WIN, DIL = 32, 32, 8, 2
TM = 256
HM = TM // 2
NB = S // TM
HD = D // 2
FC = 256
NCH = F // 2 // FC
HALO = 16
NG = D // 128
EPS = 1e-5
NEG = -1e9
BF = jnp.bfloat16
F32 = jnp.float32
U32 = jnp.uint32
LOG2E = 1.4426950408889634
NA = 8
TA = (S - TM) // NA
NSTEPS = 17
WC = 512
NWC = 3 * D // WC
N_EUP = 3
N_EUP0 = 2
CHAIN_HALVES = True
XOR_TOK = False


def _dot(a, b):
    return jnp.dot(a, b, preferred_element_type=F32)


def _butterfly(vs):
    lane = lax.broadcasted_iota(jnp.int32, vs[0].shape, 1)
    for b in range(3):
        sh = 4 << b
        bit = (lane & sh) != 0
        new = list(vs)
        for i0 in range(NG):
            if i0 & (1 << b):
                continue
            i1 = i0 | (1 << b)
            new[i0] = jnp.where(bit, pltpu.roll(vs[i1], sh, 1), vs[i0])
            new[i1] = jnp.where(bit, vs[i1], pltpu.roll(vs[i0], 128 - sh, 1))
        vs = new
    return vs


def _sum4(x):
    lane = lax.broadcasted_iota(jnp.int32, x.shape, 1)
    x = x + jnp.where((lane & 1) != 0, pltpu.roll(x, 1, 1), pltpu.roll(x, 127, 1))
    x = x + jnp.where((lane & 2) != 0, pltpu.roll(x, 2, 1), pltpu.roll(x, 126, 1))
    return x


def _dep32(x, tok, never):
    return jnp.where(never, pltpu.bitcast(tok, x.dtype), x)


def _gate(m, tok, never):
    t = pltpu.bitcast(m[0:16, 0:128], F32)
    t = pltpu.bitcast(_dep32(t, tok, never), BF)
    top = jnp.concatenate([t, m[0:16, 128:]], axis=1)
    if m.shape[0] == 16:
        return top
    return jnp.concatenate([top, m[16:]], axis=0)


def _pack(y):
    return pltpu.bitcast(y.astype(BF), U32)


def _unpack(w):
    return pltpu.bitcast(w, BF).astype(F32)


def _lhs_combos(a11, a12, a21, a22):
    return [a11 + a22, a21 + a22, a11, a22, a11 + a12, a21 - a11, a12 - a22]


def _strassen_out(m):
    return (m[0] + m[3] - m[4] + m[6], m[2] + m[4], m[1] + m[3], m[0] - m[1] + m[2] + m[5])


def _layernorm(x):
    x = x.astype(F32)
    mean = jnp.mean(x, axis=-1, keepdims=True)
    xc = x - mean
    var = jnp.mean(xc * xc, axis=-1, keepdims=True)
    return xc * lax.rsqrt(var + EPS)


def _kernel(x_hbm, wqkv_hbm, wo_hbm, wg_hbm, wu_hbm, wd_hbm, o_ref,
            x_scr, wqkv, wo, rawg, rawu, rawd, cq, cg, cu, cd,
            xn_scr, s_scr, q_scr, kv_scr, o_scr,
            sem_x, sem_w, sem_raw):
    s = pl.program_id(0)
    k_scr = kv_scr.at[0]
    v_scr = kv_scr.at[1]

    def x_copy(b):
        return pltpu.make_async_copy(x_hbm.at[pl.ds(b * TM, TM), :], x_scr.at[pl.ds(b * TM, TM), :], sem_x.at[b])

    def wqkv_copy(k):
        return pltpu.make_async_copy(wqkv_hbm.at[:, pl.ds(k * WC, WC)], wqkv.at[k], sem_w.at[k])

    def wo_copy():
        return pltpu.make_async_copy(wo_hbm, wo, sem_w.at[NWC])

    def raw_copies(c):
        return [
            pltpu.make_async_copy(wg_hbm.at[:, pl.ds(c * FC, FC)], rawg.at[c, :, pl.ds(0, FC)], sem_raw.at[c, 0]),
            pltpu.make_async_copy(wg_hbm.at[:, pl.ds(F // 2 + c * FC, FC)], rawg.at[c, :, pl.ds(FC, FC)], sem_raw.at[c, 1]),
            pltpu.make_async_copy(wu_hbm.at[:, pl.ds(c * FC, FC)], rawu.at[c, :, pl.ds(0, FC)], sem_raw.at[c, 2]),
            pltpu.make_async_copy(wu_hbm.at[:, pl.ds(F // 2 + c * FC, FC)], rawu.at[c, :, pl.ds(FC, FC)], sem_raw.at[c, 3]),
            pltpu.make_async_copy(wd_hbm.at[pl.ds(c * FC, FC), :], rawd.at[c, pl.ds(0, FC), :], sem_raw.at[c, 4]),
            pltpu.make_async_copy(wd_hbm.at[pl.ds(F // 2 + c * FC, FC), :], rawd.at[c, pl.ds(FC, FC), :], sem_raw.at[c, 5]),
        ]

    never = lax.broadcasted_iota(jnp.int32, (8, 128), 0) < jnp.minimum(s, 0)

    def ln_unit(b, r, tok):
        RC = 16
        r0 = pl.multiple_of(b * TM + r, RC)
        xt = x_scr[pl.ds(r0, RC), :]
        xb = x_scr[pl.ds(r0 + HM, RC), :]
        if tok is not None:
            xt = _gate(xt, tok, never)
            xb = _gate(xb, tok, never)
        top = _layernorm(xt)
        bot = _layernorm(xb)
        xn_scr[pl.ds(r0, RC), :] = top.astype(BF)
        xn_scr[pl.ds(r0 + HM, RC), :] = bot.astype(BF)
        cs = _lhs_combos(top[:, :HD], top[:, HD:], bot[:, :HD], bot[:, HD:])
        for j in range(7):
            s_scr[b, j, pl.ds(r, RC), :] = cs[j].astype(BF)
        return top[0:8, 0:128] + bot[0:8, 0:128]

    def ln_block(b, chain=False):
        tok = None
        for r in range(0, HM, 16):
            t = ln_unit(b, r, tok)
            tok = t if chain else None
        return tok

    def store_kv(y, dst, r0):
        for r in range(0, y.shape[0], 16):
            vs = _butterfly([_pack(y[r:r + 16, g * 128:(g + 1) * 128]) for g in range(NG)])
            for g in range(NG):
                dst[g, pl.ds(r0 + HALO + r, 16), :] = _unpack(vs[g])

    def store_q(y, r0):
        p0 = pl.multiple_of(r0 // 2, 8)
        for g in range(NG):
            q_scr[g, pl.ds(p0, y.shape[0] // 2), :] = _pack(y[:, g * 128:(g + 1) * 128])

    never4 = lax.broadcasted_iota(jnp.int32, (4, 128), 0) < jnp.minimum(s, 0)

    def build_tiles(ld8, st16, positions, tok, n_eup):
        for r, n0 in positions:
            for _ in range(n_eup):
                tok = jnp.exp2(tok)
            tok4 = tok[0:4]

            def ld(q, rr):
                t = pltpu.bitcast(ld8(q, rr, n0), F32)
                return pltpu.bitcast(_dep32(t, tok4, never4), BF).astype(F32)

            b11, b12, b21, b22 = [jnp.concatenate([ld(q, r), ld(q, r + 8)], axis=0) for q in range(4)]
            outs = [(b11 + b22).astype(BF), (b12 - b22).astype(BF), (b21 - b11).astype(BF),
                    (b11 + b12).astype(BF), (b21 + b22).astype(BF)]
            for j in range(5):
                st16(j, r, n0, outs[j])
            tok = pltpu.bitcast(outs[0], F32)
        return tok

    def build_qkv(sec, kl, kr, rb, n_eup):
        def ld8(q, r, n):
            return wqkv[kl if q in (0, 2) else kr, pl.ds((HD if q >= 2 else 0) + rb + r, 8), n:n + 128]

        def st16(j, r, n, val):
            cq[sec, j, pl.ds(rb + r, 16), n:n + 128] = val

        build_tiles(ld8, st16, [(r, n) for r in range(0, HD // 2, 16) for n in range(0, WC, 128)],
                    jnp.zeros((8, 128), F32), n_eup)

    @pl.when(s == 0)
    def _():
        x_copy(0).start(priority=1)

        def issue(j, carry):
            @pl.when(j == 1)
            def _():
                x_copy(1).start(priority=1)

            wqkv_copy(lax.rem(j + 2, NWC)).start(priority=1)
            return carry

        lax.fori_loop(0, NWC, issue, 0)
        x_copy(2).start(priority=1)
        k_scr[:, 0:HALO, :] = jnp.zeros((NG, HALO, 128), F32)
        v_scr[:, 0:HALO, :] = jnp.zeros((NG, HALO, 128), F32)
        x_copy(0).wait()
        ln_block(0)
        xn = xn_scr[0:TM, :]

        def body(j, carry):
            k = lax.rem(j + 2, NWC)
            wqkv_copy(k).wait()

            @pl.when(j == 1)
            def _():
                x_copy(1).wait()

            half = lax.rem(j, 2)
            sec = jnp.maximum(lax.div(j, 2) - 1, 0)
            src = pl.multiple_of(((sec + 1) * TM + half * HM) // 2, HM // 2)
            dstr = pl.multiple_of(HALO + half * HM, 16)
            for r in range(0, HM // 2, 8):
                vs = _butterfly([q_scr[g, pl.ds(src + r, 8), :] for g in range(NG)])
                for g in range(NG):
                    kv_scr[sec, g, pl.ds(dstr + 2 * r, 16), :] = _unpack(vs[g])
            lb = jnp.minimum(j, 1)
            u0 = 2 * jnp.clip(j - 1, 0, 3)
            tok = ln_unit(lb, pl.multiple_of(u0 * 16, 16), None)
            ln_unit(lb, pl.multiple_of(u0 * 16 + 16, 16), tok)
            jm = jnp.maximum(j - 1, 0)
            bsec = lax.div(jm, 2)
            kl = lax.rem(2 * bsec + 2, NWC)
            kr = jnp.where(j == 0, kl, kl + 1)
            bh = jnp.where(j == 0, 1, lax.rem(jm, 2))
            build_qkv(bsec, kl, kr, pl.multiple_of(bh * (HD // 2), HD // 2), N_EUP0)
            y = _dot(xn, wqkv[k])
            rb = pl.multiple_of(lax.rem(lax.div(j, 2) + 1, 3) * (TM // 2), TM // 2)
            for gg in range(WC // 128):
                q_scr[half * (WC // 128) + gg, pl.ds(rb, TM // 2), :] = _pack(y[:, gg * 128:(gg + 1) * 128])
            return carry

        lax.fori_loop(0, NWC, body, 0)
        build_qkv(2, 0, 1, HD // 2, 0)

    @pl.when(s <= NA + 1)
    def _():
        @pl.when(s < NCH)
        def _():
            for cp in raw_copies(s):
                cp.start(priority=1)

        @pl.when(s < NB - 3)
        def _():
            x_copy(s + 3).start(priority=1)

        @pl.when(s == NCH)
        def _():
            wo_copy().start(priority=1)

        @pl.when(jnp.logical_and(s >= 2, s <= NA))
        def _():
            for cp in raw_copies(s - 2):
                cp.wait()

        @pl.when(jnp.logical_and(s >= 1, s < NB - 1))
        def _():
            x_copy(s + 1).wait()

        @pl.when(s == NA + 1)
        def _():
            wo_copy().wait()

    @pl.when(jnp.logical_and(s >= 1, s <= NA))
    def _():
        r0 = pl.multiple_of(TM + (s - 1) * TA, 16)
        HA = TA // 2
        a11 = xn_scr[pl.ds(r0, HA), 0:HD]
        a12 = xn_scr[pl.ds(r0, HA), HD:D]
        a21 = xn_scr[pl.ds(r0 + HA, HA), 0:HD]
        a22 = xn_scr[pl.ds(r0 + HA, HA), HD:D]
        la = [t.astype(BF) for t in _lhs_combos(a11.astype(F32), a12.astype(F32), a21.astype(F32), a22.astype(F32))]
        la[2], la[3] = a11, a22
        ys = []
        for sec in range(3):
            kl = (2 * sec + 2) % NWC
            wl = [cq[sec, 0], wqkv[kl, 0:HD, :], cq[sec, 1], cq[sec, 2], wqkv[kl + 1, HD:D, :], cq[sec, 3], cq[sec, 4]]
            c11, c12, c21, c22 = _strassen_out([_dot(la[j], wl[j]) for j in range(7)])
            ys.append((jnp.concatenate([c11, c12], axis=1), jnp.concatenate([c21, c22], axis=1)))
        ln_block(jnp.minimum(s + 1, NB - 1), chain=True)
        c = lax.rem(s + (NCH - 2), NCH)

        def build(raw, cmb, kq, nq, tok):
            def ld8(q, r, n):
                return raw[c, pl.ds((kq if q >= 2 else 0) + r, 8), pl.ds((nq if q % 2 else 0) + n, 128)]

            def st16(j, r, n, val):
                cmb[c, j, r:r + 16, n:n + 128] = val

            return build_tiles(ld8, st16, [(r, n) for r in range(0, kq, 16) for n in range(0, nq, 128)], tok, N_EUP)

        tok = jnp.zeros((8, 128), F32)
        tok = build(rawg, cg, HD, FC, tok)
        tok = build(rawu, cu, HD, FC, tok)
        tok = build(rawd, cd, FC, HD, tok)
        for h in range(2):
            rh = pl.multiple_of(r0 + h * HA, 16)
            store_kv(ys[0][h], k_scr, rh)
            store_kv(ys[1][h], v_scr, rh)
            store_q(ys[2][h], rh)

    if NSTEPS < NA + 1 + NB:
        @pl.when(s == NSTEPS - 1)
        def _():
            l = NSTEPS - 1
            for c in (l - 1, l):
                if 0 <= c < NCH:
                    for cp in raw_copies(c):
                        cp.wait()
            for b in (l + 2, l + 3):
                if b < NB:
                    x_copy(b).wait()
            if NCH <= l <= NA:
                wo_copy().wait()

    @pl.when(s > NA)
    def _():
        i = s - (NA + 1)
        r0 = pl.multiple_of(i * TM, TM)

        def wlist(raw, cmb, c, kq, nq):
            return [cmb[c, 0], raw[c, 0:kq, 0:nq], cmb[c, 1], cmb[c, 2],
                    raw[c, kq:2 * kq, nq:2 * nq], cmb[c, 3], cmb[c, 4]]

        RA = 16
        cexp = (DH ** -0.5) * LOG2E
        p0 = pl.multiple_of(r0 // 2, 8)
        never16 = lax.broadcasted_iota(jnp.int32, (16, 128), 0) < jnp.minimum(s, 0)

        def attn_half(q, r):
            sw = []
            for w in range(WIN):
                acc = None
                for g in range(NG):
                    t = q[g] * k_scr[g, pl.ds(r0 + r + HALO - DIL * w, 8), :]
                    acc = t if acc is None else acc + t
                acc = _sum4(acc)
                if r < HALO and w > 0:
                    row = lax.broadcasted_iota(jnp.int32, (8, 128), 0) + (r0 + r)
                    acc = jnp.where(row >= DIL * w, acc, NEG)
                sw.append(acc)
            m = sw[0]
            for w in range(1, WIN):
                m = jnp.maximum(m, sw[w])
            e = [jnp.exp2((sw[w] - m) * cexp) for w in range(WIN)]
            den = e[0]
            for w in range(1, WIN):
                den = den + e[w]
            inv = 1.0 / den
            p = [e[w] * inv for w in range(WIN)]
            o = []
            for g in range(NG):
                acc = None
                for w in range(WIN):
                    t = p[w] * v_scr[g, pl.ds(r0 + r + HALO - DIL * w, 8), :]
                    acc = t if acc is None else acc + t
                o.append(acc)
            return o

        def attn_rows(r, tok):
            qp = [q_scr[g, pl.ds(p0 + r // 2, 8), :] for g in range(NG)]
            if tok is not None:
                qp = [_dep32(t, tok, never) for t in qp]
            q = [_unpack(t) for t in _butterfly(qp)]
            o0 = attn_half([t[0:8] for t in q], r)
            q1 = [t[8:16] for t in q]
            if CHAIN_HALVES:
                q1 = [_dep32(t, o0[NG - 1], never) for t in q1]
            o1 = attn_half(q1, r + 8)
            o = _butterfly([_pack(jnp.concatenate([o0[g], o1[g]], axis=0)) for g in range(NG)])
            for g in range(NG):
                o_scr[r:r + RA, g * 128:(g + 1) * 128] = pltpu.bitcast(o[g], BF)
            tok = o[0]
            if XOR_TOK:
                for g in range(1, NG):
                    tok = tok ^ o[g]
            return tok

        sl = [s_scr[i, j] for j in range(7)]
        acc = [None] * 7
        o_parts = []
        n_att = TM // RA
        per = 3
        tok = None
        for c in range(NCH):
            wg_l = wlist(rawg, cg, c, HD, FC)
            wu_l = wlist(rawu, cu, c, HD, FC)
            wd_l = wlist(rawd, cd, c, FC, HD)
            slc = sl
            g = _strassen_out([_dot(slc[j], wg_l[j]) for j in range(7)])
            u = _strassen_out([_dot(slc[j], wu_l[j]) for j in range(7)])
            hq = [g[t] * u[t] for t in range(4)]
            hl = [t.astype(BF) for t in _lhs_combos(*hq)]
            for j in range(7):
                y = _dot(hl[j], wd_l[j])
                acc[j] = y if acc[j] is None else acc[j] + y
            for a in range(c * per, min((c + 1) * per, n_att)):
                tok = attn_rows(a * RA, tok)
        ao = _dot(o_scr[...], wo[...])
        y11, y12, y21, y22 = _strassen_out(acc)
        x = x_scr[pl.ds(r0, TM), :].astype(F32)
        o_ref[0:HM, 0:HD] = (x[0:HM, 0:HD] + ao[0:HM, 0:HD] + y11).astype(o_ref.dtype)
        o_ref[0:HM, HD:D] = (x[0:HM, HD:D] + ao[0:HM, HD:D] + y12).astype(o_ref.dtype)
        o_ref[HM:TM, 0:HD] = (x[HM:TM, 0:HD] + ao[HM:TM, 0:HD] + y21).astype(o_ref.dtype)
        o_ref[HM:TM, HD:D] = (x[HM:TM, HD:D] + ao[HM:TM, HD:D] + y22).astype(o_ref.dtype)


@jax.jit
def pallas_parallel_sum__sliding_local_dilated__glu_gated_bilinear__prompt_kernel(
    A_x: jax.Array,
    A_wqkv: jax.Array,
    A_wo: jax.Array,
    B_x: jax.Array,
    B_w_gate: jax.Array,
    B_w_up: jax.Array,
    B_w_down: jax.Array,
):
    del B_x
    x = A_x.reshape(S, D)
    hbm = pl.BlockSpec(memory_space=pl.ANY)
    out = pl.pallas_call(
        _kernel,
        grid=(NSTEPS,),
        in_specs=[hbm] * 6,
        out_specs=pl.BlockSpec((TM, D), lambda s: (jnp.maximum(s - (NA + 1), 0), 0)),
        out_shape=jax.ShapeDtypeStruct((S, D), A_x.dtype),
        scratch_shapes=[
            pltpu.VMEM((S, D), BF),
            pltpu.VMEM((NWC, D, WC), BF),
            pltpu.VMEM((D, D), BF),
            pltpu.VMEM((NCH, D, 2 * FC), BF),
            pltpu.VMEM((NCH, D, 2 * FC), BF),
            pltpu.VMEM((NCH, 2 * FC, D), BF),
            pltpu.VMEM((3, 5, HD, WC), BF),
            pltpu.VMEM((NCH, 5, HD, FC), BF),
            pltpu.VMEM((NCH, 5, HD, FC), BF),
            pltpu.VMEM((NCH, 5, FC, HD), BF),
            pltpu.VMEM((S, D), BF),
            pltpu.VMEM((NB, 7, HM, HD), BF),
            pltpu.VMEM((NG, S // 2, 128), U32),
            pltpu.VMEM((2, NG, S + HALO, 128), F32),
            pltpu.VMEM((TM, D), BF),
            pltpu.SemaphoreType.DMA((NB,)),
            pltpu.SemaphoreType.DMA((NWC + 1,)),
            pltpu.SemaphoreType.DMA((NCH, 6)),
        ],
        compiler_params=pltpu.CompilerParams(
            dimension_semantics=("arbitrary",),
            vmem_limit_bytes=124 * 1024 * 1024,
            disable_bounds_checks=True,
        ),
        name="fused_attn_ffn",
    )(x, A_wqkv, A_wo, B_w_gate, B_w_up, B_w_down)
    return out.reshape(A_x.shape)
```

```python
import functools

import jax
import jax.numpy as jnp
from jax import lax
from jax.experimental import pallas as pl
from jax.experimental.pallas import tpu as pltpu

S, D, F = 2048, 1024, 3584
H, DH, WIN, DIL = 32, 32, 8, 2
TM = 256
HM = TM // 2
NB = S // TM
HD = D // 2
FC = 256
NCH = F // 2 // FC
HALO = 16
NG = D // 128
EPS = 1e-5
NEG = -1e9
BF = jnp.bfloat16
F32 = jnp.float32
U32 = jnp.uint32
LOG2E = 1.4426950408889634
NA = 8
TA = (S - TM) // NA
NSTEPS = 17
WC = 512
NWC = 3 * D // WC
N_EUP = 3
N_EUP0 = 2
CHAIN_HALVES = True
XOR_TOK = False


def _dot(a, b):
    return jnp.dot(a, b, preferred_element_type=F32)


def _butterfly(vs):
    lane = lax.broadcasted_iota(jnp.int32, vs[0].shape, 1)
    for b in range(3):
        sh = 4 << b
        bit = (lane & sh) != 0
        new = list(vs)
        for i0 in range(NG):
            if i0 & (1 << b):
                continue
            i1 = i0 | (1 << b)
            new[i0] = jnp.where(bit, pltpu.roll(vs[i1], sh, 1), vs[i0])
            new[i1] = jnp.where(bit, vs[i1], pltpu.roll(vs[i0], 128 - sh, 1))
        vs = new
    return vs


def _sum4(x):
    lane = lax.broadcasted_iota(jnp.int32, x.shape, 1)
    x = x + jnp.where((lane & 1) != 0, pltpu.roll(x, 1, 1), pltpu.roll(x, 127, 1))
    x = x + jnp.where((lane & 2) != 0, pltpu.roll(x, 2, 1), pltpu.roll(x, 126, 1))
    return x


def _dep32(x, tok, never):
    return jnp.where(never, pltpu.bitcast(tok, x.dtype), x)


def _gate(m, tok, never):
    t = pltpu.bitcast(m[0:16, 0:128], F32)
    t = pltpu.bitcast(_dep32(t, tok, never), BF)
    top = jnp.concatenate([t, m[0:16, 128:]], axis=1)
    if m.shape[0] == 16:
        return top
    return jnp.concatenate([top, m[16:]], axis=0)


def _pack(y):
    return pltpu.bitcast(y.astype(BF), U32)


def _as_bf16(w):
    return pltpu.bitcast(w, BF)


def _unpack(w):
    return pltpu.bitcast(w, BF).astype(F32)


def _lhs_combos(a11, a12, a21, a22):
    return [a11 + a22, a21 + a22, a11, a22, a11 + a12, a21 - a11, a12 - a22]


def _strassen_out(m):
    return (m[0] + m[3] - m[4] + m[6], m[2] + m[4], m[1] + m[3], m[0] - m[1] + m[2] + m[5])


def _layernorm(x):
    x = x.astype(F32)
    mean = jnp.mean(x, axis=-1, keepdims=True)
    xc = x - mean
    var = jnp.mean(xc * xc, axis=-1, keepdims=True)
    return xc * lax.rsqrt(var + EPS)


def _kernel(x_hbm, wqkv_hbm, wo_hbm, wg_hbm, wu_hbm, wd_hbm, o_ref,
            x_scr, wqkv, wo, rawg, rawu, rawd, cq, cg, cu, cd,
            xn_scr, s_scr, q_scr, kv_scr, o_scr,
            sem_x, sem_w, sem_raw):
    s = pl.program_id(0)
    k_scr = kv_scr.at[0]
    v_scr = kv_scr.at[1]

    def x_copy(b):
        return pltpu.make_async_copy(x_hbm.at[pl.ds(b * TM, TM), :], x_scr.at[pl.ds(b * TM, TM), :], sem_x.at[b])

    def wqkv_copy(k):
        return pltpu.make_async_copy(wqkv_hbm.at[:, pl.ds(k * WC, WC)], wqkv.at[k], sem_w.at[k])

    def wo_copy():
        return pltpu.make_async_copy(wo_hbm, wo, sem_w.at[NWC])

    def raw_copies(c):
        return [
            pltpu.make_async_copy(wg_hbm.at[:, pl.ds(c * FC, FC)], rawg.at[c, :, pl.ds(0, FC)], sem_raw.at[c, 0]),
            pltpu.make_async_copy(wg_hbm.at[:, pl.ds(F // 2 + c * FC, FC)], rawg.at[c, :, pl.ds(FC, FC)], sem_raw.at[c, 1]),
            pltpu.make_async_copy(wu_hbm.at[:, pl.ds(c * FC, FC)], rawu.at[c, :, pl.ds(0, FC)], sem_raw.at[c, 2]),
            pltpu.make_async_copy(wu_hbm.at[:, pl.ds(F // 2 + c * FC, FC)], rawu.at[c, :, pl.ds(FC, FC)], sem_raw.at[c, 3]),
            pltpu.make_async_copy(wd_hbm.at[pl.ds(c * FC, FC), :], rawd.at[c, pl.ds(0, FC), :], sem_raw.at[c, 4]),
            pltpu.make_async_copy(wd_hbm.at[pl.ds(F // 2 + c * FC, FC), :], rawd.at[c, pl.ds(FC, FC), :], sem_raw.at[c, 5]),
        ]

    never = lax.broadcasted_iota(jnp.int32, (8, 128), 0) < jnp.minimum(s, 0)

    def ln_unit(b, r, tok):
        RC = 16
        r0 = pl.multiple_of(b * TM + r, RC)
        xt = x_scr[pl.ds(r0, RC), :]
        xb = x_scr[pl.ds(r0 + HM, RC), :]
        if tok is not None:
            xt = _gate(xt, tok, never)
            xb = _gate(xb, tok, never)
        top = _layernorm(xt)
        bot = _layernorm(xb)
        p0 = pl.multiple_of(r0 // 2, RC // 2)
        xn_scr[pl.ds(p0, RC // 2), :] = _pack(top)
        xn_scr[pl.ds(p0 + HM // 2, RC // 2), :] = _pack(bot)
        cs = _lhs_combos(top[:, :HD], top[:, HD:], bot[:, :HD], bot[:, HD:])
        pr = r // 2 if isinstance(r, int) else pl.multiple_of(r // 2, RC // 2)
        for j in range(7):
            s_scr[b, j, pl.ds(pr, RC // 2), :] = _pack(cs[j])
        return top[0:8, 0:128] + bot[0:8, 0:128]

    def ln_block(b, chain=False):
        tok = None
        for r in range(0, HM, 16):
            t = ln_unit(b, r, tok)
            tok = t if chain else None
        return tok

    def store_kv(y, dst, r0):
        for r in range(0, y.shape[0], 16):
            vs = _butterfly([_pack(y[r:r + 16, g * 128:(g + 1) * 128]) for g in range(NG)])
            for g in range(NG):
                dst[g, pl.ds(r0 + HALO + r, 16), :] = _unpack(vs[g])

    def store_q(y, r0):
        p0 = pl.multiple_of(r0 // 2, 8)
        for g in range(NG):
            q_scr[g, pl.ds(p0, y.shape[0] // 2), :] = _pack(y[:, g * 128:(g + 1) * 128])

    never4 = lax.broadcasted_iota(jnp.int32, (4, 128), 0) < jnp.minimum(s, 0)

    def build_tiles(ld8, st16, positions, tok, n_eup):
        for r, n0 in positions:
            for _ in range(n_eup or 0):
                tok = jnp.exp2(tok)
            tok4 = tok[0:4]

            def ld(q, rr):
                if n_eup is None:
                    return ld8(q, rr, n0).astype(F32)
                t = pltpu.bitcast(ld8(q, rr, n0), F32)
                return pltpu.bitcast(_dep32(t, tok4, never4), BF).astype(F32)

            b11, b12, b21, b22 = [jnp.concatenate([ld(q, r), ld(q, r + 8)], axis=0) for q in range(4)]
            outs = [_pack(b11 + b22), _pack(b12 - b22), _pack(b21 - b11), _pack(b11 + b12), _pack(b21 + b22)]
            for j in range(5):
                st16(j, r, n0, outs[j])
            tok = pltpu.bitcast(outs[0], F32)
        return tok

    def build_qkv(sec, kl, kr, bh, n_eup):
        rb = bh * (HD // 2)

        def row(r, m):
            return rb + r if isinstance(rb, int) else pl.multiple_of(rb + r, m)

        def ld8(q, r, n):
            return wqkv[kl if q in (0, 2) else kr, pl.ds(row((HD if q >= 2 else 0) + r, 8), 8), n:n + 128]

        def st16(j, r, n, val):
            cq[sec, bh, j, r // 2:r // 2 + 8, n:n + 128] = val

        build_tiles(ld8, st16, [(r, n) for r in range(0, HD // 2, 16) for n in range(0, WC, 128)],
                    jnp.zeros((8, 128), F32), n_eup)

    @pl.when(s == 0)
    def _():
        x_copy(0).start(priority=1)

        def issue(j, carry):
            @pl.when(j == 1)
            def _():
                x_copy(1).start(priority=1)

            wqkv_copy(lax.rem(j + 2, NWC)).start(priority=1)
            return carry

        lax.fori_loop(0, NWC, issue, 0)
        x_copy(2).start(priority=1)
        k_scr[:, 0:HALO, :] = jnp.zeros((NG, HALO, 128), F32)
        v_scr[:, 0:HALO, :] = jnp.zeros((NG, HALO, 128), F32)
        x_copy(0).wait()
        ln_block(0)
        xn = _as_bf16(xn_scr[0:TM // 2, :])

        def body(j, carry):
            k = lax.rem(j + 2, NWC)
            wqkv_copy(k).wait()

            @pl.when(j == 1)
            def _():
                x_copy(1).wait()

            y = _dot(xn, wqkv[k])
            half = lax.rem(j, 2)
            sec = jnp.maximum(lax.div(j, 2) - 1, 0)
            src = pl.multiple_of(((sec + 1) * TM + half * HM) // 2, HM // 2)
            dstr = pl.multiple_of(HALO + half * HM, 16)
            for r in range(0, HM // 2, 8):
                vs = _butterfly([q_scr[g, pl.ds(src + r, 8), :] for g in range(NG)])
                for g in range(NG):
                    kv_scr[sec, g, pl.ds(dstr + 2 * r, 16), :] = _unpack(vs[g])
            lb = jnp.minimum(j, 1)
            u0 = 2 * jnp.clip(j - 1, 0, 3)
            tok = ln_unit(lb, pl.multiple_of(u0 * 16, 16), None)
            ln_unit(lb, pl.multiple_of(u0 * 16 + 16, 16), tok)
            jm = jnp.maximum(j - 1, 0)
            bsec = lax.div(jm, 2)
            kl = lax.rem(2 * bsec + 2, NWC)
            kr = jnp.where(j == 0, kl, kl + 1)
            bh = jnp.where(j == 0, 1, lax.rem(jm, 2))
            build_qkv(bsec, kl, kr, bh, N_EUP0)
            rb = pl.multiple_of(lax.rem(lax.div(j, 2) + 1, 3) * (TM // 2), TM // 2)
            for gg in range(WC // 128):
                q_scr[half * (WC // 128) + gg, pl.ds(rb, TM // 2), :] = _pack(y[:, gg * 128:(gg + 1) * 128])
            return carry

        lax.fori_loop(0, NWC, body, 0)
        build_qkv(2, 0, 1, 1, None)

    @pl.when(s <= NA + 1)
    def _():
        @pl.when(s < NCH)
        def _():
            for cp in raw_copies(s):
                cp.start(priority=1)

        @pl.when(s < NB - 3)
        def _():
            x_copy(s + 3).start(priority=1)

        @pl.when(s == NCH)
        def _():
            wo_copy().start(priority=1)

        @pl.when(jnp.logical_and(s >= 2, s <= NA))
        def _():
            for cp in raw_copies(s - 2):
                cp.wait()

        @pl.when(jnp.logical_and(s >= 1, s < NB - 1))
        def _():
            x_copy(s + 1).wait()

        @pl.when(s == NA + 1)
        def _():
            wo_copy().wait()

    @pl.when(jnp.logical_and(s >= 1, s <= NA))
    def _():
        r0 = pl.multiple_of(TM + (s - 1) * TA, 16)
        HA = TA // 2
        pt = pl.multiple_of(r0 // 2, 8)
        pb = pl.multiple_of((r0 + HA) // 2, 8)
        a11 = _as_bf16(xn_scr[pl.ds(pt, HA // 2), 0:HD])
        a12 = _as_bf16(xn_scr[pl.ds(pt, HA // 2), HD:D])
        a21 = _as_bf16(xn_scr[pl.ds(pb, HA // 2), 0:HD])
        a22 = _as_bf16(xn_scr[pl.ds(pb, HA // 2), HD:D])
        la = [t.astype(BF) for t in _lhs_combos(a11.astype(F32), a12.astype(F32), a21.astype(F32), a22.astype(F32))]
        la[2], la[3] = a11, a22
        ys = []
        for sec in range(3):
            kl = (2 * sec + 2) % NWC
            cw = [_as_bf16(jnp.concatenate([cq[sec, 0, j], cq[sec, 1, j]], axis=0)) for j in range(5)]
            wl = [cw[0], wqkv[kl, 0:HD, :], cw[1], cw[2], wqkv[kl + 1, HD:D, :], cw[3], cw[4]]
            c11, c12, c21, c22 = _strassen_out([_dot(la[j], wl[j]) for j in range(7)])
            ys.append((jnp.concatenate([c11, c12], axis=1), jnp.concatenate([c21, c22], axis=1)))
        ln_block(jnp.minimum(s + 1, NB - 1), chain=True)
        c = lax.rem(s + (NCH - 2), NCH)

        def build(raw, cmb, kq, nq, tok):
            def ld8(q, r, n):
                return raw[c, pl.ds((kq if q >= 2 else 0) + r, 8), pl.ds((nq if q % 2 else 0) + n, 128)]

            def st16(j, r, n, val):
                cmb[c, j, r // 2:r // 2 + 8, n:n + 128] = val

            return build_tiles(ld8, st16, [(r, n) for r in range(0, kq, 16) for n in range(0, nq, 128)], tok, N_EUP)

        tok = jnp.zeros((8, 128), F32)
        tok = build(rawg, cg, HD, FC, tok)
        tok = build(rawu, cu, HD, FC, tok)
        tok = build(rawd, cd, FC, HD, tok)
        for h in range(2):
            rh = pl.multiple_of(r0 + h * HA, 16)
            store_kv(ys[0][h], k_scr, rh)
            store_kv(ys[1][h], v_scr, rh)
            store_q(ys[2][h], rh)

    if NSTEPS < NA + 1 + NB:
        @pl.when(s == NSTEPS - 1)
        def _():
            l = NSTEPS - 1
            for c in (l - 1, l):
                if 0 <= c < NCH:
                    for cp in raw_copies(c):
                        cp.wait()
            for b in (l + 2, l + 3):
                if b < NB:
                    x_copy(b).wait()
            if NCH <= l <= NA:
                wo_copy().wait()

    @pl.when(s > NA)
    def _():
        i = s - (NA + 1)
        r0 = pl.multiple_of(i * TM, TM)

        def wlist(raw, cmb, c, kq, nq):
            cw = [_as_bf16(cmb[c, j]) for j in range(5)]
            return [cw[0], raw[c, 0:kq, 0:nq], cw[1], cw[2], raw[c, kq:2 * kq, nq:2 * nq], cw[3], cw[4]]

        RA = 16
        cexp = (DH ** -0.5) * LOG2E
        p0 = pl.multiple_of(r0 // 2, 8)
        never16 = lax.broadcasted_iota(jnp.int32, (16, 128), 0) < jnp.minimum(s, 0)

        def attn_half(q, r):
            sw = []
            for w in range(WIN):
                acc = None
                for g in range(NG):
                    t = q[g] * k_scr[g, pl.ds(r0 + r + HALO - DIL * w, 8), :]
                    acc = t if acc is None else acc + t
                acc = _sum4(acc)
                if r < HALO and w > 0:
                    row = lax.broadcasted_iota(jnp.int32, (8, 128), 0) + (r0 + r)
                    acc = jnp.where(row >= DIL * w, acc, NEG)
                sw.append(acc)
            m = sw[0]
            for w in range(1, WIN):
                m = jnp.maximum(m, sw[w])
            e = [jnp.exp2((sw[w] - m) * cexp) for w in range(WIN)]
            den = e[0]
            for w in range(1, WIN):
                den = den + e[w]
            inv = 1.0 / den
            p = [e[w] * inv for w in range(WIN)]
            o = []
            for g in range(NG):
                acc = None
                for w in range(WIN):
                    t = p[w] * v_scr[g, pl.ds(r0 + r + HALO - DIL * w, 8), :]
                    acc = t if acc is None else acc + t
                o.append(acc)
            return o

        def attn_rows(r, tok):
            qp = [q_scr[g, pl.ds(p0 + r // 2, 8), :] for g in range(NG)]
            if tok is not None:
                qp = [_dep32(t, tok, never) for t in qp]
            q = [_unpack(t) for t in _butterfly(qp)]
            o0 = attn_half([t[0:8] for t in q], r)
            q1 = [t[8:16] for t in q]
            if CHAIN_HALVES:
                q1 = [_dep32(t, o0[NG - 1], never) for t in q1]
            o1 = attn_half(q1, r + 8)
            o = _butterfly([_pack(jnp.concatenate([o0[g], o1[g]], axis=0)) for g in range(NG)])
            for g in range(NG):
                o_scr[r // 2:r // 2 + 8, g * 128:(g + 1) * 128] = o[g]
            tok = o[0]
            if XOR_TOK:
                for g in range(1, NG):
                    tok = tok ^ o[g]
            return tok

        sl = [_as_bf16(s_scr[i, j]) for j in range(7)]
        acc = [None] * 7
        o_parts = []
        n_att = TM // RA
        per = 3
        tok = None
        for c in range(NCH):
            wg_l = wlist(rawg, cg, c, HD, FC)
            wu_l = wlist(rawu, cu, c, HD, FC)
            wd_l = wlist(rawd, cd, c, FC, HD)
            slc = sl
            g = _strassen_out([_dot(slc[j], wg_l[j]) for j in range(7)])
            u = _strassen_out([_dot(slc[j], wu_l[j]) for j in range(7)])
            hq = [g[t] * u[t] for t in range(4)]
            hl = [t.astype(BF) for t in _lhs_combos(*hq)]
            for j in range(7):
                y = _dot(hl[j], wd_l[j])
                acc[j] = y if acc[j] is None else acc[j] + y
            for a in range(c * per, min((c + 1) * per, n_att)):
                tok = attn_rows(a * RA, tok)
        ao = _dot(_as_bf16(o_scr[...]), wo[...])
        y11, y12, y21, y22 = _strassen_out(acc)
        x = x_scr[pl.ds(r0, TM), :].astype(F32)
        o_ref[0:HM, 0:HD] = (x[0:HM, 0:HD] + ao[0:HM, 0:HD] + y11).astype(o_ref.dtype)
        o_ref[0:HM, HD:D] = (x[0:HM, HD:D] + ao[0:HM, HD:D] + y12).astype(o_ref.dtype)
        o_ref[HM:TM, 0:HD] = (x[HM:TM, 0:HD] + ao[HM:TM, 0:HD] + y21).astype(o_ref.dtype)
        o_ref[HM:TM, HD:D] = (x[HM:TM, HD:D] + ao[HM:TM, HD:D] + y22).astype(o_ref.dtype)


@jax.jit
def pallas_parallel_sum__sliding_local_dilated__glu_gated_bilinear__prompt_kernel(
    A_x: jax.Array,
    A_wqkv: jax.Array,
    A_wo: jax.Array,
    B_x: jax.Array,
    B_w_gate: jax.Array,
    B_w_up: jax.Array,
    B_w_down: jax.Array,
):
    del B_x
    x = A_x.reshape(S, D)
    hbm = pl.BlockSpec(memory_space=pl.ANY)
    out = pl.pallas_call(
        _kernel,
        grid=(NSTEPS,),
        in_specs=[hbm] * 6,
        out_specs=pl.BlockSpec((TM, D), lambda s: (jnp.maximum(s - (NA + 1), 0), 0)),
        out_shape=jax.ShapeDtypeStruct((S, D), A_x.dtype),
        scratch_shapes=[
            pltpu.VMEM((S, D), BF),
            pltpu.VMEM((NWC, D, WC), BF),
            pltpu.VMEM((D, D), BF),
            pltpu.VMEM((NCH, D, 2 * FC), BF),
            pltpu.VMEM((NCH, D, 2 * FC), BF),
            pltpu.VMEM((NCH, 2 * FC, D), BF),
            pltpu.VMEM((3, 2, 5, HD // 4, WC), U32),
            pltpu.VMEM((NCH, 5, HD // 2, FC), U32),
            pltpu.VMEM((NCH, 5, HD // 2, FC), U32),
            pltpu.VMEM((NCH, 5, FC // 2, HD), U32),
            pltpu.VMEM((S // 2, D), U32),
            pltpu.VMEM((NB, 7, HM // 2, HD), U32),
            pltpu.VMEM((NG, S // 2, 128), U32),
            pltpu.VMEM((2, NG, S + HALO, 128), F32),
            pltpu.VMEM((TM // 2, D), U32),
            pltpu.SemaphoreType.DMA((NB,)),
            pltpu.SemaphoreType.DMA((NWC + 1,)),
            pltpu.SemaphoreType.DMA((NCH, 6)),
        ],
        compiler_params=pltpu.CompilerParams(
            dimension_semantics=("arbitrary",),
            vmem_limit_bytes=124 * 1024 * 1024,
            disable_bounds_checks=True,
        ),
        name="fused_attn_ffn",
    )(x, A_wqkv, A_wo, B_w_gate, B_w_up, B_w_down)
    return out.reshape(A_x.shape)
```

```python
import functools

import jax
import jax.numpy as jnp
from jax import lax
from jax.experimental import pallas as pl
from jax.experimental.pallas import tpu as pltpu

S, D, F = 2048, 1024, 3584
H, DH, WIN, DIL = 32, 32, 8, 2
TM = 256
HM = TM // 2
NB = S // TM
HD = D // 2
FC = 256
NCH = F // 2 // FC
HALO = 16
NG = D // 128
EPS = 1e-5
NEG = -1e9
BF = jnp.bfloat16
F32 = jnp.float32
U32 = jnp.uint32
LOG2E = 1.4426950408889634
NA = 7
TA = 224
R0 = S - NA * TA
NSTEPS = 16
WC = 512
NWC = 3 * D // WC
N_EUP = 3
N_EUP0 = 2
BUILD_XOR = False
R0_BOUNDED = False
CHAIN_HALVES = True
XOR_TOK = False


def _dot(a, b):
    return jnp.dot(a, b, preferred_element_type=F32)


def _butterfly(vs):
    lane = lax.broadcasted_iota(jnp.int32, vs[0].shape, 1)
    for b in range(3):
        sh = 4 << b
        bit = (lane & sh) != 0
        new = list(vs)
        for i0 in range(NG):
            if i0 & (1 << b):
                continue
            i1 = i0 | (1 << b)
            new[i0] = jnp.where(bit, pltpu.roll(vs[i1], sh, 1), vs[i0])
            new[i1] = jnp.where(bit, vs[i1], pltpu.roll(vs[i0], 128 - sh, 1))
        vs = new
    return vs


def _sum4(x):
    lane = lax.broadcasted_iota(jnp.int32, x.shape, 1)
    x = x + jnp.where((lane & 1) != 0, pltpu.roll(x, 1, 1), pltpu.roll(x, 127, 1))
    x = x + jnp.where((lane & 2) != 0, pltpu.roll(x, 2, 1), pltpu.roll(x, 126, 1))
    return x


def _dep32(x, tok, never):
    return jnp.where(never, pltpu.bitcast(tok, x.dtype), x)


def _gate(m, tok, never):
    t = pltpu.bitcast(m[0:16, 0:128], F32)
    t = pltpu.bitcast(_dep32(t, tok, never), BF)
    top = jnp.concatenate([t, m[0:16, 128:]], axis=1)
    if m.shape[0] == 16:
        return top
    return jnp.concatenate([top, m[16:]], axis=0)


def _pack(y):
    return pltpu.bitcast(y.astype(BF), U32)


def _as_bf16(w):
    return pltpu.bitcast(w, BF)


def _unpack(w):
    return pltpu.bitcast(w, BF).astype(F32)


def _lhs_combos(a11, a12, a21, a22):
    return [a11 + a22, a21 + a22, a11, a22, a11 + a12, a21 - a11, a12 - a22]


def _strassen_out(m):
    return (m[0] + m[3] - m[4] + m[6], m[2] + m[4], m[1] + m[3], m[0] - m[1] + m[2] + m[5])


def _layernorm(x):
    x = x.astype(F32)
    mean = jnp.mean(x, axis=-1, keepdims=True)
    xc = x - mean
    var = jnp.mean(xc * xc, axis=-1, keepdims=True)
    return xc * lax.rsqrt(var + EPS)


def _kernel(x_hbm, wqkv_hbm, wo_hbm, wg_hbm, wu_hbm, wd_hbm, o_ref,
            x_scr, wqkv, wo, rawg, rawu, rawd, cq, cwo, cg, cu, cd,
            xn_scr, s_scr, q_scr, kv_scr, o_scr,
            sem_x, sem_w, sem_raw):
    s = pl.program_id(0)
    k_scr = kv_scr.at[0]
    v_scr = kv_scr.at[1]

    def x_copy(b):
        return pltpu.make_async_copy(x_hbm.at[pl.ds(b * TM, TM), :], x_scr.at[pl.ds(b * TM, TM), :], sem_x.at[b])

    def wqkv_copy(k):
        return pltpu.make_async_copy(wqkv_hbm.at[:, pl.ds(k * WC, WC)], wqkv.at[k], sem_w.at[k])

    def wo_copy():
        return pltpu.make_async_copy(wo_hbm, wo, sem_w.at[NWC])

    def raw_copies(c):
        return [
            pltpu.make_async_copy(wg_hbm.at[:, pl.ds(c * FC, FC)], rawg.at[c, :, pl.ds(0, FC)], sem_raw.at[c, 0]),
            pltpu.make_async_copy(wg_hbm.at[:, pl.ds(F // 2 + c * FC, FC)], rawg.at[c, :, pl.ds(FC, FC)], sem_raw.at[c, 1]),
            pltpu.make_async_copy(wu_hbm.at[:, pl.ds(c * FC, FC)], rawu.at[c, :, pl.ds(0, FC)], sem_raw.at[c, 2]),
            pltpu.make_async_copy(wu_hbm.at[:, pl.ds(F // 2 + c * FC, FC)], rawu.at[c, :, pl.ds(FC, FC)], sem_raw.at[c, 3]),
            pltpu.make_async_copy(wd_hbm.at[pl.ds(c * FC, FC), :], rawd.at[c, pl.ds(0, FC), :], sem_raw.at[c, 4]),
            pltpu.make_async_copy(wd_hbm.at[pl.ds(F // 2 + c * FC, FC), :], rawd.at[c, pl.ds(FC, FC), :], sem_raw.at[c, 5]),
        ]

    never = lax.broadcasted_iota(jnp.int32, (8, 128), 0) < jnp.minimum(s, 0)

    def ln_unit(b, r, tok):
        RC = 16
        r0 = pl.multiple_of(b * TM + r, RC)
        xt = x_scr[pl.ds(r0, RC), :]
        xb = x_scr[pl.ds(r0 + HM, RC), :]
        if tok is not None:
            xt = _gate(xt, tok, never)
            xb = _gate(xb, tok, never)
        top = _layernorm(xt)
        bot = _layernorm(xb)
        p0 = pl.multiple_of(r0 // 2, RC // 2)
        xn_scr[pl.ds(p0, RC // 2), :] = _pack(top)
        xn_scr[pl.ds(p0 + HM // 2, RC // 2), :] = _pack(bot)
        cs = _lhs_combos(top[:, :HD], top[:, HD:], bot[:, :HD], bot[:, HD:])
        pr = r // 2 if isinstance(r, int) else pl.multiple_of(r // 2, RC // 2)
        for j in range(7):
            s_scr[b, j, pl.ds(pr, RC // 2), :] = _pack(cs[j])
        return top[0:8, 0:128] + bot[0:8, 0:128]

    def ln_block(b, chain=False):
        tok = None
        for r in range(0, HM, 16):
            t = ln_unit(b, r, tok)
            tok = t if chain else None
        return tok

    def store_kv(y, dst, r0):
        for r in range(0, y.shape[0], 16):
            vs = _butterfly([_pack(y[r:r + 16, g * 128:(g + 1) * 128]) for g in range(NG)])
            for g in range(NG):
                dst[g, pl.ds(r0 + HALO + r, 16), :] = _unpack(vs[g])

    def store_q(y, r0):
        p0 = pl.multiple_of(r0 // 2, 8)
        for g in range(NG):
            q_scr[g, pl.ds(p0, y.shape[0] // 2), :] = _pack(y[:, g * 128:(g + 1) * 128])

    def build_tiles(ld16, st16, positions, tok, n_eup):
        for r, n0 in positions:
            for _ in range(n_eup or 0):
                tok = jnp.exp2(tok)

            def ld(q):
                w = pltpu.bitcast(ld16(q, r, n0), U32)
                if n_eup is not None:
                    w = _dep32(w, tok, never)
                return (pltpu.bitcast(w << 16, F32), pltpu.bitcast(w & jnp.uint32(0xFFFF0000), F32))

            b11, b12, b21, b22 = [ld(q) for q in range(4)]

            def comb(x, y, sign):
                ev, od = (x[0] + y[0], x[1] + y[1]) if sign > 0 else (x[0] - y[0], x[1] - y[1])
                return pltpu.bitcast(pltpu.pack_elementwise([ev, od], packed_dtype=BF), U32)

            outs = [comb(b11, b22, 1), comb(b12, b22, -1), comb(b21, b11, -1), comb(b11, b12, 1), comb(b21, b22, 1)]
            for j in range(5):
                st16(j, r, n0, outs[j])
            t = outs[0]
            if BUILD_XOR:
                t = (t ^ outs[1]) ^ (outs[2] ^ outs[3]) ^ outs[4]
            tok = pltpu.bitcast(t, F32)
        return tok

    def build_qkv(sec, kl, kr, bh, n_eup):
        rb = bh * (HD // 2)

        def row(r, m):
            return rb + r if isinstance(rb, int) else pl.multiple_of(rb + r, m)

        def ld8(q, r, n):
            return wqkv[kl if q in (0, 2) else kr, pl.ds(row((HD if q >= 2 else 0) + r, 16), 16), n:n + 128]

        def st16(j, r, n, val):
            cq[sec, bh, j, r // 2:r // 2 + 8, n:n + 128] = val

        build_tiles(ld8, st16, [(r, n) for r in range(0, HD // 2, 16) for n in range(0, WC, 128)],
                    jnp.zeros((8, 128), F32), n_eup)

    @pl.when(s == 0)
    def _():
        def issue_x(b, carry):
            x_copy(b).start(priority=1)
            return carry

        lax.fori_loop(0, 2, issue_x, 0)

        def issue_w(j, carry):
            @pl.when(j == 1)
            def _():
                x_copy(2).start(priority=1)

            wqkv_copy(lax.rem(j + 2, NWC)).start(priority=1)
            return carry

        lax.fori_loop(0, NWC, issue_w, 0)

        def issue_rest(j, carry):
            for cp in raw_copies(0):
                cp.start(priority=1)
            return carry

        lax.fori_loop(0, jnp.maximum(s, 1), issue_rest, 0)
        wo_copy().start(priority=1)
        x_copy(3).start(priority=1)
        k_scr[:, 0:HALO, :] = jnp.zeros((NG, HALO, 128), F32)
        v_scr[:, 0:HALO, :] = jnp.zeros((NG, HALO, 128), F32)
        x_copy(0).wait()
        ln_block(0)
        x_copy(1).wait()
        ln_block(1)
        P0 = R0 // 2
        xn = _as_bf16(xn_scr[0:P0, :])

        def body(j, carry):
            k = lax.rem(j + 2, NWC)
            wqkv_copy(k).wait()

            @pl.when(j == 1)
            def _():
                x_copy(2).wait()

            y = _dot(xn, wqkv[k])
            half = lax.rem(j, 2)
            sec = jnp.maximum(lax.div(j, 2) - 1, 0)
            src = pl.multiple_of((sec + 1) * P0 + half * (P0 // 2), 8)
            dstr = pl.multiple_of(HALO + half * P0, 16)
            for r in range(0, P0 // 2, 8):
                vs = _butterfly([q_scr[g, pl.ds(src + r, 8), :] for g in range(NG)])
                for g in range(NG):
                    kv_scr[sec, g, pl.ds(dstr + 2 * r, 16), :] = _unpack(vs[g])
            lb = jnp.minimum(j + 1, 2)
            u0 = 2 * jnp.clip(j - 1, 0, 3)
            tok = ln_unit(lb, pl.multiple_of(u0 * 16, 16), None)
            ln_unit(lb, pl.multiple_of(u0 * 16 + 16, 16), tok)
            jm = jnp.maximum(j - 1, 0)
            bsec = lax.div(jm, 2)
            kl = lax.rem(2 * bsec + 2, NWC)
            kr = jnp.where(j == 0, kl, kl + 1)
            bh = jnp.where(j == 0, 1, lax.rem(jm, 2))
            build_qkv(bsec, kl, kr, bh, N_EUP0)
            rb = pl.multiple_of(lax.rem(lax.div(j, 2) + 1, 3) * P0, 8)
            for gg in range(WC // 128):
                q_scr[half * (WC // 128) + gg, pl.ds(rb, P0), :] = _pack(y[:, gg * 128:(gg + 1) * 128])
            return carry

        lax.fori_loop(0, NWC, body, 0)
        build_qkv(2, 0, 1, 1, None)
        wo_copy().wait()

        def wo_ld8(q, r, n):
            return wo[pl.ds((HD if q >= 2 else 0) + r, 16), pl.ds((HD if q % 2 else 0) + n, 128)]

        def wo_st16(j, r, n, val):
            cwo[j, r // 2:r // 2 + 8, n:n + 128] = val

        build_tiles(wo_ld8, wo_st16, [(r, n) for r in range(0, HD, 16) for n in range(0, HD, 128)],
                    jnp.zeros((8, 128), F32), None)

    @pl.when(s <= NA)
    def _():
        @pl.when(s + 1 < NCH)
        def _():
            for cp in raw_copies(s + 1):
                cp.start(priority=1)

        @pl.when(s + 4 < NB)
        def _():
            x_copy(s + 4).start(priority=1)

        @pl.when(s >= 1)
        def _():
            for cp in raw_copies(s - 1):
                cp.wait()

        @pl.when(jnp.logical_and(s >= 1, s + 2 < NB))
        def _():
            x_copy(s + 2).wait()

    @pl.when(jnp.logical_and(s >= 1, s <= NA))
    def _():
        c = lax.rem(s + (NA - 1), NA)
        r0 = pl.multiple_of(R0 + (c if R0_BOUNDED else s - 1) * TA, 16)
        HA = TA // 2
        pt = pl.multiple_of(r0 // 2, 8)
        pb = pl.multiple_of((r0 + HA) // 2, 8)
        a11 = _as_bf16(xn_scr[pl.ds(pt, HA // 2), 0:HD])
        a12 = _as_bf16(xn_scr[pl.ds(pt, HA // 2), HD:D])
        a21 = _as_bf16(xn_scr[pl.ds(pb, HA // 2), 0:HD])
        a22 = _as_bf16(xn_scr[pl.ds(pb, HA // 2), HD:D])
        la = [t.astype(BF) for t in _lhs_combos(a11.astype(F32), a12.astype(F32), a21.astype(F32), a22.astype(F32))]
        la[2], la[3] = a11, a22

        def ffn_part(raw, cmb, kq, nq):
            def ld8(q, r, n):
                return raw[c, pl.ds((kq if q >= 2 else 0) + r, 16), pl.ds((nq if q % 2 else 0) + n, 128)]

            def st16(j, r, n, val):
                cmb[c, j, r // 2:r // 2 + 8, n:n + 128] = val

            return [(ld8, st16, (r, n)) for r in range(0, kq, 16) for n in range(0, nq, 128)]

        work = ffn_part(rawg, cg, HD, FC) + ffn_part(rawu, cu, HD, FC) + ffn_part(rawd, cd, FC, HD)
        ys = []
        for sec in range(3):
            kl = (2 * sec + 2) % NWC
            cw = [_as_bf16(jnp.concatenate([cq[sec, 0, j], cq[sec, 1, j]], axis=0)) for j in range(5)]
            wl = [cw[0], wqkv[kl, 0:HD, :], cw[1], cw[2], wqkv[kl + 1, HD:D, :], cw[3], cw[4]]
            c11, c12, c21, c22 = _strassen_out([_dot(la[j], wl[j]) for j in range(7)])
            ys.append((jnp.concatenate([c11, c12], axis=1), jnp.concatenate([c21, c22], axis=1)))
        ln_block(jnp.minimum(s + 2, NB - 1), chain=True)
        tok = jnp.zeros((8, 128), F32)
        for ld8, st16, pos in work:
            tok = build_tiles(ld8, st16, [pos], tok, N_EUP)
        for h in range(2):
            rh = pl.multiple_of(r0 + h * HA, 16)
            store_kv(ys[0][h], k_scr, rh)
            store_kv(ys[1][h], v_scr, rh)
            store_q(ys[2][h], rh)

    if NSTEPS < NA + 1 + NB:
        @pl.when(s == NSTEPS - 1)
        def _():
            l = NSTEPS - 1
            for c in (l, l + 1):
                if 0 <= c < NCH:
                    for cp in raw_copies(c):
                        cp.wait()
            for b in (l + 3, l + 4):
                if b < NB:
                    x_copy(b).wait()

    @pl.when(s > NA)
    def _():
        i = lax.rem(s + (NB - NA - 1), NB)
        r0 = pl.multiple_of(i * TM, TM)

        def wlist(raw, cmb, c, kq, nq):
            cw = [_as_bf16(cmb[c, j]) for j in range(5)]
            return [cw[0], raw[c, 0:kq, 0:nq], cw[1], cw[2], raw[c, kq:2 * kq, nq:2 * nq], cw[3], cw[4]]

        RA = 16
        cexp = (DH ** -0.5) * LOG2E
        p0 = pl.multiple_of(r0 // 2, 8)
        never16 = lax.broadcasted_iota(jnp.int32, (16, 128), 0) < jnp.minimum(s, 0)

        def attn_half(q, r):
            sw = []
            for w in range(WIN):
                acc = None
                for g in range(NG):
                    t = q[g] * k_scr[g, pl.ds(r0 + r + HALO - DIL * w, 8), :]
                    acc = t if acc is None else acc + t
                acc = _sum4(acc)
                if r < HALO and w > 0:
                    row = lax.broadcasted_iota(jnp.int32, (8, 128), 0) + (r0 + r)
                    acc = jnp.where(row >= DIL * w, acc, NEG)
                sw.append(acc)
            m = sw[0]
            for w in range(1, WIN):
                m = jnp.maximum(m, sw[w])
            e = [jnp.exp2((sw[w] - m) * cexp) for w in range(WIN)]
            den = e[0]
            for w in range(1, WIN):
                den = den + e[w]
            inv = 1.0 / den
            p = [e[w] * inv for w in range(WIN)]
            o = []
            for g in range(NG):
                acc = None
                for w in range(WIN):
                    t = p[w] * v_scr[g, pl.ds(r0 + r + HALO - DIL * w, 8), :]
                    acc = t if acc is None else acc + t
                o.append(acc)
            return o

        def attn_rows(r, tok):
            qp = [q_scr[g, pl.ds(p0 + r // 2, 8), :] for g in range(NG)]
            if tok is not None:
                qp = [_dep32(t, tok, never) for t in qp]
            q = [_unpack(t) for t in _butterfly(qp)]
            o0 = attn_half([t[0:8] for t in q], r)
            q1 = [t[8:16] for t in q]
            if CHAIN_HALVES:
                q1 = [_dep32(t, o0[NG - 1], never) for t in q1]
            o1 = attn_half(q1, r + 8)
            o = _butterfly([_pack(jnp.concatenate([o0[g], o1[g]], axis=0)) for g in range(NG)])
            for g in range(NG):
                o_scr[r // 2:r // 2 + 8, g * 128:(g + 1) * 128] = o[g]
            tok = o[0]
            if XOR_TOK:
                for g in range(1, NG):
                    tok = tok ^ o[g]
            return tok

        sl = [_as_bf16(s_scr[i, j]) for j in range(7)]
        acc = [None] * 7
        o_parts = []
        n_att = TM // RA
        per = 3
        tok = None
        for c in range(NCH):
            wg_l = wlist(rawg, cg, c, HD, FC)
            wu_l = wlist(rawu, cu, c, HD, FC)
            wd_l = wlist(rawd, cd, c, FC, HD)
            slc = sl
            g = _strassen_out([_dot(slc[j], wg_l[j]) for j in range(7)])
            u = _strassen_out([_dot(slc[j], wu_l[j]) for j in range(7)])
            hq = [g[t] * u[t] for t in range(4)]
            hl = [t.astype(BF) for t in _lhs_combos(*hq)]
            for j in range(7):
                y = _dot(hl[j], wd_l[j])
                acc[j] = y if acc[j] is None else acc[j] + y
            for a in range(c * per, min((c + 1) * per, n_att)):
                tok = attn_rows(a * RA, tok)
        oq = [_as_bf16(o_scr[rr:rr + HM // 2, cc:cc + HD]) for rr in (0, HM // 2) for cc in (0, HD)]
        ol = [t.astype(BF) for t in _lhs_combos(*[t.astype(F32) for t in oq])]
        ol[2], ol[3] = oq[0], oq[3]
        cw = [_as_bf16(cwo[j]) for j in range(5)]
        wo_l = [cw[0], wo[0:HD, 0:HD], cw[1], cw[2], wo[HD:D, HD:D], cw[3], cw[4]]
        acc = [acc[j] + _dot(ol[j], wo_l[j]) for j in range(7)]
        y11, y12, y21, y22 = _strassen_out(acc)
        x = x_scr[pl.ds(r0, TM), :].astype(F32)
        o_ref[0:HM, 0:HD] = (x[0:HM, 0:HD] + y11).astype(o_ref.dtype)
        o_ref[0:HM, HD:D] = (x[0:HM, HD:D] + y12).astype(o_ref.dtype)
        o_ref[HM:TM, 0:HD] = (x[HM:TM, 0:HD] + y21).astype(o_ref.dtype)
        o_ref[HM:TM, HD:D] = (x[HM:TM, HD:D] + y22).astype(o_ref.dtype)


@jax.jit
def pallas_parallel_sum__sliding_local_dilated__glu_gated_bilinear__prompt_kernel(
    A_x: jax.Array,
    A_wqkv: jax.Array,
    A_wo: jax.Array,
    B_x: jax.Array,
    B_w_gate: jax.Array,
    B_w_up: jax.Array,
    B_w_down: jax.Array,
):
    del B_x
    x = A_x.reshape(S, D)
    hbm = pl.BlockSpec(memory_space=pl.ANY)
    out = pl.pallas_call(
        _kernel,
        grid=(NSTEPS,),
        in_specs=[hbm] * 6,
        out_specs=pl.BlockSpec((TM, D), lambda s: (jnp.maximum(s - (NA + 1), 0), 0)),
        out_shape=jax.ShapeDtypeStruct((S, D), A_x.dtype),
        scratch_shapes=[
            pltpu.VMEM((S, D), BF),
            pltpu.VMEM((NWC, D, WC), BF),
            pltpu.VMEM((D, D), BF),
            pltpu.VMEM((NCH, D, 2 * FC), BF),
            pltpu.VMEM((NCH, D, 2 * FC), BF),
            pltpu.VMEM((NCH, 2 * FC, D), BF),
            pltpu.VMEM((3, 2, 5, HD // 4, WC), U32),
            pltpu.VMEM((5, HD // 2, HD), U32),
            pltpu.VMEM((NCH, 5, HD // 2, FC), U32),
            pltpu.VMEM((NCH, 5, HD // 2, FC), U32),
            pltpu.VMEM((NCH, 5, FC // 2, HD), U32),
            pltpu.VMEM((S // 2, D), U32),
            pltpu.VMEM((NB, 7, HM // 2, HD), U32),
            pltpu.VMEM((NG, S // 2, 128), U32),
            pltpu.VMEM((2, NG, S + HALO, 128), F32),
            pltpu.VMEM((TM // 2, D), U32),
            pltpu.SemaphoreType.DMA((NB,)),
            pltpu.SemaphoreType.DMA((NWC + 1,)),
            pltpu.SemaphoreType.DMA((NCH, 6)),
        ],
        compiler_params=pltpu.CompilerParams(
            dimension_semantics=("arbitrary",),
            vmem_limit_bytes=124 * 1024 * 1024,
            disable_bounds_checks=True,
        ),
        name="fused_attn_ffn",
    )(x, A_wqkv, A_wo, B_w_gate, B_w_up, B_w_down)
    return out.reshape(A_x.shape)
```

```python
import functools

import jax
import jax.numpy as jnp
from jax import lax
from jax.experimental import pallas as pl
from jax.experimental.pallas import tpu as pltpu

S, D, F = 2048, 1024, 3584
H, DH, WIN, DIL = 32, 32, 8, 2
TM = 256
HM = TM // 2
NB = S // TM
HD = D // 2
FC = 256
NCH = F // 2 // FC
HALO = 16
NG = D // 128
EPS = 1e-5
NEG = -1e9
BF = jnp.bfloat16
F32 = jnp.float32
U32 = jnp.uint32
LOG2E = 1.4426950408889634
NA = 7
TA = 224
R0 = S - NA * TA
NSTEPS = 16
WC = 512
NWC = 3 * D // WC
N_EUP = 3
N_EUP0 = 2
BUILD_XOR = False
R0_BOUNDED = False
WO_AT = 6
CHAIN_HALVES = True
XOR_TOK = False


def _dot(a, b):
    return jnp.dot(a, b, preferred_element_type=F32)


def _butterfly(vs):
    lane = lax.broadcasted_iota(jnp.int32, vs[0].shape, 1)
    for b in range(3):
        sh = 4 << b
        bit = (lane & sh) != 0
        new = list(vs)
        for i0 in range(NG):
            if i0 & (1 << b):
                continue
            i1 = i0 | (1 << b)
            new[i0] = jnp.where(bit, pltpu.roll(vs[i1], sh, 1), vs[i0])
            new[i1] = jnp.where(bit, vs[i1], pltpu.roll(vs[i0], 128 - sh, 1))
        vs = new
    return vs


def _sum4(x):
    lane = lax.broadcasted_iota(jnp.int32, x.shape, 1)
    x = x + jnp.where((lane & 1) != 0, pltpu.roll(x, 1, 1), pltpu.roll(x, 127, 1))
    x = x + jnp.where((lane & 2) != 0, pltpu.roll(x, 2, 1), pltpu.roll(x, 126, 1))
    return x


def _dep32(x, tok, never):
    return jnp.where(never, pltpu.bitcast(tok, x.dtype), x)


def _gate(m, tok, never):
    t = pltpu.bitcast(m[0:16, 0:128], F32)
    t = pltpu.bitcast(_dep32(t, tok, never), BF)
    top = jnp.concatenate([t, m[0:16, 128:]], axis=1)
    if m.shape[0] == 16:
        return top
    return jnp.concatenate([top, m[16:]], axis=0)


def _pack(y):
    return pltpu.bitcast(y.astype(BF), U32)


def _as_bf16(w):
    return pltpu.bitcast(w, BF)


def _unpack(w):
    return pltpu.bitcast(w, BF).astype(F32)


def _lhs_combos(a11, a12, a21, a22):
    return [a11 + a22, a21 + a22, a11, a22, a11 + a12, a21 - a11, a12 - a22]


def _strassen_out(m):
    return (m[0] + m[3] - m[4] + m[6], m[2] + m[4], m[1] + m[3], m[0] - m[1] + m[2] + m[5])


def _layernorm(x):
    x = x.astype(F32)
    mean = jnp.mean(x, axis=-1, keepdims=True)
    xc = x - mean
    var = jnp.mean(xc * xc, axis=-1, keepdims=True)
    return xc * lax.rsqrt(var + EPS)


def _kernel(x_hbm, wqkv_hbm, wo_hbm, wg_hbm, wu_hbm, wd_hbm, o_ref,
            x_scr, wqkv, wo, rawg, rawu, rawd, cq, cwo, cg, cu, cd,
            xn_scr, s_scr, q_scr, kv_scr, o_scr,
            sem_x, sem_w, sem_raw):
    s = pl.program_id(0)
    k_scr = kv_scr.at[0]
    v_scr = kv_scr.at[1]

    def x_copy(b):
        return pltpu.make_async_copy(x_hbm.at[pl.ds(b * TM, TM), :], x_scr.at[pl.ds(b * TM, TM), :], sem_x.at[b])

    def wqkv_copy(k):
        return pltpu.make_async_copy(wqkv_hbm.at[:, pl.ds(k * WC, WC)], wqkv.at[k], sem_w.at[k])

    def wo_copy():
        return pltpu.make_async_copy(wo_hbm, wo, sem_w.at[NWC])

    def raw_copies(c):
        return [
            pltpu.make_async_copy(wg_hbm.at[:, pl.ds(c * FC, FC)], rawg.at[c, :, pl.ds(0, FC)], sem_raw.at[c, 0]),
            pltpu.make_async_copy(wg_hbm.at[:, pl.ds(F // 2 + c * FC, FC)], rawg.at[c, :, pl.ds(FC, FC)], sem_raw.at[c, 1]),
            pltpu.make_async_copy(wu_hbm.at[:, pl.ds(c * FC, FC)], rawu.at[c, :, pl.ds(0, FC)], sem_raw.at[c, 2]),
            pltpu.make_async_copy(wu_hbm.at[:, pl.ds(F // 2 + c * FC, FC)], rawu.at[c, :, pl.ds(FC, FC)], sem_raw.at[c, 3]),
            pltpu.make_async_copy(wd_hbm.at[pl.ds(c * FC, FC), :], rawd.at[c, pl.ds(0, FC), :], sem_raw.at[c, 4]),
            pltpu.make_async_copy(wd_hbm.at[pl.ds(F // 2 + c * FC, FC), :], rawd.at[c, pl.ds(FC, FC), :], sem_raw.at[c, 5]),
        ]

    never = lax.broadcasted_iota(jnp.int32, (8, 128), 0) < jnp.minimum(s, 0)

    def ln_unit(b, r, tok):
        RC = 16
        r0 = pl.multiple_of(b * TM + r, RC)
        xt = x_scr[pl.ds(r0, RC), :]
        xb = x_scr[pl.ds(r0 + HM, RC), :]
        if tok is not None:
            xt = _gate(xt, tok, never)
            xb = _gate(xb, tok, never)
        top = _layernorm(xt)
        bot = _layernorm(xb)
        p0 = pl.multiple_of(r0 // 2, RC // 2)
        xn_scr[pl.ds(p0, RC // 2), :] = _pack(top)
        xn_scr[pl.ds(p0 + HM // 2, RC // 2), :] = _pack(bot)
        cs = _lhs_combos(top[:, :HD], top[:, HD:], bot[:, :HD], bot[:, HD:])
        pr = r // 2 if isinstance(r, int) else pl.multiple_of(r // 2, RC // 2)
        for j in range(7):
            s_scr[b, j, pl.ds(pr, RC // 2), :] = _pack(cs[j])
        return top[0:8, 0:128] + bot[0:8, 0:128]

    def ln_block(b, chain=False):
        tok = None
        for r in range(0, HM, 16):
            t = ln_unit(b, r, tok)
            tok = t if chain else None
        return tok

    def store_kv(y, dst, r0):
        for r in range(0, y.shape[0], 16):
            vs = _butterfly([_pack(y[r:r + 16, g * 128:(g + 1) * 128]) for g in range(NG)])
            for g in range(NG):
                dst[g, pl.ds(r0 + HALO + r, 16), :] = _unpack(vs[g])

    def store_q(y, r0):
        p0 = pl.multiple_of(r0 // 2, 8)
        for g in range(NG):
            q_scr[g, pl.ds(p0, y.shape[0] // 2), :] = _pack(y[:, g * 128:(g + 1) * 128])

    def build_tiles(ld16, st16, positions, tok, n_eup):
        for r, n0 in positions:
            for _ in range(n_eup or 0):
                tok = jnp.exp2(tok)

            def ld(q):
                w = pltpu.bitcast(ld16(q, r, n0), U32)
                if n_eup is not None:
                    w = _dep32(w, tok, never)
                return (pltpu.bitcast(w << 16, F32), pltpu.bitcast(w & jnp.uint32(0xFFFF0000), F32))

            b11, b12, b21, b22 = [ld(q) for q in range(4)]

            def comb(x, y, sign):
                ev, od = (x[0] + y[0], x[1] + y[1]) if sign > 0 else (x[0] - y[0], x[1] - y[1])
                return pltpu.bitcast(pltpu.pack_elementwise([ev, od], packed_dtype=BF), U32)

            outs = [comb(b11, b22, 1), comb(b12, b22, -1), comb(b21, b11, -1), comb(b11, b12, 1), comb(b21, b22, 1)]
            for j in range(5):
                st16(j, r, n0, outs[j])
            t = outs[0]
            if BUILD_XOR:
                t = (t ^ outs[1]) ^ (outs[2] ^ outs[3]) ^ outs[4]
            tok = pltpu.bitcast(t, F32)
        return tok

    def build_qkv(sec, kl, kr, bh, n_eup):
        rb = bh * (HD // 2)

        def row(r, m):
            return rb + r if isinstance(rb, int) else pl.multiple_of(rb + r, m)

        def ld8(q, r, n):
            return wqkv[kl if q in (0, 2) else kr, pl.ds(row((HD if q >= 2 else 0) + r, 16), 16), n:n + 128]

        def st16(j, r, n, val):
            cq[sec, bh, j, r // 2:r // 2 + 8, n:n + 128] = val

        build_tiles(ld8, st16, [(r, n) for r in range(0, HD // 2, 16) for n in range(0, WC, 128)],
                    jnp.zeros((8, 128), F32), n_eup)

    @pl.when(s == 0)
    def _():
        def issue_x(b, carry):
            x_copy(b).start(priority=1)
            return carry

        lax.fori_loop(0, 2, issue_x, 0)

        def issue_w(j, carry):
            @pl.when(j == 1)
            def _():
                x_copy(2).start(priority=1)

            wqkv_copy(lax.rem(j + 2, NWC)).start(priority=1)
            return carry

        lax.fori_loop(0, NWC, issue_w, 0)

        def issue_rest(j, carry):
            for cp in raw_copies(0):
                cp.start(priority=1)
            return carry

        lax.fori_loop(0, jnp.maximum(s, 1), issue_rest, 0)
        wo_copy().start(priority=1)
        x_copy(3).start(priority=1)
        k_scr[:, 0:HALO, :] = jnp.zeros((NG, HALO, 128), F32)
        v_scr[:, 0:HALO, :] = jnp.zeros((NG, HALO, 128), F32)
        x_copy(0).wait()
        ln_block(0)
        x_copy(1).wait()
        ln_block(1)
        P0 = R0 // 2
        xn = _as_bf16(xn_scr[0:P0, :])

        def body(j, carry):
            k = lax.rem(j + 2, NWC)
            wqkv_copy(k).wait()

            @pl.when(j == 1)
            def _():
                x_copy(2).wait()

            y = _dot(xn, wqkv[k])
            half = lax.rem(j, 2)
            sec = jnp.maximum(lax.div(j, 2) - 1, 0)
            src = pl.multiple_of((sec + 1) * P0 + half * (P0 // 2), 8)
            dstr = pl.multiple_of(HALO + half * P0, 16)
            for r in range(0, P0 // 2, 8):
                vs = _butterfly([q_scr[g, pl.ds(src + r, 8), :] for g in range(NG)])
                for g in range(NG):
                    kv_scr[sec, g, pl.ds(dstr + 2 * r, 16), :] = _unpack(vs[g])
            lb = jnp.minimum(j + 1, 2)
            u0 = 2 * jnp.clip(j - 1, 0, 3)
            tok = ln_unit(lb, pl.multiple_of(u0 * 16, 16), None)
            ln_unit(lb, pl.multiple_of(u0 * 16 + 16, 16), tok)
            jm = jnp.maximum(j - 1, 0)
            bsec = lax.div(jm, 2)
            kl = lax.rem(2 * bsec + 2, NWC)
            kr = jnp.where(j == 0, kl, kl + 1)
            bh = jnp.where(j == 0, 1, lax.rem(jm, 2))
            build_qkv(bsec, kl, kr, bh, N_EUP0)
            rb = pl.multiple_of(lax.rem(lax.div(j, 2) + 1, 3) * P0, 8)
            for gg in range(WC // 128):
                q_scr[half * (WC // 128) + gg, pl.ds(rb, P0), :] = _pack(y[:, gg * 128:(gg + 1) * 128])
            return carry

        lax.fori_loop(0, NWC, body, 0)
        build_qkv(2, 0, 1, 1, None)
        wo_copy().wait()

        def wo_ld8(q, r, n):
            return wo[pl.ds((HD if q >= 2 else 0) + r, 16), pl.ds((HD if q % 2 else 0) + n, 128)]

        def wo_st16(j, r, n, val):
            cwo[j, r // 2:r // 2 + 8, n:n + 128] = val

        build_tiles(wo_ld8, wo_st16, [(r, n) for r in range(0, HD, 16) for n in range(0, HD, 128)],
                    jnp.zeros((8, 128), F32), None)

    @pl.when(s <= NA)
    def _():
        @pl.when(s + 1 < NCH)
        def _():
            for cp in raw_copies(s + 1):
                cp.start(priority=1)

        @pl.when(s + 4 < NB)
        def _():
            x_copy(s + 4).start(priority=1)

        @pl.when(s >= 1)
        def _():
            for cp in raw_copies(s - 1):
                cp.wait()

        @pl.when(jnp.logical_and(s >= 1, s + 2 < NB))
        def _():
            x_copy(s + 2).wait()

    @pl.when(jnp.logical_and(s >= 1, s <= NA))
    def _():
        c = lax.rem(s + (NA - 1), NA)
        r0 = pl.multiple_of(R0 + (c if R0_BOUNDED else s - 1) * TA, 16)
        HA = TA // 2
        pt = pl.multiple_of(r0 // 2, 8)
        pb = pl.multiple_of((r0 + HA) // 2, 8)
        a11 = _as_bf16(xn_scr[pl.ds(pt, HA // 2), 0:HD])
        a12 = _as_bf16(xn_scr[pl.ds(pt, HA // 2), HD:D])
        a21 = _as_bf16(xn_scr[pl.ds(pb, HA // 2), 0:HD])
        a22 = _as_bf16(xn_scr[pl.ds(pb, HA // 2), HD:D])
        la = [t.astype(BF) for t in _lhs_combos(a11.astype(F32), a12.astype(F32), a21.astype(F32), a22.astype(F32))]
        la[2], la[3] = a11, a22

        def ffn_part(raw, cmb, kq, nq):
            def ld8(q, r, n):
                return raw[c, pl.ds((kq if q >= 2 else 0) + r, 16), pl.ds((nq if q % 2 else 0) + n, 128)]

            def st16(j, r, n, val):
                cmb[c, j, r // 2:r // 2 + 8, n:n + 128] = val

            return [(ld8, st16, (r, n)) for r in range(0, kq, 16) for n in range(0, nq, 128)]

        work = ffn_part(rawg, cg, HD, FC) + ffn_part(rawu, cu, HD, FC) + ffn_part(rawd, cd, FC, HD)
        ys = []
        for sec in range(3):
            kl = (2 * sec + 2) % NWC
            cw = [_as_bf16(jnp.concatenate([cq[sec, 0, j], cq[sec, 1, j]], axis=0)) for j in range(5)]
            wl = [cw[0], wqkv[kl, 0:HD, :], cw[1], cw[2], wqkv[kl + 1, HD:D, :], cw[3], cw[4]]
            c11, c12, c21, c22 = _strassen_out([_dot(la[j], wl[j]) for j in range(7)])
            ys.append((jnp.concatenate([c11, c12], axis=1), jnp.concatenate([c21, c22], axis=1)))
        ln_block(jnp.minimum(s + 2, NB - 1), chain=True)
        tok = jnp.zeros((8, 128), F32)
        for ld8, st16, pos in work:
            tok = build_tiles(ld8, st16, [pos], tok, N_EUP)
        for h in range(2):
            rh = pl.multiple_of(r0 + h * HA, 16)
            store_kv(ys[0][h], k_scr, rh)
            store_kv(ys[1][h], v_scr, rh)
            store_q(ys[2][h], rh)

    if NSTEPS < NA + 1 + NB:
        @pl.when(s == NSTEPS - 1)
        def _():
            l = NSTEPS - 1
            for c in (l, l + 1):
                if 0 <= c < NCH:
                    for cp in raw_copies(c):
                        cp.wait()
            for b in (l + 3, l + 4):
                if b < NB:
                    x_copy(b).wait()

    @pl.when(s > NA)
    def _():
        i = lax.rem(s + (NB - NA - 1), NB)
        r0 = pl.multiple_of(i * TM, TM)

        def wlist(raw, cmb, c, kq, nq):
            cw = [_as_bf16(cmb[c, j]) for j in range(5)]
            return [cw[0], raw[c, 0:kq, 0:nq], cw[1], cw[2], raw[c, kq:2 * kq, nq:2 * nq], cw[3], cw[4]]

        RA = 16
        cexp = (DH ** -0.5) * LOG2E
        p0 = pl.multiple_of(r0 // 2, 8)
        never16 = lax.broadcasted_iota(jnp.int32, (16, 128), 0) < jnp.minimum(s, 0)

        def attn_half(q, r):
            sw = []
            for w in range(WIN):
                acc = None
                for g in range(NG):
                    t = q[g] * k_scr[g, pl.ds(r0 + r + HALO - DIL * w, 8), :]
                    acc = t if acc is None else acc + t
                acc = _sum4(acc)
                if r < HALO and w > 0:
                    row = lax.broadcasted_iota(jnp.int32, (8, 128), 0) + (r0 + r)
                    acc = jnp.where(row >= DIL * w, acc, NEG)
                sw.append(acc)
            m = sw[0]
            for w in range(1, WIN):
                m = jnp.maximum(m, sw[w])
            e = [jnp.exp2((sw[w] - m) * cexp) for w in range(WIN)]
            den = e[0]
            for w in range(1, WIN):
                den = den + e[w]
            inv = 1.0 / den
            p = [e[w] * inv for w in range(WIN)]
            o = []
            for g in range(NG):
                acc = None
                for w in range(WIN):
                    t = p[w] * v_scr[g, pl.ds(r0 + r + HALO - DIL * w, 8), :]
                    acc = t if acc is None else acc + t
                o.append(acc)
            return o

        def attn_rows(r, tok):
            qp = [q_scr[g, pl.ds(p0 + r // 2, 8), :] for g in range(NG)]
            if tok is not None:
                qp = [_dep32(t, tok, never) for t in qp]
            q = [_unpack(t) for t in _butterfly(qp)]
            o0 = attn_half([t[0:8] for t in q], r)
            q1 = [t[8:16] for t in q]
            if CHAIN_HALVES:
                q1 = [_dep32(t, o0[NG - 1], never) for t in q1]
            o1 = attn_half(q1, r + 8)
            o = _butterfly([_pack(jnp.concatenate([o0[g], o1[g]], axis=0)) for g in range(NG)])
            for g in range(NG):
                o_scr[r // 2:r // 2 + 8, g * 128:(g + 1) * 128] = o[g]
            tok = o[0]
            if XOR_TOK:
                for g in range(1, NG):
                    tok = tok ^ o[g]
            return tok

        sl = [_as_bf16(s_scr[i, j]) for j in range(7)]
        acc = [None] * 7
        o_parts = []
        n_att = TM // RA
        per = 3
        tok = None
        for c in range(NCH):
            wg_l = wlist(rawg, cg, c, HD, FC)
            wu_l = wlist(rawu, cu, c, HD, FC)
            wd_l = wlist(rawd, cd, c, FC, HD)
            slc = sl
            g = _strassen_out([_dot(slc[j], wg_l[j]) for j in range(7)])
            u = _strassen_out([_dot(slc[j], wu_l[j]) for j in range(7)])
            hq = [g[t] * u[t] for t in range(4)]
            hl = [t.astype(BF) for t in _lhs_combos(*hq)]
            for j in range(7):
                y = _dot(hl[j], wd_l[j])
                acc[j] = y if acc[j] is None else acc[j] + y
            for a in range(c * per, min((c + 1) * per, n_att)):
                tok = attn_rows(a * RA, tok)
            if c == WO_AT:
                oq = [_as_bf16(o_scr[rr:rr + HM // 2, cc:cc + HD]) for rr in (0, HM // 2) for cc in (0, HD)]
                ol = [t.astype(BF) for t in _lhs_combos(*[t.astype(F32) for t in oq])]
                ol[2], ol[3] = oq[0], oq[3]
                cw = [_as_bf16(cwo[j]) for j in range(5)]
                wo_l = [cw[0], wo[0:HD, 0:HD], cw[1], cw[2], wo[HD:D, HD:D], cw[3], cw[4]]
                acc = [acc[j] + _dot(ol[j], wo_l[j]) for j in range(7)]
        y11, y12, y21, y22 = _strassen_out(acc)
        x = x_scr[pl.ds(r0, TM), :].astype(F32)
        o_ref[0:HM, 0:HD] = (x[0:HM, 0:HD] + y11).astype(o_ref.dtype)
        o_ref[0:HM, HD:D] = (x[0:HM, HD:D] + y12).astype(o_ref.dtype)
        o_ref[HM:TM, 0:HD] = (x[HM:TM, 0:HD] + y21).astype(o_ref.dtype)
        o_ref[HM:TM, HD:D] = (x[HM:TM, HD:D] + y22).astype(o_ref.dtype)


@jax.jit
def pallas_parallel_sum__sliding_local_dilated__glu_gated_bilinear__prompt_kernel(
    A_x: jax.Array,
    A_wqkv: jax.Array,
    A_wo: jax.Array,
    B_x: jax.Array,
    B_w_gate: jax.Array,
    B_w_up: jax.Array,
    B_w_down: jax.Array,
):
    del B_x
    x = A_x.reshape(S, D)
    hbm = pl.BlockSpec(memory_space=pl.ANY)
    out = pl.pallas_call(
        _kernel,
        grid=(NSTEPS,),
        in_specs=[hbm] * 6,
        out_specs=pl.BlockSpec((TM, D), lambda s: (jnp.maximum(s - (NA + 1), 0), 0)),
        out_shape=jax.ShapeDtypeStruct((S, D), A_x.dtype),
        scratch_shapes=[
            pltpu.VMEM((S, D), BF),
            pltpu.VMEM((NWC, D, WC), BF),
            pltpu.VMEM((D, D), BF),
            pltpu.VMEM((NCH, D, 2 * FC), BF),
            pltpu.VMEM((NCH, D, 2 * FC), BF),
            pltpu.VMEM((NCH, 2 * FC, D), BF),
            pltpu.VMEM((3, 2, 5, HD // 4, WC), U32),
            pltpu.VMEM((5, HD // 2, HD), U32),
            pltpu.VMEM((NCH, 5, HD // 2, FC), U32),
            pltpu.VMEM((NCH, 5, HD // 2, FC), U32),
            pltpu.VMEM((NCH, 5, FC // 2, HD), U32),
            pltpu.VMEM((S // 2, D), U32),
            pltpu.VMEM((NB, 7, HM // 2, HD), U32),
            pltpu.VMEM((NG, S // 2, 128), U32),
            pltpu.VMEM((2, NG, S + HALO, 128), F32),
            pltpu.VMEM((TM // 2, D), U32),
            pltpu.SemaphoreType.DMA((NB,)),
            pltpu.SemaphoreType.DMA((NWC + 1,)),
            pltpu.SemaphoreType.DMA((NCH, 6)),
        ],
        compiler_params=pltpu.CompilerParams(
            dimension_semantics=("arbitrary",),
            vmem_limit_bytes=124 * 1024 * 1024,
            disable_bounds_checks=True,
        ),
        name="fused_attn_ffn",
    )(x, A_wqkv, A_wo, B_w_gate, B_w_up, B_w_down)
    return out.reshape(A_x.shape)
```

```python
import functools

import jax
import jax.numpy as jnp
from jax import lax
from jax.experimental import pallas as pl
from jax.experimental.pallas import tpu as pltpu

S, D, F = 2048, 1024, 3584
H, DH, WIN, DIL = 32, 32, 8, 2
TM = 256
HM = TM // 2
NB = S // TM
HD = D // 2
FC = 256
NCH = F // 2 // FC
HALO = 16
NG = D // 128
EPS = 1e-5
NEG = -1e9
BF = jnp.bfloat16
F32 = jnp.float32
U32 = jnp.uint32
LOG2E = 1.4426950408889634
NA = 7
TA = 224
R0 = S - NA * TA
NSTEPS = 16
WC = 512
NWC = 3 * D // WC
N_EUP = 3
N_EUP0 = 2
BUILD_XOR = False
R0_BOUNDED = False
WO_AT = 6
WO_GATE = False
DOWN_GROUP = 2
CHAIN_HALVES = True
XOR_TOK = False


def _dot(a, b):
    return jnp.dot(a, b, preferred_element_type=F32)


def _butterfly(vs):
    lane = lax.broadcasted_iota(jnp.int32, vs[0].shape, 1)
    for b in range(3):
        sh = 4 << b
        bit = (lane & sh) != 0
        new = list(vs)
        for i0 in range(NG):
            if i0 & (1 << b):
                continue
            i1 = i0 | (1 << b)
            new[i0] = jnp.where(bit, pltpu.roll(vs[i1], sh, 1), vs[i0])
            new[i1] = jnp.where(bit, vs[i1], pltpu.roll(vs[i0], 128 - sh, 1))
        vs = new
    return vs


def _sum4(x):
    lane = lax.broadcasted_iota(jnp.int32, x.shape, 1)
    x = x + jnp.where((lane & 1) != 0, pltpu.roll(x, 1, 1), pltpu.roll(x, 127, 1))
    x = x + jnp.where((lane & 2) != 0, pltpu.roll(x, 2, 1), pltpu.roll(x, 126, 1))
    return x


def _dep32(x, tok, never):
    return jnp.where(never, pltpu.bitcast(tok, x.dtype), x)


def _gate(m, tok, never):
    t = pltpu.bitcast(m[0:16, 0:128], F32)
    t = pltpu.bitcast(_dep32(t, tok, never), BF)
    top = jnp.concatenate([t, m[0:16, 128:]], axis=1)
    if m.shape[0] == 16:
        return top
    return jnp.concatenate([top, m[16:]], axis=0)


def _pack(y):
    return pltpu.bitcast(y.astype(BF), U32)


def _as_bf16(w):
    return pltpu.bitcast(w, BF)


def _unpack(w):
    return pltpu.bitcast(w, BF).astype(F32)


def _lhs_combos(a11, a12, a21, a22):
    return [a11 + a22, a21 + a22, a11, a22, a11 + a12, a21 - a11, a12 - a22]


def _strassen_out(m):
    return (m[0] + m[3] - m[4] + m[6], m[2] + m[4], m[1] + m[3], m[0] - m[1] + m[2] + m[5])


def _layernorm(x):
    x = x.astype(F32)
    mean = jnp.mean(x, axis=-1, keepdims=True)
    xc = x - mean
    var = jnp.mean(xc * xc, axis=-1, keepdims=True)
    return xc * lax.rsqrt(var + EPS)


def _kernel(x_hbm, wqkv_hbm, wo_hbm, wg_hbm, wu_hbm, wd_hbm, o_ref,
            x_scr, wqkv, wo, rawg, rawu, rawd, cq, cwo, cg, cu, cd,
            xn_scr, s_scr, q_scr, kv_scr, o_scr,
            sem_x, sem_w, sem_raw):
    s = pl.program_id(0)
    k_scr = kv_scr.at[0]
    v_scr = kv_scr.at[1]

    def x_copy(b):
        return pltpu.make_async_copy(x_hbm.at[pl.ds(b * TM, TM), :], x_scr.at[pl.ds(b * TM, TM), :], sem_x.at[b])

    def wqkv_copy(k):
        return pltpu.make_async_copy(wqkv_hbm.at[:, pl.ds(k * WC, WC)], wqkv.at[k], sem_w.at[k])

    def wo_copy():
        return pltpu.make_async_copy(wo_hbm, wo, sem_w.at[NWC])

    def raw_copies(c):
        return [
            pltpu.make_async_copy(wg_hbm.at[:, pl.ds(c * FC, FC)], rawg.at[c, :, pl.ds(0, FC)], sem_raw.at[c, 0]),
            pltpu.make_async_copy(wg_hbm.at[:, pl.ds(F // 2 + c * FC, FC)], rawg.at[c, :, pl.ds(FC, FC)], sem_raw.at[c, 1]),
            pltpu.make_async_copy(wu_hbm.at[:, pl.ds(c * FC, FC)], rawu.at[c, :, pl.ds(0, FC)], sem_raw.at[c, 2]),
            pltpu.make_async_copy(wu_hbm.at[:, pl.ds(F // 2 + c * FC, FC)], rawu.at[c, :, pl.ds(FC, FC)], sem_raw.at[c, 3]),
            pltpu.make_async_copy(wd_hbm.at[pl.ds(c * FC, FC), :], rawd.at[c, pl.ds(0, FC), :], sem_raw.at[c, 4]),
            pltpu.make_async_copy(wd_hbm.at[pl.ds(F // 2 + c * FC, FC), :], rawd.at[c, pl.ds(FC, FC), :], sem_raw.at[c, 5]),
        ]

    never = lax.broadcasted_iota(jnp.int32, (8, 128), 0) < jnp.minimum(s, 0)

    def ln_unit(b, r, tok):
        RC = 16
        r0 = pl.multiple_of(b * TM + r, RC)
        xt = x_scr[pl.ds(r0, RC), :]
        xb = x_scr[pl.ds(r0 + HM, RC), :]
        if tok is not None:
            xt = _gate(xt, tok, never)
            xb = _gate(xb, tok, never)
        top = _layernorm(xt)
        bot = _layernorm(xb)
        p0 = pl.multiple_of(r0 // 2, RC // 2)
        xn_scr[pl.ds(p0, RC // 2), :] = _pack(top)
        xn_scr[pl.ds(p0 + HM // 2, RC // 2), :] = _pack(bot)
        cs = _lhs_combos(top[:, :HD], top[:, HD:], bot[:, :HD], bot[:, HD:])
        pr = r // 2 if isinstance(r, int) else pl.multiple_of(r // 2, RC // 2)
        for j in range(7):
            s_scr[b, j, pl.ds(pr, RC // 2), :] = _pack(cs[j])
        return top[0:8, 0:128] + bot[0:8, 0:128]

    def ln_block(b, chain=False):
        tok = None
        for r in range(0, HM, 16):
            t = ln_unit(b, r, tok)
            tok = t if chain else None
        return tok

    def store_kv(y, dst, r0):
        for r in range(0, y.shape[0], 16):
            vs = _butterfly([_pack(y[r:r + 16, g * 128:(g + 1) * 128]) for g in range(NG)])
            for g in range(NG):
                dst[g, pl.ds(r0 + HALO + r, 16), :] = _unpack(vs[g])

    def store_q(y, r0):
        p0 = pl.multiple_of(r0 // 2, 8)
        for g in range(NG):
            q_scr[g, pl.ds(p0, y.shape[0] // 2), :] = _pack(y[:, g * 128:(g + 1) * 128])

    def build_tiles(ld16, st16, positions, tok, n_eup):
        for r, n0 in positions:
            for _ in range(n_eup or 0):
                tok = jnp.exp2(tok)

            def ld(q):
                w = pltpu.bitcast(ld16(q, r, n0), U32)
                if n_eup is not None:
                    w = _dep32(w, tok, never)
                return (pltpu.bitcast(w << 16, F32), pltpu.bitcast(w & jnp.uint32(0xFFFF0000), F32))

            b11, b12, b21, b22 = [ld(q) for q in range(4)]

            def comb(x, y, sign):
                ev, od = (x[0] + y[0], x[1] + y[1]) if sign > 0 else (x[0] - y[0], x[1] - y[1])
                return pltpu.bitcast(pltpu.pack_elementwise([ev, od], packed_dtype=BF), U32)

            outs = [comb(b11, b22, 1), comb(b12, b22, -1), comb(b21, b11, -1), comb(b11, b12, 1), comb(b21, b22, 1)]
            for j in range(5):
                st16(j, r, n0, outs[j])
            t = outs[0]
            if BUILD_XOR:
                t = (t ^ outs[1]) ^ (outs[2] ^ outs[3]) ^ outs[4]
            tok = pltpu.bitcast(t, F32)
        return tok

    def build_qkv(sec, kl, kr, bh, n_eup):
        rb = bh * (HD // 2)

        def row(r, m):
            return rb + r if isinstance(rb, int) else pl.multiple_of(rb + r, m)

        def ld8(q, r, n):
            return wqkv[kl if q in (0, 2) else kr, pl.ds(row((HD if q >= 2 else 0) + r, 16), 16), n:n + 128]

        def st16(j, r, n, val):
            cq[sec, bh, j, r // 2:r // 2 + 8, n:n + 128] = val

        build_tiles(ld8, st16, [(r, n) for r in range(0, HD // 2, 16) for n in range(0, WC, 128)],
                    jnp.zeros((8, 128), F32), n_eup)

    @pl.when(s == 0)
    def _():
        def issue_x(b, carry):
            x_copy(b).start(priority=1)
            return carry

        lax.fori_loop(0, 2, issue_x, 0)

        def issue_w(j, carry):
            @pl.when(j == 1)
            def _():
                x_copy(2).start(priority=1)

            wqkv_copy(lax.rem(j + 2, NWC)).start(priority=1)
            return carry

        lax.fori_loop(0, NWC, issue_w, 0)

        def issue_rest(j, carry):
            for cp in raw_copies(0):
                cp.start(priority=1)
            return carry

        lax.fori_loop(0, jnp.maximum(s, 1), issue_rest, 0)
        wo_copy().start(priority=1)
        x_copy(3).start(priority=1)
        k_scr[:, 0:HALO, :] = jnp.zeros((NG, HALO, 128), F32)
        v_scr[:, 0:HALO, :] = jnp.zeros((NG, HALO, 128), F32)
        x_copy(0).wait()
        ln_block(0)
        x_copy(1).wait()
        ln_block(1)
        P0 = R0 // 2
        xn = _as_bf16(xn_scr[0:P0, :])

        def body(j, carry):
            k = lax.rem(j + 2, NWC)
            wqkv_copy(k).wait()

            @pl.when(j == 1)
            def _():
                x_copy(2).wait()

            y = _dot(xn, wqkv[k])
            half = lax.rem(j, 2)
            sec = jnp.maximum(lax.div(j, 2) - 1, 0)
            src = pl.multiple_of((sec + 1) * P0 + half * (P0 // 2), 8)
            dstr = pl.multiple_of(HALO + half * P0, 16)
            for r in range(0, P0 // 2, 8):
                vs = _butterfly([q_scr[g, pl.ds(src + r, 8), :] for g in range(NG)])
                for g in range(NG):
                    kv_scr[sec, g, pl.ds(dstr + 2 * r, 16), :] = _unpack(vs[g])
            lb = jnp.minimum(j + 1, 2)
            u0 = 2 * jnp.clip(j - 1, 0, 3)
            tok = ln_unit(lb, pl.multiple_of(u0 * 16, 16), None)
            ln_unit(lb, pl.multiple_of(u0 * 16 + 16, 16), tok)
            jm = jnp.maximum(j - 1, 0)
            bsec = lax.div(jm, 2)
            kl = lax.rem(2 * bsec + 2, NWC)
            kr = jnp.where(j == 0, kl, kl + 1)
            bh = jnp.where(j == 0, 1, lax.rem(jm, 2))
            build_qkv(bsec, kl, kr, bh, N_EUP0)
            rb = pl.multiple_of(lax.rem(lax.div(j, 2) + 1, 3) * P0, 8)
            for gg in range(WC // 128):
                q_scr[half * (WC // 128) + gg, pl.ds(rb, P0), :] = _pack(y[:, gg * 128:(gg + 1) * 128])
            return carry

        lax.fori_loop(0, NWC, body, 0)
        build_qkv(2, 0, 1, 1, None)
        wo_copy().wait()

        def wo_ld8(q, r, n):
            return wo[pl.ds((HD if q >= 2 else 0) + r, 16), pl.ds((HD if q % 2 else 0) + n, 128)]

        def wo_st16(j, r, n, val):
            cwo[j, r // 2:r // 2 + 8, n:n + 128] = val

        build_tiles(wo_ld8, wo_st16, [(r, n) for r in range(0, HD, 16) for n in range(0, HD, 128)],
                    jnp.zeros((8, 128), F32), None)

    @pl.when(s <= NA)
    def _():
        @pl.when(s + 1 < NCH)
        def _():
            for cp in raw_copies(s + 1):
                cp.start(priority=1)

        @pl.when(s + 4 < NB)
        def _():
            x_copy(s + 4).start(priority=1)

        @pl.when(s >= 1)
        def _():
            for cp in raw_copies(s - 1):
                cp.wait()

        @pl.when(jnp.logical_and(s >= 1, s + 2 < NB))
        def _():
            x_copy(s + 2).wait()

    @pl.when(jnp.logical_and(s >= 1, s <= NA))
    def _():
        c = lax.rem(s + (NA - 1), NA)
        r0 = pl.multiple_of(R0 + (c if R0_BOUNDED else s - 1) * TA, 16)
        HA = TA // 2
        pt = pl.multiple_of(r0 // 2, 8)
        pb = pl.multiple_of((r0 + HA) // 2, 8)
        a11 = _as_bf16(xn_scr[pl.ds(pt, HA // 2), 0:HD])
        a12 = _as_bf16(xn_scr[pl.ds(pt, HA // 2), HD:D])
        a21 = _as_bf16(xn_scr[pl.ds(pb, HA // 2), 0:HD])
        a22 = _as_bf16(xn_scr[pl.ds(pb, HA // 2), HD:D])
        la = [t.astype(BF) for t in _lhs_combos(a11.astype(F32), a12.astype(F32), a21.astype(F32), a22.astype(F32))]
        la[2], la[3] = a11, a22

        def ffn_part(raw, cmb, kq, nq):
            def ld8(q, r, n):
                return raw[c, pl.ds((kq if q >= 2 else 0) + r, 16), pl.ds((nq if q % 2 else 0) + n, 128)]

            def st16(j, r, n, val):
                cmb[c, j, r // 2:r // 2 + 8, n:n + 128] = val

            return [(ld8, st16, (r, n)) for r in range(0, kq, 16) for n in range(0, nq, 128)]

        work = ffn_part(rawg, cg, HD, FC) + ffn_part(rawu, cu, HD, FC) + ffn_part(rawd, cd, FC, HD)
        ys = []
        for sec in range(3):
            kl = (2 * sec + 2) % NWC
            cw = [_as_bf16(jnp.concatenate([cq[sec, 0, j], cq[sec, 1, j]], axis=0)) for j in range(5)]
            wl = [cw[0], wqkv[kl, 0:HD, :], cw[1], cw[2], wqkv[kl + 1, HD:D, :], cw[3], cw[4]]
            c11, c12, c21, c22 = _strassen_out([_dot(la[j], wl[j]) for j in range(7)])
            ys.append((jnp.concatenate([c11, c12], axis=1), jnp.concatenate([c21, c22], axis=1)))
        ln_block(jnp.minimum(s + 2, NB - 1), chain=True)
        tok = jnp.zeros((8, 128), F32)
        for ld8, st16, pos in work:
            tok = build_tiles(ld8, st16, [pos], tok, N_EUP)
        for h in range(2):
            rh = pl.multiple_of(r0 + h * HA, 16)
            store_kv(ys[0][h], k_scr, rh)
            store_kv(ys[1][h], v_scr, rh)
            store_q(ys[2][h], rh)

    if NSTEPS < NA + 1 + NB:
        @pl.when(s == NSTEPS - 1)
        def _():
            l = NSTEPS - 1
            for c in (l, l + 1):
                if 0 <= c < NCH:
                    for cp in raw_copies(c):
                        cp.wait()
            for b in (l + 3, l + 4):
                if b < NB:
                    x_copy(b).wait()

    @pl.when(s > NA)
    def _():
        i = lax.rem(s + (NB - NA - 1), NB)
        r0 = pl.multiple_of(i * TM, TM)

        def wlist(raw, cmb, c, kq, nq):
            cw = [_as_bf16(cmb[c, j]) for j in range(5)]
            return [cw[0], raw[c, 0:kq, 0:nq], cw[1], cw[2], raw[c, kq:2 * kq, nq:2 * nq], cw[3], cw[4]]

        RA = 16
        cexp = (DH ** -0.5) * LOG2E
        p0 = pl.multiple_of(r0 // 2, 8)
        never16 = lax.broadcasted_iota(jnp.int32, (16, 128), 0) < jnp.minimum(s, 0)

        def attn_half(q, r):
            sw = []
            for w in range(WIN):
                acc = None
                for g in range(NG):
                    t = q[g] * k_scr[g, pl.ds(r0 + r + HALO - DIL * w, 8), :]
                    acc = t if acc is None else acc + t
                acc = _sum4(acc)
                if r < HALO and w > 0:
                    row = lax.broadcasted_iota(jnp.int32, (8, 128), 0) + (r0 + r)
                    acc = jnp.where(row >= DIL * w, acc, NEG)
                sw.append(acc)
            m = sw[0]
            for w in range(1, WIN):
                m = jnp.maximum(m, sw[w])
            e = [jnp.exp2((sw[w] - m) * cexp) for w in range(WIN)]
            den = e[0]
            for w in range(1, WIN):
                den = den + e[w]
            inv = 1.0 / den
            p = [e[w] * inv for w in range(WIN)]
            o = []
            for g in range(NG):
                acc = None
                for w in range(WIN):
                    t = p[w] * v_scr[g, pl.ds(r0 + r + HALO - DIL * w, 8), :]
                    acc = t if acc is None else acc + t
                o.append(acc)
            return o

        def attn_rows(r, tok):
            qp = [q_scr[g, pl.ds(p0 + r // 2, 8), :] for g in range(NG)]
            if tok is not None:
                qp = [_dep32(t, tok, never) for t in qp]
            q = [_unpack(t) for t in _butterfly(qp)]
            o0 = attn_half([t[0:8] for t in q], r)
            q1 = [t[8:16] for t in q]
            if CHAIN_HALVES:
                q1 = [_dep32(t, o0[NG - 1], never) for t in q1]
            o1 = attn_half(q1, r + 8)
            o = _butterfly([_pack(jnp.concatenate([o0[g], o1[g]], axis=0)) for g in range(NG)])
            for g in range(NG):
                o_scr[r // 2:r // 2 + 8, g * 128:(g + 1) * 128] = o[g]
            tok = o[0]
            if XOR_TOK:
                for g in range(1, NG):
                    tok = tok ^ o[g]
            return tok

        sl = [_as_bf16(s_scr[i, j]) for j in range(7)]
        acc = [None] * 7
        o_parts = []
        n_att = TM // RA
        per = 3
        tok = None
        pend = []
        for c in range(NCH):
            wg_l = wlist(rawg, cg, c, HD, FC)
            wu_l = wlist(rawu, cu, c, HD, FC)
            wd_l = wlist(rawd, cd, c, FC, HD)
            slc = sl
            g = _strassen_out([_dot(slc[j], wg_l[j]) for j in range(7)])
            u = _strassen_out([_dot(slc[j], wu_l[j]) for j in range(7)])
            hq = [g[t] * u[t] for t in range(4)]
            pend.append(([t.astype(BF) for t in _lhs_combos(*hq)], wd_l))
            if len(pend) == DOWN_GROUP or c == NCH - 1:
                for j in range(7):
                    y = _dot(jnp.concatenate([p[0][j] for p in pend], axis=1),
                             jnp.concatenate([p[1][j] for p in pend], axis=0))
                    acc[j] = y if acc[j] is None else acc[j] + y
                pend = []
            for a in range(c * per, min((c + 1) * per, n_att)):
                tok = attn_rows(a * RA, tok)
            if c == WO_AT:
                oq = [_as_bf16(o_scr[rr:rr + HM // 2, cc:cc + HD]) for rr in (0, HM // 2) for cc in (0, HD)]
                ol = [t.astype(BF) for t in _lhs_combos(*[t.astype(F32) for t in oq])]
                ol[2], ol[3] = oq[0], oq[3]
                if WO_GATE:
                    ol = [_gate(t, y[0:8, 0:128], never) for t in ol]
                cw = [_as_bf16(cwo[j]) for j in range(5)]
                wo_l = [cw[0], wo[0:HD, 0:HD], cw[1], cw[2], wo[HD:D, HD:D], cw[3], cw[4]]
                acc = [acc[j] + _dot(ol[j], wo_l[j]) for j in range(7)]
        y11, y12, y21, y22 = _strassen_out(acc)
        x = x_scr[pl.ds(r0, TM), :].astype(F32)
        o_ref[0:HM, 0:HD] = (x[0:HM, 0:HD] + y11).astype(o_ref.dtype)
        o_ref[0:HM, HD:D] = (x[0:HM, HD:D] + y12).astype(o_ref.dtype)
        o_ref[HM:TM, 0:HD] = (x[HM:TM, 0:HD] + y21).astype(o_ref.dtype)
        o_ref[HM:TM, HD:D] = (x[HM:TM, HD:D] + y22).astype(o_ref.dtype)


@jax.jit
def pallas_parallel_sum__sliding_local_dilated__glu_gated_bilinear__prompt_kernel(
    A_x: jax.Array,
    A_wqkv: jax.Array,
    A_wo: jax.Array,
    B_x: jax.Array,
    B_w_gate: jax.Array,
    B_w_up: jax.Array,
    B_w_down: jax.Array,
):
    del B_x
    x = A_x.reshape(S, D)
    hbm = pl.BlockSpec(memory_space=pl.ANY)
    out = pl.pallas_call(
        _kernel,
        grid=(NSTEPS,),
        in_specs=[hbm] * 6,
        out_specs=pl.BlockSpec((TM, D), lambda s: (jnp.maximum(s - (NA + 1), 0), 0)),
        out_shape=jax.ShapeDtypeStruct((S, D), A_x.dtype),
        scratch_shapes=[
            pltpu.VMEM((S, D), BF),
            pltpu.VMEM((NWC, D, WC), BF),
            pltpu.VMEM((D, D), BF),
            pltpu.VMEM((NCH, D, 2 * FC), BF),
            pltpu.VMEM((NCH, D, 2 * FC), BF),
            pltpu.VMEM((NCH, 2 * FC, D), BF),
            pltpu.VMEM((3, 2, 5, HD // 4, WC), U32),
            pltpu.VMEM((5, HD // 2, HD), U32),
            pltpu.VMEM((NCH, 5, HD // 2, FC), U32),
            pltpu.VMEM((NCH, 5, HD // 2, FC), U32),
            pltpu.VMEM((NCH, 5, FC // 2, HD), U32),
            pltpu.VMEM((S // 2, D), U32),
            pltpu.VMEM((NB, 7, HM // 2, HD), U32),
            pltpu.VMEM((NG, S // 2, 128), U32),
            pltpu.VMEM((2, NG, S + HALO, 128), F32),
            pltpu.VMEM((TM // 2, D), U32),
            pltpu.SemaphoreType.DMA((NB,)),
            pltpu.SemaphoreType.DMA((NWC + 1,)),
            pltpu.SemaphoreType.DMA((NCH, 6)),
        ],
        compiler_params=pltpu.CompilerParams(
            dimension_semantics=("arbitrary",),
            vmem_limit_bytes=124 * 1024 * 1024,
            disable_bounds_checks=True,
        ),
        name="fused_attn_ffn",
    )(x, A_wqkv, A_wo, B_w_gate, B_w_up, B_w_down)
    return out.reshape(A_x.shape)
```

```python
import functools

import jax
import jax.numpy as jnp
from jax import lax
from jax.experimental import pallas as pl
from jax.experimental.pallas import tpu as pltpu

S, D, F = 2048, 1024, 3584
H, DH, WIN, DIL = 32, 32, 8, 2
TM = 256
HM = TM // 2
NB = S // TM
HD = D // 2
FC = 256
NCH = F // 2 // FC
HALO = 16
NG = D // 128
EPS = 1e-5
NEG = -1e9
BF = jnp.bfloat16
F32 = jnp.float32
U32 = jnp.uint32
LOG2E = 1.4426950408889634
NA = 7
TA = 224
R0 = S - NA * TA
NSTEPS = 16
WC = 512
NWC = 3 * D // WC
N_EUP = 3
N_EUP0 = 2
BUILD_XOR = False
R0_BOUNDED = False
WO_AT = 6
WO_GATE = False
DOWN_GROUP = 2
CHAIN_HALVES = True
XOR_TOK = False


def _dot(a, b):
    return jnp.dot(a, b, preferred_element_type=F32)


def _butterfly(vs):
    lane = lax.broadcasted_iota(jnp.int32, vs[0].shape, 1)
    for b in range(3):
        sh = 4 << b
        bit = (lane & sh) != 0
        new = list(vs)
        for i0 in range(NG):
            if i0 & (1 << b):
                continue
            i1 = i0 | (1 << b)
            new[i0] = jnp.where(bit, pltpu.roll(vs[i1], sh, 1), vs[i0])
            new[i1] = jnp.where(bit, vs[i1], pltpu.roll(vs[i0], 128 - sh, 1))
        vs = new
    return vs


def _sum4(x):
    lane = lax.broadcasted_iota(jnp.int32, x.shape, 1)
    x = x + jnp.where((lane & 1) != 0, pltpu.roll(x, 1, 1), pltpu.roll(x, 127, 1))
    x = x + jnp.where((lane & 2) != 0, pltpu.roll(x, 2, 1), pltpu.roll(x, 126, 1))
    return x


def _dep32(x, tok, never):
    return jnp.where(never, pltpu.bitcast(tok, x.dtype), x)


def _gate(m, tok, never):
    t = pltpu.bitcast(m[0:16, 0:128], F32)
    t = pltpu.bitcast(_dep32(t, tok, never), BF)
    top = jnp.concatenate([t, m[0:16, 128:]], axis=1)
    if m.shape[0] == 16:
        return top
    return jnp.concatenate([top, m[16:]], axis=0)


def _pack(y):
    return pltpu.bitcast(y.astype(BF), U32)


def _as_bf16(w):
    return pltpu.bitcast(w, BF)


def _unpack(w):
    return pltpu.bitcast(w, BF).astype(F32)


def _lhs_combos(a11, a12, a21, a22):
    return [a11 + a22, a21 + a22, a11, a22, a11 + a12, a21 - a11, a12 - a22]


def _strassen_out(m):
    return (m[0] + m[3] - m[4] + m[6], m[2] + m[4], m[1] + m[3], m[0] - m[1] + m[2] + m[5])


def _layernorm(x):
    x = x.astype(F32)
    mean = jnp.mean(x, axis=-1, keepdims=True)
    xc = x - mean
    var = jnp.mean(xc * xc, axis=-1, keepdims=True)
    return xc * lax.rsqrt(var + EPS)


def _kernel(x_hbm, wqkv_hbm, wo_hbm, wg_hbm, wu_hbm, wd_hbm, o_hbm,
            x_scr, wqkv, wo, rawg, rawu, rawd, cq, cwo, cg, cu, cd,
            xn_scr, s_scr, q_scr, kv_scr, o_scr, ob0, ob1, ob2, ob3,
            sem_x, sem_w, sem_raw, sem_o):
    s = pl.program_id(0)
    k_scr = kv_scr.at[0]
    v_scr = kv_scr.at[1]

    def x_copy(b):
        return pltpu.make_async_copy(x_hbm.at[pl.ds(b * TM, TM), :], x_scr.at[pl.ds(b * TM, TM), :], sem_x.at[b])

    def wqkv_copy(k):
        return pltpu.make_async_copy(wqkv_hbm.at[:, pl.ds(k * WC, WC)], wqkv.at[k], sem_w.at[k])

    def wo_copy():
        return pltpu.make_async_copy(wo_hbm, wo, sem_w.at[NWC])

    def raw_copies(c):
        return [
            pltpu.make_async_copy(wg_hbm.at[:, pl.ds(c * FC, FC)], rawg.at[c, :, pl.ds(0, FC)], sem_raw.at[c, 0]),
            pltpu.make_async_copy(wg_hbm.at[:, pl.ds(F // 2 + c * FC, FC)], rawg.at[c, :, pl.ds(FC, FC)], sem_raw.at[c, 1]),
            pltpu.make_async_copy(wu_hbm.at[:, pl.ds(c * FC, FC)], rawu.at[c, :, pl.ds(0, FC)], sem_raw.at[c, 2]),
            pltpu.make_async_copy(wu_hbm.at[:, pl.ds(F // 2 + c * FC, FC)], rawu.at[c, :, pl.ds(FC, FC)], sem_raw.at[c, 3]),
            pltpu.make_async_copy(wd_hbm.at[pl.ds(c * FC, FC), :], rawd.at[c, pl.ds(0, FC), :], sem_raw.at[c, 4]),
            pltpu.make_async_copy(wd_hbm.at[pl.ds(F // 2 + c * FC, FC), :], rawd.at[c, pl.ds(FC, FC), :], sem_raw.at[c, 5]),
        ]

    def out_copy(i, q):
        slot = lax.rem(i, 2)
        rr, cc = (q // 2) * HM, (q % 2) * HD
        return pltpu.make_async_copy((ob0, ob1, ob2, ob3)[q].at[slot],
                                     o_hbm.at[pl.ds(i * TM + rr, HM), pl.ds(cc, HD)], sem_o.at[slot, q])

    never = lax.broadcasted_iota(jnp.int32, (8, 128), 0) < jnp.minimum(s, 0)

    def ln_unit(b, r, tok):
        RC = 16
        r0 = pl.multiple_of(b * TM + r, RC)
        xt = x_scr[pl.ds(r0, RC), :]
        xb = x_scr[pl.ds(r0 + HM, RC), :]
        if tok is not None:
            xt = _gate(xt, tok, never)
            xb = _gate(xb, tok, never)
        top = _layernorm(xt)
        bot = _layernorm(xb)
        p0 = pl.multiple_of(r0 // 2, RC // 2)
        xn_scr[pl.ds(p0, RC // 2), :] = _pack(top)
        xn_scr[pl.ds(p0 + HM // 2, RC // 2), :] = _pack(bot)
        cs = _lhs_combos(top[:, :HD], top[:, HD:], bot[:, :HD], bot[:, HD:])
        pr = r // 2 if isinstance(r, int) else pl.multiple_of(r // 2, RC // 2)
        for j in range(7):
            s_scr[b, j, pl.ds(pr, RC // 2), :] = _pack(cs[j])
        return top[0:8, 0:128] + bot[0:8, 0:128]

    def ln_block(b, chain=False):
        tok = None
        for r in range(0, HM, 16):
            t = ln_unit(b, r, tok)
            tok = t if chain else None
        return tok

    def store_kv(y, dst, r0):
        for r in range(0, y.shape[0], 16):
            vs = _butterfly([_pack(y[r:r + 16, g * 128:(g + 1) * 128]) for g in range(NG)])
            for g in range(NG):
                dst[g, pl.ds(r0 + HALO + r, 16), :] = _unpack(vs[g])

    def store_q(y, r0):
        p0 = pl.multiple_of(r0 // 2, 8)
        for g in range(NG):
            q_scr[g, pl.ds(p0, y.shape[0] // 2), :] = _pack(y[:, g * 128:(g + 1) * 128])

    def build_tiles(ld16, st16, positions, tok, n_eup):
        for r, n0 in positions:
            for _ in range(n_eup or 0):
                tok = jnp.exp2(tok)

            def ld(q):
                w = pltpu.bitcast(ld16(q, r, n0), U32)
                if n_eup is not None:
                    w = _dep32(w, tok, never)
                return (pltpu.bitcast(w << 16, F32), pltpu.bitcast(w & jnp.uint32(0xFFFF0000), F32))

            b11, b12, b21, b22 = [ld(q) for q in range(4)]

            def comb(x, y, sign):
                ev, od = (x[0] + y[0], x[1] + y[1]) if sign > 0 else (x[0] - y[0], x[1] - y[1])
                return pltpu.bitcast(pltpu.pack_elementwise([ev, od], packed_dtype=BF), U32)

            outs = [comb(b11, b22, 1), comb(b12, b22, -1), comb(b21, b11, -1), comb(b11, b12, 1), comb(b21, b22, 1)]
            for j in range(5):
                st16(j, r, n0, outs[j])
            t = outs[0]
            if BUILD_XOR:
                t = (t ^ outs[1]) ^ (outs[2] ^ outs[3]) ^ outs[4]
            tok = pltpu.bitcast(t, F32)
        return tok

    def build_qkv(sec, kl, kr, bh, n_eup):
        rb = bh * (HD // 2)

        def row(r, m):
            return rb + r if isinstance(rb, int) else pl.multiple_of(rb + r, m)

        def ld8(q, r, n):
            return wqkv[kl if q in (0, 2) else kr, pl.ds(row((HD if q >= 2 else 0) + r, 16), 16), n:n + 128]

        def st16(j, r, n, val):
            cq[sec, bh, j, r // 2:r // 2 + 8, n:n + 128] = val

        build_tiles(ld8, st16, [(r, n) for r in range(0, HD // 2, 16) for n in range(0, WC, 128)],
                    jnp.zeros((8, 128), F32), n_eup)

    @pl.when(s == 0)
    def _():
        def issue_x(b, carry):
            x_copy(b).start(priority=1)
            return carry

        lax.fori_loop(0, 2, issue_x, 0)

        def issue_w(j, carry):
            @pl.when(j == 1)
            def _():
                x_copy(2).start(priority=1)

            wqkv_copy(lax.rem(j + 2, NWC)).start(priority=1)
            return carry

        lax.fori_loop(0, NWC, issue_w, 0)

        def issue_rest(j, carry):
            for cp in raw_copies(0):
                cp.start(priority=1)
            return carry

        lax.fori_loop(0, jnp.maximum(s, 1), issue_rest, 0)
        wo_copy().start(priority=1)
        x_copy(3).start(priority=1)
        k_scr[:, 0:HALO, :] = jnp.zeros((NG, HALO, 128), F32)
        v_scr[:, 0:HALO, :] = jnp.zeros((NG, HALO, 128), F32)
        x_copy(0).wait()
        ln_block(0)
        x_copy(1).wait()
        ln_block(1)
        P0 = R0 // 2
        xn = _as_bf16(xn_scr[0:P0, :])

        def body(j, carry):
            k = lax.rem(j + 2, NWC)
            wqkv_copy(k).wait()

            @pl.when(j == 1)
            def _():
                x_copy(2).wait()

            y = _dot(xn, wqkv[k])
            half = lax.rem(j, 2)
            sec = jnp.maximum(lax.div(j, 2) - 1, 0)
            src = pl.multiple_of((sec + 1) * P0 + half * (P0 // 2), 8)
            dstr = pl.multiple_of(HALO + half * P0, 16)
            for r in range(0, P0 // 2, 8):
                vs = _butterfly([q_scr[g, pl.ds(src + r, 8), :] for g in range(NG)])
                for g in range(NG):
                    kv_scr[sec, g, pl.ds(dstr + 2 * r, 16), :] = _unpack(vs[g])
            lb = jnp.minimum(j + 1, 2)
            u0 = 2 * jnp.clip(j - 1, 0, 3)
            tok = ln_unit(lb, pl.multiple_of(u0 * 16, 16), None)
            ln_unit(lb, pl.multiple_of(u0 * 16 + 16, 16), tok)
            jm = jnp.maximum(j - 1, 0)
            bsec = lax.div(jm, 2)
            kl = lax.rem(2 * bsec + 2, NWC)
            kr = jnp.where(j == 0, kl, kl + 1)
            bh = jnp.where(j == 0, 1, lax.rem(jm, 2))
            build_qkv(bsec, kl, kr, bh, N_EUP0)
            rb = pl.multiple_of(lax.rem(lax.div(j, 2) + 1, 3) * P0, 8)
            for gg in range(WC // 128):
                q_scr[half * (WC // 128) + gg, pl.ds(rb, P0), :] = _pack(y[:, gg * 128:(gg + 1) * 128])
            return carry

        lax.fori_loop(0, NWC, body, 0)
        build_qkv(2, 0, 1, 1, None)
        wo_copy().wait()

        def wo_ld8(q, r, n):
            return wo[pl.ds((HD if q >= 2 else 0) + r, 16), pl.ds((HD if q % 2 else 0) + n, 128)]

        def wo_st16(j, r, n, val):
            cwo[j, r // 2:r // 2 + 8, n:n + 128] = val

        build_tiles(wo_ld8, wo_st16, [(r, n) for r in range(0, HD, 16) for n in range(0, HD, 128)],
                    jnp.zeros((8, 128), F32), None)

    @pl.when(s <= NA)
    def _():
        @pl.when(s + 1 < NCH)
        def _():
            for cp in raw_copies(s + 1):
                cp.start(priority=1)

        @pl.when(s + 4 < NB)
        def _():
            x_copy(s + 4).start(priority=1)

        @pl.when(s >= 1)
        def _():
            for cp in raw_copies(s - 1):
                cp.wait()

        @pl.when(jnp.logical_and(s >= 1, s + 2 < NB))
        def _():
            x_copy(s + 2).wait()

    @pl.when(s >= NA + 3)
    def _():
        for q in range(4):
            out_copy(s - (NA + 3), q).wait()

    @pl.when(jnp.logical_and(s >= 1, s <= NA))
    def _():
        c = lax.rem(s + (NA - 1), NA)
        r0 = pl.multiple_of(R0 + (c if R0_BOUNDED else s - 1) * TA, 16)
        HA = TA // 2
        pt = pl.multiple_of(r0 // 2, 8)
        pb = pl.multiple_of((r0 + HA) // 2, 8)
        a11 = _as_bf16(xn_scr[pl.ds(pt, HA // 2), 0:HD])
        a12 = _as_bf16(xn_scr[pl.ds(pt, HA // 2), HD:D])
        a21 = _as_bf16(xn_scr[pl.ds(pb, HA // 2), 0:HD])
        a22 = _as_bf16(xn_scr[pl.ds(pb, HA // 2), HD:D])
        la = [t.astype(BF) for t in _lhs_combos(a11.astype(F32), a12.astype(F32), a21.astype(F32), a22.astype(F32))]
        la[2], la[3] = a11, a22

        def ffn_part(raw, cmb, kq, nq):
            def ld8(q, r, n):
                return raw[c, pl.ds((kq if q >= 2 else 0) + r, 16), pl.ds((nq if q % 2 else 0) + n, 128)]

            def st16(j, r, n, val):
                cmb[c, j, r // 2:r // 2 + 8, n:n + 128] = val

            return [(ld8, st16, (r, n)) for r in range(0, kq, 16) for n in range(0, nq, 128)]

        work = ffn_part(rawg, cg, HD, FC) + ffn_part(rawu, cu, HD, FC) + ffn_part(rawd, cd, FC, HD)
        ys = []
        for sec in range(3):
            kl = (2 * sec + 2) % NWC
            cw = [_as_bf16(jnp.concatenate([cq[sec, 0, j], cq[sec, 1, j]], axis=0)) for j in range(5)]
            wl = [cw[0], wqkv[kl, 0:HD, :], cw[1], cw[2], wqkv[kl + 1, HD:D, :], cw[3], cw[4]]
            c11, c12, c21, c22 = _strassen_out([_dot(la[j], wl[j]) for j in range(7)])
            ys.append((jnp.concatenate([c11, c12], axis=1), jnp.concatenate([c21, c22], axis=1)))
        ln_block(jnp.minimum(s + 2, NB - 1), chain=True)
        tok = jnp.zeros((8, 128), F32)
        for ld8, st16, pos in work:
            tok = build_tiles(ld8, st16, [pos], tok, N_EUP)
        for h in range(2):
            rh = pl.multiple_of(r0 + h * HA, 16)
            store_kv(ys[0][h], k_scr, rh)
            store_kv(ys[1][h], v_scr, rh)
            store_q(ys[2][h], rh)

    if NSTEPS < NA + 1 + NB:
        @pl.when(s == NSTEPS - 1)
        def _():
            l = NSTEPS - 1
            for c in (l, l + 1):
                if 0 <= c < NCH:
                    for cp in raw_copies(c):
                        cp.wait()
            for b in (l + 3, l + 4):
                if b < NB:
                    x_copy(b).wait()

    @pl.when(s > NA)
    def _():
        i = lax.rem(s + (NB - NA - 1), NB)
        r0 = pl.multiple_of(i * TM, TM)

        def wlist(raw, cmb, c, kq, nq):
            cw = [_as_bf16(cmb[c, j]) for j in range(5)]
            return [cw[0], raw[c, 0:kq, 0:nq], cw[1], cw[2], raw[c, kq:2 * kq, nq:2 * nq], cw[3], cw[4]]

        RA = 16
        cexp = (DH ** -0.5) * LOG2E
        p0 = pl.multiple_of(r0 // 2, 8)
        never16 = lax.broadcasted_iota(jnp.int32, (16, 128), 0) < jnp.minimum(s, 0)

        def attn_half(q, r):
            sw = []
            for w in range(WIN):
                acc = None
                for g in range(NG):
                    t = q[g] * k_scr[g, pl.ds(r0 + r + HALO - DIL * w, 8), :]
                    acc = t if acc is None else acc + t
                acc = _sum4(acc)
                if r < HALO and w > 0:
                    row = lax.broadcasted_iota(jnp.int32, (8, 128), 0) + (r0 + r)
                    acc = jnp.where(row >= DIL * w, acc, NEG)
                sw.append(acc)
            m = sw[0]
            for w in range(1, WIN):
                m = jnp.maximum(m, sw[w])
            e = [jnp.exp2((sw[w] - m) * cexp) for w in range(WIN)]
            den = e[0]
            for w in range(1, WIN):
                den = den + e[w]
            inv = 1.0 / den
            p = [e[w] * inv for w in range(WIN)]
            o = []
            for g in range(NG):
                acc = None
                for w in range(WIN):
                    t = p[w] * v_scr[g, pl.ds(r0 + r + HALO - DIL * w, 8), :]
                    acc = t if acc is None else acc + t
                o.append(acc)
            return o

        def attn_rows(r, tok):
            qp = [q_scr[g, pl.ds(p0 + r // 2, 8), :] for g in range(NG)]
            if tok is not None:
                qp = [_dep32(t, tok, never) for t in qp]
            q = [_unpack(t) for t in _butterfly(qp)]
            o0 = attn_half([t[0:8] for t in q], r)
            q1 = [t[8:16] for t in q]
            if CHAIN_HALVES:
                q1 = [_dep32(t, o0[NG - 1], never) for t in q1]
            o1 = attn_half(q1, r + 8)
            o = _butterfly([_pack(jnp.concatenate([o0[g], o1[g]], axis=0)) for g in range(NG)])
            for g in range(NG):
                o_scr[r // 2:r // 2 + 8, g * 128:(g + 1) * 128] = o[g]
            tok = o[0]
            if XOR_TOK:
                for g in range(1, NG):
                    tok = tok ^ o[g]
            return tok

        sl = [_as_bf16(s_scr[i, j]) for j in range(7)]
        acc = [None] * 7
        o_parts = []
        n_att = TM // RA
        per = 3
        tok = None
        pend = []
        for c in range(NCH):
            wg_l = wlist(rawg, cg, c, HD, FC)
            wu_l = wlist(rawu, cu, c, HD, FC)
            wd_l = wlist(rawd, cd, c, FC, HD)
            slc = sl
            g = _strassen_out([_dot(slc[j], wg_l[j]) for j in range(7)])
            u = _strassen_out([_dot(slc[j], wu_l[j]) for j in range(7)])
            hq = [g[t] * u[t] for t in range(4)]
            pend.append(([t.astype(BF) for t in _lhs_combos(*hq)], wd_l))
            if len(pend) == DOWN_GROUP or c == NCH - 1:
                for j in range(7):
                    y = _dot(jnp.concatenate([p[0][j] for p in pend], axis=1),
                             jnp.concatenate([p[1][j] for p in pend], axis=0))
                    acc[j] = y if acc[j] is None else acc[j] + y
                pend = []
            for a in range(c * per, min((c + 1) * per, n_att)):
                tok = attn_rows(a * RA, tok)
            if c == WO_AT:
                oq = [_as_bf16(o_scr[rr:rr + HM // 2, cc:cc + HD]) for rr in (0, HM // 2) for cc in (0, HD)]
                ol = [t.astype(BF) for t in _lhs_combos(*[t.astype(F32) for t in oq])]
                ol[2], ol[3] = oq[0], oq[3]
                if WO_GATE:
                    ol = [_gate(t, y[0:8, 0:128], never) for t in ol]
                cw = [_as_bf16(cwo[j]) for j in range(5)]
                wo_l = [cw[0], wo[0:HD, 0:HD], cw[1], cw[2], wo[HD:D, HD:D], cw[3], cw[4]]
                acc = [acc[j] + _dot(ol[j], wo_l[j]) for j in range(7)]
        ys = _strassen_out(acc)
        x = x_scr[pl.ds(r0, TM), :].astype(F32)
        slot = lax.rem(i, 2)
        for q in range(4):
            rr, cc = (q // 2) * HM, (q % 2) * HD
            (ob0, ob1, ob2, ob3)[q][slot] = (x[rr:rr + HM, cc:cc + HD] + ys[q]).astype(BF)
            out_copy(i, q).start()

        @pl.when(i == NB - 1)
        def _():
            for q in range(4):
                out_copy(i - 1, q).wait()
            for q in range(4):
                out_copy(i, q).wait()


@jax.jit
def pallas_parallel_sum__sliding_local_dilated__glu_gated_bilinear__prompt_kernel(
    A_x: jax.Array,
    A_wqkv: jax.Array,
    A_wo: jax.Array,
    B_x: jax.Array,
    B_w_gate: jax.Array,
    B_w_up: jax.Array,
    B_w_down: jax.Array,
):
    del B_x
    x = A_x.reshape(S, D)
    hbm = pl.BlockSpec(memory_space=pl.ANY)
    out = pl.pallas_call(
        _kernel,
        grid=(NSTEPS,),
        in_specs=[hbm] * 6,
        out_specs=hbm,
        out_shape=jax.ShapeDtypeStruct((S, D), A_x.dtype),
        scratch_shapes=[
            pltpu.VMEM((S, D), BF),
            pltpu.VMEM((NWC, D, WC), BF),
            pltpu.VMEM((D, D), BF),
            pltpu.VMEM((NCH, D, 2 * FC), BF),
            pltpu.VMEM((NCH, D, 2 * FC), BF),
            pltpu.VMEM((NCH, 2 * FC, D), BF),
            pltpu.VMEM((3, 2, 5, HD // 4, WC), U32),
            pltpu.VMEM((5, HD // 2, HD), U32),
            pltpu.VMEM((NCH, 5, HD // 2, FC), U32),
            pltpu.VMEM((NCH, 5, HD // 2, FC), U32),
            pltpu.VMEM((NCH, 5, FC // 2, HD), U32),
            pltpu.VMEM((S // 2, D), U32),
            pltpu.VMEM((NB, 7, HM // 2, HD), U32),
            pltpu.VMEM((NG, S // 2, 128), U32),
            pltpu.VMEM((2, NG, S + HALO, 128), F32),
            pltpu.VMEM((TM // 2, D), U32),
            pltpu.VMEM((2, HM, HD), BF),
            pltpu.VMEM((2, HM, HD), BF),
            pltpu.VMEM((2, HM, HD), BF),
            pltpu.VMEM((2, HM, HD), BF),
            pltpu.SemaphoreType.DMA((NB,)),
            pltpu.SemaphoreType.DMA((NWC + 1,)),
            pltpu.SemaphoreType.DMA((NCH, 6)),
            pltpu.SemaphoreType.DMA((2, 4)),
        ],
        compiler_params=pltpu.CompilerParams(
            dimension_semantics=("arbitrary",),
            vmem_limit_bytes=124 * 1024 * 1024,
            disable_bounds_checks=True,
        ),
        name="fused_attn_ffn",
    )(x, A_wqkv, A_wo, B_w_gate, B_w_up, B_w_down)
    return out.reshape(A_x.shape)
```

```python
import functools

import jax
import jax.numpy as jnp
from jax import lax
from jax.experimental import pallas as pl
from jax.experimental.pallas import tpu as pltpu

S, D, F = 2048, 1024, 3584
H, DH, WIN, DIL = 32, 32, 8, 2
TM = 256
HM = TM // 2
NB = S // TM
HD = D // 2
FC = 256
NCH = F // 2 // FC
HALO = 16
NG = D // 128
EPS = 1e-5
NEG = -1e9
BF = jnp.bfloat16
F32 = jnp.float32
U32 = jnp.uint32
LOG2E = 1.4426950408889634
NA = 7
TA = 224
R0 = S - NA * TA
NSTEPS = 16
NWP = 8
WC = 512
NWC = 3 * D // WC
N_EUP = 3
N_EUP0 = 2
BUILD_XOR = False
R0_BOUNDED = False
WO_AT = 6
WO_GATE = False
DOWN_GROUP = 2
CHAIN_HALVES = True
XOR_TOK = False


def _dot(a, b):
    return jnp.dot(a, b, preferred_element_type=F32)


def _butterfly(vs):
    lane = lax.broadcasted_iota(jnp.int32, vs[0].shape, 1)
    for b in range(3):
        sh = 4 << b
        bit = (lane & sh) != 0
        new = list(vs)
        for i0 in range(NG):
            if i0 & (1 << b):
                continue
            i1 = i0 | (1 << b)
            new[i0] = jnp.where(bit, pltpu.roll(vs[i1], sh, 1), vs[i0])
            new[i1] = jnp.where(bit, vs[i1], pltpu.roll(vs[i0], 128 - sh, 1))
        vs = new
    return vs


def _sum4(x):
    lane = lax.broadcasted_iota(jnp.int32, x.shape, 1)
    x = x + jnp.where((lane & 1) != 0, pltpu.roll(x, 1, 1), pltpu.roll(x, 127, 1))
    x = x + jnp.where((lane & 2) != 0, pltpu.roll(x, 2, 1), pltpu.roll(x, 126, 1))
    return x


def _dep32(x, tok, never):
    return jnp.where(never, pltpu.bitcast(tok, x.dtype), x)


def _gate(m, tok, never):
    t = pltpu.bitcast(m[0:16, 0:128], F32)
    t = pltpu.bitcast(_dep32(t, tok, never), BF)
    top = jnp.concatenate([t, m[0:16, 128:]], axis=1)
    if m.shape[0] == 16:
        return top
    return jnp.concatenate([top, m[16:]], axis=0)


def _pack(y):
    return pltpu.bitcast(y.astype(BF), U32)


def _as_bf16(w):
    return pltpu.bitcast(w, BF)


def _unpack(w):
    return pltpu.bitcast(w, BF).astype(F32)


def _lhs_combos(a11, a12, a21, a22):
    return [a11 + a22, a21 + a22, a11, a22, a11 + a12, a21 - a11, a12 - a22]


def _strassen_out(m):
    return (m[0] + m[3] - m[4] + m[6], m[2] + m[4], m[1] + m[3], m[0] - m[1] + m[2] + m[5])


def _layernorm(x):
    x = x.astype(F32)
    mean = jnp.mean(x, axis=-1, keepdims=True)
    xc = x - mean
    var = jnp.mean(xc * xc, axis=-1, keepdims=True)
    return xc * lax.rsqrt(var + EPS)


def _kernel(x_hbm, wqkv_hbm, wo_hbm, wg_hbm, wu_hbm, wd_hbm, o_hbm,
            x_scr, wqkv, wo, rawg, rawu, rawd, cq, cwo, cg, cu, cd,
            xn_scr, s_scr, q_scr, kv_scr, o_scr, ob0, ob1, ob2, ob3,
            sem_x, sem_w, sem_raw, sem_o):
    s = pl.program_id(0)
    k_scr = kv_scr.at[0]
    v_scr = kv_scr.at[1]

    def x_copy(b):
        return pltpu.make_async_copy(x_hbm.at[pl.ds(b * TM, TM), :], x_scr.at[pl.ds(b * TM, TM), :], sem_x.at[b])

    def wqkv_copy(k):
        return pltpu.make_async_copy(wqkv_hbm.at[:, pl.ds(k * WC, WC)], wqkv.at[k], sem_w.at[k])

    def wo_copy():
        return pltpu.make_async_copy(wo_hbm, wo, sem_w.at[NWC])

    def raw_copies(c):
        return [
            pltpu.make_async_copy(wg_hbm.at[:, pl.ds(c * FC, FC)], rawg.at[c, :, pl.ds(0, FC)], sem_raw.at[c, 0]),
            pltpu.make_async_copy(wg_hbm.at[:, pl.ds(F // 2 + c * FC, FC)], rawg.at[c, :, pl.ds(FC, FC)], sem_raw.at[c, 1]),
            pltpu.make_async_copy(wu_hbm.at[:, pl.ds(c * FC, FC)], rawu.at[c, :, pl.ds(0, FC)], sem_raw.at[c, 2]),
            pltpu.make_async_copy(wu_hbm.at[:, pl.ds(F // 2 + c * FC, FC)], rawu.at[c, :, pl.ds(FC, FC)], sem_raw.at[c, 3]),
            pltpu.make_async_copy(wd_hbm.at[pl.ds(c * FC, FC), :], rawd.at[c, pl.ds(0, FC), :], sem_raw.at[c, 4]),
            pltpu.make_async_copy(wd_hbm.at[pl.ds(F // 2 + c * FC, FC), :], rawd.at[c, pl.ds(FC, FC), :], sem_raw.at[c, 5]),
        ]

    def out_copy(i, q):
        slot = lax.rem(i, 2)
        rr, cc = (q // 2) * HM, (q % 2) * HD
        return pltpu.make_async_copy((ob0, ob1, ob2, ob3)[q].at[slot],
                                     o_hbm.at[pl.ds(i * TM + rr, HM), pl.ds(cc, HD)], sem_o.at[slot, q])

    never = lax.broadcasted_iota(jnp.int32, (8, 128), 0) < jnp.minimum(s, 0)

    def ln_unit(b, r, tok):
        RC = 16
        r0 = pl.multiple_of(b * TM + r, RC)
        xt = x_scr[pl.ds(r0, RC), :]
        xb = x_scr[pl.ds(r0 + HM, RC), :]
        if tok is not None:
            xt = _gate(xt, tok, never)
            xb = _gate(xb, tok, never)
        top = _layernorm(xt)
        bot = _layernorm(xb)
        p0 = pl.multiple_of(r0 // 2, RC // 2)
        xn_scr[pl.ds(p0, RC // 2), :] = _pack(top)
        xn_scr[pl.ds(p0 + HM // 2, RC // 2), :] = _pack(bot)
        cs = _lhs_combos(top[:, :HD], top[:, HD:], bot[:, :HD], bot[:, HD:])
        pr = r // 2 if isinstance(r, int) else pl.multiple_of(r // 2, RC // 2)
        for j in range(7):
            s_scr[b, j, pl.ds(pr, RC // 2), :] = _pack(cs[j])
        return top[0:8, 0:128] + bot[0:8, 0:128]

    def ln_block(b, chain=False):
        tok = None
        for r in range(0, HM, 16):
            t = ln_unit(b, r, tok)
            tok = t if chain else None
        return tok

    def store_kv(y, dst, r0):
        for r in range(0, y.shape[0], 16):
            vs = _butterfly([_pack(y[r:r + 16, g * 128:(g + 1) * 128]) for g in range(NG)])
            for g in range(NG):
                dst[g, pl.ds(r0 + HALO + r, 16), :] = _unpack(vs[g])

    def store_q(y, r0):
        p0 = pl.multiple_of(r0 // 2, 8)
        for g in range(NG):
            q_scr[g, pl.ds(p0, y.shape[0] // 2), :] = _pack(y[:, g * 128:(g + 1) * 128])

    def build_tiles(ld16, st16, positions, tok, n_eup):
        for r, n0 in positions:
            for _ in range(n_eup or 0):
                tok = jnp.exp2(tok)

            def ld(q):
                w = pltpu.bitcast(ld16(q, r, n0), U32)
                if n_eup is not None:
                    w = _dep32(w, tok, never)
                return (pltpu.bitcast(w << 16, F32), pltpu.bitcast(w & jnp.uint32(0xFFFF0000), F32))

            b11, b12, b21, b22 = [ld(q) for q in range(4)]

            def comb(x, y, sign):
                ev, od = (x[0] + y[0], x[1] + y[1]) if sign > 0 else (x[0] - y[0], x[1] - y[1])
                return pltpu.bitcast(pltpu.pack_elementwise([ev, od], packed_dtype=BF), U32)

            outs = [comb(b11, b22, 1), comb(b12, b22, -1), comb(b21, b11, -1), comb(b11, b12, 1), comb(b21, b22, 1)]
            for j in range(5):
                st16(j, r, n0, outs[j])
            t = outs[0]
            if BUILD_XOR:
                t = (t ^ outs[1]) ^ (outs[2] ^ outs[3]) ^ outs[4]
            tok = pltpu.bitcast(t, F32)
        return tok

    def build_qkv(sec, kl, kr, bh, n_eup):
        rb = bh * (HD // 2)

        def row(r, m):
            return rb + r if isinstance(rb, int) else pl.multiple_of(rb + r, m)

        def ld8(q, r, n):
            return wqkv[kl if q in (0, 2) else kr, pl.ds(row((HD if q >= 2 else 0) + r, 16), 16), n:n + 128]

        def st16(j, r, n, val):
            cq[sec, bh, j, r // 2:r // 2 + 8, n:n + 128] = val

        build_tiles(ld8, st16, [(r, n) for r in range(0, HD // 2, 16) for n in range(0, WC, 128)],
                    jnp.zeros((8, 128), F32), n_eup)

    def wo_part(t):
        def ld16(q, r, n):
            return wo[q // 2, t, r:r + 16, pl.ds((HD if q % 2 else 0) + n, 128)]

        def st16(j, r, n, val):
            cwo[t, j, r // 2:r // 2 + 8, n:n + 128] = val

        return [(ld16, st16, (r, n)) for r in range(0, HD // NWP, 16) for n in range(0, HD, 128)]

    @pl.when(s == 0)
    def _():
        def issue_x(b, carry):
            x_copy(b).start(priority=1)
            return carry

        lax.fori_loop(0, 2, issue_x, 0)

        def issue_w(j, carry):
            @pl.when(j == 1)
            def _():
                x_copy(2).start(priority=1)

            wqkv_copy(lax.rem(j + 2, NWC)).start(priority=1)
            return carry

        lax.fori_loop(0, NWC, issue_w, 0)

        def issue_rest(j, carry):
            for cp in raw_copies(0):
                cp.start(priority=1)
            return carry

        lax.fori_loop(0, jnp.maximum(s, 1), issue_rest, 0)
        wo_copy().start(priority=1)
        x_copy(3).start(priority=1)
        k_scr[:, 0:HALO, :] = jnp.zeros((NG, HALO, 128), F32)
        v_scr[:, 0:HALO, :] = jnp.zeros((NG, HALO, 128), F32)
        x_copy(0).wait()
        ln_block(0)
        x_copy(1).wait()
        ln_block(1)
        P0 = R0 // 2
        xn = _as_bf16(xn_scr[0:P0, :])

        def body(j, carry):
            k = lax.rem(j + 2, NWC)
            wqkv_copy(k).wait()

            @pl.when(j == 1)
            def _():
                x_copy(2).wait()

            y = _dot(xn, wqkv[k])
            half = lax.rem(j, 2)
            sec = jnp.maximum(lax.div(j, 2) - 1, 0)
            src = pl.multiple_of((sec + 1) * P0 + half * (P0 // 2), 8)
            dstr = pl.multiple_of(HALO + half * P0, 16)
            for r in range(0, P0 // 2, 8):
                vs = _butterfly([q_scr[g, pl.ds(src + r, 8), :] for g in range(NG)])
                for g in range(NG):
                    kv_scr[sec, g, pl.ds(dstr + 2 * r, 16), :] = _unpack(vs[g])
            lb = jnp.minimum(j + 1, 2)
            u0 = 2 * jnp.clip(j - 1, 0, 3)
            tok = ln_unit(lb, pl.multiple_of(u0 * 16, 16), None)
            ln_unit(lb, pl.multiple_of(u0 * 16 + 16, 16), tok)
            jm = jnp.maximum(j - 1, 0)
            bsec = lax.div(jm, 2)
            kl = lax.rem(2 * bsec + 2, NWC)
            kr = jnp.where(j == 0, kl, kl + 1)
            bh = jnp.where(j == 0, 1, lax.rem(jm, 2))
            build_qkv(bsec, kl, kr, bh, N_EUP0)
            rb = pl.multiple_of(lax.rem(lax.div(j, 2) + 1, 3) * P0, 8)
            for gg in range(WC // 128):
                q_scr[half * (WC // 128) + gg, pl.ds(rb, P0), :] = _pack(y[:, gg * 128:(gg + 1) * 128])
            return carry

        lax.fori_loop(0, NWC, body, 0)
        build_qkv(2, 0, 1, 1, None)
        wo_copy().wait()
        for ld16, st16, pos in wo_part(NWP - 1):
            build_tiles(ld16, st16, [pos], jnp.zeros((8, 128), F32), None)

    @pl.when(s <= NA)
    def _():
        @pl.when(s + 1 < NCH)
        def _():
            for cp in raw_copies(s + 1):
                cp.start(priority=1)

        @pl.when(s + 4 < NB)
        def _():
            x_copy(s + 4).start(priority=1)

        @pl.when(s >= 1)
        def _():
            for cp in raw_copies(s - 1):
                cp.wait()

        @pl.when(jnp.logical_and(s >= 1, s + 2 < NB))
        def _():
            x_copy(s + 2).wait()

    @pl.when(s >= NA + 3)
    def _():
        for q in range(4):
            out_copy(s - (NA + 3), q).wait()

    @pl.when(jnp.logical_and(s >= 1, s <= NA))
    def _():
        c = lax.rem(s + (NA - 1), NA)
        r0 = pl.multiple_of(R0 + (c if R0_BOUNDED else s - 1) * TA, 16)
        HA = TA // 2
        pt = pl.multiple_of(r0 // 2, 8)
        pb = pl.multiple_of((r0 + HA) // 2, 8)
        a11 = _as_bf16(xn_scr[pl.ds(pt, HA // 2), 0:HD])
        a12 = _as_bf16(xn_scr[pl.ds(pt, HA // 2), HD:D])
        a21 = _as_bf16(xn_scr[pl.ds(pb, HA // 2), 0:HD])
        a22 = _as_bf16(xn_scr[pl.ds(pb, HA // 2), HD:D])
        la = [t.astype(BF) for t in _lhs_combos(a11.astype(F32), a12.astype(F32), a21.astype(F32), a22.astype(F32))]
        la[2], la[3] = a11, a22

        def ffn_part(raw, cmb, kq, nq):
            def ld8(q, r, n):
                return raw[c, pl.ds((kq if q >= 2 else 0) + r, 16), pl.ds((nq if q % 2 else 0) + n, 128)]

            def st16(j, r, n, val):
                cmb[c, j, r // 2:r // 2 + 8, n:n + 128] = val

            return [(ld8, st16, (r, n)) for r in range(0, kq, 16) for n in range(0, nq, 128)]

        work = ffn_part(rawg, cg, HD, FC) + ffn_part(rawu, cu, HD, FC) + ffn_part(rawd, cd, FC, HD) + wo_part(c)
        ys = []
        for sec in range(3):
            kl = (2 * sec + 2) % NWC
            cw = [_as_bf16(jnp.concatenate([cq[sec, 0, j], cq[sec, 1, j]], axis=0)) for j in range(5)]
            wl = [cw[0], wqkv[kl, 0:HD, :], cw[1], cw[2], wqkv[kl + 1, HD:D, :], cw[3], cw[4]]
            c11, c12, c21, c22 = _strassen_out([_dot(la[j], wl[j]) for j in range(7)])
            ys.append((jnp.concatenate([c11, c12], axis=1), jnp.concatenate([c21, c22], axis=1)))
        ln_block(jnp.minimum(s + 2, NB - 1), chain=True)
        tok = jnp.zeros((8, 128), F32)
        for ld8, st16, pos in work:
            tok = build_tiles(ld8, st16, [pos], tok, N_EUP)
        for h in range(2):
            rh = pl.multiple_of(r0 + h * HA, 16)
            store_kv(ys[0][h], k_scr, rh)
            store_kv(ys[1][h], v_scr, rh)
            store_q(ys[2][h], rh)

    if NSTEPS < NA + 1 + NB:
        @pl.when(s == NSTEPS - 1)
        def _():
            l = NSTEPS - 1
            for c in (l, l + 1):
                if 0 <= c < NCH:
                    for cp in raw_copies(c):
                        cp.wait()
            for b in (l + 3, l + 4):
                if b < NB:
                    x_copy(b).wait()

    @pl.when(s > NA)
    def _():
        i = lax.rem(s + (NB - NA - 1), NB)
        r0 = pl.multiple_of(i * TM, TM)

        def wlist(raw, cmb, c, kq, nq):
            cw = [_as_bf16(cmb[c, j]) for j in range(5)]
            return [cw[0], raw[c, 0:kq, 0:nq], cw[1], cw[2], raw[c, kq:2 * kq, nq:2 * nq], cw[3], cw[4]]

        RA = 16
        cexp = (DH ** -0.5) * LOG2E
        p0 = pl.multiple_of(r0 // 2, 8)
        never16 = lax.broadcasted_iota(jnp.int32, (16, 128), 0) < jnp.minimum(s, 0)

        def attn_half(q, r):
            sw = []
            for w in range(WIN):
                acc = None
                for g in range(NG):
                    t = q[g] * k_scr[g, pl.ds(r0 + r + HALO - DIL * w, 8), :]
                    acc = t if acc is None else acc + t
                acc = _sum4(acc)
                if r < HALO and w > 0:
                    row = lax.broadcasted_iota(jnp.int32, (8, 128), 0) + (r0 + r)
                    acc = jnp.where(row >= DIL * w, acc, NEG)
                sw.append(acc)
            m = sw[0]
            for w in range(1, WIN):
                m = jnp.maximum(m, sw[w])
            e = [jnp.exp2((sw[w] - m) * cexp) for w in range(WIN)]
            den = e[0]
            for w in range(1, WIN):
                den = den + e[w]
            inv = 1.0 / den
            p = [e[w] * inv for w in range(WIN)]
            o = []
            for g in range(NG):
                acc = None
                for w in range(WIN):
                    t = p[w] * v_scr[g, pl.ds(r0 + r + HALO - DIL * w, 8), :]
                    acc = t if acc is None else acc + t
                o.append(acc)
            return o

        def attn_rows(r, tok):
            qp = [q_scr[g, pl.ds(p0 + r // 2, 8), :] for g in range(NG)]
            if tok is not None:
                qp = [_dep32(t, tok, never) for t in qp]
            q = [_unpack(t) for t in _butterfly(qp)]
            o0 = attn_half([t[0:8] for t in q], r)
            q1 = [t[8:16] for t in q]
            if CHAIN_HALVES:
                q1 = [_dep32(t, o0[NG - 1], never) for t in q1]
            o1 = attn_half(q1, r + 8)
            o = _butterfly([_pack(jnp.concatenate([o0[g], o1[g]], axis=0)) for g in range(NG)])
            for g in range(NG):
                o_scr[r // 2:r // 2 + 8, g * 128:(g + 1) * 128] = o[g]
            tok = o[0]
            if XOR_TOK:
                for g in range(1, NG):
                    tok = tok ^ o[g]
            return tok

        sl = [_as_bf16(s_scr[i, j]) for j in range(7)]
        acc = [None] * 7
        o_parts = []
        n_att = TM // RA
        per = 3
        tok = None
        pend = []
        for c in range(NCH):
            wg_l = wlist(rawg, cg, c, HD, FC)
            wu_l = wlist(rawu, cu, c, HD, FC)
            wd_l = wlist(rawd, cd, c, FC, HD)
            slc = sl
            g = _strassen_out([_dot(slc[j], wg_l[j]) for j in range(7)])
            u = _strassen_out([_dot(slc[j], wu_l[j]) for j in range(7)])
            hq = [g[t] * u[t] for t in range(4)]
            pend.append(([t.astype(BF) for t in _lhs_combos(*hq)], wd_l))
            if len(pend) == DOWN_GROUP or c == NCH - 1:
                for j in range(7):
                    y = _dot(jnp.concatenate([p[0][j] for p in pend], axis=1),
                             jnp.concatenate([p[1][j] for p in pend], axis=0))
                    acc[j] = y if acc[j] is None else acc[j] + y
                pend = []
            for a in range(c * per, min((c + 1) * per, n_att)):
                tok = attn_rows(a * RA, tok)
            if c == WO_AT:
                oq = [_as_bf16(o_scr[rr:rr + HM // 2, cc:cc + HD]) for rr in (0, HM // 2) for cc in (0, HD)]
                ol = [t.astype(BF) for t in _lhs_combos(*[t.astype(F32) for t in oq])]
                ol[2], ol[3] = oq[0], oq[3]
                if WO_GATE:
                    ol = [_gate(t, y[0:8, 0:128], never) for t in ol]
                cw = [_as_bf16(jnp.concatenate([cwo[t, j] for t in range(NWP)], axis=0)) for j in range(5)]
                b11 = jnp.concatenate([wo[0, t, :, 0:HD] for t in range(NWP)], axis=0)
                b22 = jnp.concatenate([wo[1, t, :, HD:D] for t in range(NWP)], axis=0)
                wo_l = [cw[0], b11, cw[1], cw[2], b22, cw[3], cw[4]]
                acc = [acc[j] + _dot(ol[j], wo_l[j]) for j in range(7)]
        ys = _strassen_out(acc)
        x = x_scr[pl.ds(r0, TM), :].astype(F32)
        slot = lax.rem(i, 2)
        for q in range(4):
            rr, cc = (q // 2) * HM, (q % 2) * HD
            (ob0, ob1, ob2, ob3)[q][slot] = (x[rr:rr + HM, cc:cc + HD] + ys[q]).astype(BF)
            out_copy(i, q).start()

        @pl.when(i == NB - 1)
        def _():
            for q in range(4):
                out_copy(i - 1, q).wait()
            for q in range(4):
                out_copy(i, q).wait()


@jax.jit
def pallas_parallel_sum__sliding_local_dilated__glu_gated_bilinear__prompt_kernel(
    A_x: jax.Array,
    A_wqkv: jax.Array,
    A_wo: jax.Array,
    B_x: jax.Array,
    B_w_gate: jax.Array,
    B_w_up: jax.Array,
    B_w_down: jax.Array,
):
    del B_x
    x = A_x.reshape(S, D)
    hbm = pl.BlockSpec(memory_space=pl.ANY)
    out = pl.pallas_call(
        _kernel,
        grid=(NSTEPS,),
        in_specs=[hbm] * 6,
        out_specs=hbm,
        out_shape=jax.ShapeDtypeStruct((S, D), A_x.dtype),
        scratch_shapes=[
            pltpu.VMEM((S, D), BF),
            pltpu.VMEM((NWC, D, WC), BF),
            pltpu.VMEM((2, NWP, HD // NWP, D), BF),
            pltpu.VMEM((NCH, D, 2 * FC), BF),
            pltpu.VMEM((NCH, D, 2 * FC), BF),
            pltpu.VMEM((NCH, 2 * FC, D), BF),
            pltpu.VMEM((3, 2, 5, HD // 4, WC), U32),
            pltpu.VMEM((NWP, 5, HD // NWP // 2, HD), U32),
            pltpu.VMEM((NCH, 5, HD // 2, FC), U32),
            pltpu.VMEM((NCH, 5, HD // 2, FC), U32),
            pltpu.VMEM((NCH, 5, FC // 2, HD), U32),
            pltpu.VMEM((S // 2, D), U32),
            pltpu.VMEM((NB, 7, HM // 2, HD), U32),
            pltpu.VMEM((NG, S // 2, 128), U32),
            pltpu.VMEM((2, NG, S + HALO, 128), F32),
            pltpu.VMEM((TM // 2, D), U32),
            pltpu.VMEM((2, HM, HD), BF),
            pltpu.VMEM((2, HM, HD), BF),
            pltpu.VMEM((2, HM, HD), BF),
            pltpu.VMEM((2, HM, HD), BF),
            pltpu.SemaphoreType.DMA((NB,)),
            pltpu.SemaphoreType.DMA((NWC + 1,)),
            pltpu.SemaphoreType.DMA((NCH, 6)),
            pltpu.SemaphoreType.DMA((2, 4)),
        ],
        compiler_params=pltpu.CompilerParams(
            dimension_semantics=("arbitrary",),
            vmem_limit_bytes=124 * 1024 * 1024,
            disable_bounds_checks=True,
        ),
        name="fused_attn_ffn",
    )(x, A_wqkv, A_wo.reshape(2, NWP, HD // NWP, D), B_w_gate, B_w_up, B_w_down)
    return out.reshape(A_x.shape)
```

```python
import functools

import jax
import jax.numpy as jnp
from jax import lax
from jax.experimental import pallas as pl
from jax.experimental.pallas import tpu as pltpu

S, D, F = 2048, 1024, 3584
H, DH, WIN, DIL = 32, 32, 8, 2
TM = 256
HM = TM // 2
NB = S // TM
HD = D // 2
FC = 256
NCH = F // 2 // FC
HALO = 16
NG = D // 128
EPS = 1e-5
NEG = -1e9
BF = jnp.bfloat16
F32 = jnp.float32
U32 = jnp.uint32
LOG2E = 1.4426950408889634
NA = 7
TA = 224
R0 = S - NA * TA
NSTEPS = 16
NWP = 8
WC = 512
NWC = 3 * D // WC
N_EUP = 3
N_EUP0 = 2
BUILD_XOR = False
R0_BOUNDED = False
WO_AT = 6
WO_GATE = False
DOWN_GROUP = 2
CHAIN_HALVES = True
TOK_MODE = 3


def _dot(a, b):
    return jnp.dot(a, b, preferred_element_type=F32)


def _butterfly(vs):
    lane = lax.broadcasted_iota(jnp.int32, vs[0].shape, 1)
    for b in range(3):
        sh = 4 << b
        bit = (lane & sh) != 0
        new = list(vs)
        for i0 in range(NG):
            if i0 & (1 << b):
                continue
            i1 = i0 | (1 << b)
            new[i0] = jnp.where(bit, pltpu.roll(vs[i1], sh, 1), vs[i0])
            new[i1] = jnp.where(bit, vs[i1], pltpu.roll(vs[i0], 128 - sh, 1))
        vs = new
    return vs


def _sum4(x):
    lane = lax.broadcasted_iota(jnp.int32, x.shape, 1)
    x = x + jnp.where((lane & 1) != 0, pltpu.roll(x, 1, 1), pltpu.roll(x, 127, 1))
    x = x + jnp.where((lane & 2) != 0, pltpu.roll(x, 2, 1), pltpu.roll(x, 126, 1))
    return x


def _dep32(x, tok, never):
    return jnp.where(never, pltpu.bitcast(tok, x.dtype), x)


def _gate(m, tok, never):
    t = pltpu.bitcast(m[0:16, 0:128], F32)
    t = pltpu.bitcast(_dep32(t, tok, never), BF)
    top = jnp.concatenate([t, m[0:16, 128:]], axis=1)
    if m.shape[0] == 16:
        return top
    return jnp.concatenate([top, m[16:]], axis=0)


def _pack(y):
    return pltpu.bitcast(y.astype(BF), U32)


def _as_bf16(w):
    return pltpu.bitcast(w, BF)


def _unpack(w):
    return pltpu.bitcast(w, BF).astype(F32)


def _lhs_combos(a11, a12, a21, a22):
    return [a11 + a22, a21 + a22, a11, a22, a11 + a12, a21 - a11, a12 - a22]


def _strassen_out(m):
    return (m[0] + m[3] - m[4] + m[6], m[2] + m[4], m[1] + m[3], m[0] - m[1] + m[2] + m[5])


def _layernorm(x):
    x = x.astype(F32)
    mean = jnp.mean(x, axis=-1, keepdims=True)
    xc = x - mean
    var = jnp.mean(xc * xc, axis=-1, keepdims=True)
    return xc * lax.rsqrt(var + EPS)


def _kernel(x_hbm, wqkv_hbm, wo_hbm, wg_hbm, wu_hbm, wd_hbm, o_hbm,
            x_scr, wqkv, wo, rawg, rawu, rawd, cq, cwo, cg, cu, cd,
            xn_scr, s_scr, q_scr, kv_scr, o_scr, ob0, ob1, ob2, ob3,
            sem_x, sem_w, sem_raw, sem_o):
    s = pl.program_id(0)
    k_scr = kv_scr.at[0]
    v_scr = kv_scr.at[1]

    def x_copy(b):
        return pltpu.make_async_copy(x_hbm.at[pl.ds(b * TM, TM), :], x_scr.at[pl.ds(b * TM, TM), :], sem_x.at[b])

    def wqkv_copy(k):
        return pltpu.make_async_copy(wqkv_hbm.at[:, pl.ds(k * WC, WC)], wqkv.at[k], sem_w.at[k])

    def wo_copy():
        return pltpu.make_async_copy(wo_hbm, wo, sem_w.at[NWC])

    def raw_copies(c):
        return [
            pltpu.make_async_copy(wg_hbm.at[:, pl.ds(c * FC, FC)], rawg.at[c, :, pl.ds(0, FC)], sem_raw.at[c, 0]),
            pltpu.make_async_copy(wg_hbm.at[:, pl.ds(F // 2 + c * FC, FC)], rawg.at[c, :, pl.ds(FC, FC)], sem_raw.at[c, 1]),
            pltpu.make_async_copy(wu_hbm.at[:, pl.ds(c * FC, FC)], rawu.at[c, :, pl.ds(0, FC)], sem_raw.at[c, 2]),
            pltpu.make_async_copy(wu_hbm.at[:, pl.ds(F // 2 + c * FC, FC)], rawu.at[c, :, pl.ds(FC, FC)], sem_raw.at[c, 3]),
            pltpu.make_async_copy(wd_hbm.at[pl.ds(c * FC, FC), :], rawd.at[c, pl.ds(0, FC), :], sem_raw.at[c, 4]),
            pltpu.make_async_copy(wd_hbm.at[pl.ds(F // 2 + c * FC, FC), :], rawd.at[c, pl.ds(FC, FC), :], sem_raw.at[c, 5]),
        ]

    def out_copy(i, q):
        slot = lax.rem(i, 2)
        rr, cc = (q // 2) * HM, (q % 2) * HD
        return pltpu.make_async_copy((ob0, ob1, ob2, ob3)[q].at[slot],
                                     o_hbm.at[pl.ds(i * TM + rr, HM), pl.ds(cc, HD)], sem_o.at[slot, q])

    never = lax.broadcasted_iota(jnp.int32, (8, 128), 0) < jnp.minimum(s, 0)

    def ln_unit(b, r, tok):
        RC = 16
        r0 = pl.multiple_of(b * TM + r, RC)
        xt = x_scr[pl.ds(r0, RC), :]
        xb = x_scr[pl.ds(r0 + HM, RC), :]
        if tok is not None:
            xt = _gate(xt, tok, never)
            xb = _gate(xb, tok, never)
        top = _layernorm(xt)
        bot = _layernorm(xb)
        p0 = pl.multiple_of(r0 // 2, RC // 2)
        xn_scr[pl.ds(p0, RC // 2), :] = _pack(top)
        xn_scr[pl.ds(p0 + HM // 2, RC // 2), :] = _pack(bot)
        cs = _lhs_combos(top[:, :HD], top[:, HD:], bot[:, :HD], bot[:, HD:])
        pr = r // 2 if isinstance(r, int) else pl.multiple_of(r // 2, RC // 2)
        for j in range(7):
            s_scr[b, j, pl.ds(pr, RC // 2), :] = _pack(cs[j])
        return top[0:8, 0:128] + bot[0:8, 0:128]

    def ln_block(b, chain=False):
        tok = None
        for r in range(0, HM, 16):
            t = ln_unit(b, r, tok)
            tok = t if chain else None
        return tok

    def store_kv(y, dst, r0):
        for r in range(0, y.shape[0], 16):
            vs = _butterfly([_pack(y[r:r + 16, g * 128:(g + 1) * 128]) for g in range(NG)])
            for g in range(NG):
                dst[g, pl.ds(r0 + HALO + r, 16), :] = _unpack(vs[g])

    def store_q(y, r0):
        p0 = pl.multiple_of(r0 // 2, 8)
        for g in range(NG):
            q_scr[g, pl.ds(p0, y.shape[0] // 2), :] = _pack(y[:, g * 128:(g + 1) * 128])

    def build_tiles(ld16, st16, positions, tok, n_eup):
        for r, n0 in positions:
            for _ in range(n_eup or 0):
                tok = jnp.exp2(tok)

            def ld(q):
                w = pltpu.bitcast(ld16(q, r, n0), U32)
                if n_eup is not None:
                    w = _dep32(w, tok, never)
                return (pltpu.bitcast(w << 16, F32), pltpu.bitcast(w & jnp.uint32(0xFFFF0000), F32))

            b11, b12, b21, b22 = [ld(q) for q in range(4)]

            def comb(x, y, sign):
                ev, od = (x[0] + y[0], x[1] + y[1]) if sign > 0 else (x[0] - y[0], x[1] - y[1])
                return pltpu.bitcast(pltpu.pack_elementwise([ev, od], packed_dtype=BF), U32)

            outs = [comb(b11, b22, 1), comb(b12, b22, -1), comb(b21, b11, -1), comb(b11, b12, 1), comb(b21, b22, 1)]
            for j in range(5):
                st16(j, r, n0, outs[j])
            t = outs[0]
            if BUILD_XOR:
                t = (t ^ outs[1]) ^ (outs[2] ^ outs[3]) ^ outs[4]
            tok = pltpu.bitcast(t, F32)
        return tok

    def build_qkv(sec, kl, kr, bh, n_eup):
        rb = bh * (HD // 2)

        def row(r, m):
            return rb + r if isinstance(rb, int) else pl.multiple_of(rb + r, m)

        def ld8(q, r, n):
            return wqkv[kl if q in (0, 2) else kr, pl.ds(row((HD if q >= 2 else 0) + r, 16), 16), n:n + 128]

        def st16(j, r, n, val):
            cq[sec, bh, j, r // 2:r // 2 + 8, n:n + 128] = val

        build_tiles(ld8, st16, [(r, n) for r in range(0, HD // 2, 16) for n in range(0, WC, 128)],
                    jnp.zeros((8, 128), F32), n_eup)

    def wo_part(t):
        def ld16(q, r, n):
            return wo[q // 2, t, r:r + 16, pl.ds((HD if q % 2 else 0) + n, 128)]

        def st16(j, r, n, val):
            cwo[t, j, r // 2:r // 2 + 8, n:n + 128] = val

        return [(ld16, st16, (r, n)) for r in range(0, HD // NWP, 16) for n in range(0, HD, 128)]

    @pl.when(s == 0)
    def _():
        def issue_x(b, carry):
            x_copy(b).start(priority=1)
            return carry

        lax.fori_loop(0, 2, issue_x, 0)

        def issue_w(j, carry):
            @pl.when(j == 1)
            def _():
                x_copy(2).start(priority=1)

            wqkv_copy(lax.rem(j + 2, NWC)).start(priority=1)
            return carry

        lax.fori_loop(0, NWC, issue_w, 0)

        def issue_rest(j, carry):
            for cp in raw_copies(0):
                cp.start(priority=1)
            return carry

        lax.fori_loop(0, jnp.maximum(s, 1), issue_rest, 0)
        wo_copy().start(priority=1)
        x_copy(3).start(priority=1)
        k_scr[:, 0:HALO, :] = jnp.zeros((NG, HALO, 128), F32)
        v_scr[:, 0:HALO, :] = jnp.zeros((NG, HALO, 128), F32)
        x_copy(0).wait()
        ln_block(0)
        x_copy(1).wait()
        ln_block(1)
        P0 = R0 // 2
        xn = _as_bf16(xn_scr[0:P0, :])

        def body(j, carry):
            k = lax.rem(j + 2, NWC)
            wqkv_copy(k).wait()

            @pl.when(j == 1)
            def _():
                x_copy(2).wait()

            y = _dot(xn, wqkv[k])
            half = lax.rem(j, 2)
            sec = jnp.maximum(lax.div(j, 2) - 1, 0)
            src = pl.multiple_of((sec + 1) * P0 + half * (P0 // 2), 8)
            dstr = pl.multiple_of(HALO + half * P0, 16)
            for r in range(0, P0 // 2, 8):
                vs = _butterfly([q_scr[g, pl.ds(src + r, 8), :] for g in range(NG)])
                for g in range(NG):
                    kv_scr[sec, g, pl.ds(dstr + 2 * r, 16), :] = _unpack(vs[g])
            lb = jnp.minimum(j + 1, 2)
            u0 = 2 * jnp.clip(j - 1, 0, 3)
            tok = ln_unit(lb, pl.multiple_of(u0 * 16, 16), None)
            ln_unit(lb, pl.multiple_of(u0 * 16 + 16, 16), tok)
            jm = jnp.maximum(j - 1, 0)
            bsec = lax.div(jm, 2)
            kl = lax.rem(2 * bsec + 2, NWC)
            kr = jnp.where(j == 0, kl, kl + 1)
            bh = jnp.where(j == 0, 1, lax.rem(jm, 2))
            build_qkv(bsec, kl, kr, bh, N_EUP0)
            rb = pl.multiple_of(lax.rem(lax.div(j, 2) + 1, 3) * P0, 8)
            for gg in range(WC // 128):
                q_scr[half * (WC // 128) + gg, pl.ds(rb, P0), :] = _pack(y[:, gg * 128:(gg + 1) * 128])
            return carry

        lax.fori_loop(0, NWC, body, 0)
        build_qkv(2, 0, 1, 1, None)
        wo_copy().wait()
        for ld16, st16, pos in wo_part(NWP - 1):
            build_tiles(ld16, st16, [pos], jnp.zeros((8, 128), F32), None)

    @pl.when(s <= NA)
    def _():
        @pl.when(s + 1 < NCH)
        def _():
            for cp in raw_copies(s + 1):
                cp.start(priority=1)

        @pl.when(s + 4 < NB)
        def _():
            x_copy(s + 4).start(priority=1)

        @pl.when(s >= 1)
        def _():
            for cp in raw_copies(s - 1):
                cp.wait()

        @pl.when(jnp.logical_and(s >= 1, s + 2 < NB))
        def _():
            x_copy(s + 2).wait()

    @pl.when(s >= NA + 3)
    def _():
        for q in range(4):
            out_copy(s - (NA + 3), q).wait()

    @pl.when(jnp.logical_and(s >= 1, s <= NA))
    def _():
        c = lax.rem(s + (NA - 1), NA)
        r0 = pl.multiple_of(R0 + (c if R0_BOUNDED else s - 1) * TA, 16)
        HA = TA // 2
        pt = pl.multiple_of(r0 // 2, 8)
        pb = pl.multiple_of((r0 + HA) // 2, 8)
        a11 = _as_bf16(xn_scr[pl.ds(pt, HA // 2), 0:HD])
        a12 = _as_bf16(xn_scr[pl.ds(pt, HA // 2), HD:D])
        a21 = _as_bf16(xn_scr[pl.ds(pb, HA // 2), 0:HD])
        a22 = _as_bf16(xn_scr[pl.ds(pb, HA // 2), HD:D])
        la = [t.astype(BF) for t in _lhs_combos(a11.astype(F32), a12.astype(F32), a21.astype(F32), a22.astype(F32))]
        la[2], la[3] = a11, a22

        def ffn_part(raw, cmb, kq, nq):
            def ld8(q, r, n):
                return raw[c, pl.ds((kq if q >= 2 else 0) + r, 16), pl.ds((nq if q % 2 else 0) + n, 128)]

            def st16(j, r, n, val):
                cmb[c, j, r // 2:r // 2 + 8, n:n + 128] = val

            return [(ld8, st16, (r, n)) for r in range(0, kq, 16) for n in range(0, nq, 128)]

        work = ffn_part(rawg, cg, HD, FC) + ffn_part(rawu, cu, HD, FC) + ffn_part(rawd, cd, FC, HD) + wo_part(c)
        ys = []
        for sec in range(3):
            kl = (2 * sec + 2) % NWC
            cw = [_as_bf16(jnp.concatenate([cq[sec, 0, j], cq[sec, 1, j]], axis=0)) for j in range(5)]
            wl = [cw[0], wqkv[kl, 0:HD, :], cw[1], cw[2], wqkv[kl + 1, HD:D, :], cw[3], cw[4]]
            c11, c12, c21, c22 = _strassen_out([_dot(la[j], wl[j]) for j in range(7)])
            ys.append((jnp.concatenate([c11, c12], axis=1), jnp.concatenate([c21, c22], axis=1)))
        ln_block(jnp.minimum(s + 2, NB - 1), chain=True)
        tok = jnp.zeros((8, 128), F32)
        for ld8, st16, pos in work:
            tok = build_tiles(ld8, st16, [pos], tok, N_EUP)
        for h in range(2):
            rh = pl.multiple_of(r0 + h * HA, 16)
            store_kv(ys[0][h], k_scr, rh)
            store_kv(ys[1][h], v_scr, rh)
            store_q(ys[2][h], rh)

    if NSTEPS < NA + 1 + NB:
        @pl.when(s == NSTEPS - 1)
        def _():
            l = NSTEPS - 1
            for c in (l, l + 1):
                if 0 <= c < NCH:
                    for cp in raw_copies(c):
                        cp.wait()
            for b in (l + 3, l + 4):
                if b < NB:
                    x_copy(b).wait()

    @pl.when(s > NA)
    def _():
        i = lax.rem(s + (NB - NA - 1), NB)
        r0 = pl.multiple_of(i * TM, TM)

        def wlist(raw, cmb, c, kq, nq):
            cw = [_as_bf16(cmb[c, j]) for j in range(5)]
            return [cw[0], raw[c, 0:kq, 0:nq], cw[1], cw[2], raw[c, kq:2 * kq, nq:2 * nq], cw[3], cw[4]]

        RA = 16
        cexp = (DH ** -0.5) * LOG2E
        p0 = pl.multiple_of(r0 // 2, 8)
        never16 = lax.broadcasted_iota(jnp.int32, (16, 128), 0) < jnp.minimum(s, 0)

        def attn_half(q, r):
            sw = []
            for w in range(WIN):
                acc = None
                for g in range(NG):
                    t = q[g] * k_scr[g, pl.ds(r0 + r + HALO - DIL * w, 8), :]
                    acc = t if acc is None else acc + t
                acc = _sum4(acc)
                if r < HALO and w > 0:
                    row = lax.broadcasted_iota(jnp.int32, (8, 128), 0) + (r0 + r)
                    acc = jnp.where(row >= DIL * w, acc, NEG)
                sw.append(acc)
            m = sw[0]
            for w in range(1, WIN):
                m = jnp.maximum(m, sw[w])
            e = [jnp.exp2((sw[w] - m) * cexp) for w in range(WIN)]
            den = e[0]
            for w in range(1, WIN):
                den = den + e[w]
            inv = 1.0 / den
            p = [e[w] * inv for w in range(WIN)]
            o = []
            for g in range(NG):
                acc = None
                for w in range(WIN):
                    t = p[w] * v_scr[g, pl.ds(r0 + r + HALO - DIL * w, 8), :]
                    acc = t if acc is None else acc + t
                o.append(acc)
            return o

        prev_fin = [None]

        def attn_rows(r, tok):
            qp = [q_scr[g, pl.ds(p0 + r // 2, 8), :] for g in range(NG)]
            if tok is not None:
                qp = [_dep32(t, tok, never) for t in qp]
            q = [_unpack(t) for t in _butterfly(qp)]
            o0 = attn_half([t[0:8] for t in q], r)
            q1 = [t[8:16] for t in q]
            if CHAIN_HALVES:
                q1 = [_dep32(t, o0[NG - 1], never) for t in q1]
            o1 = attn_half(q1, r + 8)
            o = _butterfly([_pack(jnp.concatenate([o0[g], o1[g]], axis=0)) for g in range(NG)])
            for g in range(NG):
                o_scr[r // 2:r // 2 + 8, g * 128:(g + 1) * 128] = o[g]
            if TOK_MODE == 0:
                return o[0]
            fin = o[0]
            for g in range(1, NG):
                fin = fin ^ o[g]
            if TOK_MODE == 1:
                return fin
            tok = pltpu.bitcast(o1[NG - 1], U32) if TOK_MODE == 2 else o[0]
            if prev_fin[0] is not None:
                tok = tok ^ prev_fin[0]
            prev_fin[0] = fin
            return tok

        sl = [_as_bf16(s_scr[i, j]) for j in range(7)]
        acc = [None] * 7
        o_parts = []
        n_att = TM // RA
        per = 3
        tok = None
        pend = []
        for c in range(NCH):
            wg_l = wlist(rawg, cg, c, HD, FC)
            wu_l = wlist(rawu, cu, c, HD, FC)
            wd_l = wlist(rawd, cd, c, FC, HD)
            slc = sl
            g = _strassen_out([_dot(slc[j], wg_l[j]) for j in range(7)])
            u = _strassen_out([_dot(slc[j], wu_l[j]) for j in range(7)])
            hq = [g[t] * u[t] for t in range(4)]
            pend.append(([t.astype(BF) for t in _lhs_combos(*hq)], wd_l))
            if len(pend) == DOWN_GROUP or c == NCH - 1:
                for j in range(7):
                    y = _dot(jnp.concatenate([p[0][j] for p in pend], axis=1),
                             jnp.concatenate([p[1][j] for p in pend], axis=0))
                    acc[j] = y if acc[j] is None else acc[j] + y
                pend = []
            for a in range(c * per, min((c + 1) * per, n_att)):
                tok = attn_rows(a * RA, tok)
            if c == WO_AT:
                oq = [_as_bf16(o_scr[rr:rr + HM // 2, cc:cc + HD]) for rr in (0, HM // 2) for cc in (0, HD)]
                ol = [t.astype(BF) for t in _lhs_combos(*[t.astype(F32) for t in oq])]
                ol[2], ol[3] = oq[0], oq[3]
                if WO_GATE:
                    ol = [_gate(t, y[0:8, 0:128], never) for t in ol]
                cw = [_as_bf16(jnp.concatenate([cwo[t, j] for t in range(NWP)], axis=0)) for j in range(5)]
                b11 = jnp.concatenate([wo[0, t, :, 0:HD] for t in range(NWP)], axis=0)
                b22 = jnp.concatenate([wo[1, t, :, HD:D] for t in range(NWP)], axis=0)
                wo_l = [cw[0], b11, cw[1], cw[2], b22, cw[3], cw[4]]
                acc = [acc[j] + _dot(ol[j], wo_l[j]) for j in range(7)]
        ys = _strassen_out(acc)
        x = x_scr[pl.ds(r0, TM), :].astype(F32)
        slot = lax.rem(i, 2)
        for q in range(4):
            rr, cc = (q // 2) * HM, (q % 2) * HD
            (ob0, ob1, ob2, ob3)[q][slot] = (x[rr:rr + HM, cc:cc + HD] + ys[q]).astype(BF)
            out_copy(i, q).start()

        @pl.when(i == NB - 1)
        def _():
            for q in range(4):
                out_copy(i - 1, q).wait()
            for q in range(4):
                out_copy(i, q).wait()


@jax.jit
def pallas_parallel_sum__sliding_local_dilated__glu_gated_bilinear__prompt_kernel(
    A_x: jax.Array,
    A_wqkv: jax.Array,
    A_wo: jax.Array,
    B_x: jax.Array,
    B_w_gate: jax.Array,
    B_w_up: jax.Array,
    B_w_down: jax.Array,
):
    del B_x
    x = A_x.reshape(S, D)
    hbm = pl.BlockSpec(memory_space=pl.ANY)
    out = pl.pallas_call(
        _kernel,
        grid=(NSTEPS,),
        in_specs=[hbm] * 6,
        out_specs=hbm,
        out_shape=jax.ShapeDtypeStruct((S, D), A_x.dtype),
        scratch_shapes=[
            pltpu.VMEM((S, D), BF),
            pltpu.VMEM((NWC, D, WC), BF),
            pltpu.VMEM((2, NWP, HD // NWP, D), BF),
            pltpu.VMEM((NCH, D, 2 * FC), BF),
            pltpu.VMEM((NCH, D, 2 * FC), BF),
            pltpu.VMEM((NCH, 2 * FC, D), BF),
            pltpu.VMEM((3, 2, 5, HD // 4, WC), U32),
            pltpu.VMEM((NWP, 5, HD // NWP // 2, HD), U32),
            pltpu.VMEM((NCH, 5, HD // 2, FC), U32),
            pltpu.VMEM((NCH, 5, HD // 2, FC), U32),
            pltpu.VMEM((NCH, 5, FC // 2, HD), U32),
            pltpu.VMEM((S // 2, D), U32),
            pltpu.VMEM((NB, 7, HM // 2, HD), U32),
            pltpu.VMEM((NG, S // 2, 128), U32),
            pltpu.VMEM((2, NG, S + HALO, 128), F32),
            pltpu.VMEM((TM // 2, D), U32),
            pltpu.VMEM((2, HM, HD), BF),
            pltpu.VMEM((2, HM, HD), BF),
            pltpu.VMEM((2, HM, HD), BF),
            pltpu.VMEM((2, HM, HD), BF),
            pltpu.SemaphoreType.DMA((NB,)),
            pltpu.SemaphoreType.DMA((NWC + 1,)),
            pltpu.SemaphoreType.DMA((NCH, 6)),
            pltpu.SemaphoreType.DMA((2, 4)),
        ],
        compiler_params=pltpu.CompilerParams(
            dimension_semantics=("arbitrary",),
            vmem_limit_bytes=124 * 1024 * 1024,
            disable_bounds_checks=True,
        ),
        name="fused_attn_ffn",
    )(x, A_wqkv, A_wo.reshape(2, NWP, HD // NWP, D), B_w_gate, B_w_up, B_w_down)
    return out.reshape(A_x.shape)
```

```python
import jax
import jax.numpy as jnp
from jax import lax
from jax.experimental import pallas as pl
from jax.experimental.pallas import tpu as pltpu

S, D, F = 2048, 1024, 3584
DH, WIN, DIL = 32, 8, 2
TM = 256
HM = TM // 2
NB = S // TM
HD = D // 2
FC = 256
NCH = F // 2 // FC
HALO = 16
NG = D // 128
EPS = 1e-5
NEG = -1e9
BF = jnp.bfloat16
F32 = jnp.float32
U32 = jnp.uint32
LOG2E = 1.4426950408889634
NA = 7
TA = 224
R0 = S - NA * TA
NSTEPS = 1 + NA + NB
NWP = 8
WC = 512
NWC = 3 * D // WC
N_EUP = 3
N_EUP0 = 2
DOWN_GROUP = 2

def _dot(a, b):
    return jnp.dot(a, b, preferred_element_type=F32)


def _butterfly(vs):
    lane = lax.broadcasted_iota(jnp.int32, vs[0].shape, 1)
    for b in range(3):
        sh = 4 << b
        bit = (lane & sh) != 0
        new = list(vs)
        for i0 in range(NG):
            if i0 & (1 << b):
                continue
            i1 = i0 | (1 << b)
            new[i0] = jnp.where(bit, pltpu.roll(vs[i1], sh, 1), vs[i0])
            new[i1] = jnp.where(bit, vs[i1], pltpu.roll(vs[i0], 128 - sh, 1))
        vs = new
    return vs


def _sum4(x):
    lane = lax.broadcasted_iota(jnp.int32, x.shape, 1)
    x = x + jnp.where((lane & 1) != 0, pltpu.roll(x, 1, 1), pltpu.roll(x, 127, 1))
    x = x + jnp.where((lane & 2) != 0, pltpu.roll(x, 2, 1), pltpu.roll(x, 126, 1))
    return x


def _dep32(x, tok, never):
    return jnp.where(never, pltpu.bitcast(tok, x.dtype), x)


def _gate(m, tok, never):
    t = pltpu.bitcast(m[0:16, 0:128], F32)
    t = pltpu.bitcast(_dep32(t, tok, never), BF)
    top = jnp.concatenate([t, m[0:16, 128:]], axis=1)
    if m.shape[0] == 16:
        return top
    return jnp.concatenate([top, m[16:]], axis=0)


def _pack(y):
    return pltpu.bitcast(y.astype(BF), U32)


def _as_bf16(w):
    return pltpu.bitcast(w, BF)


def _unpack(w):
    return pltpu.bitcast(w, BF).astype(F32)


def _lhs_combos(a11, a12, a21, a22):
    return [a11 + a22, a21 + a22, a11, a22, a11 + a12, a21 - a11, a12 - a22]


def _strassen_out(m):
    return (m[0] + m[3] - m[4] + m[6], m[2] + m[4], m[1] + m[3], m[0] - m[1] + m[2] + m[5])


def _layernorm(x):
    x = x.astype(F32)
    mean = jnp.mean(x, axis=-1, keepdims=True)
    xc = x - mean
    var = jnp.mean(xc * xc, axis=-1, keepdims=True)
    return xc * lax.rsqrt(var + EPS)


def _kernel(x_hbm, wqkv_hbm, wo_hbm, wg_hbm, wu_hbm, wd_hbm, o_hbm,
            x_scr, wqkv, wo, rawg, rawu, rawd, cq, cwo, cg, cu, cd,
            xn_scr, s_scr, q_scr, kv_scr, o_scr, ob0, ob1, ob2, ob3,
            sem_x, sem_w, sem_raw, sem_o):
    s = pl.program_id(0)
    k_scr = kv_scr.at[0]
    v_scr = kv_scr.at[1]

    def x_copy(b):
        return pltpu.make_async_copy(x_hbm.at[pl.ds(b * TM, TM), :], x_scr.at[pl.ds(b * TM, TM), :], sem_x.at[b])

    def wqkv_copy(k):
        return pltpu.make_async_copy(wqkv_hbm.at[:, pl.ds(k * WC, WC)], wqkv.at[k], sem_w.at[k])

    def wo_copy():
        return pltpu.make_async_copy(wo_hbm, wo, sem_w.at[NWC])

    def raw_copies(c):
        return [
            pltpu.make_async_copy(wg_hbm.at[:, pl.ds(c * FC, FC)], rawg.at[c, :, pl.ds(0, FC)], sem_raw.at[c, 0]),
            pltpu.make_async_copy(wg_hbm.at[:, pl.ds(F // 2 + c * FC, FC)], rawg.at[c, :, pl.ds(FC, FC)], sem_raw.at[c, 1]),
            pltpu.make_async_copy(wu_hbm.at[:, pl.ds(c * FC, FC)], rawu.at[c, :, pl.ds(0, FC)], sem_raw.at[c, 2]),
            pltpu.make_async_copy(wu_hbm.at[:, pl.ds(F // 2 + c * FC, FC)], rawu.at[c, :, pl.ds(FC, FC)], sem_raw.at[c, 3]),
            pltpu.make_async_copy(wd_hbm.at[pl.ds(c * FC, FC), :], rawd.at[c, pl.ds(0, FC), :], sem_raw.at[c, 4]),
            pltpu.make_async_copy(wd_hbm.at[pl.ds(F // 2 + c * FC, FC), :], rawd.at[c, pl.ds(FC, FC), :], sem_raw.at[c, 5]),
        ]

    def out_copy(i, q):
        slot = lax.rem(i, 2)
        rr, cc = (q // 2) * HM, (q % 2) * HD
        return pltpu.make_async_copy((ob0, ob1, ob2, ob3)[q].at[slot],
                                     o_hbm.at[pl.ds(i * TM + rr, HM), pl.ds(cc, HD)], sem_o.at[slot, q])

    never = lax.broadcasted_iota(jnp.int32, (8, 128), 0) < jnp.minimum(s, 0)

    def ln_unit(b, r, tok):
        RC = 16
        r0 = pl.multiple_of(b * TM + r, RC)
        xt = x_scr[pl.ds(r0, RC), :]
        xb = x_scr[pl.ds(r0 + HM, RC), :]
        if tok is not None:
            xt = _gate(xt, tok, never)
            xb = _gate(xb, tok, never)
        top = _layernorm(xt)
        bot = _layernorm(xb)
        p0 = pl.multiple_of(r0 // 2, RC // 2)
        xn_scr[pl.ds(p0, RC // 2), :] = _pack(top)
        xn_scr[pl.ds(p0 + HM // 2, RC // 2), :] = _pack(bot)
        cs = _lhs_combos(top[:, :HD], top[:, HD:], bot[:, :HD], bot[:, HD:])
        pr = r // 2 if isinstance(r, int) else pl.multiple_of(r // 2, RC // 2)
        for j in range(7):
            s_scr[b, j, pl.ds(pr, RC // 2), :] = _pack(cs[j])
        return top[0:8, 0:128] + bot[0:8, 0:128]

    def ln_block(b, chain=False):
        tok = None
        for r in range(0, HM, 16):
            t = ln_unit(b, r, tok)
            tok = t if chain else None
        return tok

    def store_kv(y, dst, r0):
        for r in range(0, y.shape[0], 16):
            vs = _butterfly([_pack(y[r:r + 16, g * 128:(g + 1) * 128]) for g in range(NG)])
            for g in range(NG):
                dst[g, pl.ds(r0 + HALO + r, 16), :] = _unpack(vs[g])

    def store_q(y, r0):
        p0 = pl.multiple_of(r0 // 2, 8)
        for g in range(NG):
            q_scr[g, pl.ds(p0, y.shape[0] // 2), :] = _pack(y[:, g * 128:(g + 1) * 128])

    def build_tiles(ld16, st16, positions, tok, n_eup):
        for r, n0 in positions:
            for _ in range(n_eup or 0):
                tok = jnp.exp2(tok)

            def ld(q):
                w = pltpu.bitcast(ld16(q, r, n0), U32)
                if n_eup is not None:
                    w = _dep32(w, tok, never)
                return (pltpu.bitcast(w << 16, F32), pltpu.bitcast(w & jnp.uint32(0xFFFF0000), F32))

            b11, b12, b21, b22 = [ld(q) for q in range(4)]

            def comb(x, y, sign):
                ev, od = (x[0] + y[0], x[1] + y[1]) if sign > 0 else (x[0] - y[0], x[1] - y[1])
                return pltpu.bitcast(pltpu.pack_elementwise([ev, od], packed_dtype=BF), U32)

            outs = [comb(b11, b22, 1), comb(b12, b22, -1), comb(b21, b11, -1), comb(b11, b12, 1), comb(b21, b22, 1)]
            for j in range(5):
                st16(j, r, n0, outs[j])
            tok = pltpu.bitcast(outs[0], F32)
        return tok

    def build_qkv(sec, kl, kr, bh, n_eup):
        rb = bh * (HD // 2)

        def row(r, m):
            return rb + r if isinstance(rb, int) else pl.multiple_of(rb + r, m)

        def ld8(q, r, n):
            return wqkv[kl if q in (0, 2) else kr, pl.ds(row((HD if q >= 2 else 0) + r, 16), 16), n:n + 128]

        def st16(j, r, n, val):
            cq[sec, bh, j, r // 2:r // 2 + 8, n:n + 128] = val

        build_tiles(ld8, st16, [(r, n) for r in range(0, HD // 2, 16) for n in range(0, WC, 128)],
                    jnp.zeros((8, 128), F32), n_eup)

    def wo_part(t):
        def ld16(q, r, n):
            return wo[q // 2, t, r:r + 16, pl.ds((HD if q % 2 else 0) + n, 128)]

        def st16(j, r, n, val):
            cwo[t, j, r // 2:r // 2 + 8, n:n + 128] = val

        return [(ld16, st16, (r, n)) for r in range(0, HD // NWP, 16) for n in range(0, HD, 128)]

    @pl.when(s == 0)
    def _():
        def issue_x(b, carry):
            x_copy(b).start(priority=1)
            return carry

        lax.fori_loop(0, 2, issue_x, 0)

        def issue_w(j, carry):
            @pl.when(j == 1)
            def _():
                x_copy(2).start(priority=1)

            wqkv_copy(lax.rem(j + 2, NWC)).start(priority=1)
            return carry

        lax.fori_loop(0, NWC, issue_w, 0)

        def issue_rest(j, carry):
            for cp in raw_copies(0):
                cp.start(priority=1)
            return carry

        lax.fori_loop(0, jnp.maximum(s, 1), issue_rest, 0)
        wo_copy().start(priority=1)
        x_copy(3).start(priority=1)
        k_scr[:, 0:HALO, :] = jnp.zeros((NG, HALO, 128), F32)
        v_scr[:, 0:HALO, :] = jnp.zeros((NG, HALO, 128), F32)
        x_copy(0).wait()
        ln_block(0)
        x_copy(1).wait()
        ln_block(1)
        P0 = R0 // 2
        xn = _as_bf16(xn_scr[0:P0, :])

        def body(j, carry):
            k = lax.rem(j + 2, NWC)
            wqkv_copy(k).wait()

            @pl.when(j == 1)
            def _():
                x_copy(2).wait()

            y = _dot(xn, wqkv[k])
            half = lax.rem(j, 2)
            sec = jnp.maximum(lax.div(j, 2) - 1, 0)
            src = pl.multiple_of((sec + 1) * P0 + half * (P0 // 2), 8)
            dstr = pl.multiple_of(HALO + half * P0, 16)
            for r in range(0, P0 // 2, 8):
                vs = _butterfly([q_scr[g, pl.ds(src + r, 8), :] for g in range(NG)])
                for g in range(NG):
                    kv_scr[sec, g, pl.ds(dstr + 2 * r, 16), :] = _unpack(vs[g])
            lb = jnp.minimum(j + 1, 2)
            u0 = 2 * jnp.clip(j - 1, 0, 3)
            tok = ln_unit(lb, pl.multiple_of(u0 * 16, 16), None)
            ln_unit(lb, pl.multiple_of(u0 * 16 + 16, 16), tok)
            jm = jnp.maximum(j - 1, 0)
            bsec = lax.div(jm, 2)
            kl = lax.rem(2 * bsec + 2, NWC)
            kr = jnp.where(j == 0, kl, kl + 1)
            bh = jnp.where(j == 0, 1, lax.rem(jm, 2))
            build_qkv(bsec, kl, kr, bh, N_EUP0)
            rb = pl.multiple_of(lax.rem(lax.div(j, 2) + 1, 3) * P0, 8)
            for gg in range(WC // 128):
                q_scr[half * (WC // 128) + gg, pl.ds(rb, P0), :] = _pack(y[:, gg * 128:(gg + 1) * 128])
            return carry

        lax.fori_loop(0, NWC, body, 0)
        build_qkv(2, 0, 1, 1, None)
        wo_copy().wait()
        for ld16, st16, pos in wo_part(NWP - 1):
            build_tiles(ld16, st16, [pos], jnp.zeros((8, 128), F32), None)

    @pl.when(s <= NA)
    def _():
        @pl.when(s + 1 < NCH)
        def _():
            for cp in raw_copies(s + 1):
                cp.start(priority=1)

        @pl.when(s + 4 < NB)
        def _():
            x_copy(s + 4).start(priority=1)

        @pl.when(s >= 1)
        def _():
            for cp in raw_copies(s - 1):
                cp.wait()

        @pl.when(jnp.logical_and(s >= 1, s + 2 < NB))
        def _():
            x_copy(s + 2).wait()

    @pl.when(s >= NA + 3)
    def _():
        for q in range(4):
            out_copy(s - (NA + 3), q).wait()

    @pl.when(jnp.logical_and(s >= 1, s <= NA))
    def _():
        c = lax.rem(s + (NA - 1), NA)
        r0 = pl.multiple_of(R0 + (s - 1) * TA, 16)
        HA = TA // 2
        pt = pl.multiple_of(r0 // 2, 8)
        pb = pl.multiple_of((r0 + HA) // 2, 8)
        a11 = _as_bf16(xn_scr[pl.ds(pt, HA // 2), 0:HD])
        a12 = _as_bf16(xn_scr[pl.ds(pt, HA // 2), HD:D])
        a21 = _as_bf16(xn_scr[pl.ds(pb, HA // 2), 0:HD])
        a22 = _as_bf16(xn_scr[pl.ds(pb, HA // 2), HD:D])
        la = [t.astype(BF) for t in _lhs_combos(a11.astype(F32), a12.astype(F32), a21.astype(F32), a22.astype(F32))]
        la[2], la[3] = a11, a22

        def ffn_part(raw, cmb, kq, nq):
            def ld8(q, r, n):
                return raw[c, pl.ds((kq if q >= 2 else 0) + r, 16), pl.ds((nq if q % 2 else 0) + n, 128)]

            def st16(j, r, n, val):
                cmb[c, j, r // 2:r // 2 + 8, n:n + 128] = val

            return [(ld8, st16, (r, n)) for r in range(0, kq, 16) for n in range(0, nq, 128)]

        work = ffn_part(rawg, cg, HD, FC) + ffn_part(rawu, cu, HD, FC) + ffn_part(rawd, cd, FC, HD) + wo_part(c)
        ys = []
        for sec in range(3):
            kl = (2 * sec + 2) % NWC
            cw = [_as_bf16(jnp.concatenate([cq[sec, 0, j], cq[sec, 1, j]], axis=0)) for j in range(5)]
            wl = [cw[0], wqkv[kl, 0:HD, :], cw[1], cw[2], wqkv[kl + 1, HD:D, :], cw[3], cw[4]]
            c11, c12, c21, c22 = _strassen_out([_dot(la[j], wl[j]) for j in range(7)])
            ys.append((jnp.concatenate([c11, c12], axis=1), jnp.concatenate([c21, c22], axis=1)))
        ln_block(jnp.minimum(s + 2, NB - 1), chain=True)
        tok = jnp.zeros((8, 128), F32)
        for ld8, st16, pos in work:
            tok = build_tiles(ld8, st16, [pos], tok, N_EUP)
        for h in range(2):
            rh = pl.multiple_of(r0 + h * HA, 16)
            store_kv(ys[0][h], k_scr, rh)
            store_kv(ys[1][h], v_scr, rh)
            store_q(ys[2][h], rh)

    @pl.when(s > NA)
    def _():
        i = lax.rem(s + (NB - NA - 1), NB)
        r0 = pl.multiple_of(i * TM, TM)

        def wlist(raw, cmb, c, kq, nq):
            cw = [_as_bf16(cmb[c, j]) for j in range(5)]
            return [cw[0], raw[c, 0:kq, 0:nq], cw[1], cw[2], raw[c, kq:2 * kq, nq:2 * nq], cw[3], cw[4]]

        RA = 16
        cexp = (DH ** -0.5) * LOG2E
        p0 = pl.multiple_of(r0 // 2, 8)

        def attn_half(q, r):
            sw = []
            for w in range(WIN):
                acc = None
                for g in range(NG):
                    t = q[g] * k_scr[g, pl.ds(r0 + r + HALO - DIL * w, 8), :]
                    acc = t if acc is None else acc + t
                acc = _sum4(acc)
                if r < HALO and w > 0:
                    row = lax.broadcasted_iota(jnp.int32, (8, 128), 0) + (r0 + r)
                    acc = jnp.where(row >= DIL * w, acc, NEG)
                sw.append(acc)
            m = sw[0]
            for w in range(1, WIN):
                m = jnp.maximum(m, sw[w])
            e = [jnp.exp2((sw[w] - m) * cexp) for w in range(WIN)]
            den = e[0]
            for w in range(1, WIN):
                den = den + e[w]
            inv = 1.0 / den
            p = [e[w] * inv for w in range(WIN)]
            o = []
            for g in range(NG):
                acc = None
                for w in range(WIN):
                    t = p[w] * v_scr[g, pl.ds(r0 + r + HALO - DIL * w, 8), :]
                    acc = t if acc is None else acc + t
                o.append(acc)
            return o

        prev_fin = [None]

        def attn_rows(r, tok):
            qp = [q_scr[g, pl.ds(p0 + r // 2, 8), :] for g in range(NG)]
            if tok is not None:
                qp = [_dep32(t, tok, never) for t in qp]
            q = [_unpack(t) for t in _butterfly(qp)]
            o0 = attn_half([t[0:8] for t in q], r)
            q1 = [t[8:16] for t in q]
            q1 = [_dep32(t, o0[NG - 1], never) for t in q1]
            o1 = attn_half(q1, r + 8)
            o = _butterfly([_pack(jnp.concatenate([o0[g], o1[g]], axis=0)) for g in range(NG)])
            for g in range(NG):
                o_scr[r // 2:r // 2 + 8, g * 128:(g + 1) * 128] = o[g]
            fin = o[0]
            for g in range(1, NG):
                fin = fin ^ o[g]
            tok = o[0]
            if prev_fin[0] is not None:
                tok = tok ^ prev_fin[0]
            prev_fin[0] = fin
            return tok

        sl = [_as_bf16(s_scr[i, j]) for j in range(7)]
        acc = [None] * 7
        n_att = TM // RA
        per = 3
        tok = None
        pend = []
        for c in range(NCH):
            wg_l = wlist(rawg, cg, c, HD, FC)
            wu_l = wlist(rawu, cu, c, HD, FC)
            wd_l = wlist(rawd, cd, c, FC, HD)
            g = _strassen_out([_dot(sl[j], wg_l[j]) for j in range(7)])
            u = _strassen_out([_dot(sl[j], wu_l[j]) for j in range(7)])
            hq = [g[t] * u[t] for t in range(4)]
            pend.append(([t.astype(BF) for t in _lhs_combos(*hq)], wd_l))
            if len(pend) == DOWN_GROUP or c == NCH - 1:
                for j in range(7):
                    y = _dot(jnp.concatenate([p[0][j] for p in pend], axis=1),
                             jnp.concatenate([p[1][j] for p in pend], axis=0))
                    acc[j] = y if acc[j] is None else acc[j] + y
                pend = []
            for a in range(c * per, min((c + 1) * per, n_att)):
                tok = attn_rows(a * RA, tok)
            if c == NCH - 1:
                oq = [_as_bf16(o_scr[rr:rr + HM // 2, cc:cc + HD]) for rr in (0, HM // 2) for cc in (0, HD)]
                ol = [t.astype(BF) for t in _lhs_combos(*[t.astype(F32) for t in oq])]
                ol[2], ol[3] = oq[0], oq[3]
                cw = [_as_bf16(jnp.concatenate([cwo[t, j] for t in range(NWP)], axis=0)) for j in range(5)]
                b11 = jnp.concatenate([wo[0, t, :, 0:HD] for t in range(NWP)], axis=0)
                b22 = jnp.concatenate([wo[1, t, :, HD:D] for t in range(NWP)], axis=0)
                wo_l = [cw[0], b11, cw[1], cw[2], b22, cw[3], cw[4]]
                acc = [acc[j] + _dot(ol[j], wo_l[j]) for j in range(7)]
        ys = _strassen_out(acc)
        x = x_scr[pl.ds(r0, TM), :].astype(F32)
        slot = lax.rem(i, 2)
        for q in range(4):
            rr, cc = (q // 2) * HM, (q % 2) * HD
            (ob0, ob1, ob2, ob3)[q][slot] = (x[rr:rr + HM, cc:cc + HD] + ys[q]).astype(BF)
            out_copy(i, q).start()

        @pl.when(i == NB - 1)
        def _():
            for q in range(4):
                out_copy(i - 1, q).wait()
            for q in range(4):
                out_copy(i, q).wait()


@jax.jit
def pallas_parallel_sum__sliding_local_dilated__glu_gated_bilinear__prompt_kernel(
    A_x: jax.Array,
    A_wqkv: jax.Array,
    A_wo: jax.Array,
    B_x: jax.Array,
    B_w_gate: jax.Array,
    B_w_up: jax.Array,
    B_w_down: jax.Array,
):
    del B_x
    x = A_x.reshape(S, D)
    hbm = pl.BlockSpec(memory_space=pl.ANY)
    out = pl.pallas_call(
        _kernel,
        grid=(NSTEPS,),
        in_specs=[hbm] * 6,
        out_specs=hbm,
        out_shape=jax.ShapeDtypeStruct((S, D), A_x.dtype),
        scratch_shapes=[
            pltpu.VMEM((S, D), BF),
            pltpu.VMEM((NWC, D, WC), BF),
            pltpu.VMEM((2, NWP, HD // NWP, D), BF),
            pltpu.VMEM((NCH, D, 2 * FC), BF),
            pltpu.VMEM((NCH, D, 2 * FC), BF),
            pltpu.VMEM((NCH, 2 * FC, D), BF),
            pltpu.VMEM((3, 2, 5, HD // 4, WC), U32),
            pltpu.VMEM((NWP, 5, HD // NWP // 2, HD), U32),
            pltpu.VMEM((NCH, 5, HD // 2, FC), U32),
            pltpu.VMEM((NCH, 5, HD // 2, FC), U32),
            pltpu.VMEM((NCH, 5, FC // 2, HD), U32),
            pltpu.VMEM((S // 2, D), U32),
            pltpu.VMEM((NB, 7, HM // 2, HD), U32),
            pltpu.VMEM((NG, S // 2, 128), U32),
            pltpu.VMEM((2, NG, S + HALO, 128), F32),
            pltpu.VMEM((TM // 2, D), U32),
            pltpu.VMEM((2, HM, HD), BF),
            pltpu.VMEM((2, HM, HD), BF),
            pltpu.VMEM((2, HM, HD), BF),
            pltpu.VMEM((2, HM, HD), BF),
            pltpu.SemaphoreType.DMA((NB,)),
            pltpu.SemaphoreType.DMA((NWC + 1,)),
            pltpu.SemaphoreType.DMA((NCH, 6)),
            pltpu.SemaphoreType.DMA((2, 4)),
        ],
        compiler_params=pltpu.CompilerParams(
            dimension_semantics=("arbitrary",),
            vmem_limit_bytes=124 * 1024 * 1024,
            disable_bounds_checks=True,
        ),
        name="fused_attn_ffn",
    )(x, A_wqkv, A_wo.reshape(2, NWP, HD // NWP, D), B_w_gate, B_w_up, B_w_down)
    return out.reshape(A_x.shape)
```

```python
import jax
import jax.numpy as jnp
from jax import lax
from jax.experimental import pallas as pl
from jax.experimental.pallas import tpu as pltpu

S, D, F = 2048, 1024, 3584
DH, WIN, DIL = 32, 8, 2
TM = 256
HM = TM // 2
NB = S // TM
HD = D // 2
FC = 256
NCH = F // 2 // FC
HALO = 16
NG = D // 128
EPS = 1e-5
NEG = -1e9
BF = jnp.bfloat16
F32 = jnp.float32
U32 = jnp.uint32
LOG2E = 1.4426950408889634
NA = 7
TA = 224
R0 = S - NA * TA
NSTEPS = 1 + NA + NB
NWP = 8
WC = 512
NWC = 3 * D // WC
N_EUP = 3
N_EUP0 = 2
BUILD_XOR = True
QN = 256
DOWN_GROUP = 2

def _dot(a, b):
    return jnp.dot(a, b, preferred_element_type=F32)


def _butterfly(vs):
    lane = lax.broadcasted_iota(jnp.int32, vs[0].shape, 1)
    for b in range(3):
        sh = 4 << b
        bit = (lane & sh) != 0
        new = list(vs)
        for i0 in range(NG):
            if i0 & (1 << b):
                continue
            i1 = i0 | (1 << b)
            new[i0] = jnp.where(bit, pltpu.roll(vs[i1], sh, 1), vs[i0])
            new[i1] = jnp.where(bit, vs[i1], pltpu.roll(vs[i0], 128 - sh, 1))
        vs = new
    return vs


def _sum4(x):
    lane = lax.broadcasted_iota(jnp.int32, x.shape, 1)
    x = x + jnp.where((lane & 1) != 0, pltpu.roll(x, 1, 1), pltpu.roll(x, 127, 1))
    x = x + jnp.where((lane & 2) != 0, pltpu.roll(x, 2, 1), pltpu.roll(x, 126, 1))
    return x


def _dep32(x, tok, never):
    return jnp.where(never, pltpu.bitcast(tok, x.dtype), x)


def _gate(m, tok, never):
    t = pltpu.bitcast(m[0:16, 0:128], F32)
    t = pltpu.bitcast(_dep32(t, tok, never), BF)
    top = jnp.concatenate([t, m[0:16, 128:]], axis=1)
    if m.shape[0] == 16:
        return top
    return jnp.concatenate([top, m[16:]], axis=0)


def _pack(y):
    return pltpu.bitcast(y.astype(BF), U32)


def _as_bf16(w):
    return pltpu.bitcast(w, BF)


def _unpack(w):
    return pltpu.bitcast(w, BF).astype(F32)


def _lhs_combos(a11, a12, a21, a22):
    return [a11 + a22, a21 + a22, a11, a22, a11 + a12, a21 - a11, a12 - a22]


def _strassen_out(m):
    return (m[0] + m[3] - m[4] + m[6], m[2] + m[4], m[1] + m[3], m[0] - m[1] + m[2] + m[5])


def _layernorm(x):
    x = x.astype(F32)
    mean = jnp.mean(x, axis=-1, keepdims=True)
    xc = x - mean
    var = jnp.mean(xc * xc, axis=-1, keepdims=True)
    return xc * lax.rsqrt(var + EPS)


def _kernel(x_hbm, wqkv_hbm, wo_hbm, wg_hbm, wu_hbm, wd_hbm, o_hbm,
            x_scr, wqkv, wo, rawg, rawu, rawd, cq, cwo, cg, cu, cd,
            xn_scr, s_scr, q_scr, kv_scr, o_scr, ob0, ob1, ob2, ob3,
            sem_x, sem_w, sem_raw, sem_o):
    s = pl.program_id(0)
    k_scr = kv_scr.at[0]
    v_scr = kv_scr.at[1]

    def x_copy(b):
        return pltpu.make_async_copy(x_hbm.at[pl.ds(b * TM, TM), :], x_scr.at[pl.ds(b * TM, TM), :], sem_x.at[b])

    def wqkv_copy(k):
        return pltpu.make_async_copy(wqkv_hbm.at[:, pl.ds(k * WC, WC)], wqkv.at[k], sem_w.at[k])

    def wo_copy():
        return pltpu.make_async_copy(wo_hbm, wo, sem_w.at[NWC])

    def raw_copies(c):
        return [
            pltpu.make_async_copy(wg_hbm.at[:, pl.ds(c * FC, FC)], rawg.at[c, :, pl.ds(0, FC)], sem_raw.at[c, 0]),
            pltpu.make_async_copy(wg_hbm.at[:, pl.ds(F // 2 + c * FC, FC)], rawg.at[c, :, pl.ds(FC, FC)], sem_raw.at[c, 1]),
            pltpu.make_async_copy(wu_hbm.at[:, pl.ds(c * FC, FC)], rawu.at[c, :, pl.ds(0, FC)], sem_raw.at[c, 2]),
            pltpu.make_async_copy(wu_hbm.at[:, pl.ds(F // 2 + c * FC, FC)], rawu.at[c, :, pl.ds(FC, FC)], sem_raw.at[c, 3]),
            pltpu.make_async_copy(wd_hbm.at[pl.ds(c * FC, FC), :], rawd.at[c, pl.ds(0, FC), :], sem_raw.at[c, 4]),
            pltpu.make_async_copy(wd_hbm.at[pl.ds(F // 2 + c * FC, FC), :], rawd.at[c, pl.ds(FC, FC), :], sem_raw.at[c, 5]),
        ]

    def out_copy(i, q):
        slot = lax.rem(i, 2)
        rr, cc = (q // 2) * HM, (q % 2) * HD
        return pltpu.make_async_copy((ob0, ob1, ob2, ob3)[q].at[slot],
                                     o_hbm.at[pl.ds(i * TM + rr, HM), pl.ds(cc, HD)], sem_o.at[slot, q])

    never = lax.broadcasted_iota(jnp.int32, (8, 128), 0) < jnp.minimum(s, 0)

    def ln_unit(b, r, tok):
        RC = 16
        r0 = pl.multiple_of(b * TM + r, RC)
        xt = x_scr[pl.ds(r0, RC), :]
        xb = x_scr[pl.ds(r0 + HM, RC), :]
        if tok is not None:
            xt = _gate(xt, tok, never)
            xb = _gate(xb, tok, never)
        top = _layernorm(xt)
        bot = _layernorm(xb)
        p0 = pl.multiple_of(r0 // 2, RC // 2)
        xn_scr[pl.ds(p0, RC // 2), :] = _pack(top)
        xn_scr[pl.ds(p0 + HM // 2, RC // 2), :] = _pack(bot)
        cs = _lhs_combos(top[:, :HD], top[:, HD:], bot[:, :HD], bot[:, HD:])
        pr = r // 2 if isinstance(r, int) else pl.multiple_of(r // 2, RC // 2)
        for j in range(7):
            s_scr[b, j, pl.ds(pr, RC // 2), :] = _pack(cs[j])
        return top[0:8, 0:128] + bot[0:8, 0:128]

    def ln_block(b, chain=False):
        tok = None
        for r in range(0, HM, 16):
            t = ln_unit(b, r, tok)
            tok = t if chain else None
        return tok

    def store_kv(y, dst, r0):
        for r in range(0, y.shape[0], 16):
            vs = _butterfly([_pack(y[r:r + 16, g * 128:(g + 1) * 128]) for g in range(NG)])
            for g in range(NG):
                dst[g, pl.ds(r0 + HALO + r, 16), :] = _unpack(vs[g])

    def store_q(y, r0):
        p0 = pl.multiple_of(r0 // 2, 8)
        for g in range(NG):
            q_scr[g, pl.ds(p0, y.shape[0] // 2), :] = _pack(y[:, g * 128:(g + 1) * 128])

    def build_tiles(ld16, st16, positions, tok, n_eup):
        for r, n0 in positions:
            for _ in range(n_eup or 0):
                tok = jnp.exp2(tok)

            def ld(q):
                w = pltpu.bitcast(ld16(q, r, n0), U32)
                if n_eup is not None:
                    w = _dep32(w, tok, never)
                return (pltpu.bitcast(w << 16, F32), pltpu.bitcast(w & jnp.uint32(0xFFFF0000), F32))

            b11, b12, b21, b22 = [ld(q) for q in range(4)]

            def comb(x, y, sign):
                ev, od = (x[0] + y[0], x[1] + y[1]) if sign > 0 else (x[0] - y[0], x[1] - y[1])
                return pltpu.bitcast(pltpu.pack_elementwise([ev, od], packed_dtype=BF), U32)

            outs = [comb(b11, b22, 1), comb(b12, b22, -1), comb(b21, b11, -1), comb(b11, b12, 1), comb(b21, b22, 1)]
            for j in range(5):
                st16(j, r, n0, outs[j])
            t = outs[0]
            if n_eup is not None and BUILD_XOR:
                t = (t ^ outs[1]) ^ (outs[2] ^ outs[3]) ^ outs[4]
            tok = pltpu.bitcast(t, F32)
        return tok

    def build_qkv(sec, kl, kr, bh, n_eup):
        rb = bh * (HD // 2)

        def row(r, m):
            return rb + r if isinstance(rb, int) else pl.multiple_of(rb + r, m)

        def ld8(q, r, n):
            return wqkv[kl if q in (0, 2) else kr, pl.ds(row((HD if q >= 2 else 0) + r, 16), 16), n:n + 128]

        def st16(j, r, n, val):
            cq[sec, bh, j, r // 2:r // 2 + 8, n:n + 128] = val

        build_tiles(ld8, st16, [(r, n) for r in range(0, HD // 2, 16) for n in range(0, WC, 128)],
                    jnp.zeros((8, 128), F32), n_eup)

    def wo_part(t):
        def ld16(q, r, n):
            return wo[q // 2, t, r:r + 16, pl.ds((HD if q % 2 else 0) + n, 128)]

        def st16(j, r, n, val):
            cwo[t, j, r // 2:r // 2 + 8, n:n + 128] = val

        return [(ld16, st16, (r, n)) for r in range(0, HD // NWP, 16) for n in range(0, HD, 128)]

    @pl.when(s == 0)
    def _():
        def issue_x(b, carry):
            x_copy(b).start(priority=1)
            return carry

        lax.fori_loop(0, 2, issue_x, 0)

        def issue_w(j, carry):
            @pl.when(j == 1)
            def _():
                x_copy(2).start(priority=1)

            wqkv_copy(lax.rem(j + 2, NWC)).start(priority=1)
            return carry

        lax.fori_loop(0, NWC, issue_w, 0)

        def issue_rest(j, carry):
            for cp in raw_copies(0):
                cp.start(priority=1)
            return carry

        lax.fori_loop(0, jnp.maximum(s, 1), issue_rest, 0)
        wo_copy().start(priority=1)
        x_copy(3).start(priority=1)
        k_scr[:, 0:HALO, :] = jnp.zeros((NG, HALO, 128), F32)
        v_scr[:, 0:HALO, :] = jnp.zeros((NG, HALO, 128), F32)
        x_copy(0).wait()
        ln_block(0)
        x_copy(1).wait()
        ln_block(1)
        P0 = R0 // 2
        xn = _as_bf16(xn_scr[0:P0, :])

        def body(j, carry):
            k = lax.rem(j + 2, NWC)
            wqkv_copy(k).wait()

            @pl.when(j == 1)
            def _():
                x_copy(2).wait()

            y = _dot(xn, wqkv[k])
            half = lax.rem(j, 2)
            sec = jnp.maximum(lax.div(j, 2) - 1, 0)
            src = pl.multiple_of((sec + 1) * P0 + half * (P0 // 2), 8)
            dstr = pl.multiple_of(HALO + half * P0, 16)
            for r in range(0, P0 // 2, 8):
                vs = _butterfly([q_scr[g, pl.ds(src + r, 8), :] for g in range(NG)])
                for g in range(NG):
                    kv_scr[sec, g, pl.ds(dstr + 2 * r, 16), :] = _unpack(vs[g])
            lb = jnp.minimum(j + 1, 2)
            u0 = 2 * jnp.clip(j - 1, 0, 3)
            tok = ln_unit(lb, pl.multiple_of(u0 * 16, 16), None)
            ln_unit(lb, pl.multiple_of(u0 * 16 + 16, 16), tok)
            jm = jnp.maximum(j - 1, 0)
            bsec = lax.div(jm, 2)
            kl = lax.rem(2 * bsec + 2, NWC)
            kr = jnp.where(j == 0, kl, kl + 1)
            bh = jnp.where(j == 0, 1, lax.rem(jm, 2))
            build_qkv(bsec, kl, kr, bh, N_EUP0)
            rb = pl.multiple_of(lax.rem(lax.div(j, 2) + 1, 3) * P0, 8)
            for gg in range(WC // 128):
                q_scr[half * (WC // 128) + gg, pl.ds(rb, P0), :] = _pack(y[:, gg * 128:(gg + 1) * 128])
            return carry

        lax.fori_loop(0, NWC, body, 0)
        build_qkv(2, 0, 1, 1, None)
        wo_copy().wait()
        for ld16, st16, pos in wo_part(NWP - 1):
            build_tiles(ld16, st16, [pos], jnp.zeros((8, 128), F32), None)

    @pl.when(s <= NA)
    def _():
        @pl.when(s + 1 < NCH)
        def _():
            for cp in raw_copies(s + 1):
                cp.start(priority=1)

        @pl.when(s + 4 < NB)
        def _():
            x_copy(s + 4).start(priority=1)

        @pl.when(s >= 1)
        def _():
            for cp in raw_copies(s - 1):
                cp.wait()

        @pl.when(jnp.logical_and(s >= 1, s + 2 < NB))
        def _():
            x_copy(s + 2).wait()

    @pl.when(s >= NA + 3)
    def _():
        for q in range(4):
            out_copy(s - (NA + 3), q).wait()

    @pl.when(jnp.logical_and(s >= 1, s <= NA))
    def _():
        c = lax.rem(s + (NA - 1), NA)
        r0 = pl.multiple_of(R0 + (s - 1) * TA, 16)
        HA = TA // 2
        pt = pl.multiple_of(r0 // 2, 8)
        pb = pl.multiple_of((r0 + HA) // 2, 8)
        a11 = _as_bf16(xn_scr[pl.ds(pt, HA // 2), 0:HD])
        a12 = _as_bf16(xn_scr[pl.ds(pt, HA // 2), HD:D])
        a21 = _as_bf16(xn_scr[pl.ds(pb, HA // 2), 0:HD])
        a22 = _as_bf16(xn_scr[pl.ds(pb, HA // 2), HD:D])
        la = [t.astype(BF) for t in _lhs_combos(a11.astype(F32), a12.astype(F32), a21.astype(F32), a22.astype(F32))]
        la[2], la[3] = a11, a22

        def ffn_part(raw, cmb, kq, nq):
            def ld8(q, r, n):
                return raw[c, pl.ds((kq if q >= 2 else 0) + r, 16), pl.ds((nq if q % 2 else 0) + n, 128)]

            def st16(j, r, n, val):
                cmb[c, j, r // 2:r // 2 + 8, n:n + 128] = val

            return [(ld8, st16, (r, n)) for r in range(0, kq, 16) for n in range(0, nq, 128)]

        work = ffn_part(rawg, cg, HD, FC) + ffn_part(rawu, cu, HD, FC) + ffn_part(rawd, cd, FC, HD) + wo_part(c)
        ys = []
        for sec in range(3):
            kl = (2 * sec + 2) % NWC
            cw = [_as_bf16(jnp.concatenate([cq[sec, 0, j], cq[sec, 1, j]], axis=0)) for j in range(5)]
            wl = [cw[0], wqkv[kl, 0:HD, :], cw[1], cw[2], wqkv[kl + 1, HD:D, :], cw[3], cw[4]]
            parts = [_strassen_out([_dot(la[j], wl[j][:, n:n + QN]) for j in range(7)]) for n in range(0, WC, QN)]
            c11, c12, c21, c22 = [jnp.concatenate([p[t] for p in parts], axis=1) for t in range(4)]
            ys.append((jnp.concatenate([c11, c12], axis=1), jnp.concatenate([c21, c22], axis=1)))
        ln_block(jnp.minimum(s + 2, NB - 1), chain=True)
        tok = jnp.zeros((8, 128), F32)
        for ld8, st16, pos in work:
            tok = build_tiles(ld8, st16, [pos], tok, N_EUP)
        for h in range(2):
            rh = pl.multiple_of(r0 + h * HA, 16)
            store_kv(ys[0][h], k_scr, rh)
            store_kv(ys[1][h], v_scr, rh)
            store_q(ys[2][h], rh)

    @pl.when(s > NA)
    def _():
        i = lax.rem(s + (NB - NA - 1), NB)
        r0 = pl.multiple_of(i * TM, TM)

        def wlist(raw, cmb, c, kq, nq):
            cw = [_as_bf16(cmb[c, j]) for j in range(5)]
            return [cw[0], raw[c, 0:kq, 0:nq], cw[1], cw[2], raw[c, kq:2 * kq, nq:2 * nq], cw[3], cw[4]]

        RA = 16
        cexp = (DH ** -0.5) * LOG2E
        p0 = pl.multiple_of(r0 // 2, 8)

        def attn_half(q, r):
            sw = []
            for w in range(WIN):
                acc = None
                for g in range(NG):
                    t = q[g] * k_scr[g, pl.ds(r0 + r + HALO - DIL * w, 8), :]
                    acc = t if acc is None else acc + t
                acc = _sum4(acc)
                if r < HALO and w > 0:
                    row = lax.broadcasted_iota(jnp.int32, (8, 128), 0) + (r0 + r)
                    acc = jnp.where(row >= DIL * w, acc, NEG)
                sw.append(acc)
            m = sw[0]
            for w in range(1, WIN):
                m = jnp.maximum(m, sw[w])
            e = [jnp.exp2((sw[w] - m) * cexp) for w in range(WIN)]
            den = e[0]
            for w in range(1, WIN):
                den = den + e[w]
            inv = 1.0 / den
            p = [e[w] * inv for w in range(WIN)]
            o = []
            for g in range(NG):
                acc = None
                for w in range(WIN):
                    t = p[w] * v_scr[g, pl.ds(r0 + r + HALO - DIL * w, 8), :]
                    acc = t if acc is None else acc + t
                o.append(acc)
            return o

        prev_fin = [None]

        def attn_rows(r, tok):
            qp = [q_scr[g, pl.ds(p0 + r // 2, 8), :] for g in range(NG)]
            if tok is not None:
                qp = [_dep32(t, tok, never) for t in qp]
            q = [_unpack(t) for t in _butterfly(qp)]
            o0 = attn_half([t[0:8] for t in q], r)
            q1 = [t[8:16] for t in q]
            q1 = [_dep32(t, o0[NG - 1], never) for t in q1]
            o1 = attn_half(q1, r + 8)
            o = _butterfly([_pack(jnp.concatenate([o0[g], o1[g]], axis=0)) for g in range(NG)])
            for g in range(NG):
                o_scr[r // 2:r // 2 + 8, g * 128:(g + 1) * 128] = o[g]
            fin = o[0]
            for g in range(1, NG):
                fin = fin ^ o[g]
            tok = o[0]
            if prev_fin[0] is not None:
                tok = tok ^ prev_fin[0]
            prev_fin[0] = fin
            return tok

        sl = [_as_bf16(s_scr[i, j]) for j in range(7)]
        acc = [None] * 7
        n_att = TM // RA
        per = 3
        tok = None
        pend = []
        for c in range(NCH):
            wg_l = wlist(rawg, cg, c, HD, FC)
            wu_l = wlist(rawu, cu, c, HD, FC)
            wd_l = wlist(rawd, cd, c, FC, HD)
            g = _strassen_out([_dot(sl[j], wg_l[j]) for j in range(7)])
            u = _strassen_out([_dot(sl[j], wu_l[j]) for j in range(7)])
            hq = [g[t] * u[t] for t in range(4)]
            pend.append(([t.astype(BF) for t in _lhs_combos(*hq)], wd_l))
            if len(pend) == DOWN_GROUP or c == NCH - 1:
                for j in range(7):
                    y = _dot(jnp.concatenate([p[0][j] for p in pend], axis=1),
                             jnp.concatenate([p[1][j] for p in pend], axis=0))
                    acc[j] = y if acc[j] is None else acc[j] + y
                pend = []
            for a in range(c * per, min((c + 1) * per, n_att)):
                tok = attn_rows(a * RA, tok)
            if c == NCH - 1:
                oq = [_as_bf16(o_scr[rr:rr + HM // 2, cc:cc + HD]) for rr in (0, HM // 2) for cc in (0, HD)]
                ol = [t.astype(BF) for t in _lhs_combos(*[t.astype(F32) for t in oq])]
                ol[2], ol[3] = oq[0], oq[3]
                cw = [_as_bf16(jnp.concatenate([cwo[t, j] for t in range(NWP)], axis=0)) for j in range(5)]
                b11 = jnp.concatenate([wo[0, t, :, 0:HD] for t in range(NWP)], axis=0)
                b22 = jnp.concatenate([wo[1, t, :, HD:D] for t in range(NWP)], axis=0)
                wo_l = [cw[0], b11, cw[1], cw[2], b22, cw[3], cw[4]]
                acc = [acc[j] + _dot(ol[j], wo_l[j]) for j in range(7)]
        ys = _strassen_out(acc)
        x = x_scr[pl.ds(r0, TM), :].astype(F32)
        slot = lax.rem(i, 2)
        for q in range(4):
            rr, cc = (q // 2) * HM, (q % 2) * HD
            (ob0, ob1, ob2, ob3)[q][slot] = (x[rr:rr + HM, cc:cc + HD] + ys[q]).astype(BF)
            out_copy(i, q).start()

        @pl.when(i == NB - 1)
        def _():
            for q in range(4):
                out_copy(i - 1, q).wait()
            for q in range(4):
                out_copy(i, q).wait()


@jax.jit
def pallas_parallel_sum__sliding_local_dilated__glu_gated_bilinear__prompt_kernel(
    A_x: jax.Array,
    A_wqkv: jax.Array,
    A_wo: jax.Array,
    B_x: jax.Array,
    B_w_gate: jax.Array,
    B_w_up: jax.Array,
    B_w_down: jax.Array,
):
    del B_x
    x = A_x.reshape(S, D)
    hbm = pl.BlockSpec(memory_space=pl.ANY)
    out = pl.pallas_call(
        _kernel,
        grid=(NSTEPS,),
        in_specs=[hbm] * 6,
        out_specs=hbm,
        out_shape=jax.ShapeDtypeStruct((S, D), A_x.dtype),
        scratch_shapes=[
            pltpu.VMEM((S, D), BF),
            pltpu.VMEM((NWC, D, WC), BF),
            pltpu.VMEM((2, NWP, HD // NWP, D), BF),
            pltpu.VMEM((NCH, D, 2 * FC), BF),
            pltpu.VMEM((NCH, D, 2 * FC), BF),
            pltpu.VMEM((NCH, 2 * FC, D), BF),
            pltpu.VMEM((3, 2, 5, HD // 4, WC), U32),
            pltpu.VMEM((NWP, 5, HD // NWP // 2, HD), U32),
            pltpu.VMEM((NCH, 5, HD // 2, FC), U32),
            pltpu.VMEM((NCH, 5, HD // 2, FC), U32),
            pltpu.VMEM((NCH, 5, FC // 2, HD), U32),
            pltpu.VMEM((S // 2, D), U32),
            pltpu.VMEM((NB, 7, HM // 2, HD), U32),
            pltpu.VMEM((NG, S // 2, 128), U32),
            pltpu.VMEM((2, NG, S + HALO, 128), F32),
            pltpu.VMEM((TM // 2, D), U32),
            pltpu.VMEM((2, HM, HD), BF),
            pltpu.VMEM((2, HM, HD), BF),
            pltpu.VMEM((2, HM, HD), BF),
            pltpu.VMEM((2, HM, HD), BF),
            pltpu.SemaphoreType.DMA((NB,)),
            pltpu.SemaphoreType.DMA((NWC + 1,)),
            pltpu.SemaphoreType.DMA((NCH, 6)),
            pltpu.SemaphoreType.DMA((2, 4)),
        ],
        compiler_params=pltpu.CompilerParams(
            dimension_semantics=("arbitrary",),
            vmem_limit_bytes=124 * 1024 * 1024,
            disable_bounds_checks=True,
        ),
        name="fused_attn_ffn",
    )(x, A_wqkv, A_wo.reshape(2, NWP, HD // NWP, D), B_w_gate, B_w_up, B_w_down)
    return out.reshape(A_x.shape)
```

```python
import jax
import jax.numpy as jnp
from jax import lax
from jax.experimental import pallas as pl
from jax.experimental.pallas import tpu as pltpu

S, D, F = 2048, 1024, 3584
DH, WIN, DIL = 32, 8, 2
TM = 256
HM = TM // 2
NB = S // TM
HD = D // 2
FC = 256
NCH = F // 2 // FC
HALO = 16
NG = D // 128
EPS = 1e-5
NEG = -1e9
BF = jnp.bfloat16
F32 = jnp.float32
U32 = jnp.uint32
LOG2E = 1.4426950408889634
NA = 7
TA = 224
R0 = S - NA * TA
NSTEPS = 1 + NA + NB
NWP = 8
WC = 512
NWC = 3 * D // WC
N_EUP = 3
N_EUP0 = 3
QN = 128
DOWN_GROUP = 3

def _dot(a, b):
    return jnp.dot(a, b, preferred_element_type=F32)


def _butterfly(vs):
    lane = lax.broadcasted_iota(jnp.int32, vs[0].shape, 1)
    for b in range(3):
        sh = 4 << b
        bit = (lane & sh) != 0
        new = list(vs)
        for i0 in range(NG):
            if i0 & (1 << b):
                continue
            i1 = i0 | (1 << b)
            new[i0] = jnp.where(bit, pltpu.roll(vs[i1], sh, 1), vs[i0])
            new[i1] = jnp.where(bit, vs[i1], pltpu.roll(vs[i0], 128 - sh, 1))
        vs = new
    return vs


def _sum4(x):
    lane = lax.broadcasted_iota(jnp.int32, x.shape, 1)
    x = x + jnp.where((lane & 1) != 0, pltpu.roll(x, 1, 1), pltpu.roll(x, 127, 1))
    x = x + jnp.where((lane & 2) != 0, pltpu.roll(x, 2, 1), pltpu.roll(x, 126, 1))
    return x


def _dep32(x, tok, never):
    return jnp.where(never, pltpu.bitcast(tok, x.dtype), x)


def _gate(m, tok, never):
    t = pltpu.bitcast(m[0:16, 0:128], F32)
    t = pltpu.bitcast(_dep32(t, tok, never), BF)
    top = jnp.concatenate([t, m[0:16, 128:]], axis=1)
    if m.shape[0] == 16:
        return top
    return jnp.concatenate([top, m[16:]], axis=0)


def _pack(y):
    return pltpu.bitcast(y.astype(BF), U32)


def _as_bf16(w):
    return pltpu.bitcast(w, BF)


def _unpack(w):
    return pltpu.bitcast(w, BF).astype(F32)


def _lhs_combos(a11, a12, a21, a22):
    return [a11 + a22, a21 + a22, a11, a22, a11 + a12, a21 - a11, a12 - a22]


def _strassen_out(m):
    return (m[0] + m[3] - m[4] + m[6], m[2] + m[4], m[1] + m[3], m[0] - m[1] + m[2] + m[5])


def _layernorm(x):
    x = x.astype(F32)
    mean = jnp.mean(x, axis=-1, keepdims=True)
    xc = x - mean
    var = jnp.mean(xc * xc, axis=-1, keepdims=True)
    return xc * lax.rsqrt(var + EPS)


def _kernel(x_hbm, wqkv_hbm, wo_hbm, wg_hbm, wu_hbm, wd_hbm, o_ref,
            x_scr, wqkv, wo, rawg, rawu, rawd, cq, cwo, cg, cu, cd,
            xn_scr, s_scr, q_scr, kv_scr, o_scr,
            sem_x, sem_w, sem_raw):
    s = pl.program_id(0)
    k_scr = kv_scr.at[0]
    v_scr = kv_scr.at[1]

    def x_copy(b):
        return pltpu.make_async_copy(x_hbm.at[pl.ds(b * TM, TM), :], x_scr.at[pl.ds(b * TM, TM), :], sem_x.at[b])

    def wqkv_copy(k):
        return pltpu.make_async_copy(wqkv_hbm.at[:, pl.ds(k * WC, WC)], wqkv.at[k], sem_w.at[k])

    def wo_copy():
        return pltpu.make_async_copy(wo_hbm, wo, sem_w.at[NWC])

    def raw_copies(c):
        return [
            pltpu.make_async_copy(wg_hbm.at[:, pl.ds(c * FC, FC)], rawg.at[c, :, pl.ds(0, FC)], sem_raw.at[c, 0]),
            pltpu.make_async_copy(wg_hbm.at[:, pl.ds(F // 2 + c * FC, FC)], rawg.at[c, :, pl.ds(FC, FC)], sem_raw.at[c, 1]),
            pltpu.make_async_copy(wu_hbm.at[:, pl.ds(c * FC, FC)], rawu.at[c, :, pl.ds(0, FC)], sem_raw.at[c, 2]),
            pltpu.make_async_copy(wu_hbm.at[:, pl.ds(F // 2 + c * FC, FC)], rawu.at[c, :, pl.ds(FC, FC)], sem_raw.at[c, 3]),
            pltpu.make_async_copy(wd_hbm.at[pl.ds(c * FC, FC), :], rawd.at[c, pl.ds(0, FC), :], sem_raw.at[c, 4]),
            pltpu.make_async_copy(wd_hbm.at[pl.ds(F // 2 + c * FC, FC), :], rawd.at[c, pl.ds(FC, FC), :], sem_raw.at[c, 5]),
        ]

    never = lax.broadcasted_iota(jnp.int32, (8, 128), 0) < jnp.minimum(s, 0)

    def ln_unit(b, r, tok):
        RC = 16
        r0 = pl.multiple_of(b * TM + r, RC)
        xt = x_scr[pl.ds(r0, RC), :]
        xb = x_scr[pl.ds(r0 + HM, RC), :]
        if tok is not None:
            xt = _gate(xt, tok, never)
            xb = _gate(xb, tok, never)
        top = _layernorm(xt)
        bot = _layernorm(xb)
        p0 = pl.multiple_of(r0 // 2, RC // 2)
        xn_scr[pl.ds(p0, RC // 2), :] = _pack(top)
        xn_scr[pl.ds(p0 + HM // 2, RC // 2), :] = _pack(bot)
        cs = _lhs_combos(top[:, :HD], top[:, HD:], bot[:, :HD], bot[:, HD:])
        pr = r // 2 if isinstance(r, int) else pl.multiple_of(r // 2, RC // 2)
        for j in range(7):
            s_scr[b, j, pl.ds(pr, RC // 2), :] = _pack(cs[j])
        return top[0:8, 0:128] + bot[0:8, 0:128]

    def ln_block(b, chain=False):
        tok = None
        for r in range(0, HM, 16):
            t = ln_unit(b, r, tok)
            tok = t if chain else None
        return tok

    def store_kv(y, dst, r0):
        for r in range(0, y.shape[0], 16):
            vs = _butterfly([_pack(y[r:r + 16, g * 128:(g + 1) * 128]) for g in range(NG)])
            for g in range(NG):
                dst[g, pl.ds(r0 + HALO + r, 16), :] = _unpack(vs[g])

    def store_q(y, r0):
        p0 = pl.multiple_of(r0 // 2, 8)
        for g in range(NG):
            q_scr[g, pl.ds(p0, y.shape[0] // 2), :] = _pack(y[:, g * 128:(g + 1) * 128])

    def build_tiles(ld16, st16, positions, tok, n_eup):
        for r, n0 in positions:
            for _ in range(n_eup or 0):
                tok = jnp.exp2(tok)

            def ld(q):
                w = pltpu.bitcast(ld16(q, r, n0), U32)
                if n_eup is not None:
                    w = _dep32(w, tok, never)
                return (pltpu.bitcast(w << 16, F32), pltpu.bitcast(w & jnp.uint32(0xFFFF0000), F32))

            b11, b12, b21, b22 = [ld(q) for q in range(4)]

            def comb(x, y, sign):
                ev, od = (x[0] + y[0], x[1] + y[1]) if sign > 0 else (x[0] - y[0], x[1] - y[1])
                return pltpu.bitcast(pltpu.pack_elementwise([ev, od], packed_dtype=BF), U32)

            outs = [comb(b11, b22, 1), comb(b12, b22, -1), comb(b21, b11, -1), comb(b11, b12, 1), comb(b21, b22, 1)]
            for j in range(5):
                st16(j, r, n0, outs[j])
            t = outs[0]
            if n_eup is not None:
                t = (t ^ outs[1]) ^ (outs[2] ^ outs[3]) ^ outs[4]
            tok = pltpu.bitcast(t, F32)
        return tok

    def build_qkv(sec, kl, kr, bh, n_eup):
        rb = bh * (HD // 2)

        def row(r, m):
            return rb + r if isinstance(rb, int) else pl.multiple_of(rb + r, m)

        def ld8(q, r, n):
            return wqkv[kl if q in (0, 2) else kr, pl.ds(row((HD if q >= 2 else 0) + r, 16), 16), n:n + 128]

        def st16(j, r, n, val):
            cq[sec, bh, j, r // 2:r // 2 + 8, n:n + 128] = val

        build_tiles(ld8, st16, [(r, n) for r in range(0, HD // 2, 16) for n in range(0, WC, 128)],
                    jnp.zeros((8, 128), F32), n_eup)

    def wo_part(t):
        def ld16(q, r, n):
            return wo[q // 2, t, r:r + 16, pl.ds((HD if q % 2 else 0) + n, 128)]

        def st16(j, r, n, val):
            cwo[t, j, r // 2:r // 2 + 8, n:n + 128] = val

        return [(ld16, st16, (r, n)) for r in range(0, HD // NWP, 16) for n in range(0, HD, 128)]

    @pl.when(s == 0)
    def _():
        def issue_x(b, carry):
            x_copy(b).start(priority=1)
            return carry

        lax.fori_loop(0, 2, issue_x, 0)

        def issue_w(j, carry):
            @pl.when(j == 1)
            def _():
                x_copy(2).start(priority=1)

            wqkv_copy(lax.rem(j + 2, NWC)).start(priority=1)
            return carry

        lax.fori_loop(0, NWC, issue_w, 0)

        def issue_rest(j, carry):
            for cp in raw_copies(0):
                cp.start(priority=1)
            return carry

        lax.fori_loop(0, jnp.maximum(s, 1), issue_rest, 0)
        wo_copy().start(priority=1)
        x_copy(3).start(priority=1)
        k_scr[:, 0:HALO, :] = jnp.zeros((NG, HALO, 128), F32)
        v_scr[:, 0:HALO, :] = jnp.zeros((NG, HALO, 128), F32)
        x_copy(0).wait()
        ln_block(0)
        x_copy(1).wait()
        ln_block(1)
        P0 = R0 // 2
        xn = _as_bf16(xn_scr[0:P0, :])

        def body(j, carry):
            k = lax.rem(j + 2, NWC)
            wqkv_copy(k).wait()

            @pl.when(j == 1)
            def _():
                x_copy(2).wait()

            y = _dot(xn, wqkv[k])
            half = lax.rem(j, 2)
            sec = jnp.maximum(lax.div(j, 2) - 1, 0)
            src = pl.multiple_of((sec + 1) * P0 + half * (P0 // 2), 8)
            dstr = pl.multiple_of(HALO + half * P0, 16)
            for r in range(0, P0 // 2, 8):
                vs = _butterfly([q_scr[g, pl.ds(src + r, 8), :] for g in range(NG)])
                for g in range(NG):
                    kv_scr[sec, g, pl.ds(dstr + 2 * r, 16), :] = _unpack(vs[g])
            lb = jnp.minimum(j + 1, 2)
            u0 = 2 * jnp.clip(j - 1, 0, 3)
            tok = ln_unit(lb, pl.multiple_of(u0 * 16, 16), None)
            ln_unit(lb, pl.multiple_of(u0 * 16 + 16, 16), tok)
            jm = jnp.maximum(j - 1, 0)
            bsec = lax.div(jm, 2)
            kl = lax.rem(2 * bsec + 2, NWC)
            kr = jnp.where(j == 0, kl, kl + 1)
            bh = jnp.where(j == 0, 1, lax.rem(jm, 2))
            build_qkv(bsec, kl, kr, bh, N_EUP0)
            rb = pl.multiple_of(lax.rem(lax.div(j, 2) + 1, 3) * P0, 8)
            for gg in range(WC // 128):
                q_scr[half * (WC // 128) + gg, pl.ds(rb, P0), :] = _pack(y[:, gg * 128:(gg + 1) * 128])
            return carry

        lax.fori_loop(0, NWC, body, 0)
        build_qkv(2, 0, 1, 1, None)
        wo_copy().wait()
        for ld16, st16, pos in wo_part(NWP - 1):
            build_tiles(ld16, st16, [pos], jnp.zeros((8, 128), F32), None)

    @pl.when(s <= NA)
    def _():
        @pl.when(s + 1 < NCH)
        def _():
            for cp in raw_copies(s + 1):
                cp.start(priority=1)

        @pl.when(s + 4 < NB)
        def _():
            x_copy(s + 4).start(priority=1)

        @pl.when(s >= 1)
        def _():
            for cp in raw_copies(s - 1):
                cp.wait()

        @pl.when(jnp.logical_and(s >= 1, s + 2 < NB))
        def _():
            x_copy(s + 2).wait()

    @pl.when(jnp.logical_and(s >= 1, s <= NA))
    def _():
        c = lax.rem(s + (NA - 1), NA)
        r0 = pl.multiple_of(R0 + (s - 1) * TA, 16)
        HA = TA // 2
        pt = pl.multiple_of(r0 // 2, 8)
        pb = pl.multiple_of((r0 + HA) // 2, 8)
        a11 = _as_bf16(xn_scr[pl.ds(pt, HA // 2), 0:HD])
        a12 = _as_bf16(xn_scr[pl.ds(pt, HA // 2), HD:D])
        a21 = _as_bf16(xn_scr[pl.ds(pb, HA // 2), 0:HD])
        a22 = _as_bf16(xn_scr[pl.ds(pb, HA // 2), HD:D])
        la = [t.astype(BF) for t in _lhs_combos(a11.astype(F32), a12.astype(F32), a21.astype(F32), a22.astype(F32))]
        la[2], la[3] = a11, a22

        def ffn_part(raw, cmb, kq, nq):
            def ld8(q, r, n):
                return raw[c, pl.ds((kq if q >= 2 else 0) + r, 16), pl.ds((nq if q % 2 else 0) + n, 128)]

            def st16(j, r, n, val):
                cmb[c, j, r // 2:r // 2 + 8, n:n + 128] = val

            return [(ld8, st16, (r, n)) for r in range(0, kq, 16) for n in range(0, nq, 128)]

        work = ffn_part(rawg, cg, HD, FC) + ffn_part(rawu, cu, HD, FC) + ffn_part(rawd, cd, FC, HD) + wo_part(c)
        def stores(sec):
            for h in range(2):
                rh = pl.multiple_of(r0 + h * HA, 16)
                if sec == 2:
                    store_q(ys[2][h], rh)
                else:
                    store_kv(ys[sec][h], k_scr if sec == 0 else v_scr, rh)

        ys = []
        for sec in range(3):
            kl = (2 * sec + 2) % NWC
            cw = [_as_bf16(jnp.concatenate([cq[sec, 0, j], cq[sec, 1, j]], axis=0)) for j in range(5)]
            wl = [cw[0], wqkv[kl, 0:HD, :], cw[1], cw[2], wqkv[kl + 1, HD:D, :], cw[3], cw[4]]
            parts = [_strassen_out([_dot(la[j], wl[j][:, n:n + QN]) for j in range(7)]) for n in range(0, WC, QN)]
            c11, c12, c21, c22 = [jnp.concatenate([p[t] for p in parts], axis=1) for t in range(4)]
            ys.append((jnp.concatenate([c11, c12], axis=1), jnp.concatenate([c21, c22], axis=1)))
            stores(sec)
        ln_block(jnp.minimum(s + 2, NB - 1), chain=True)
        tok = jnp.zeros((8, 128), F32)
        for ld8, st16, pos in work:
            tok = build_tiles(ld8, st16, [pos], tok, N_EUP)

    @pl.when(s > NA)
    def _():
        i = lax.rem(s + (NB - NA - 1), NB)
        r0 = pl.multiple_of(i * TM, TM)

        def wlist(raw, cmb, c, kq, nq):
            cw = [_as_bf16(cmb[c, j]) for j in range(5)]
            return [cw[0], raw[c, 0:kq, 0:nq], cw[1], cw[2], raw[c, kq:2 * kq, nq:2 * nq], cw[3], cw[4]]

        RA = 16
        cexp = (DH ** -0.5) * LOG2E
        p0 = pl.multiple_of(r0 // 2, 8)

        def attn_half(q, r):
            sw = []
            for w in range(WIN):
                acc = None
                for g in range(NG):
                    t = q[g] * k_scr[g, pl.ds(r0 + r + HALO - DIL * w, 8), :]
                    acc = t if acc is None else acc + t
                acc = _sum4(acc)
                if r < HALO and w > 0:
                    row = lax.broadcasted_iota(jnp.int32, (8, 128), 0) + (r0 + r)
                    acc = jnp.where(row >= DIL * w, acc, NEG)
                sw.append(acc)
            m = sw[0]
            for w in range(1, WIN):
                m = jnp.maximum(m, sw[w])
            e = [jnp.exp2((sw[w] - m) * cexp) for w in range(WIN)]
            den = e[0]
            for w in range(1, WIN):
                den = den + e[w]
            inv = 1.0 / den
            p = [e[w] * inv for w in range(WIN)]
            o = []
            for g in range(NG):
                acc = None
                for w in range(WIN):
                    t = p[w] * v_scr[g, pl.ds(r0 + r + HALO - DIL * w, 8), :]
                    acc = t if acc is None else acc + t
                o.append(acc)
            return o

        prev_fin = [None]

        def attn_rows(r, tok):
            qp = [q_scr[g, pl.ds(p0 + r // 2, 8), :] for g in range(NG)]
            if tok is not None:
                qp = [_dep32(t, tok, never) for t in qp]
            q = [_unpack(t) for t in _butterfly(qp)]
            o0 = attn_half([t[0:8] for t in q], r)
            q1 = [t[8:16] for t in q]
            q1 = [_dep32(t, o0[NG - 1], never) for t in q1]
            o1 = attn_half(q1, r + 8)
            o = _butterfly([_pack(jnp.concatenate([o0[g], o1[g]], axis=0)) for g in range(NG)])
            for g in range(NG):
                o_scr[r // 2:r // 2 + 8, g * 128:(g + 1) * 128] = o[g]
            fin = o[0]
            for g in range(1, NG):
                fin = fin ^ o[g]
            tok = o[0]
            if prev_fin[0] is not None:
                tok = tok ^ prev_fin[0]
            prev_fin[0] = fin
            return tok

        sl = [_as_bf16(s_scr[i, j]) for j in range(7)]
        acc = [None] * 7
        n_att = TM // RA
        per = 3
        tok = None
        pend = []
        for c in range(NCH):
            wg_l = wlist(rawg, cg, c, HD, FC)
            wu_l = wlist(rawu, cu, c, HD, FC)
            wd_l = wlist(rawd, cd, c, FC, HD)
            g = _strassen_out([_dot(sl[j], wg_l[j]) for j in range(7)])
            u = _strassen_out([_dot(sl[j], wu_l[j]) for j in range(7)])
            hq = [g[t] * u[t] for t in range(4)]
            pend.append(([t.astype(BF) for t in _lhs_combos(*hq)], wd_l))
            if len(pend) == DOWN_GROUP or c == NCH - 1:
                for j in range(7):
                    y = _dot(jnp.concatenate([p[0][j] for p in pend], axis=1),
                             jnp.concatenate([p[1][j] for p in pend], axis=0))
                    acc[j] = y if acc[j] is None else acc[j] + y
                pend = []
            for a in range(c * per, min((c + 1) * per, n_att)):
                tok = attn_rows(a * RA, tok)
            if c == NCH - 1:
                oq = [_as_bf16(o_scr[rr:rr + HM // 2, cc:cc + HD]) for rr in (0, HM // 2) for cc in (0, HD)]
                ol = [t.astype(BF) for t in _lhs_combos(*[t.astype(F32) for t in oq])]
                ol[2], ol[3] = oq[0], oq[3]
                cw = [_as_bf16(jnp.concatenate([cwo[t, j] for t in range(NWP)], axis=0)) for j in range(5)]
                b11 = jnp.concatenate([wo[0, t, :, 0:HD] for t in range(NWP)], axis=0)
                b22 = jnp.concatenate([wo[1, t, :, HD:D] for t in range(NWP)], axis=0)
                wo_l = [cw[0], b11, cw[1], cw[2], b22, cw[3], cw[4]]
                acc = [acc[j] + _dot(ol[j], wo_l[j]) for j in range(7)]
        ys = _strassen_out(acc)
        x = x_scr[pl.ds(r0, TM), :].astype(F32)
        for q in range(4):
            rr, cc = (q // 2) * HM, (q % 2) * HD
            o_ref[rr:rr + HM, cc:cc + HD] = (x[rr:rr + HM, cc:cc + HD] + ys[q]).astype(o_ref.dtype)


@jax.jit
def pallas_parallel_sum__sliding_local_dilated__glu_gated_bilinear__prompt_kernel(
    A_x: jax.Array,
    A_wqkv: jax.Array,
    A_wo: jax.Array,
    B_x: jax.Array,
    B_w_gate: jax.Array,
    B_w_up: jax.Array,
    B_w_down: jax.Array,
):
    del B_x
    x = A_x.reshape(S, D)
    hbm = pl.BlockSpec(memory_space=pl.ANY)
    out = pl.pallas_call(
        _kernel,
        grid=(NSTEPS,),
        in_specs=[hbm] * 6,
        out_specs=pl.BlockSpec((TM, D), lambda s: (jnp.maximum(s - (NA + 1), 0), 0)),
        out_shape=jax.ShapeDtypeStruct((S, D), A_x.dtype),
        scratch_shapes=[
            pltpu.VMEM((S, D), BF),
            pltpu.VMEM((NWC, D, WC), BF),
            pltpu.VMEM((2, NWP, HD // NWP, D), BF),
            pltpu.VMEM((NCH, D, 2 * FC), BF),
            pltpu.VMEM((NCH, D, 2 * FC), BF),
            pltpu.VMEM((NCH, 2 * FC, D), BF),
            pltpu.VMEM((3, 2, 5, HD // 4, WC), U32),
            pltpu.VMEM((NWP, 5, HD // NWP // 2, HD), U32),
            pltpu.VMEM((NCH, 5, HD // 2, FC), U32),
            pltpu.VMEM((NCH, 5, HD // 2, FC), U32),
            pltpu.VMEM((NCH, 5, FC // 2, HD), U32),
            pltpu.VMEM((S // 2, D), U32),
            pltpu.VMEM((NB, 7, HM // 2, HD), U32),
            pltpu.VMEM((NG, S // 2, 128), U32),
            pltpu.VMEM((2, NG, S + HALO, 128), F32),
            pltpu.VMEM((TM // 2, D), U32),
            pltpu.SemaphoreType.DMA((NB,)),
            pltpu.SemaphoreType.DMA((NWC + 1,)),
            pltpu.SemaphoreType.DMA((NCH, 6)),
        ],
        compiler_params=pltpu.CompilerParams(
            dimension_semantics=("arbitrary",),
            vmem_limit_bytes=124 * 1024 * 1024,
            disable_bounds_checks=True,
        ),
        name="fused_attn_ffn",
    )(x, A_wqkv, A_wo.reshape(2, NWP, HD // NWP, D), B_w_gate, B_w_up, B_w_down)
    return out.reshape(A_x.shape)
```

```python
import jax
import jax.numpy as jnp
from jax import lax
from jax.experimental import pallas as pl
from jax.experimental.pallas import tpu as pltpu

S, D, F = 2048, 1024, 3584
DH, WIN, DIL = 32, 8, 2
TM = 256
HM = TM // 2
NB = S // TM
HD = D // 2
FC = 256
NCH = F // 2 // FC
HALO = 16
NG = D // 128
EPS = 1e-5
NEG = -1e9
BF = jnp.bfloat16
F32 = jnp.float32
U32 = jnp.uint32
LOG2E = 1.4426950408889634
NA = 7
TA = 224
R0 = S - NA * TA
NSTEPS = 1 + NA + NB
NWP = 8
WC = 512
NWC = 3 * D // WC
N_EUP = 3
N_EUP0 = 3
QN = 128
DOWN_GROUP = 4

def _dot(a, b):
    return jnp.dot(a, b, preferred_element_type=F32)


def _butterfly(vs):
    lane = lax.broadcasted_iota(jnp.int32, vs[0].shape, 1)
    for b in range(3):
        sh = 4 << b
        bit = (lane & sh) != 0
        new = list(vs)
        for i0 in range(NG):
            if i0 & (1 << b):
                continue
            i1 = i0 | (1 << b)
            new[i0] = jnp.where(bit, pltpu.roll(vs[i1], sh, 1), vs[i0])
            new[i1] = jnp.where(bit, vs[i1], pltpu.roll(vs[i0], 128 - sh, 1))
        vs = new
    return vs


def _sum4(x):
    lane = lax.broadcasted_iota(jnp.int32, x.shape, 1)
    x = x + jnp.where((lane & 1) != 0, pltpu.roll(x, 1, 1), pltpu.roll(x, 127, 1))
    x = x + jnp.where((lane & 2) != 0, pltpu.roll(x, 2, 1), pltpu.roll(x, 126, 1))
    return x


def _dep32(x, tok, never):
    return jnp.where(never, pltpu.bitcast(tok, x.dtype), x)


def _gate(m, tok, never):
    t = pltpu.bitcast(m[0:16, 0:128], F32)
    t = pltpu.bitcast(_dep32(t, tok, never), BF)
    top = jnp.concatenate([t, m[0:16, 128:]], axis=1)
    if m.shape[0] == 16:
        return top
    return jnp.concatenate([top, m[16:]], axis=0)


def _pack(y):
    return pltpu.bitcast(y.astype(BF), U32)


def _as_bf16(w):
    return pltpu.bitcast(w, BF)


def _unpack(w):
    return pltpu.bitcast(w, BF).astype(F32)


def _lhs_combos(a11, a12, a21, a22):
    return [a11 + a22, a21 + a22, a11, a22, a11 + a12, a21 - a11, a12 - a22]


def _strassen_out(m):
    return (m[0] + m[3] - m[4] + m[6], m[2] + m[4], m[1] + m[3], m[0] - m[1] + m[2] + m[5])


def _layernorm(x):
    x = x.astype(F32)
    mean = jnp.mean(x, axis=-1, keepdims=True)
    xc = x - mean
    var = jnp.mean(xc * xc, axis=-1, keepdims=True)
    return xc * lax.rsqrt(var + EPS)


def _kernel(x_hbm, wqkv_hbm, wo_hbm, wg_hbm, wu_hbm, wd_hbm, o_ref,
            x_scr, wqkv, wo, rawg, rawu, rawd, cq, cwo, cg, cu, cd,
            xn_scr, s_scr, q_scr, kv_scr, o_scr,
            sem_x, sem_w, sem_raw):
    s = pl.program_id(0)
    k_scr = kv_scr.at[0]
    v_scr = kv_scr.at[1]

    def x_copy(b):
        return pltpu.make_async_copy(x_hbm.at[pl.ds(b * TM, TM), :], x_scr.at[pl.ds(b * TM, TM), :], sem_x.at[b])

    def wqkv_copy(k):
        return pltpu.make_async_copy(wqkv_hbm.at[:, pl.ds(k * WC, WC)], wqkv.at[k], sem_w.at[k])

    def wo_copy():
        return pltpu.make_async_copy(wo_hbm, wo, sem_w.at[NWC])

    def raw_copies(c):
        return [
            pltpu.make_async_copy(wg_hbm.at[:, pl.ds(c * FC, FC)], rawg.at[c, :, pl.ds(0, FC)], sem_raw.at[c, 0]),
            pltpu.make_async_copy(wg_hbm.at[:, pl.ds(F // 2 + c * FC, FC)], rawg.at[c, :, pl.ds(FC, FC)], sem_raw.at[c, 1]),
            pltpu.make_async_copy(wu_hbm.at[:, pl.ds(c * FC, FC)], rawu.at[c, :, pl.ds(0, FC)], sem_raw.at[c, 2]),
            pltpu.make_async_copy(wu_hbm.at[:, pl.ds(F // 2 + c * FC, FC)], rawu.at[c, :, pl.ds(FC, FC)], sem_raw.at[c, 3]),
            pltpu.make_async_copy(wd_hbm.at[pl.ds(c * FC, FC), :], rawd.at[c, pl.ds(0, FC), :], sem_raw.at[c, 4]),
            pltpu.make_async_copy(wd_hbm.at[pl.ds(F // 2 + c * FC, FC), :], rawd.at[c, pl.ds(FC, FC), :], sem_raw.at[c, 5]),
        ]

    never = lax.broadcasted_iota(jnp.int32, (8, 128), 0) < jnp.minimum(s, 0)

    def ln_unit(b, r, tok):
        RC = 16
        r0 = pl.multiple_of(b * TM + r, RC)
        xt = x_scr[pl.ds(r0, RC), :]
        xb = x_scr[pl.ds(r0 + HM, RC), :]
        if tok is not None:
            xt = _gate(xt, tok, never)
            xb = _gate(xb, tok, never)
        top = _layernorm(xt)
        bot = _layernorm(xb)
        p0 = pl.multiple_of(r0 // 2, RC // 2)
        xn_scr[pl.ds(p0, RC // 2), :] = _pack(top)
        xn_scr[pl.ds(p0 + HM // 2, RC // 2), :] = _pack(bot)
        cs = _lhs_combos(top[:, :HD], top[:, HD:], bot[:, :HD], bot[:, HD:])
        pr = r // 2 if isinstance(r, int) else pl.multiple_of(r // 2, RC // 2)
        for j in range(7):
            s_scr[b, j, pl.ds(pr, RC // 2), :] = _pack(cs[j])
        return top[0:8, 0:128] + bot[0:8, 0:128]

    def ln_block(b, chain=False):
        tok = None
        for r in range(0, HM, 16):
            t = ln_unit(b, r, tok)
            tok = t if chain else None
        return tok

    def store_kv(y, dst, r0):
        prev = None
        for r in range(0, y.shape[0], 16):
            ws = [_pack(y[r:r + 16, g * 128:(g + 1) * 128]) for g in range(NG)]
            if prev is not None:
                ws = [_dep32(w, prev, never) for w in ws]
            vs = _butterfly(ws)
            prev = vs[0]
            for g in range(NG):
                dst[g, pl.ds(r0 + HALO + r, 16), :] = _unpack(vs[g])

    def store_q(y, r0):
        p0 = pl.multiple_of(r0 // 2, 8)
        for g in range(NG):
            q_scr[g, pl.ds(p0, y.shape[0] // 2), :] = _pack(y[:, g * 128:(g + 1) * 128])

    def build_tiles(ld16, st16, positions, tok, n_eup):
        for r, n0 in positions:
            for _ in range(n_eup or 0):
                tok = jnp.exp2(tok)

            def ld(q):
                w = pltpu.bitcast(ld16(q, r, n0), U32)
                if n_eup is not None:
                    w = _dep32(w, tok, never)
                return (pltpu.bitcast(w << 16, F32), pltpu.bitcast(w & jnp.uint32(0xFFFF0000), F32))

            b11, b12, b21, b22 = [ld(q) for q in range(4)]

            def comb(x, y, sign):
                ev, od = (x[0] + y[0], x[1] + y[1]) if sign > 0 else (x[0] - y[0], x[1] - y[1])
                return pltpu.bitcast(pltpu.pack_elementwise([ev, od], packed_dtype=BF), U32)

            outs = [comb(b11, b22, 1), comb(b12, b22, -1), comb(b21, b11, -1), comb(b11, b12, 1), comb(b21, b22, 1)]
            for j in range(5):
                st16(j, r, n0, outs[j])
            t = outs[0]
            if n_eup is not None:
                t = (t ^ outs[1]) ^ (outs[2] ^ outs[3]) ^ outs[4]
            tok = pltpu.bitcast(t, F32)
        return tok

    def build_qkv(sec, kl, kr, bh, n_eup):
        rb = bh * (HD // 2)

        def row(r, m):
            return rb + r if isinstance(rb, int) else pl.multiple_of(rb + r, m)

        def ld8(q, r, n):
            return wqkv[kl if q in (0, 2) else kr, pl.ds(row((HD if q >= 2 else 0) + r, 16), 16), n:n + 128]

        def st16(j, r, n, val):
            cq[sec, bh, j, r // 2:r // 2 + 8, n:n + 128] = val

        build_tiles(ld8, st16, [(r, n) for r in range(0, HD // 2, 16) for n in range(0, WC, 128)],
                    jnp.zeros((8, 128), F32), n_eup)

    def wo_part(t):
        def ld16(q, r, n):
            return wo[q // 2, t, r:r + 16, pl.ds((HD if q % 2 else 0) + n, 128)]

        def st16(j, r, n, val):
            cwo[t, j, r // 2:r // 2 + 8, n:n + 128] = val

        return [(ld16, st16, (r, n)) for r in range(0, HD // NWP, 16) for n in range(0, HD, 128)]

    @pl.when(s == 0)
    def _():
        def issue_x(b, carry):
            x_copy(b).start(priority=1)
            return carry

        lax.fori_loop(0, 2, issue_x, 0)

        def issue_w(j, carry):
            @pl.when(j == 1)
            def _():
                x_copy(2).start(priority=1)

            wqkv_copy(lax.rem(j + 2, NWC)).start(priority=1)
            return carry

        lax.fori_loop(0, NWC, issue_w, 0)

        def issue_rest(j, carry):
            for cp in raw_copies(0):
                cp.start(priority=1)
            return carry

        lax.fori_loop(0, jnp.maximum(s, 1), issue_rest, 0)
        wo_copy().start(priority=1)
        x_copy(3).start(priority=1)
        k_scr[:, 0:HALO, :] = jnp.zeros((NG, HALO, 128), F32)
        v_scr[:, 0:HALO, :] = jnp.zeros((NG, HALO, 128), F32)
        x_copy(0).wait()
        ln_block(0)
        x_copy(1).wait()
        ln_block(1)
        P0 = R0 // 2
        xn = _as_bf16(xn_scr[0:P0, :])

        def body(j, carry):
            k = lax.rem(j + 2, NWC)
            wqkv_copy(k).wait()

            @pl.when(j == 1)
            def _():
                x_copy(2).wait()

            y = _dot(xn, wqkv[k])
            half = lax.rem(j, 2)
            sec = jnp.maximum(lax.div(j, 2) - 1, 0)
            src = pl.multiple_of((sec + 1) * P0 + half * (P0 // 2), 8)
            dstr = pl.multiple_of(HALO + half * P0, 16)
            for r in range(0, P0 // 2, 8):
                vs = _butterfly([q_scr[g, pl.ds(src + r, 8), :] for g in range(NG)])
                for g in range(NG):
                    kv_scr[sec, g, pl.ds(dstr + 2 * r, 16), :] = _unpack(vs[g])
            lb = jnp.minimum(j + 1, 2)
            u0 = 2 * jnp.clip(j - 1, 0, 3)
            tok = ln_unit(lb, pl.multiple_of(u0 * 16, 16), None)
            ln_unit(lb, pl.multiple_of(u0 * 16 + 16, 16), tok)
            jm = jnp.maximum(j - 1, 0)
            bsec = lax.div(jm, 2)
            kl = lax.rem(2 * bsec + 2, NWC)
            kr = jnp.where(j == 0, kl, kl + 1)
            bh = jnp.where(j == 0, 1, lax.rem(jm, 2))
            build_qkv(bsec, kl, kr, bh, N_EUP0)
            rb = pl.multiple_of(lax.rem(lax.div(j, 2) + 1, 3) * P0, 8)
            for gg in range(WC // 128):
                q_scr[half * (WC // 128) + gg, pl.ds(rb, P0), :] = _pack(y[:, gg * 128:(gg + 1) * 128])
            return carry

        lax.fori_loop(0, NWC, body, 0)
        build_qkv(2, 0, 1, 1, None)
        wo_copy().wait()
        for ld16, st16, pos in wo_part(NWP - 1):
            build_tiles(ld16, st16, [pos], jnp.zeros((8, 128), F32), None)

    @pl.when(s <= NA)
    def _():
        @pl.when(s + 1 < NCH)
        def _():
            for cp in raw_copies(s + 1):
                cp.start(priority=1)

        @pl.when(s + 4 < NB)
        def _():
            x_copy(s + 4).start(priority=1)

        @pl.when(s >= 1)
        def _():
            for cp in raw_copies(s - 1):
                cp.wait()

        @pl.when(jnp.logical_and(s >= 1, s + 2 < NB))
        def _():
            x_copy(s + 2).wait()

    @pl.when(jnp.logical_and(s >= 1, s <= NA))
    def _():
        c = lax.rem(s + (NA - 1), NA)
        r0 = pl.multiple_of(R0 + (s - 1) * TA, 16)
        HA = TA // 2
        pt = pl.multiple_of(r0 // 2, 8)
        pb = pl.multiple_of((r0 + HA) // 2, 8)
        a11 = _as_bf16(xn_scr[pl.ds(pt, HA // 2), 0:HD])
        a12 = _as_bf16(xn_scr[pl.ds(pt, HA // 2), HD:D])
        a21 = _as_bf16(xn_scr[pl.ds(pb, HA // 2), 0:HD])
        a22 = _as_bf16(xn_scr[pl.ds(pb, HA // 2), HD:D])
        la = [t.astype(BF) for t in _lhs_combos(a11.astype(F32), a12.astype(F32), a21.astype(F32), a22.astype(F32))]
        la[2], la[3] = a11, a22

        def ffn_part(raw, cmb, kq, nq):
            def ld8(q, r, n):
                return raw[c, pl.ds((kq if q >= 2 else 0) + r, 16), pl.ds((nq if q % 2 else 0) + n, 128)]

            def st16(j, r, n, val):
                cmb[c, j, r // 2:r // 2 + 8, n:n + 128] = val

            return [(ld8, st16, (r, n)) for r in range(0, kq, 16) for n in range(0, nq, 128)]

        work = ffn_part(rawg, cg, HD, FC) + ffn_part(rawu, cu, HD, FC) + ffn_part(rawd, cd, FC, HD) + wo_part(c)
        def stores(sec):
            for h in range(2):
                rh = pl.multiple_of(r0 + h * HA, 16)
                if sec == 2:
                    store_q(ys[2][h], rh)
                else:
                    store_kv(ys[sec][h], k_scr if sec == 0 else v_scr, rh)

        ys = []
        for sec in range(3):
            kl = (2 * sec + 2) % NWC
            cw = [_as_bf16(jnp.concatenate([cq[sec, 0, j], cq[sec, 1, j]], axis=0)) for j in range(5)]
            wl = [cw[0], wqkv[kl, 0:HD, :], cw[1], cw[2], wqkv[kl + 1, HD:D, :], cw[3], cw[4]]
            parts = [_strassen_out([_dot(la[j], wl[j][:, n:n + QN]) for j in range(7)]) for n in range(0, WC, QN)]
            c11, c12, c21, c22 = [jnp.concatenate([p[t] for p in parts], axis=1) for t in range(4)]
            ys.append((jnp.concatenate([c11, c12], axis=1), jnp.concatenate([c21, c22], axis=1)))
            stores(sec)
        ln_block(jnp.minimum(s + 2, NB - 1), chain=True)
        tok = jnp.zeros((8, 128), F32)
        for ld8, st16, pos in work:
            tok = build_tiles(ld8, st16, [pos], tok, N_EUP)

    @pl.when(s > NA)
    def _():
        i = lax.rem(s + (NB - NA - 1), NB)
        r0 = pl.multiple_of(i * TM, TM)

        def wlist(raw, cmb, c, kq, nq):
            cw = [_as_bf16(cmb[c, j]) for j in range(5)]
            return [cw[0], raw[c, 0:kq, 0:nq], cw[1], cw[2], raw[c, kq:2 * kq, nq:2 * nq], cw[3], cw[4]]

        RA = 16
        cexp = (DH ** -0.5) * LOG2E
        p0 = pl.multiple_of(r0 // 2, 8)

        def attn_half(q, r):
            sw = []
            for w in range(WIN):
                acc = None
                for g in range(NG):
                    t = q[g] * k_scr[g, pl.ds(r0 + r + HALO - DIL * w, 8), :]
                    acc = t if acc is None else acc + t
                acc = _sum4(acc)
                if r < HALO and w > 0:
                    row = lax.broadcasted_iota(jnp.int32, (8, 128), 0) + (r0 + r)
                    acc = jnp.where(row >= DIL * w, acc, NEG)
                sw.append(acc)
            m = sw[0]
            for w in range(1, WIN):
                m = jnp.maximum(m, sw[w])
            e = [jnp.exp2((sw[w] - m) * cexp) for w in range(WIN)]
            den = e[0]
            for w in range(1, WIN):
                den = den + e[w]
            inv = 1.0 / den
            p = [e[w] * inv for w in range(WIN)]
            o = []
            for g in range(NG):
                acc = None
                for w in range(WIN):
                    t = p[w] * v_scr[g, pl.ds(r0 + r + HALO - DIL * w, 8), :]
                    acc = t if acc is None else acc + t
                o.append(acc)
            return o

        prev_fin = [None]

        def attn_rows(r, tok):
            qp = [q_scr[g, pl.ds(p0 + r // 2, 8), :] for g in range(NG)]
            if tok is not None:
                qp = [_dep32(t, tok, never) for t in qp]
            q = [_unpack(t) for t in _butterfly(qp)]
            o0 = attn_half([t[0:8] for t in q], r)
            q1 = [t[8:16] for t in q]
            q1 = [_dep32(t, o0[NG - 1], never) for t in q1]
            o1 = attn_half(q1, r + 8)
            o = _butterfly([_pack(jnp.concatenate([o0[g], o1[g]], axis=0)) for g in range(NG)])
            for g in range(NG):
                o_scr[r // 2:r // 2 + 8, g * 128:(g + 1) * 128] = o[g]
            fin = o[0]
            for g in range(1, NG):
                fin = fin ^ o[g]
            tok = o[0]
            if prev_fin[0] is not None:
                tok = tok ^ prev_fin[0]
            prev_fin[0] = fin
            return tok

        sl = [_as_bf16(s_scr[i, j]) for j in range(7)]
        acc = [None] * 7
        n_att = TM // RA
        per = 3
        tok = None
        pend = []
        for c in range(NCH):
            wg_l = wlist(rawg, cg, c, HD, FC)
            wu_l = wlist(rawu, cu, c, HD, FC)
            wd_l = wlist(rawd, cd, c, FC, HD)
            g = _strassen_out([_dot(sl[j], wg_l[j]) for j in range(7)])
            u = _strassen_out([_dot(sl[j], wu_l[j]) for j in range(7)])
            hq = [g[t] * u[t] for t in range(4)]
            pend.append(([t.astype(BF) for t in _lhs_combos(*hq)], wd_l))
            if len(pend) == DOWN_GROUP or c == NCH - 1:
                for j in range(7):
                    y = _dot(jnp.concatenate([p[0][j] for p in pend], axis=1),
                             jnp.concatenate([p[1][j] for p in pend], axis=0))
                    acc[j] = y if acc[j] is None else acc[j] + y
                pend = []
            for a in range(c * per, min((c + 1) * per, n_att)):
                tok = attn_rows(a * RA, tok)
            if c == NCH - 1:
                oq = [_as_bf16(o_scr[rr:rr + HM // 2, cc:cc + HD]) for rr in (0, HM // 2) for cc in (0, HD)]
                ol = [t.astype(BF) for t in _lhs_combos(*[t.astype(F32) for t in oq])]
                ol[2], ol[3] = oq[0], oq[3]
                cw = [_as_bf16(jnp.concatenate([cwo[t, j] for t in range(NWP)], axis=0)) for j in range(5)]
                b11 = jnp.concatenate([wo[0, t, :, 0:HD] for t in range(NWP)], axis=0)
                b22 = jnp.concatenate([wo[1, t, :, HD:D] for t in range(NWP)], axis=0)
                wo_l = [cw[0], b11, cw[1], cw[2], b22, cw[3], cw[4]]
                acc = [acc[j] + _dot(ol[j], wo_l[j]) for j in range(7)]
        ys = _strassen_out(acc)
        x = x_scr[pl.ds(r0, TM), :].astype(F32)
        for q in range(4):
            rr, cc = (q // 2) * HM, (q % 2) * HD
            o_ref[rr:rr + HM, cc:cc + HD] = (x[rr:rr + HM, cc:cc + HD] + ys[q]).astype(o_ref.dtype)


@jax.jit
def pallas_parallel_sum__sliding_local_dilated__glu_gated_bilinear__prompt_kernel(
    A_x: jax.Array,
    A_wqkv: jax.Array,
    A_wo: jax.Array,
    B_x: jax.Array,
    B_w_gate: jax.Array,
    B_w_up: jax.Array,
    B_w_down: jax.Array,
):
    del B_x
    x = A_x.reshape(S, D)
    hbm = pl.BlockSpec(memory_space=pl.ANY)
    out = pl.pallas_call(
        _kernel,
        grid=(NSTEPS,),
        in_specs=[hbm] * 6,
        out_specs=pl.BlockSpec((TM, D), lambda s: (jnp.maximum(s - (NA + 1), 0), 0)),
        out_shape=jax.ShapeDtypeStruct((S, D), A_x.dtype),
        scratch_shapes=[
            pltpu.VMEM((S, D), BF),
            pltpu.VMEM((NWC, D, WC), BF),
            pltpu.VMEM((2, NWP, HD // NWP, D), BF),
            pltpu.VMEM((NCH, D, 2 * FC), BF),
            pltpu.VMEM((NCH, D, 2 * FC), BF),
            pltpu.VMEM((NCH, 2 * FC, D), BF),
            pltpu.VMEM((3, 2, 5, HD // 4, WC), U32),
            pltpu.VMEM((NWP, 5, HD // NWP // 2, HD), U32),
            pltpu.VMEM((NCH, 5, HD // 2, FC), U32),
            pltpu.VMEM((NCH, 5, HD // 2, FC), U32),
            pltpu.VMEM((NCH, 5, FC // 2, HD), U32),
            pltpu.VMEM((S // 2, D), U32),
            pltpu.VMEM((NB, 7, HM // 2, HD), U32),
            pltpu.VMEM((NG, S // 2, 128), U32),
            pltpu.VMEM((2, NG, S + HALO, 128), F32),
            pltpu.VMEM((TM // 2, D), U32),
            pltpu.SemaphoreType.DMA((NB,)),
            pltpu.SemaphoreType.DMA((NWC + 1,)),
            pltpu.SemaphoreType.DMA((NCH, 6)),
        ],
        compiler_params=pltpu.CompilerParams(
            dimension_semantics=("arbitrary",),
            vmem_limit_bytes=124 * 1024 * 1024,
            disable_bounds_checks=True,
        ),
        name="fused_attn_ffn",
    )(x, A_wqkv, A_wo.reshape(2, NWP, HD // NWP, D), B_w_gate, B_w_up, B_w_down)
    return out.reshape(A_x.shape)
```

```python
import jax
import jax.numpy as jnp
from jax import lax
from jax.experimental import pallas as pl
from jax.experimental.pallas import tpu as pltpu

S, D, F = 2048, 1024, 3584
DH, WIN, DIL = 32, 8, 2
TM = 256
HM = TM // 2
NB = S // TM
HD = D // 2
FC = 256
NCH = F // 2 // FC
HALO = 16
NG = D // 128
EPS = 1e-5
NEG = -1e9
BF = jnp.bfloat16
F32 = jnp.float32
U32 = jnp.uint32
LOG2E = 1.4426950408889634
NA = 7
TA = 224
R0 = S - NA * TA
NSTEPS = 1 + NA + NB
NWP = 8
WC = 512
NWC = 3 * D // WC
N_EUP = 3
N_EUP0 = 2
QN = 128
DOWN_GROUP = 4

def _dot(a, b):
    return jnp.dot(a, b, preferred_element_type=F32)


def _butterfly(vs):
    lane = lax.broadcasted_iota(jnp.int32, vs[0].shape, 1)
    for b in range(3):
        sh = 4 << b
        bit = (lane & sh) != 0
        new = list(vs)
        for i0 in range(NG):
            if i0 & (1 << b):
                continue
            i1 = i0 | (1 << b)
            new[i0] = jnp.where(bit, pltpu.roll(vs[i1], sh, 1), vs[i0])
            new[i1] = jnp.where(bit, vs[i1], pltpu.roll(vs[i0], 128 - sh, 1))
        vs = new
    return vs


def _sum4(x):
    lane = lax.broadcasted_iota(jnp.int32, x.shape, 1)
    x = x + jnp.where((lane & 1) != 0, pltpu.roll(x, 1, 1), pltpu.roll(x, 127, 1))
    x = x + jnp.where((lane & 2) != 0, pltpu.roll(x, 2, 1), pltpu.roll(x, 126, 1))
    return x


def _dep32(x, tok, never):
    return jnp.where(never, pltpu.bitcast(tok, x.dtype), x)


def _gate(m, tok, never):
    t = pltpu.bitcast(m[0:16, 0:128], F32)
    t = pltpu.bitcast(_dep32(t, tok, never), BF)
    top = jnp.concatenate([t, m[0:16, 128:]], axis=1)
    if m.shape[0] == 16:
        return top
    return jnp.concatenate([top, m[16:]], axis=0)


def _pack(y):
    return pltpu.bitcast(y.astype(BF), U32)


def _as_bf16(w):
    return pltpu.bitcast(w, BF)


def _unpack(w):
    return pltpu.bitcast(w, BF).astype(F32)


def _lhs_combos(a11, a12, a21, a22):
    return [a11 + a22, a21 + a22, a11, a22, a11 + a12, a21 - a11, a12 - a22]


def _strassen_out(m):
    return (m[0] + m[3] - m[4] + m[6], m[2] + m[4], m[1] + m[3], m[0] - m[1] + m[2] + m[5])


def _layernorm(x):
    x = x.astype(F32)
    mean = jnp.mean(x, axis=-1, keepdims=True)
    xc = x - mean
    var = jnp.mean(xc * xc, axis=-1, keepdims=True)
    return xc * lax.rsqrt(var + EPS)


def _kernel(x_hbm, wqkv_hbm, wo_hbm, wg_hbm, wu_hbm, wd_hbm, o_ref,
            x_scr, wqkv, wo, rawg, rawu, rawd, cq, cwo, cg, cu, cd,
            xn_scr, s_scr, q_scr, kv_scr, o_scr,
            sem_x, sem_w, sem_raw):
    s = pl.program_id(0)
    k_scr = kv_scr.at[0]
    v_scr = kv_scr.at[1]

    def x_copy(b):
        return pltpu.make_async_copy(x_hbm.at[pl.ds(b * TM, TM), :], x_scr.at[pl.ds(b * TM, TM), :], sem_x.at[b])

    def wqkv_copy(k):
        return pltpu.make_async_copy(wqkv_hbm.at[:, pl.ds(k * WC, WC)], wqkv.at[k], sem_w.at[k])

    def wo_copy():
        return pltpu.make_async_copy(wo_hbm, wo, sem_w.at[NWC])

    def raw_copies(c):
        return [
            pltpu.make_async_copy(wg_hbm.at[:, pl.ds(c * FC, FC)], rawg.at[c, :, pl.ds(0, FC)], sem_raw.at[c, 0]),
            pltpu.make_async_copy(wg_hbm.at[:, pl.ds(F // 2 + c * FC, FC)], rawg.at[c, :, pl.ds(FC, FC)], sem_raw.at[c, 1]),
            pltpu.make_async_copy(wu_hbm.at[:, pl.ds(c * FC, FC)], rawu.at[c, :, pl.ds(0, FC)], sem_raw.at[c, 2]),
            pltpu.make_async_copy(wu_hbm.at[:, pl.ds(F // 2 + c * FC, FC)], rawu.at[c, :, pl.ds(FC, FC)], sem_raw.at[c, 3]),
            pltpu.make_async_copy(wd_hbm.at[pl.ds(c * FC, FC), :], rawd.at[c, pl.ds(0, FC), :], sem_raw.at[c, 4]),
            pltpu.make_async_copy(wd_hbm.at[pl.ds(F // 2 + c * FC, FC), :], rawd.at[c, pl.ds(FC, FC), :], sem_raw.at[c, 5]),
        ]

    never = lax.broadcasted_iota(jnp.int32, (8, 128), 0) < jnp.minimum(s, 0)

    def ln_unit(b, r, tok):
        RC = 16
        r0 = pl.multiple_of(b * TM + r, RC)
        xt = x_scr[pl.ds(r0, RC), :]
        if tok is not None:
            xt = _gate(xt, tok, never)
        y = _layernorm(xt)
        xn_scr[pl.ds(pl.multiple_of(r0 // 2, RC // 2), RC // 2), :] = _pack(y)
        return y[0:8, 0:128]

    def ln_block(b, chain=False):
        tok = None
        for r in range(0, TM, 16):
            t = ln_unit(b, r, tok)
            tok = t if chain else None
        return tok

    def s_block(b, tok):
        p0 = b * (TM // 2)
        for r in range(0, HM // 2, 8):
            for n in range(0, HD, 128):
                def ld(half, cc):
                    w = xn_scr[pl.ds(pl.multiple_of(p0 + half * (HM // 2) + r, 8), 8), cc + n:cc + n + 128]
                    if tok is not None:
                        w = _dep32(w, tok, never)
                    return (pltpu.bitcast(w << 16, F32), pltpu.bitcast(w & jnp.uint32(0xFFFF0000), F32))

                a11, a12, a21, a22 = ld(0, 0), ld(0, HD), ld(1, 0), ld(1, HD)

                def comb(x, y, sign):
                    ev, od = (x[0] + y[0], x[1] + y[1]) if sign > 0 else (x[0] - y[0], x[1] - y[1])
                    return pltpu.bitcast(pltpu.pack_elementwise([ev, od], packed_dtype=BF), U32)

                outs = [comb(a11, a22, 1), comb(a21, a22, 1), comb(a11, a12, 1), comb(a21, a11, -1), comb(a12, a22, -1)]
                for j in range(5):
                    s_scr[b, j, r:r + 8, n:n + 128] = outs[j]
                if tok is not None:
                    t = (outs[0] ^ outs[1]) ^ (outs[2] ^ outs[3]) ^ outs[4]
                    tok = jnp.exp2(pltpu.bitcast(t, F32))
        return tok

    def store_kv(y, dst, r0):
        prev = None
        for r in range(0, y.shape[0], 16):
            ws = [_pack(y[r:r + 16, g * 128:(g + 1) * 128]) for g in range(NG)]
            if prev is not None:
                ws = [_dep32(w, prev, never) for w in ws]
            vs = _butterfly(ws)
            prev = vs[0]
            for g in range(NG):
                dst[g, pl.ds(r0 + HALO + r, 16), :] = _unpack(vs[g])

    def store_q(y, r0):
        p0 = pl.multiple_of(r0 // 2, 8)
        for g in range(NG):
            q_scr[g, pl.ds(p0, y.shape[0] // 2), :] = _pack(y[:, g * 128:(g + 1) * 128])

    def build_tiles(ld16, st16, positions, tok, n_eup):
        for r, n0 in positions:
            for _ in range(n_eup or 0):
                tok = jnp.exp2(tok)

            def ld(q):
                w = pltpu.bitcast(ld16(q, r, n0), U32)
                if n_eup is not None:
                    w = _dep32(w, tok, never)
                return (pltpu.bitcast(w << 16, F32), pltpu.bitcast(w & jnp.uint32(0xFFFF0000), F32))

            b11, b12, b21, b22 = [ld(q) for q in range(4)]

            def comb(x, y, sign):
                ev, od = (x[0] + y[0], x[1] + y[1]) if sign > 0 else (x[0] - y[0], x[1] - y[1])
                return pltpu.bitcast(pltpu.pack_elementwise([ev, od], packed_dtype=BF), U32)

            outs = [comb(b11, b22, 1), comb(b12, b22, -1), comb(b21, b11, -1), comb(b11, b12, 1), comb(b21, b22, 1)]
            for j in range(5):
                st16(j, r, n0, outs[j])
            t = outs[0]
            if n_eup is not None:
                t = (t ^ outs[1]) ^ (outs[2] ^ outs[3]) ^ outs[4]
            tok = pltpu.bitcast(t, F32)
        return tok

    def build_qkv(sec, kl, kr, bh, n_eup):
        rb = bh * (HD // 2)

        def row(r, m):
            return rb + r if isinstance(rb, int) else pl.multiple_of(rb + r, m)

        def ld8(q, r, n):
            return wqkv[kl if q in (0, 2) else kr, pl.ds(row((HD if q >= 2 else 0) + r, 16), 16), n:n + 128]

        def st16(j, r, n, val):
            cq[sec, bh, j, r // 2:r // 2 + 8, n:n + 128] = val

        build_tiles(ld8, st16, [(r, n) for r in range(0, HD // 2, 16) for n in range(0, WC, 128)],
                    jnp.zeros((8, 128), F32), n_eup)

    def wo_part(t):
        def ld16(q, r, n):
            return wo[q // 2, t, r:r + 16, pl.ds((HD if q % 2 else 0) + n, 128)]

        def st16(j, r, n, val):
            cwo[t, j, r // 2:r // 2 + 8, n:n + 128] = val

        return [(ld16, st16, (r, n)) for r in range(0, HD // NWP, 16) for n in range(0, HD, 128)]

    @pl.when(s == 0)
    def _():
        def issue_x(b, carry):
            x_copy(b).start(priority=1)
            return carry

        lax.fori_loop(0, 2, issue_x, 0)

        def issue_w(j, carry):
            @pl.when(j == 1)
            def _():
                x_copy(2).start(priority=1)

            wqkv_copy(lax.rem(j + 2, NWC)).start(priority=1)
            return carry

        lax.fori_loop(0, NWC, issue_w, 0)

        def issue_rest(j, carry):
            for cp in raw_copies(0):
                cp.start(priority=1)
            return carry

        lax.fori_loop(0, jnp.maximum(s, 1), issue_rest, 0)
        wo_copy().start(priority=1)
        x_copy(3).start(priority=1)
        k_scr[:, 0:HALO, :] = jnp.zeros((NG, HALO, 128), F32)
        v_scr[:, 0:HALO, :] = jnp.zeros((NG, HALO, 128), F32)
        x_copy(0).wait()
        ln_block(0)
        x_copy(1).wait()
        ln_block(1)
        s_block(0, None)
        P0 = R0 // 2
        xn = _as_bf16(xn_scr[0:P0, :])

        def body(j, carry):
            k = lax.rem(j + 2, NWC)
            wqkv_copy(k).wait()

            @pl.when(j == 1)
            def _():
                x_copy(2).wait()

            y = _dot(xn, wqkv[k])
            half = lax.rem(j, 2)
            sec = jnp.maximum(lax.div(j, 2) - 1, 0)
            src = pl.multiple_of((sec + 1) * P0 + half * (P0 // 2), 8)
            dstr = pl.multiple_of(HALO + half * P0, 16)
            for r in range(0, P0 // 2, 8):
                vs = _butterfly([q_scr[g, pl.ds(src + r, 8), :] for g in range(NG)])
                for g in range(NG):
                    kv_scr[sec, g, pl.ds(dstr + 2 * r, 16), :] = _unpack(vs[g])
            lb = jnp.minimum(j + 1, 2)
            u0 = 2 * jnp.clip(j - 1, 0, 3)
            for k4 in range(4):
                ln_unit(lb, pl.multiple_of(u0 * 32 + 16 * k4, 16), None)
            jm = jnp.maximum(j - 1, 0)
            bsec = lax.div(jm, 2)
            kl = lax.rem(2 * bsec + 2, NWC)
            kr = jnp.where(j == 0, kl, kl + 1)
            bh = jnp.where(j == 0, 1, lax.rem(jm, 2))
            build_qkv(bsec, kl, kr, bh, N_EUP0)
            rb = pl.multiple_of(lax.rem(lax.div(j, 2) + 1, 3) * P0, 8)
            for gg in range(WC // 128):
                q_scr[half * (WC // 128) + gg, pl.ds(rb, P0), :] = _pack(y[:, gg * 128:(gg + 1) * 128])
            return carry

        lax.fori_loop(0, NWC, body, 0)
        build_qkv(2, 0, 1, 1, None)
        wo_copy().wait()
        for ld16, st16, pos in wo_part(NWP - 1):
            build_tiles(ld16, st16, [pos], jnp.zeros((8, 128), F32), None)

    @pl.when(s <= NA)
    def _():
        @pl.when(s + 1 < NCH)
        def _():
            for cp in raw_copies(s + 1):
                cp.start(priority=1)

        @pl.when(s + 4 < NB)
        def _():
            x_copy(s + 4).start(priority=1)

        @pl.when(s >= 1)
        def _():
            for cp in raw_copies(s - 1):
                cp.wait()

        @pl.when(jnp.logical_and(s >= 1, s + 2 < NB))
        def _():
            x_copy(s + 2).wait()

    @pl.when(jnp.logical_and(s >= 1, s <= NA))
    def _():
        c = lax.rem(s + (NA - 1), NA)
        r0 = pl.multiple_of(R0 + (s - 1) * TA, 16)
        HA = TA // 2
        pt = pl.multiple_of(r0 // 2, 8)
        pb = pl.multiple_of((r0 + HA) // 2, 8)
        a11 = _as_bf16(xn_scr[pl.ds(pt, HA // 2), 0:HD])
        a12 = _as_bf16(xn_scr[pl.ds(pt, HA // 2), HD:D])
        a21 = _as_bf16(xn_scr[pl.ds(pb, HA // 2), 0:HD])
        a22 = _as_bf16(xn_scr[pl.ds(pb, HA // 2), HD:D])
        la = [t.astype(BF) for t in _lhs_combos(a11.astype(F32), a12.astype(F32), a21.astype(F32), a22.astype(F32))]
        la[2], la[3] = a11, a22

        def ffn_part(raw, cmb, kq, nq):
            def ld8(q, r, n):
                return raw[c, pl.ds((kq if q >= 2 else 0) + r, 16), pl.ds((nq if q % 2 else 0) + n, 128)]

            def st16(j, r, n, val):
                cmb[c, j, r // 2:r // 2 + 8, n:n + 128] = val

            return [(ld8, st16, (r, n)) for r in range(0, kq, 16) for n in range(0, nq, 128)]

        work = ffn_part(rawg, cg, HD, FC) + ffn_part(rawu, cu, HD, FC) + ffn_part(rawd, cd, FC, HD) + wo_part(c)
        def stores(sec):
            for h in range(2):
                rh = pl.multiple_of(r0 + h * HA, 16)
                if sec == 2:
                    store_q(ys[2][h], rh)
                else:
                    store_kv(ys[sec][h], k_scr if sec == 0 else v_scr, rh)

        ys = []
        for sec in range(3):
            kl = (2 * sec + 2) % NWC
            cw = [_as_bf16(jnp.concatenate([cq[sec, 0, j], cq[sec, 1, j]], axis=0)) for j in range(5)]
            wl = [cw[0], wqkv[kl, 0:HD, :], cw[1], cw[2], wqkv[kl + 1, HD:D, :], cw[3], cw[4]]
            parts = [_strassen_out([_dot(la[j], wl[j][:, n:n + QN]) for j in range(7)]) for n in range(0, WC, QN)]
            c11, c12, c21, c22 = [jnp.concatenate([p[t] for p in parts], axis=1) for t in range(4)]
            ys.append((jnp.concatenate([c11, c12], axis=1), jnp.concatenate([c21, c22], axis=1)))
            stores(sec)
        ln_block(jnp.minimum(s + 2, NB - 1), chain=True)
        tok = jnp.zeros((8, 128), F32)
        for ld8, st16, pos in work:
            tok = build_tiles(ld8, st16, [pos], tok, N_EUP)

    @pl.when(s > NA)
    def _():
        i = lax.rem(s + (NB - NA - 1), NB)
        r0 = pl.multiple_of(i * TM, TM)

        def wlist(raw, cmb, c, kq, nq):
            cw = [_as_bf16(cmb[c, j]) for j in range(5)]
            return [cw[0], raw[c, 0:kq, 0:nq], cw[1], cw[2], raw[c, kq:2 * kq, nq:2 * nq], cw[3], cw[4]]

        RA = 16
        cexp = (DH ** -0.5) * LOG2E
        p0 = pl.multiple_of(r0 // 2, 8)

        def attn_half(q, r):
            sw = []
            for w in range(WIN):
                acc = None
                for g in range(NG):
                    t = q[g] * k_scr[g, pl.ds(r0 + r + HALO - DIL * w, 8), :]
                    acc = t if acc is None else acc + t
                acc = _sum4(acc)
                if r < HALO and w > 0:
                    row = lax.broadcasted_iota(jnp.int32, (8, 128), 0) + (r0 + r)
                    acc = jnp.where(row >= DIL * w, acc, NEG)
                sw.append(acc)
            m = sw[0]
            for w in range(1, WIN):
                m = jnp.maximum(m, sw[w])
            e = [jnp.exp2((sw[w] - m) * cexp) for w in range(WIN)]
            den = e[0]
            for w in range(1, WIN):
                den = den + e[w]
            inv = 1.0 / den
            p = [e[w] * inv for w in range(WIN)]
            o = []
            for g in range(NG):
                acc = None
                for w in range(WIN):
                    t = p[w] * v_scr[g, pl.ds(r0 + r + HALO - DIL * w, 8), :]
                    acc = t if acc is None else acc + t
                o.append(acc)
            return o

        prev_fin = [None]

        def attn_rows(r, tok):
            qp = [q_scr[g, pl.ds(p0 + r // 2, 8), :] for g in range(NG)]
            if tok is not None:
                qp = [_dep32(t, tok, never) for t in qp]
            q = [_unpack(t) for t in _butterfly(qp)]
            o0 = attn_half([t[0:8] for t in q], r)
            q1 = [t[8:16] for t in q]
            q1 = [_dep32(t, o0[NG - 1], never) for t in q1]
            o1 = attn_half(q1, r + 8)
            o = _butterfly([_pack(jnp.concatenate([o0[g], o1[g]], axis=0)) for g in range(NG)])
            for g in range(NG):
                o_scr[r // 2:r // 2 + 8, g * 128:(g + 1) * 128] = o[g]
            fin = o[0]
            for g in range(1, NG):
                fin = fin ^ o[g]
            tok = o[0]
            if prev_fin[0] is not None:
                tok = tok ^ prev_fin[0]
            prev_fin[0] = fin
            return tok

        s5 = [_as_bf16(s_scr[i, j]) for j in range(5)]
        xa11 = _as_bf16(xn_scr[pl.ds(p0, HM // 2), 0:HD])
        xa22 = _as_bf16(xn_scr[pl.ds(pl.multiple_of(p0 + HM // 2, 8), HM // 2), HD:D])
        sl = [s5[0], s5[1], xa11, xa22, s5[2], s5[3], s5[4]]
        s_block(jnp.minimum(i + 1, NB - 1), jnp.zeros((8, 128), F32))
        acc = [None] * 7
        n_att = TM // RA
        per = 3
        tok = None
        pend = []
        for c in range(NCH):
            wg_l = wlist(rawg, cg, c, HD, FC)
            wu_l = wlist(rawu, cu, c, HD, FC)
            wd_l = wlist(rawd, cd, c, FC, HD)
            g = _strassen_out([_dot(sl[j], wg_l[j]) for j in range(7)])
            u = _strassen_out([_dot(sl[j], wu_l[j]) for j in range(7)])
            hq = [g[t] * u[t] for t in range(4)]
            pend.append(([t.astype(BF) for t in _lhs_combos(*hq)], wd_l))
            if len(pend) == DOWN_GROUP or c == NCH - 1:
                for j in range(7):
                    y = _dot(jnp.concatenate([p[0][j] for p in pend], axis=1),
                             jnp.concatenate([p[1][j] for p in pend], axis=0))
                    acc[j] = y if acc[j] is None else acc[j] + y
                pend = []
            for a in range(c * per, min((c + 1) * per, n_att)):
                tok = attn_rows(a * RA, tok)
            if c == NCH - 1:
                oq = [_as_bf16(o_scr[rr:rr + HM // 2, cc:cc + HD]) for rr in (0, HM // 2) for cc in (0, HD)]
                ol = [t.astype(BF) for t in _lhs_combos(*[t.astype(F32) for t in oq])]
                ol[2], ol[3] = oq[0], oq[3]
                cw = [_as_bf16(jnp.concatenate([cwo[t, j] for t in range(NWP)], axis=0)) for j in range(5)]
                b11 = jnp.concatenate([wo[0, t, :, 0:HD] for t in range(NWP)], axis=0)
                b22 = jnp.concatenate([wo[1, t, :, HD:D] for t in range(NWP)], axis=0)
                wo_l = [cw[0], b11, cw[1], cw[2], b22, cw[3], cw[4]]
                acc = [acc[j] + _dot(ol[j], wo_l[j]) for j in range(7)]
        ys = _strassen_out(acc)
        x = x_scr[pl.ds(r0, TM), :].astype(F32)
        for q in range(4):
            rr, cc = (q // 2) * HM, (q % 2) * HD
            o_ref[rr:rr + HM, cc:cc + HD] = (x[rr:rr + HM, cc:cc + HD] + ys[q]).astype(o_ref.dtype)


@jax.jit
def pallas_parallel_sum__sliding_local_dilated__glu_gated_bilinear__prompt_kernel(
    A_x: jax.Array,
    A_wqkv: jax.Array,
    A_wo: jax.Array,
    B_x: jax.Array,
    B_w_gate: jax.Array,
    B_w_up: jax.Array,
    B_w_down: jax.Array,
):
    del B_x
    x = A_x.reshape(S, D)
    hbm = pl.BlockSpec(memory_space=pl.ANY)
    out = pl.pallas_call(
        _kernel,
        grid=(NSTEPS,),
        in_specs=[hbm] * 6,
        out_specs=pl.BlockSpec((TM, D), lambda s: (jnp.maximum(s - (NA + 1), 0), 0)),
        out_shape=jax.ShapeDtypeStruct((S, D), A_x.dtype),
        scratch_shapes=[
            pltpu.VMEM((S, D), BF),
            pltpu.VMEM((NWC, D, WC), BF),
            pltpu.VMEM((2, NWP, HD // NWP, D), BF),
            pltpu.VMEM((NCH, D, 2 * FC), BF),
            pltpu.VMEM((NCH, D, 2 * FC), BF),
            pltpu.VMEM((NCH, 2 * FC, D), BF),
            pltpu.VMEM((3, 2, 5, HD // 4, WC), U32),
            pltpu.VMEM((NWP, 5, HD // NWP // 2, HD), U32),
            pltpu.VMEM((NCH, 5, HD // 2, FC), U32),
            pltpu.VMEM((NCH, 5, HD // 2, FC), U32),
            pltpu.VMEM((NCH, 5, FC // 2, HD), U32),
            pltpu.VMEM((S // 2, D), U32),
            pltpu.VMEM((NB, 5, HM // 2, HD), U32),
            pltpu.VMEM((NG, S // 2, 128), U32),
            pltpu.VMEM((2, NG, S + HALO, 128), F32),
            pltpu.VMEM((TM // 2, D), U32),
            pltpu.SemaphoreType.DMA((NB,)),
            pltpu.SemaphoreType.DMA((NWC + 1,)),
            pltpu.SemaphoreType.DMA((NCH, 6)),
        ],
        compiler_params=pltpu.CompilerParams(
            dimension_semantics=("arbitrary",),
            vmem_limit_bytes=124 * 1024 * 1024,
            disable_bounds_checks=True,
        ),
        name="fused_attn_ffn",
    )(x, A_wqkv, A_wo.reshape(2, NWP, HD // NWP, D), B_w_gate, B_w_up, B_w_down)
    return out.reshape(A_x.shape)
```

```python
import jax
import jax.numpy as jnp
from jax import lax
from jax.experimental import pallas as pl
from jax.experimental.pallas import tpu as pltpu

S, D, F = 2048, 1024, 3584
DH, WIN, DIL = 32, 8, 2
TM = 256
HM = TM // 2
NB = S // TM
HD = D // 2
FC = 256
NCH = F // 2 // FC
HALO = 16
NG = D // 128
EPS = 1e-5
NEG = -1e9
BF = jnp.bfloat16
F32 = jnp.float32
U32 = jnp.uint32
LOG2E = 1.4426950408889634
NA = 7
TA = 224
R0 = S - NA * TA
NSTEPS = 1 + NA + NB
NWP = 8
WC = 512
NWC = 3 * D // WC
NSX = 4
NSR = 3
N_EUP = 3
N_EUP0 = 2
QN = 128
DOWN_GROUP = 4

def _dot(a, b):
    return jnp.dot(a, b, preferred_element_type=F32)


def _butterfly(vs):
    lane = lax.broadcasted_iota(jnp.int32, vs[0].shape, 1)
    for b in range(3):
        sh = 4 << b
        bit = (lane & sh) != 0
        new = list(vs)
        for i0 in range(NG):
            if i0 & (1 << b):
                continue
            i1 = i0 | (1 << b)
            new[i0] = jnp.where(bit, pltpu.roll(vs[i1], sh, 1), vs[i0])
            new[i1] = jnp.where(bit, vs[i1], pltpu.roll(vs[i0], 128 - sh, 1))
        vs = new
    return vs


def _sum4(x):
    lane = lax.broadcasted_iota(jnp.int32, x.shape, 1)
    x = x + jnp.where((lane & 1) != 0, pltpu.roll(x, 1, 1), pltpu.roll(x, 127, 1))
    x = x + jnp.where((lane & 2) != 0, pltpu.roll(x, 2, 1), pltpu.roll(x, 126, 1))
    return x


def _dep32(x, tok, never):
    return jnp.where(never, pltpu.bitcast(tok, x.dtype), x)


def _gate(m, tok, never):
    t = pltpu.bitcast(m[0:16, 0:128], F32)
    t = pltpu.bitcast(_dep32(t, tok, never), BF)
    top = jnp.concatenate([t, m[0:16, 128:]], axis=1)
    if m.shape[0] == 16:
        return top
    return jnp.concatenate([top, m[16:]], axis=0)


def _pack(y):
    return pltpu.bitcast(y.astype(BF), U32)


def _as_bf16(w):
    return pltpu.bitcast(w, BF)


def _unpack(w):
    return pltpu.bitcast(w, BF).astype(F32)


def _lhs_combos(a11, a12, a21, a22):
    return [a11 + a22, a21 + a22, a11, a22, a11 + a12, a21 - a11, a12 - a22]


def _strassen_out(m):
    return (m[0] + m[3] - m[4] + m[6], m[2] + m[4], m[1] + m[3], m[0] - m[1] + m[2] + m[5])


def _layernorm(x):
    x = x.astype(F32)
    mean = jnp.mean(x, axis=-1, keepdims=True)
    xc = x - mean
    var = jnp.mean(xc * xc, axis=-1, keepdims=True)
    return xc * lax.rsqrt(var + EPS)


def _kernel(x_hbm, wqkv_hbm, wo_hbm, wg_hbm, wu_hbm, wd_hbm, o_ref,
            x_scr, wqkv, wo, rawg, rawu, rawd, cq, cwo, cg, cu, cd,
            xn_scr, s_scr, q_scr, kv_scr, o_scr,
            sem_x, sem_w, sem_raw):
    s = pl.program_id(0)
    k_scr = kv_scr.at[0]
    v_scr = kv_scr.at[1]

    def x_copy(b):
        return pltpu.make_async_copy(x_hbm.at[pl.ds(b * TM, TM), :], x_scr.at[pl.ds(b * TM, TM), :], sem_x.at[lax.rem(b, NSX)])

    def wqkv_copy(k):
        return pltpu.make_async_copy(wqkv_hbm.at[:, pl.ds(k * WC, WC)], wqkv.at[k], sem_w.at[k])

    def wo_copy():
        return pltpu.make_async_copy(wo_hbm, wo, sem_w.at[NWC])

    def raw_copies(c):
        sem = sem_raw.at[lax.rem(c, NSR)]
        return [
            pltpu.make_async_copy(wg_hbm.at[:, pl.ds(c * FC, FC)], rawg.at[c, :, pl.ds(0, FC)], sem),
            pltpu.make_async_copy(wg_hbm.at[:, pl.ds(F // 2 + c * FC, FC)], rawg.at[c, :, pl.ds(FC, FC)], sem),
            pltpu.make_async_copy(wu_hbm.at[:, pl.ds(c * FC, FC)], rawu.at[c, :, pl.ds(0, FC)], sem),
            pltpu.make_async_copy(wu_hbm.at[:, pl.ds(F // 2 + c * FC, FC)], rawu.at[c, :, pl.ds(FC, FC)], sem),
            pltpu.make_async_copy(wd_hbm.at[pl.ds(c * FC, FC), :], rawd.at[c, pl.ds(0, FC), :], sem),
            pltpu.make_async_copy(wd_hbm.at[pl.ds(F // 2 + c * FC, FC), :], rawd.at[c, pl.ds(FC, FC), :], sem),
        ]

    never = lax.broadcasted_iota(jnp.int32, (8, 128), 0) < jnp.minimum(s, 0)

    def ln_unit(b, r, tok):
        RC = 16
        r0 = pl.multiple_of(b * TM + r, RC)
        xt = x_scr[pl.ds(r0, RC), :]
        if tok is not None:
            xt = _gate(xt, tok, never)
        y = _layernorm(xt)
        xn_scr[pl.ds(pl.multiple_of(r0 // 2, RC // 2), RC // 2), :] = _pack(y)
        return y[0:8, 0:128]

    def ln_block(b, chain=False):
        tok = None
        for r in range(0, TM, 16):
            t = ln_unit(b, r, tok)
            tok = t if chain else None
        return tok

    def s_block(b, tok):
        p0 = b * (TM // 2)
        for r in range(0, HM // 2, 8):
            for n in range(0, HD, 128):
                def ld(half, cc):
                    w = xn_scr[pl.ds(pl.multiple_of(p0 + half * (HM // 2) + r, 8), 8), cc + n:cc + n + 128]
                    if tok is not None:
                        w = _dep32(w, tok, never)
                    return (pltpu.bitcast(w << 16, F32), pltpu.bitcast(w & jnp.uint32(0xFFFF0000), F32))

                a11, a12, a21, a22 = ld(0, 0), ld(0, HD), ld(1, 0), ld(1, HD)

                def comb(x, y, sign):
                    ev, od = (x[0] + y[0], x[1] + y[1]) if sign > 0 else (x[0] - y[0], x[1] - y[1])
                    return pltpu.bitcast(pltpu.pack_elementwise([ev, od], packed_dtype=BF), U32)

                outs = [comb(a11, a22, 1), comb(a21, a22, 1), comb(a11, a12, 1), comb(a21, a11, -1), comb(a12, a22, -1)]
                for j in range(5):
                    s_scr[b, j, r:r + 8, n:n + 128] = outs[j]
                if tok is not None:
                    t = (outs[0] ^ outs[1]) ^ (outs[2] ^ outs[3]) ^ outs[4]
                    tok = jnp.exp2(pltpu.bitcast(t, F32))
        return tok

    def store_kv(y, dst, r0):
        prev = None
        for r in range(0, y.shape[0], 16):
            ws = [_pack(y[r:r + 16, g * 128:(g + 1) * 128]) for g in range(NG)]
            if prev is not None:
                ws = [_dep32(w, prev, never) for w in ws]
            vs = _butterfly(ws)
            prev = vs[0]
            for g in range(NG):
                dst[g, pl.ds(r0 + HALO + r, 16), :] = _unpack(vs[g])

    def store_q(y, r0):
        p0 = pl.multiple_of(r0 // 2, 8)
        for g in range(NG):
            q_scr[g, pl.ds(p0, y.shape[0] // 2), :] = _pack(y[:, g * 128:(g + 1) * 128])

    def build_tiles(ld16, st16, positions, tok, n_eup):
        for r, n0 in positions:
            for _ in range(n_eup or 0):
                tok = jnp.exp2(tok)

            def ld(q):
                w = pltpu.bitcast(ld16(q, r, n0), U32)
                if n_eup is not None:
                    w = _dep32(w, tok, never)
                return (pltpu.bitcast(w << 16, F32), pltpu.bitcast(w & jnp.uint32(0xFFFF0000), F32))

            b11, b12, b21, b22 = [ld(q) for q in range(4)]

            def comb(x, y, sign):
                ev, od = (x[0] + y[0], x[1] + y[1]) if sign > 0 else (x[0] - y[0], x[1] - y[1])
                return pltpu.bitcast(pltpu.pack_elementwise([ev, od], packed_dtype=BF), U32)

            outs = [comb(b11, b22, 1), comb(b12, b22, -1), comb(b21, b11, -1), comb(b11, b12, 1), comb(b21, b22, 1)]
            for j in range(5):
                st16(j, r, n0, outs[j])
            t = outs[0]
            if n_eup is not None:
                t = (t ^ outs[1]) ^ (outs[2] ^ outs[3]) ^ outs[4]
            tok = pltpu.bitcast(t, F32)
        return tok

    def build_qkv(sec, kl, kr, bh, n_eup):
        rb = bh * (HD // 2)

        def row(r, m):
            return rb + r if isinstance(rb, int) else pl.multiple_of(rb + r, m)

        def ld8(q, r, n):
            return wqkv[kl if q in (0, 2) else kr, pl.ds(row((HD if q >= 2 else 0) + r, 16), 16), n:n + 128]

        def st16(j, r, n, val):
            cq[sec, bh, j, r // 2:r // 2 + 8, n:n + 128] = val

        build_tiles(ld8, st16, [(r, n) for r in range(0, HD // 2, 16) for n in range(0, WC, 128)],
                    jnp.zeros((8, 128), F32), n_eup)

    def wo_part(t):
        def ld16(q, r, n):
            return wo[q // 2, t, r:r + 16, pl.ds((HD if q % 2 else 0) + n, 128)]

        def st16(j, r, n, val):
            cwo[t, j, r // 2:r // 2 + 8, n:n + 128] = val

        return [(ld16, st16, (r, n)) for r in range(0, HD // NWP, 16) for n in range(0, HD, 128)]

    @pl.when(s == 0)
    def _():
        def issue_x(b, carry):
            x_copy(b).start(priority=1)
            return carry

        lax.fori_loop(0, 2, issue_x, 0)

        def issue_w(j, carry):
            @pl.when(j == 1)
            def _():
                x_copy(2).start(priority=1)

            wqkv_copy(lax.rem(j + 2, NWC)).start(priority=1)
            return carry

        lax.fori_loop(0, NWC, issue_w, 0)

        def issue_rest(j, carry):
            for cp in raw_copies(0):
                cp.start(priority=1)
            return carry

        lax.fori_loop(0, jnp.maximum(s, 1), issue_rest, 0)
        wo_copy().start(priority=1)
        x_copy(3).start(priority=1)
        k_scr[:, 0:HALO, :] = jnp.zeros((NG, HALO, 128), F32)
        v_scr[:, 0:HALO, :] = jnp.zeros((NG, HALO, 128), F32)
        x_copy(0).wait()
        ln_block(0)
        x_copy(1).wait()
        ln_block(1)
        s_block(0, None)
        P0 = R0 // 2
        xn = _as_bf16(xn_scr[0:P0, :])

        def body(j, carry):
            k = lax.rem(j + 2, NWC)
            wqkv_copy(k).wait()

            @pl.when(j == 1)
            def _():
                x_copy(2).wait()

            y = _dot(xn, wqkv[k])
            half = lax.rem(j, 2)
            sec = jnp.maximum(lax.div(j, 2) - 1, 0)
            src = pl.multiple_of((sec + 1) * P0 + half * (P0 // 2), 8)
            dstr = pl.multiple_of(HALO + half * P0, 16)
            for r in range(0, P0 // 2, 8):
                vs = _butterfly([q_scr[g, pl.ds(src + r, 8), :] for g in range(NG)])
                for g in range(NG):
                    kv_scr[sec, g, pl.ds(dstr + 2 * r, 16), :] = _unpack(vs[g])
            lb = jnp.minimum(j + 1, 2)
            u0 = 2 * jnp.clip(j - 1, 0, 3)
            for k4 in range(4):
                ln_unit(lb, pl.multiple_of(u0 * 32 + 16 * k4, 16), None)
            jm = jnp.maximum(j - 1, 0)
            bsec = lax.div(jm, 2)
            kl = lax.rem(2 * bsec + 2, NWC)
            kr = jnp.where(j == 0, kl, kl + 1)
            bh = jnp.where(j == 0, 1, lax.rem(jm, 2))
            build_qkv(bsec, kl, kr, bh, N_EUP0)
            rb = pl.multiple_of(lax.rem(lax.div(j, 2) + 1, 3) * P0, 8)
            for gg in range(WC // 128):
                q_scr[half * (WC // 128) + gg, pl.ds(rb, P0), :] = _pack(y[:, gg * 128:(gg + 1) * 128])
            return carry

        lax.fori_loop(0, NWC, body, 0)
        build_qkv(2, 0, 1, 1, None)
        wo_copy().wait()
        for ld16, st16, pos in wo_part(NWP - 1):
            build_tiles(ld16, st16, [pos], jnp.zeros((8, 128), F32), None)

    @pl.when(s <= NA)
    def _():
        @pl.when(s + 1 < NCH)
        def _():
            for cp in raw_copies(s + 1):
                cp.start(priority=1)

        @pl.when(s + 4 < NB)
        def _():
            x_copy(s + 4).start(priority=1)

        @pl.when(s >= 1)
        def _():
            for cp in raw_copies(s - 1):
                cp.wait()

        @pl.when(jnp.logical_and(s >= 1, s + 2 < NB))
        def _():
            x_copy(s + 2).wait()

    @pl.when(jnp.logical_and(s >= 1, s <= NA))
    def _():
        c = lax.rem(s + (NA - 1), NA)
        r0 = pl.multiple_of(R0 + (s - 1) * TA, 16)
        HA = TA // 2
        pt = pl.multiple_of(r0 // 2, 8)
        pb = pl.multiple_of((r0 + HA) // 2, 8)
        a11 = _as_bf16(xn_scr[pl.ds(pt, HA // 2), 0:HD])
        a12 = _as_bf16(xn_scr[pl.ds(pt, HA // 2), HD:D])
        a21 = _as_bf16(xn_scr[pl.ds(pb, HA // 2), 0:HD])
        a22 = _as_bf16(xn_scr[pl.ds(pb, HA // 2), HD:D])
        la = [t.astype(BF) for t in _lhs_combos(a11.astype(F32), a12.astype(F32), a21.astype(F32), a22.astype(F32))]
        la[2], la[3] = a11, a22

        def ffn_part(raw, cmb, kq, nq):
            def ld8(q, r, n):
                return raw[c, pl.ds((kq if q >= 2 else 0) + r, 16), pl.ds((nq if q % 2 else 0) + n, 128)]

            def st16(j, r, n, val):
                cmb[c, j, r // 2:r // 2 + 8, n:n + 128] = val

            return [(ld8, st16, (r, n)) for r in range(0, kq, 16) for n in range(0, nq, 128)]

        work = ffn_part(rawg, cg, HD, FC) + ffn_part(rawu, cu, HD, FC) + ffn_part(rawd, cd, FC, HD) + wo_part(c)
        def stores(sec):
            for h in range(2):
                rh = pl.multiple_of(r0 + h * HA, 16)
                if sec == 2:
                    store_q(ys[2][h], rh)
                else:
                    store_kv(ys[sec][h], k_scr if sec == 0 else v_scr, rh)

        ys = []
        for sec in range(3):
            kl = (2 * sec + 2) % NWC
            cw = [_as_bf16(jnp.concatenate([cq[sec, 0, j], cq[sec, 1, j]], axis=0)) for j in range(5)]
            wl = [cw[0], wqkv[kl, 0:HD, :], cw[1], cw[2], wqkv[kl + 1, HD:D, :], cw[3], cw[4]]
            parts = [_strassen_out([_dot(la[j], wl[j][:, n:n + QN]) for j in range(7)]) for n in range(0, WC, QN)]
            c11, c12, c21, c22 = [jnp.concatenate([p[t] for p in parts], axis=1) for t in range(4)]
            ys.append((jnp.concatenate([c11, c12], axis=1), jnp.concatenate([c21, c22], axis=1)))
            stores(sec)
        ln_block(jnp.minimum(s + 2, NB - 1), chain=True)
        tok = jnp.zeros((8, 128), F32)
        for ld8, st16, pos in work:
            tok = build_tiles(ld8, st16, [pos], tok, N_EUP)

    @pl.when(s > NA)
    def _():
        i = lax.rem(s + (NB - NA - 1), NB)
        r0 = pl.multiple_of(i * TM, TM)

        def wlist(raw, cmb, c, kq, nq):
            cw = [_as_bf16(cmb[c, j]) for j in range(5)]
            return [cw[0], raw[c, 0:kq, 0:nq], cw[1], cw[2], raw[c, kq:2 * kq, nq:2 * nq], cw[3], cw[4]]

        RA = 16
        cexp = (DH ** -0.5) * LOG2E
        p0 = pl.multiple_of(r0 // 2, 8)

        def attn_half(q, r):
            sw = []
            for w in range(WIN):
                acc = None
                for g in range(NG):
                    t = q[g] * k_scr[g, pl.ds(r0 + r + HALO - DIL * w, 8), :]
                    acc = t if acc is None else acc + t
                acc = _sum4(acc)
                if r < HALO and w > 0:
                    row = lax.broadcasted_iota(jnp.int32, (8, 128), 0) + (r0 + r)
                    acc = jnp.where(row >= DIL * w, acc, NEG)
                sw.append(acc)
            m = sw[0]
            for w in range(1, WIN):
                m = jnp.maximum(m, sw[w])
            e = [jnp.exp2((sw[w] - m) * cexp) for w in range(WIN)]
            den = e[0]
            for w in range(1, WIN):
                den = den + e[w]
            inv = 1.0 / den
            p = [e[w] * inv for w in range(WIN)]
            o = []
            for g in range(NG):
                acc = None
                for w in range(WIN):
                    t = p[w] * v_scr[g, pl.ds(r0 + r + HALO - DIL * w, 8), :]
                    acc = t if acc is None else acc + t
                o.append(acc)
            return o

        prev_fin = [None]

        def attn_rows(r, tok):
            qp = [q_scr[g, pl.ds(p0 + r // 2, 8), :] for g in range(NG)]
            if tok is not None:
                qp = [_dep32(t, tok, never) for t in qp]
            q = [_unpack(t) for t in _butterfly(qp)]
            o0 = attn_half([t[0:8] for t in q], r)
            q1 = [t[8:16] for t in q]
            q1 = [_dep32(t, o0[NG - 1], never) for t in q1]
            o1 = attn_half(q1, r + 8)
            o = _butterfly([_pack(jnp.concatenate([o0[g], o1[g]], axis=0)) for g in range(NG)])
            for g in range(NG):
                o_scr[r // 2:r // 2 + 8, g * 128:(g + 1) * 128] = o[g]
            fin = o[0]
            for g in range(1, NG):
                fin = fin ^ o[g]
            tok = o[0]
            if prev_fin[0] is not None:
                tok = tok ^ prev_fin[0]
            prev_fin[0] = fin
            return tok

        s5 = [_as_bf16(s_scr[i, j]) for j in range(5)]
        xa11 = _as_bf16(xn_scr[pl.ds(p0, HM // 2), 0:HD])
        xa22 = _as_bf16(xn_scr[pl.ds(pl.multiple_of(p0 + HM // 2, 8), HM // 2), HD:D])
        sl = [s5[0], s5[1], xa11, xa22, s5[2], s5[3], s5[4]]
        s_block(jnp.minimum(i + 1, NB - 1), jnp.zeros((8, 128), F32))
        acc = [None] * 7
        n_att = TM // RA
        per = 3
        tok = None
        pend = []
        for c in range(NCH):
            wg_l = wlist(rawg, cg, c, HD, FC)
            wu_l = wlist(rawu, cu, c, HD, FC)
            wd_l = wlist(rawd, cd, c, FC, HD)
            g = _strassen_out([_dot(sl[j], wg_l[j]) for j in range(7)])
            u = _strassen_out([_dot(sl[j], wu_l[j]) for j in range(7)])
            hq = [g[t] * u[t] for t in range(4)]
            pend.append(([t.astype(BF) for t in _lhs_combos(*hq)], wd_l))
            if len(pend) == DOWN_GROUP or c == NCH - 1:
                for j in range(7):
                    y = _dot(jnp.concatenate([p[0][j] for p in pend], axis=1),
                             jnp.concatenate([p[1][j] for p in pend], axis=0))
                    acc[j] = y if acc[j] is None else acc[j] + y
                pend = []
            for a in range(c * per, min((c + 1) * per, n_att)):
                tok = attn_rows(a * RA, tok)
            if c == NCH - 1:
                oq = [_as_bf16(o_scr[rr:rr + HM // 2, cc:cc + HD]) for rr in (0, HM // 2) for cc in (0, HD)]
                ol = [t.astype(BF) for t in _lhs_combos(*[t.astype(F32) for t in oq])]
                ol[2], ol[3] = oq[0], oq[3]
                cw = [_as_bf16(jnp.concatenate([cwo[t, j] for t in range(NWP)], axis=0)) for j in range(5)]
                b11 = jnp.concatenate([wo[0, t, :, 0:HD] for t in range(NWP)], axis=0)
                b22 = jnp.concatenate([wo[1, t, :, HD:D] for t in range(NWP)], axis=0)
                wo_l = [cw[0], b11, cw[1], cw[2], b22, cw[3], cw[4]]
                acc = [acc[j] + _dot(ol[j], wo_l[j]) for j in range(7)]
        ys = _strassen_out(acc)
        x = x_scr[pl.ds(r0, TM), :].astype(F32)
        for q in range(4):
            rr, cc = (q // 2) * HM, (q % 2) * HD
            o_ref[rr:rr + HM, cc:cc + HD] = (x[rr:rr + HM, cc:cc + HD] + ys[q]).astype(o_ref.dtype)


@jax.jit
def pallas_parallel_sum__sliding_local_dilated__glu_gated_bilinear__prompt_kernel(
    A_x: jax.Array,
    A_wqkv: jax.Array,
    A_wo: jax.Array,
    B_x: jax.Array,
    B_w_gate: jax.Array,
    B_w_up: jax.Array,
    B_w_down: jax.Array,
):
    del B_x
    x = A_x.reshape(S, D)
    hbm = pl.BlockSpec(memory_space=pl.ANY)
    out = pl.pallas_call(
        _kernel,
        grid=(NSTEPS,),
        in_specs=[hbm] * 6,
        out_specs=pl.BlockSpec((TM, D), lambda s: (jnp.maximum(s - (NA + 1), 0), 0)),
        out_shape=jax.ShapeDtypeStruct((S, D), A_x.dtype),
        scratch_shapes=[
            pltpu.VMEM((S, D), BF),
            pltpu.VMEM((NWC, D, WC), BF),
            pltpu.VMEM((2, NWP, HD // NWP, D), BF),
            pltpu.VMEM((NCH, D, 2 * FC), BF),
            pltpu.VMEM((NCH, D, 2 * FC), BF),
            pltpu.VMEM((NCH, 2 * FC, D), BF),
            pltpu.VMEM((3, 2, 5, HD // 4, WC), U32),
            pltpu.VMEM((NWP, 5, HD // NWP // 2, HD), U32),
            pltpu.VMEM((NCH, 5, HD // 2, FC), U32),
            pltpu.VMEM((NCH, 5, HD // 2, FC), U32),
            pltpu.VMEM((NCH, 5, FC // 2, HD), U32),
            pltpu.VMEM((S // 2, D), U32),
            pltpu.VMEM((NB, 5, HM // 2, HD), U32),
            pltpu.VMEM((NG, S // 2, 128), U32),
            pltpu.VMEM((2, NG, S + HALO, 128), F32),
            pltpu.VMEM((TM // 2, D), U32),
            pltpu.SemaphoreType.DMA((NSX,)),
            pltpu.SemaphoreType.DMA((NWC + 1,)),
            pltpu.SemaphoreType.DMA((NSR,)),
        ],
        compiler_params=pltpu.CompilerParams(
            dimension_semantics=("arbitrary",),
            vmem_limit_bytes=124 * 1024 * 1024,
            disable_bounds_checks=True,
        ),
        name="fused_attn_ffn",
    )(x, A_wqkv, A_wo.reshape(2, NWP, HD // NWP, D), B_w_gate, B_w_up, B_w_down)
    return out.reshape(A_x.shape)
```
